```python
import jax
import jax.numpy as jnp

def _softmax(x, axis=-1):
    return jax.nn.softmax(x, axis=axis)

def _gelu(x):
    return jax.nn.gelu(x, approximate=True)

def _silu(x):
    return jax.nn.silu(x)

def _sigmoid(x):
    return jax.nn.sigmoid(x)

def _layernorm(x, axis=-1, eps=1e-05):
    m = jnp.mean(x, axis=axis, keepdims=True)
    v = jnp.var(x, axis=axis, keepdims=True)
    return (x - m) / jnp.sqrt(v + eps)

def _scatter_add(tgt, idx, src, axis=0):
    return tgt.at[idx].add(src)

def _segment_sum(src, seg, n):
    return jax.ops.segment_sum(src, seg, n)

class _Rng:

    def __init__(self, key):
        self._k = key

    def _next(self):
        self._k, sub = jax.random.split(self._k)
        return sub

    def normal(self, shape):
        return jax.random.normal(self._next(), shape, dtype=jnp.bfloat16)

    def randint(self, lo, hi, shape):
        return jax.random.randint(self._next(), shape, lo, hi, dtype=jnp.int32)

    def uniform(self, shape, lo=0.0, hi=1.0):
        return jax.random.uniform(self._next(), shape, jnp.bfloat16, lo, hi)

    def permutation(self, n):
        return jax.random.permutation(self._next(), n)
kernel_name = 'concat_heads__ssm_conv_h3__memory_aug_infini_attn__prompt'

def setup_inputs():
    _rng = _Rng(jax.random.key(int.from_bytes(__import__("os").urandom(4), "little")))
    _w = lambda a: (lambda t: t.astype(jnp.bfloat16) if jnp.issubdtype(t.dtype, jnp.floating) else t)(jnp.asarray(a))

    def _A_setup():
        B, S, D = (1, 2048, 640)
        ks = 4
        return {'q': _w((lambda *s: _rng.normal(s) * 0.05)(B, S, D)), 'k': _w((lambda *s: _rng.normal(s) * 0.05)(B, S, D)), 'v': _w((lambda *s: _rng.normal(s) * 0.05)(B, S, D)), 'shift_k': _w((lambda *s: _rng.normal(s) * 0.05)(D, ks) * 0.5), 'ssm_k': _w((lambda *s: _rng.normal(s) * 0.05)(D, S) * (1.0 / S ** 0.5)), 'ssm_D': _w((lambda *s: _rng.normal(s) * 0.05)(D))}
    _A_in = _A_setup()

    def _B_setup():
        B, S, D, H = (1, 2048, 640, 32)
        N = 4
        L = max(1, S // N)
        sc = D ** (-0.5)
        return {'x': _w((lambda *s: _rng.normal(s) * 0.05)(B, N * L, D)), 'wq': _w((lambda *s: _rng.normal(s) * 0.05)(D, D) * sc), 'wk': _w((lambda *s: _rng.normal(s) * 0.05)(D, D) * sc), 'wv': _w((lambda *s: _rng.normal(s) * 0.05)(D, D) * sc), 'wo': _w((lambda *s: _rng.normal(s) * 0.05)(D, D) * sc), 'beta': _w((lambda *s: _rng.normal(s) * 0.05)(H))}
    _B_in = _B_setup()
    return {'A_q': _A_in['q'], 'A_k': _A_in['k'], 'A_v': _A_in['v'], 'A_shift_k': _A_in['shift_k'], 'A_ssm_k': _A_in['ssm_k'], 'A_ssm_D': _A_in['ssm_D'], 'B_x': _B_in['x'], 'B_wq': _B_in['wq'], 'B_wk': _B_in['wk'], 'B_wv': _B_in['wv'], 'B_wo': _B_in['wo'], 'B_beta': _B_in['beta']}

def reference(A_q, A_k, A_v, A_shift_k, A_ssm_k, A_ssm_D, B_x, B_wq, B_wk, B_wv, B_wo, B_beta):

    def _A_ref(q, k, v, shift_k, ssm_k, ssm_D):
        B, S, D = q.shape
        ks = shift_k.shape[-1]
        k_pad = jnp.pad(k, ((0, 0), (ks - 1, 0), (0, 0)))
        k_shift = jnp.zeros_like(k)
        for t in range(ks):
            k_shift = k_shift + k_pad[:, t:t + S, :] * shift_k[:, ks - 1 - t][None, None, :]
        kv = k_shift * v
        L = 2 * S
        kv_pad = jnp.pad(kv, ((0, 0), (0, S), (0, 0)))
        kf_pad = jnp.pad(ssm_k, ((0, 0), (0, S)))
        kv_f = (lambda x, axes=(-2, -1): jnp.fft.rfft2(x.astype(jnp.float32), axes=axes))(kv_pad[:, None, :, :], axes=(1, 2))
        kf_f = (lambda x, axes=(-2, -1): jnp.fft.rfft2(x.astype(jnp.float32), axes=axes))(kf_pad[:, None, :], axes=(1, 2))
        kf_f = (lambda x, *d: x.transpose(*d))(kf_f, 1, 2, 0)
        y_f = kv_f * kf_f[None, :, :, :]
        y = (lambda x, s, axes=(-2, -1): jnp.fft.irfft2(x, s=s, axes=axes).astype(jnp.bfloat16))(y_f, (1, L), axes=(1, 2))[:, 0, :S, :]
        y = y + kv * ssm_D[None, None, :]
        return q * y

    def _B_ref(x, wq, wk, wv, wo, beta):
        B, S, D = x.shape
        H = 32
        Dh = D // H
        N = 4
        L = S // N
        q = (lambda x, *d: x.transpose(*d))((x @ wq).reshape(B, S, H, Dh), 0, 2, 1, 3).reshape(B, H, N, L, Dh)
        k = (lambda x, *d: x.transpose(*d))((x @ wk).reshape(B, S, H, Dh), 0, 2, 1, 3).reshape(B, H, N, L, Dh)
        v = (lambda x, *d: x.transpose(*d))((x @ wv).reshape(B, S, H, Dh), 0, 2, 1, 3).reshape(B, H, N, L, Dh)
        phi = lambda t: jnp.where(t > 0, t + 1.0, jnp.exp(t))
        scale = Dh ** (-0.5)
        ar = jnp.arange(L)
        mask = (lambda x, dt: x.astype(dt))(ar[:, None] < ar[None, :], x.dtype) * -1000000000.0
        g = _sigmoid(beta).reshape(1, H, 1, 1)
        M = jnp.einsum('bhd,bhe->bhde', q[:, :, 0, 0, :] * 0.0, q[:, :, 0, 0, :] * 0.0)
        z = q[:, :, 0, 0, :] * 0.0
        outs = []
        for s in range(N):
            qs, ks, vs = (q[:, :, s].copy(), k[:, :, s].copy(), v[:, :, s].copy())
            logits = jnp.einsum('bhqd,bhkd->bhqk', qs, ks) * scale + mask
            p = _softmax(logits, axis=-1)
            a_dot = jnp.einsum('bhqk,bhkd->bhqd', p, vs)
            pq = phi(qs)
            num = jnp.einsum('bhld,bhde->bhle', pq, M)
            den = jnp.einsum('bhld,bhd->bhl', pq, z)[..., None] + 1e-06
            a_mem = num / den
            o = g * a_mem + (1.0 - g) * a_dot
            outs.append(o)
            pk = phi(ks)
            M = M + jnp.einsum('bhld,bhle->bhde', pk, vs)
            z = z + jnp.einsum('bhld->bhd', pk)
        o = (lambda x, *d: x.transpose(*d))(jnp.stack(outs, 2).reshape(B, H, S, Dh), 0, 2, 1, 3).reshape(B, S, D)
        return o @ wo
    a = _A_ref(A_q, A_k, A_v, A_shift_k, A_ssm_k, A_ssm_D)
    b = _B_ref(B_x, B_wq, B_wk, B_wv, B_wo, B_beta)
    return jnp.concatenate([a, b], axis=-1)
```

```python
import jax
import jax.numpy as jnp
import numpy as np
from jax import lax
from jax.experimental import pallas as pl
from jax.experimental.pallas import tpu as pltpu

f32, bf16, u32, i32 = jnp.float32, jnp.bfloat16, jnp.uint32, jnp.int32

S, D, H, DH = 2048, 640, 32, 20
NSEG, L = 4, 512
T = 128
NC = D // T
NB = S // T
NQ = L // T
NG = 8
GW = 4 * DH
NFV = 16
LOG2E = 1.4426950408889634
NEG = -1e30

NT = (((1,), (1,)), ((), ()))


def _dft_tables():
    freq = np.concatenate([np.arange(0, T, 2), np.arange(1, T, 2)])
    theta = 2.0 * np.pi * (freq[:, None] + 0.5) * np.arange(T)[None, :] / (2 * T)
    re, im = np.cos(theta), -np.sin(theta)
    fwd = np.stack([re.reshape(NFV, 8, T), im.reshape(NFV, 8, T)], axis=1).reshape(2 * T, T)
    inv = fwd.T / T
    inv = np.stack([inv[:, :T], inv[:, T:]])
    return fwd.astype(np.float32).astype(bf16), inv.astype(np.float32).astype(bf16)


_FWD, _INV = _dft_tables()


def _as_bf16(words):
    return pltpu.bitcast(words, bf16)


def _as_words(x):
    return pltpu.bitcast(x.astype(bf16), u32)


def _dot(a, b):
    return jnp.dot(a, b, preferred_element_type=f32)


def _dot_nt(a, b):
    return lax.dot_general(a, b, NT, preferred_element_type=f32)


def _phi(t):
    return jnp.where(t > 0, t + 1.0, jnp.exp(t))


def _kernel(
    shift_ref, ssmd_ref, beta_ref, fwd_ref, inv_ref,
    q_hbm, k_hbm, v_hbm, ssm_hbm, x_hbm, wq_hbm, wk_hbm, wv_hbm, wo_hbm, out_hbm,
    xs, wraw, wt, qa, ka, va, ssk, kst, uf, kf, yf, outa, outb,
    fwd, inv, gate, qm, pq, kk, pk, vt, ot, mz, sem_in, sem_out,
):
    def x_copies(s):
        return [
            pltpu.make_async_copy(
                x_hbm.at[0, pl.ds(s * L, L), pl.ds(c * T, T)],
                xs.at[c, pl.ds(s * L, L)], sem_in.at[s])
            for c in range(NC)
        ]

    def w_copy(i):
        return pltpu.make_async_copy(
            (wq_hbm, wk_hbm, wv_hbm, wo_hbm)[i], wraw.at[i], sem_in.at[4 + i])

    def conv_copies(c):
        cols = pl.ds(pl.multiple_of(c * T, T), T)
        sem = sem_in.at[8 + c]
        return [
            pltpu.make_async_copy(k_hbm.at[0, :, cols], ka.at[c], sem),
            pltpu.make_async_copy(v_hbm.at[0, :, cols], va.at[c], sem),
            pltpu.make_async_copy(ssm_hbm.at[pl.ds(pl.multiple_of(c * T, T), T), :], ssk.at[c], sem),
        ]

    def q_copy(c):
        cols = pl.ds(pl.multiple_of(c * T, T), T)
        return pltpu.make_async_copy(q_hbm.at[0, :, cols], qa.at[c], sem_in.at[13 + c])

    for i in range(3):
        w_copy(i).start()
    for cp in x_copies(0):
        cp.start()
    for c in range(NC):
        for cp in conv_copies(c):
            cp.start()
    w_copy(3).start()
    for s in range(1, NSEG):
        for cp in x_copies(s):
            cp.start()
    for c in range(NC):
        q_copy(c).start()

    fwd[...] = pltpu.bitcast(fwd_ref[...], u32)
    for half in range(2):
        inv[half] = pltpu.bitcast(inv_ref[half], u32)
    mz[...] = jnp.zeros(mz.shape, f32)
    kst[0:8, :] = jnp.zeros((8, T), f32)
    for slot in range(2):
        for n in range(NQ):
            vt[slot, n, GW // 2:, :] = _as_words(jnp.ones((16, T), f32))
    beta = jnp.concatenate([beta_ref[...].astype(f32)[None, :], jnp.zeros((1, T - H), f32)], axis=1)
    gate[...] = jax.nn.sigmoid(jnp.broadcast_to(beta, (T, T)).T[:H])

    def transpose_weight(i):
        w_copy(i).wait()

        def body(c, carry):
            rows = pl.ds(pl.multiple_of(c * T, T), T)
            for n in range(NC):
                tile = wraw[i, rows, n * T:(n + 1) * T]
                wt[i, c, n * T // 2:(n + 1) * T // 2, :] = pltpu.bitcast(tile.T, u32)
            return carry

        lax.fori_loop(0, NC, body, 0)

    sub = lax.broadcasted_iota(i32, (8, T), 0)
    low = sub < 4

    def project(unit, slot, n):
        s, g = unit // NG, unit % NG
        rows = pl.ds(pl.multiple_of(g * (GW // 2), 8), GW // 2)
        times = pl.ds(pl.multiple_of(s * L + n * T, T), T)
        acc = None
        for c in range(NC):
            w = _as_bf16(jnp.concatenate([wt[i, c, rows, :] for i in range(3)], axis=0))
            part = _dot_nt(w, xs[c, times, :])
            acc = part if acc is None else acc + part
        q_t, k_t, v_t = acc[:GW], acc[GW:2 * GW], acc[2 * GW:]
        qs = q_t * (DH ** -0.5 * LOG2E)
        r = [qs[8 * i:8 * i + 8] for i in range(10)]
        zero = jnp.zeros((8, T), f32)
        heads = [
            r[0], r[1], jnp.where(low, r[2], 0.0), zero,
            jnp.where(low, 0.0, r[2]), r[3], r[4], zero,
            zero, r[5], r[6], jnp.where(low, r[7], 0.0),
            zero, jnp.where(low, 0.0, r[7]), r[8], r[9],
        ]
        qm[slot, n] = _as_words(jnp.concatenate(heads, axis=0))
        pq[slot, n] = _as_words(_phi(q_t))
        pk[slot, n] = _as_words(_phi(k_t))
        vt[slot, n, :GW // 2, :] = _as_words(v_t)
        k_pad = jnp.concatenate([k_t.astype(bf16), jnp.zeros((T - GW, T), bf16)], axis=0)
        kk[slot, n] = pltpu.bitcast(k_pad.T, u32)

    def attend(unit, slot, fillers):
        g = unit % NG
        row = lax.broadcasted_iota(i32, (T, T), 0)
        col = lax.broadcasted_iota(i32, (T, T), 1)
        causal = row <= col
        never = sub > 100 + g
        tiles = [(qt, kt) for qt in (3, 2, 1, 0) for kt in range(qt + 1)]
        lag = 5
        logits, run_max, col_max, acc, token = {}, {}, {}, {}, {}

        state = mz[g]
        row_m = lax.broadcasted_iota(i32, (GW, T), 0)
        col_m = lax.broadcasted_iota(i32, (GW, T), 1)

        def head_of(i):
            return (i >= DH).astype(i32) + (i >= 2 * DH).astype(i32) + (i >= 3 * DH).astype(i32)

        weights = jnp.where(head_of(row_m) == head_of(col_m), state[:GW], 0.0)
        lane_head = head_of(lax.broadcasted_iota(i32, (8, T), 1))
        sub_head = jnp.where(low, 0, 1)
        z01 = jnp.where(lane_head == sub_head, state[GW:GW + 8], 0.0)
        z23 = jnp.where(lane_head == sub_head + 2, state[GW:GW + 8], 0.0)
        mem_w = jnp.concatenate([weights, z01, z23], axis=0).astype(bf16)[:, :GW]
        gates = [jnp.broadcast_to(gate[pl.ds(4 * g + j, 1), :], (8, T)) for j in range(4)]
        g01 = jnp.where(low, gates[0], gates[1])
        g23 = jnp.where(low, gates[2], gates[3])

        def qk(t, j):
            qt, kt = tiles[t]
            window = _as_bf16(qm[slot, qt, 16 * j:16 * j + 16, :])
            rhs = window if j == 0 else jnp.concatenate(
                [jnp.zeros((16 * j, T), bf16), window], axis=0)
            keys = _as_bf16(kk[slot, kt])[:, :16 * j + 32]
            sc = _dot(keys, rhs)
            token[t, j] = sc[48:56]
            if kt == qt:
                sc = jnp.where(causal, sc, NEG)
            m8 = jnp.max(sc.reshape(16, 8, T), axis=0)
            run_max[qt, j] = m8 if kt == 0 else jnp.maximum(run_max[qt, j], m8)
            if kt == qt:
                col_max[qt, j] = jnp.broadcast_to(
                    jnp.max(run_max[qt, j], axis=0, keepdims=True), (8, T))
            logits[t, j] = sc

        def pv(t, j):
            qt, kt = tiles[t]
            m = col_max[qt, j]
            if (t + lag - 1, j) in token:
                m = jnp.where(never, token[t + lag - 1, j], m)
            p = jnp.exp2(logits[t, j].reshape(16, 8, T) - m[None]).reshape(T, T).astype(bf16)
            words = vt[slot, kt, 8 * j:8 * j + 16, :]
            ones = jnp.full((8, T), 0x3F803F80, u32)
            if j < 2:
                words = jnp.concatenate([words[:8], jnp.where(low, words[8:], ones)], axis=0)
            else:
                words = jnp.concatenate([jnp.where(low, ones, words[:8]), words[8:]], axis=0)
            part = _dot(_as_bf16(words), p)
            acc[qt, j] = part if kt == 0 else acc[qt, j] + part

        def finish(qt):
            mem = _dot(mem_w, _as_bf16(pq[slot, qt]))
            c01 = g01 / (mem[GW:GW + 8] + 1e-6)
            c23 = g23 / (mem[GW + 8:] + 1e-6)
            s01, s23 = pltpu.roll(c01, 4, 0), pltpu.roll(c23, 4, 0)
            cm = [jnp.where(low, c01, s01), c01, jnp.where(low, s01, c01),
                  jnp.where(low, c23, s23), c23, jnp.where(low, s23, c23)]
            cm = [cm[i] for i in (0, 0, 1, 2, 2, 3, 3, 4, 5, 5)]
            a = []
            for j in range(4):
                w = acc[qt, j]
                scale = (1.0 - gates[j]) / (w[24:] if j < 2 else w[:8])
                a.append([(w[8 * i:8 * i + 8] * scale) for i in range(4)])
            dotp = [a[0][0], a[0][1], jnp.where(low, a[0][2], a[1][0]), a[1][1], a[1][2],
                    a[2][1], a[2][2], jnp.where(low, a[2][3], a[3][1]), a[3][2], a[3][3]]
            o = jnp.concatenate(
                [mem[8 * i:8 * i + 8] * cm[i] + dotp[i] for i in range(10)], axis=0)
            ot[qt, pl.ds(pl.multiple_of(g * (GW // 2), 8), GW // 2), :] = _as_words(o)

        n = len(tiles)
        for t in range(n + lag):
            if t < n:
                for j in range(4):
                    qk(t, j)
            for filler in fillers.get(t, ()):
                filler()
            if t >= lag:
                for j in range(4):
                    pv(t - lag, j)
        for qt in (3, 2, 1, 0):
            finish(qt)
        upd = None
        for kt in range(NQ):
            pk_t = jnp.concatenate(
                [_as_bf16(pk[slot, kt]), jnp.zeros((T - GW, T), bf16)], axis=0)
            part = _dot_nt(_as_bf16(vt[slot, kt]), pk_t)
            upd = part if upd is None else upd + part
        mz[g] = state + upd

    def out_project(s):
        def body(n, carry):
            acc = [None] * 4
            for c in range(NC):
                rhs = _as_bf16(ot[n, c * 64:(c + 1) * 64, :])
                for m in range(4):
                    part = _dot(_as_bf16(wt[3, c, 80 * m:80 * (m + 1), :]), rhs)
                    acc[m] = part if acc[m] is None else acc[m] + part
            res = jnp.concatenate(acc, axis=0).astype(bf16)
            rows = pl.ds(pl.multiple_of(n * T, T), T)
            for c in range(NC):
                outb[s, rows, c * T:(c + 1) * T] = res[c * T:(c + 1) * T].T
            return carry

        lax.fori_loop(0, NQ, body, 0)

    def outb_copy(s):
        return pltpu.make_async_copy(
            outb.at[s], out_hbm.at[0, pl.ds(pl.multiple_of(s * L, L), L), pl.ds(D, D)],
            sem_out.at[s])

    def conv_forward(c, carry):
        for cp in conv_copies(c):
            cp.wait()
        cols = pl.ds(pl.multiple_of(c * T, T), T)
        taps = shift_ref[:, cols].astype(f32)
        taps = [jnp.broadcast_to(taps[j:j + 1], (T, T)) for j in range(4)]
        skip = jnp.broadcast_to(ssmd_ref[...].astype(f32), (NC, T))
        skip = jnp.sum(
            jnp.where(lax.broadcasted_iota(i32, (NC, T), 0) == c, skip, 0.0), axis=0, keepdims=True)
        fmat = _as_bf16(fwd[...])
        prev = None
        for b in range(NB):
            rows = slice(b * T, (b + 1) * T)
            k0 = ka[c, rows, :].astype(f32)
            kst[8 + b * T:8 + (b + 1) * T, :] = k0
            shifted = k0 * taps[0]
            for j in range(1, 4):
                shifted = shifted + kst[8 + b * T - j:8 + (b + 1) * T - j, :] * taps[j]
            kv = (shifted * va[c, rows, :].astype(f32)).astype(bf16)
            uf[c, :, b] = _dot(fmat, kv).reshape(NFV, 16, T)
            spec = _dot_nt(fmat, ssk[c, :, rows]).reshape(NFV, 2, 8, T)
            re, im = spec[:, 0], spec[:, 1]
            if prev is None:
                re2, im2 = re + skip[None], im
            else:
                half = NFV // 2
                pre, pim = prev
                re2 = jnp.concatenate([re[:half] - pim[:half], re[half:] + pim[half:]], axis=0)
                im2 = jnp.concatenate([im[:half] + pre[:half], im[half:] - pre[half:]], axis=0)
            prev = (re, im)
            kf[c, :, b, 0:8, :] = re2
            kf[c, :, b, 8:16, :] = im2
        return carry

    def conv_mix(c, fv):
        def load(ref, b):
            return ref[c, fv, b, 0:8, :], ref[c, fv, b, 8:16, :]

        blk = 4
        for a0 in range(0, NB, blk):
            acc = [None] * blk
            kcache = {}
            for b in range(a0 + blk):
                ur, ui = load(uf, b)
                us = ur + ui
                for a in range(max(a0, b), a0 + blk):
                    if a - b not in kcache:
                        kr, ki = load(kf, a - b)
                        kcache[a - b] = (kr, ki - kr, kr + ki)
                    k1, k2, k3 = kcache[a - b]
                    terms = (us * k1, ur * k2, ui * k3)
                    old = acc[a - a0]
                    acc[a - a0] = terms if old is None else tuple(
                        o + t for o, t in zip(old, terms))
            for i in range(blk):
                p1, p2, p3 = acc[i]
                yf[c, fv, a0 + i] = _as_words(jnp.concatenate([p1 - p3, p1 + p2], axis=0))

    def outa_copy(c):
        cols = pl.ds(pl.multiple_of(c * T, T), T)
        return pltpu.make_async_copy(outa.at[c], out_hbm.at[0, :, cols], sem_out.at[NSEG + c])

    def conv_inverse(c, carry):
        q_copy(c).wait()
        for a in range(NB):
            spec = _as_bf16(yf[c, :, a].reshape(T, T))
            y = _dot(_as_bf16(inv[0]), spec[:T]) + _dot(_as_bf16(inv[1]), spec[T:])
            rows = slice(a * T, (a + 1) * T)
            outa[c, rows, :] = (qa[c, rows, :].astype(f32) * y).astype(bf16)
        outa_copy(c).start()
        return carry

    for i in range(3):
        transpose_weight(i)
    for cp in x_copies(0):
        cp.wait()
    for n in range(NQ):
        project(0, 0, n)
    lax.fori_loop(0, NC, conv_forward, 0)
    transpose_weight(3)

    def segment(s, carry):
        @pl.when(s + 1 < NSEG)
        def _():
            for cp in x_copies(s + 1):
                cp.wait()

        def pair(p, carry):
            i = s * 4 + p
            for slot in range(2):
                unit = 2 * i + slot
                nxt = jnp.minimum(unit + 1, NSEG * NG - 1)
                fillers = {
                    9 + n: [lambda n=n, nxt=nxt, slot=slot: project(nxt, 1 - slot, n)]
                    for n in range(NQ)
                }
                attend(unit, slot, fillers)
            for c in range(NC):
                conv_mix(c, i)
            return carry

        lax.fori_loop(0, 4, pair, 0)
        out_project(s)
        outb_copy(s).start()
        return carry

    lax.fori_loop(0, NSEG, segment, 0)
    lax.fori_loop(0, NC, conv_inverse, 0)
    for s in range(NSEG):
        outb_copy(s).wait()
    for c in range(NC):
        outa_copy(c).wait()


@jax.jit
def pallas_concat_heads__ssm_conv_h3__memory_aug_infini_attn__prompt_kernel(
    A_q: jax.Array,
    A_k: jax.Array,
    A_v: jax.Array,
    A_shift_k: jax.Array,
    A_ssm_k: jax.Array,
    A_ssm_D: jax.Array,
    B_x: jax.Array,
    B_wq: jax.Array,
    B_wk: jax.Array,
    B_wv: jax.Array,
    B_wo: jax.Array,
    B_beta: jax.Array,
):
    vmem = pl.BlockSpec(memory_space=pltpu.VMEM)
    hbm = pl.BlockSpec(memory_space=pl.ANY)
    scratch = [
        pltpu.VMEM((NC, S, T), bf16),
        pltpu.VMEM((4, D, D), bf16),
        pltpu.VMEM((4, NC, D // 2, T), u32),
        pltpu.VMEM((NC, S, T), bf16),
        pltpu.VMEM((NC, S, T), bf16),
        pltpu.VMEM((NC, S, T), bf16),
        pltpu.VMEM((NC, T, S), bf16),
        pltpu.VMEM((S + 8, T), f32),
        pltpu.VMEM((NC, NFV, NB, 16, T), f32),
        pltpu.VMEM((NC, NFV, NB, 16, T), f32),
        pltpu.VMEM((NC, NFV, NB, 8, T), u32),
        pltpu.VMEM((NC, S, T), bf16),
        pltpu.VMEM((NSEG, L, D), bf16),
        pltpu.VMEM((T, T), u32),
        pltpu.VMEM((2, T // 2, T), u32),
        pltpu.VMEM((H, T), f32),
        pltpu.VMEM((2, NQ, 64, T), u32),
        pltpu.VMEM((2, NQ, GW // 2, T), u32),
        pltpu.VMEM((2, NQ, T // 2, T), u32),
        pltpu.VMEM((2, NQ, GW // 2, T), u32),
        pltpu.VMEM((2, NQ, GW // 2 + 8, T), u32),
        pltpu.VMEM((NQ, D // 2, T), u32),
        pltpu.VMEM((NG, GW + 16, T), f32),
        pltpu.SemaphoreType.DMA((18,)),
        pltpu.SemaphoreType.DMA((NSEG + NC,)),
    ]
    return pl.pallas_call(
        _kernel,
        out_shape=jax.ShapeDtypeStruct((1, S, 2 * D), bf16),
        in_specs=[vmem] * 5 + [hbm] * 9,
        out_specs=hbm,
        scratch_shapes=scratch,
        compiler_params=pltpu.CompilerParams(vmem_limit_bytes=100 * 2**20),
    )(
        A_shift_k.T, A_ssm_D.reshape(NC, T), B_beta, _FWD, _INV,
        A_q, A_k, A_v, A_ssm_k, B_x, B_wq, B_wk, B_wv, B_wo,
    )
```

```python
import os
import jax
import jax.numpy as jnp
import numpy as np
from jax import lax
from jax.experimental import pallas as pl
from jax.experimental.pallas import tpu as pltpu

f32, bf16, u32, i32 = jnp.float32, jnp.bfloat16, jnp.uint32, jnp.int32

S, D, H, DH = 2048, 640, 32, 20
NSEG, L = 4, 512
T = 128
NC = D // T
NB = S // T
NQ = L // T
NG = 8
GW = 4 * DH
NFV = 16
LOG2E = 1.4426950408889634
NEG = -1e30
MIX_PER_ITER = 7

def _env(name, default):
    return type(default)(os.environ.get(name, default))
WA, WP, WO, WM = _env("WA", 1.0), _env("WP", 1.0), _env("WO", 1.0), _env("WM", 1.0)
SLACK = _env("SLACK", 0.97)
LAG, BACK, TOK = _env("LAG", 5), _env("BACK", 1), _env("TOK", 6)
PSTEPS = [int(v) for v in _env("PSTEPS", "9,10,11,12").split(",")]
OSTEPS = [int(v) for v in _env("OSTEPS", "0,1,2,3,4").split(",")]
ORDER = [int(v) for v in _env("ORDER", "3,2,1,0").split(",")]
FSTEPS = [int(v) for v in _env("FSTEPS", "14,14,14,14").split(",")]

NT = (((1,), (1,)), ((), ()))


def _dft_tables():
    freq = np.concatenate([np.arange(0, T, 2), np.arange(1, T, 2)])
    theta = 2.0 * np.pi * (freq[:, None] + 0.5) * np.arange(T)[None, :] / (2 * T)
    re, im = np.cos(theta), -np.sin(theta)
    fwd = np.stack([re.reshape(NFV, 8, T), im.reshape(NFV, 8, T)], axis=1).reshape(2 * T, T)
    inv = fwd.T / T
    inv = np.stack([inv[:, :T], inv[:, T:]])
    return fwd.astype(np.float32).astype(bf16), inv.astype(np.float32).astype(bf16)


_FWD, _INV = _dft_tables()


def _as_bf16(words):
    return pltpu.bitcast(words, bf16)


def _as_words(x):
    return pltpu.bitcast(x.astype(bf16), u32)


def _dot(a, b):
    return jnp.dot(a, b, preferred_element_type=f32)


def _dot_nt(a, b):
    return lax.dot_general(a, b, NT, preferred_element_type=f32)


def _phi(t):
    return jnp.where(t > 0, t + 1.0, jnp.exp(t))


def _ds(start, size, align):
    if isinstance(start, int):
        return pl.ds(start, size)
    return pl.ds(pl.multiple_of(start, align), size)


class _Side:
    def __init__(self, gen=None, steps=0, cycles=1):
        self.gen, self.rate, self.credit = gen, steps / cycles, 0.0
        if gen is not None:
            next(gen)

    def tick(self, result, lane, weight):
        nv = result.shape[0] // 8
        self.credit += self.rate * result.shape[0] / 4 * weight
        count = int(self.credit)
        self.credit -= count
        for i in range(count):
            if self.gen is None:
                return
            v = min(nv - 1, int(nv * (lane + (i + 0.5) / count) / 4))
            try:
                self.gen.send(result[8 * v:8 * v + 8])
            except StopIteration:
                self.gen = None


def _kernel(
    shift_ref, ssmd_ref, beta_ref, fwd_ref, inv_ref,
    q_hbm, k_hbm, v_hbm, ssm_hbm, x_hbm, wq_hbm, wk_hbm, wv_hbm, wo_hbm, out_hbm,
    xs, wraw, wt, wot, qa, ka, va, ssk, kst, uf, kf, yf, outa, outb,
    fwd, inv, gate, qm, pq, kk, vt, pk_keep, vt_keep, ot, mz, sem_in, sem_out,
):
    def x_copies(s):
        return [
            pltpu.make_async_copy(
                x_hbm.at[0, pl.ds(s * L, L), pl.ds(c * T, T)],
                xs.at[c, pl.ds(s * L, L)], sem_in.at[s])
            for c in range(NC)
        ]

    def w_copies(i):
        src = (wq_hbm, wk_hbm, wv_hbm, wo_hbm)[i]
        return [
            pltpu.make_async_copy(src.at[:, pl.ds(n * T, T)], wraw.at[i, n], sem_in.at[4 + i])
            for n in range(NC)
        ]

    def conv_copies(c):
        cols = _ds(c * T, T, T)
        sem = sem_in.at[8 + c]
        return [
            pltpu.make_async_copy(k_hbm.at[0, :, cols], ka.at[c], sem),
            pltpu.make_async_copy(v_hbm.at[0, :, cols], va.at[c], sem),
            pltpu.make_async_copy(ssm_hbm.at[cols, :], ssk.at[c], sem),
        ]

    def q_copy(c):
        return pltpu.make_async_copy(q_hbm.at[0, :, _ds(c * T, T, T)], qa.at[c], sem_in.at[13 + c])

    def start(copies):
        for cp in copies:
            cp.start()

    def wait(copies):
        for cp in copies:
            cp.wait()

    for i in range(3):
        start(w_copies(i))
    start(x_copies(0))
    start(x_copies(1))
    for c in range(NC):
        start(conv_copies(c))
    start(w_copies(3))
    for s in range(2, NSEG):
        start(x_copies(s))
    start([q_copy(c) for c in range(NC)])

    fwd[...] = pltpu.bitcast(fwd_ref[...], u32)
    for half in range(2):
        inv[half] = pltpu.bitcast(inv_ref[half], u32)
    mz[...] = jnp.zeros(mz.shape, f32)
    kst[0:8, :] = jnp.zeros((8, T), f32)
    beta = jnp.concatenate([beta_ref[...].astype(f32)[None, :], jnp.zeros((1, T - H), f32)], axis=1)
    gate[...] = jax.nn.sigmoid(jnp.broadcast_to(beta, (T, T)).T[:H])

    def transpose_weight(i):
        wait(w_copies(i))
        for n in range(NC):
            for c in range(NC):
                words = pltpu.bitcast(wraw[i, n, c * T:(c + 1) * T, :].T, u32)
                if i < 3:
                    wt[i, c, n * T // 2:(n + 1) * T // 2, :] = words
                else:
                    wot[c, n * T // 2:(n + 1) * T // 2, :] = words

    sub = lax.broadcasted_iota(i32, (8, T), 0)
    low = sub < 4

    def project(s, g, slot, n, side):
        rows = _ds(g * (GW // 2), GW // 2, 8)
        times = _ds(s * L + n * T, T, T)
        acc = None
        for c in range(NC):
            w = _as_bf16(jnp.concatenate([wt[i, c, rows, :] for i in range(3)], axis=0))
            part = _dot_nt(w, xs[c, times, :])
            side.tick(part, (n * NC + c) % 4, WP)
            acc = part if acc is None else acc + part
        q_t, k_t, v_t = acc[:GW], acc[GW:2 * GW], acc[2 * GW:]
        qs = q_t * (DH ** -0.5 * LOG2E)
        r = [qs[8 * i:8 * i + 8] for i in range(10)]
        zero = jnp.zeros((8, T), f32)
        heads = [
            r[0], r[1], jnp.where(low, r[2], 0.0), zero,
            jnp.where(low, 0.0, r[2]), r[3], r[4], zero,
            zero, r[5], r[6], jnp.where(low, r[7], 0.0),
            zero, jnp.where(low, 0.0, r[7]), r[8], r[9],
        ]
        qm[slot, n] = _as_words(jnp.concatenate(heads, axis=0))
        pq[slot, n] = _as_words(_phi(q_t))
        pk_keep[s % 2, g, n] = _as_words(_phi(k_t))
        v_words = _as_words(v_t)
        vt[slot, n] = v_words
        vt_keep[s % 2, g, n] = v_words
        k_pad = jnp.concatenate([k_t.astype(bf16), jnp.zeros((T - GW, T), bf16)], axis=0)
        kk[slot, n] = pltpu.bitcast(k_pad.T, u32)

    def attend(s, g, slot, fillers, side, memory):
        row = lax.broadcasted_iota(i32, (T, T), 0)
        col = lax.broadcasted_iota(i32, (T, T), 1)
        causal = row <= col
        never = sub > 100 + g
        ones = jnp.full((8, T), 0x3F803F80, u32)
        tiles = [(qt, kt) for qt in ORDER for kt in range(qt + 1)]
        logits, run_max, col_max, acc, token = {}, {}, {}, {}, {}
        gates = [jnp.broadcast_to(gate[pl.ds(4 * g + j, 1), :], (8, T)) for j in range(4)]

        if memory:
            state = mz[g]
            for kt in range(NQ):
                v_one = jnp.concatenate([vt_keep[(s + 1) % 2, g, kt], ones], axis=0)
                pk_t = jnp.concatenate(
                    [_as_bf16(pk_keep[(s + 1) % 2, g, kt]), jnp.zeros((T - GW, T), bf16)], axis=0)
                part = _dot_nt(_as_bf16(v_one), pk_t)
                side.tick(part, kt, WM)
                state = state + part
            mz[g] = state

            def head_of(i):
                return (i >= DH).astype(i32) + (i >= 2 * DH).astype(i32) + (i >= 3 * DH).astype(i32)

            row_m = lax.broadcasted_iota(i32, (GW, T), 0)
            col_m = lax.broadcasted_iota(i32, (GW, T), 1)
            weights = jnp.where(head_of(row_m) == head_of(col_m), state[:GW], 0.0)
            lane_head = head_of(lax.broadcasted_iota(i32, (8, T), 1))
            sub_head = jnp.where(low, 0, 1)
            z01 = jnp.where(lane_head == sub_head, state[GW:GW + 8], 0.0)
            z23 = jnp.where(lane_head == sub_head + 2, state[GW:GW + 8], 0.0)
            mem_w = jnp.concatenate([weights, z01, z23], axis=0).astype(bf16)[:, :GW]
            g01 = jnp.where(low, gates[0], gates[1])
            g23 = jnp.where(low, gates[2], gates[3])

        def qk(t, j):
            qt, kt = tiles[t]
            window = _as_bf16(qm[slot, qt, 16 * j:16 * j + 16, :])
            rhs = window if j == 0 else jnp.concatenate(
                [jnp.zeros((16 * j, T), bf16), window], axis=0)
            keys = _as_bf16(kk[slot, kt])[:, :16 * j + 32]
            sc = _dot(keys, rhs)
            token[t, j] = sc[8 * TOK:8 * TOK + 8]
            side.tick(sc, j, WA)
            if kt == qt:
                sc = jnp.where(causal, sc, NEG)
            m8 = jnp.max(sc.reshape(16, 8, T), axis=0)
            run_max[qt, j] = m8 if kt == 0 else jnp.maximum(run_max[qt, j], m8)
            if kt == qt:
                col_max[qt, j] = jnp.broadcast_to(
                    jnp.max(run_max[qt, j], axis=0, keepdims=True), (8, T))
            logits[t, j] = sc

        def pv(t, j):
            qt, kt = tiles[t]
            m = col_max[qt, j]
            if (t + LAG - BACK, j) in token:
                m = jnp.where(never, token[t + LAG - BACK, j], m)
            p = jnp.exp2(logits[t, j].reshape(16, 8, T) - m[None]).reshape(T, T).astype(bf16)
            words = vt[slot, kt, 8 * j:8 * j + 16, :]
            if j < 2:
                words = jnp.concatenate([words[:8], jnp.where(low, words[8:], ones)], axis=0)
            else:
                words = jnp.concatenate([jnp.where(low, ones, words[:8]), words[8:]], axis=0)
            part = _dot(_as_bf16(words), p)
            acc[qt, j] = part if kt == 0 else acc[qt, j] + part

        def finish(qt):
            a = []
            for j in range(4):
                w = acc[qt, j]
                scale = (1.0 - gates[j]) / (w[24:] if j < 2 else w[:8])
                a.append([(w[8 * i:8 * i + 8] * scale) for i in range(4)])
            o = [a[0][0], a[0][1], jnp.where(low, a[0][2], a[1][0]), a[1][1], a[1][2],
                 a[2][1], a[2][2], jnp.where(low, a[2][3], a[3][1]), a[3][2], a[3][3]]
            if memory:
                mem = _dot(mem_w, _as_bf16(pq[slot, qt]))
                side.tick(mem, qt, WM)
                c01 = g01 / (mem[GW:GW + 8] + 1e-6)
                c23 = g23 / (mem[GW + 8:] + 1e-6)
                s01, s23 = pltpu.roll(c01, 4, 0), pltpu.roll(c23, 4, 0)
                cm = [jnp.where(low, c01, s01), c01, jnp.where(low, s01, c01),
                      jnp.where(low, c23, s23), c23, jnp.where(low, s23, c23)]
                cm = [cm[i] for i in (0, 0, 1, 2, 2, 3, 3, 4, 5, 5)]
                o = [mem[8 * i:8 * i + 8] * cm[i] + o[i] for i in range(10)]
            ot[s % 2, qt, _ds(g * (GW // 2), GW // 2, 8), :] = _as_words(
                jnp.concatenate(o, axis=0))

        n = len(tiles)
        for t in range(n + LAG):
            if t < n:
                for j in range(4):
                    qk(t, j)
            for filler in fillers.get(t, ()):
                filler()
            if t >= LAG:
                for j in range(4):
                    pv(t - LAG, j)
            for qt, step in zip(ORDER, FSTEPS):
                if step == t:
                    finish(qt)

    def out_project(s, n, side):
        acc = [None] * 4

        def step(c):
            rhs = _as_bf16(ot[s % 2, n, c * 64:(c + 1) * 64, :])
            for m in range(4):
                part = _dot(_as_bf16(wot[c, 80 * m:80 * (m + 1), :]), rhs)
                side.tick(part, m, WO)
                acc[m] = part if acc[m] is None else acc[m] + part
            if c == NC - 1:
                res = jnp.concatenate(acc, axis=0).astype(bf16)
                for i in range(NC):
                    outb[s, _ds(n * T, T, T), i * T:(i + 1) * T] = res[i * T:(i + 1) * T].T

        return [lambda c=c: step(c) for c in range(NC)]

    def outb_copy(s, n):
        return pltpu.make_async_copy(
            outb.at[s, _ds(n * T, T, T)],
            out_hbm.at[0, _ds(s * L + n * T, T, T), pl.ds(D, D)],
            sem_out.at[NC + s * NQ + n])

    def conv_forward(c, carry):
        wait(conv_copies(c))
        taps = shift_ref[:, _ds(c * T, T, T)].astype(f32)
        taps = [jnp.broadcast_to(taps[j:j + 1], (T, T)) for j in range(4)]
        skip = jnp.sum(
            jnp.where(lax.broadcasted_iota(i32, (NC, T), 0) == c, ssmd_ref[...].astype(f32), 0.0),
            axis=0, keepdims=True)
        fmat = _as_bf16(fwd[...])
        prev = None
        for b in range(NB):
            rows = slice(b * T, (b + 1) * T)
            k0 = ka[c, rows, :].astype(f32)
            kst[8 + b * T:8 + (b + 1) * T, :] = k0
            shifted = k0 * taps[0]
            for j in range(1, 4):
                shifted = shifted + kst[8 + b * T - j:8 + (b + 1) * T - j, :] * taps[j]
            kv = (shifted * va[c, rows, :].astype(f32)).astype(bf16)
            spec = _dot_nt(fmat, ssk[c, :, rows]).reshape(NFV, 2, 8, T)
            uf[c, :, b] = _dot(fmat, kv).reshape(NFV, 16, T)
            re, im = spec[:, 0], spec[:, 1]
            if prev is None:
                re2, im2 = re + skip[None], im
            else:
                half = NFV // 2
                pre, pim = prev
                re2 = jnp.concatenate([re[:half] - pim[:half], re[half:] + pim[half:]], axis=0)
                im2 = jnp.concatenate([im[:half] + pre[:half], im[half:] - pre[half:]], axis=0)
            prev = (re, im)
            kf[c, :, b, 0:8, :] = re2
            kf[c, :, b, 8:16, :] = im2
        return carry

    def conv_mix(first, never, blk=4):
        for item in range(MIX_PER_ITER):
            idx = jnp.minimum(first + item, NC * NFV - 1)
            c, fv = idx // NFV, idx % NFV

            def load(ref, b):
                return ref[c, fv, b, 0:8, :], ref[c, fv, b, 8:16, :]

            for a0 in range(0, NB, blk):
                acc = [None] * blk
                kcache = {}
                for b in range(a0 + blk):
                    token = yield
                    ur, ui = load(uf, b)
                    ur = jnp.where(never, token, ur)
                    ui = jnp.where(never, token, ui)
                    us = ur + ui
                    for a in range(max(a0, b), a0 + blk):
                        if a - b not in kcache:
                            kr, ki = load(kf, a - b)
                            kcache[a - b] = (kr, ki - kr, kr + ki)
                        k1, k2, k3 = kcache[a - b]
                        terms = (us * k1, ur * k2, ui * k3)
                        old = acc[a - a0]
                        acc[a - a0] = terms if old is None else tuple(
                            o + t for o, t in zip(old, terms))
                for i in range(blk):
                    p1, p2, p3 = acc[i]
                    yf[c, fv, a0 + i] = _as_words(jnp.concatenate([p1 - p3, p1 + p2], axis=0))

    def outa_copy(c):
        return pltpu.make_async_copy(
            outa.at[c], out_hbm.at[0, :, _ds(c * T, T, T)], sem_out.at[c])

    def conv_inverse(c, carry):
        q_copy(c).wait()
        for a in range(NB):
            spec = _as_bf16(yf[c, :, a].reshape(T, T))
            y = _dot(_as_bf16(inv[0]), spec[:T]) + _dot(_as_bf16(inv[1]), spec[T:])
            rows = slice(a * T, (a + 1) * T)
            outa[c, rows, :] = (qa[c, rows, :].astype(f32) * y).astype(bf16)
        outa_copy(c).start()
        return carry

    def pair(s, p, first):
        if first:
            side = _Side()
        else:
            steps = MIX_PER_ITER * 40
            cycles = 2 * (1280 * WA + 1200 * WP + 192 * WM) + 800 * WO
            side = _Side(conv_mix(((s - 1) * 4 + p) * MIX_PER_ITER, sub > 100 + p),
                         steps, cycles * SLACK)
        for slot in range(2):
            g = 2 * p + slot
            if slot == 0:
                ns, ng = s, g + 1
            else:
                ns, ng = jnp.minimum(s + (g + 1) // NG, NSEG - 1), (g + 1) % NG
            fillers = {}
            if slot == 0 and not first:
                for step, fn in zip(OSTEPS, out_project(s - 1, p, side)):
                    fillers.setdefault(step, []).append(fn)
            for n in range(NQ):
                fillers.setdefault(PSTEPS[n], []).append(
                    lambda n=n, ns=ns, ng=ng, slot=slot: project(ns, ng, 1 - slot, n, side))
            attend(s, g, slot, fillers, side, memory=not first)
        assert side.gen is None

    for i in range(3):
        transpose_weight(i)
    wait(x_copies(0))
    for n in range(NQ):
        project(0, 0, 0, n, _Side())
    wait(x_copies(1))

    @pl.loop(0, 4)
    def _(p):
        pair(0, p, True)

    lax.fori_loop(0, NC, conv_forward, 0)
    transpose_weight(3)
    wait(x_copies(2))
    wait(x_copies(3))

    @pl.loop(4, 16)
    def _(i):
        s, p = i // 4, i % 4
        pair(s, p, False)
        outb_copy(s - 1, p).start()

    lax.fori_loop(0, NC, conv_inverse, 0)

    @pl.loop(0, NQ)
    def _(n):
        for step in out_project(NSEG - 1, n, _Side()):
            step()
        outb_copy(NSEG - 1, n).start()

    for s in range(NSEG):
        for n in range(NQ):
            outb_copy(s, n).wait()
    for c in range(NC):
        outa_copy(c).wait()


@jax.jit
def pallas_concat_heads__ssm_conv_h3__memory_aug_infini_attn__prompt_kernel(
    A_q: jax.Array,
    A_k: jax.Array,
    A_v: jax.Array,
    A_shift_k: jax.Array,
    A_ssm_k: jax.Array,
    A_ssm_D: jax.Array,
    B_x: jax.Array,
    B_wq: jax.Array,
    B_wk: jax.Array,
    B_wv: jax.Array,
    B_wo: jax.Array,
    B_beta: jax.Array,
):
    vmem = pl.BlockSpec(memory_space=pltpu.VMEM)
    hbm = pl.BlockSpec(memory_space=pl.ANY)
    scratch = [
        pltpu.VMEM((NC, S, T), bf16),
        pltpu.VMEM((4, NC, D, T), bf16),
        pltpu.VMEM((3, NC, D // 2, T), u32),
        pltpu.VMEM((NC, D // 2, T), u32),
        pltpu.VMEM((NC, S, T), bf16),
        pltpu.VMEM((NC, S, T), bf16),
        pltpu.VMEM((NC, S, T), bf16),
        pltpu.VMEM((NC, T, S), bf16),
        pltpu.VMEM((S + 8, T), f32),
        pltpu.VMEM((NC, NFV, NB, 16, T), f32),
        pltpu.VMEM((NC, NFV, NB, 16, T), f32),
        pltpu.VMEM((NC, NFV, NB, 8, T), u32),
        pltpu.VMEM((NC, S, T), bf16),
        pltpu.VMEM((NSEG, L, D), bf16),
        pltpu.VMEM((T, T), u32),
        pltpu.VMEM((2, T // 2, T), u32),
        pltpu.VMEM((H, T), f32),
        pltpu.VMEM((2, NQ, 64, T), u32),
        pltpu.VMEM((2, NQ, GW // 2, T), u32),
        pltpu.VMEM((2, NQ, T // 2, T), u32),
        pltpu.VMEM((2, NQ, GW // 2, T), u32),
        pltpu.VMEM((2, NG, NQ, GW // 2, T), u32),
        pltpu.VMEM((2, NG, NQ, GW // 2, T), u32),
        pltpu.VMEM((2, NQ, D // 2, T), u32),
        pltpu.VMEM((NG, GW + 16, T), f32),
        pltpu.SemaphoreType.DMA((18,)),
        pltpu.SemaphoreType.DMA((NC + NSEG * NQ,)),
    ]
    return pl.pallas_call(
        _kernel,
        out_shape=jax.ShapeDtypeStruct((1, S, 2 * D), bf16),
        in_specs=[vmem] * 5 + [hbm] * 9,
        out_specs=hbm,
        scratch_shapes=scratch,
        compiler_params=pltpu.CompilerParams(vmem_limit_bytes=100 * 2**20),
    )(
        A_shift_k.T, A_ssm_D.reshape(NC, T), B_beta, _FWD, _INV,
        A_q, A_k, A_v, A_ssm_k, B_x, B_wq, B_wk, B_wv, B_wo,
    )
```

```python
import os
import jax
import jax.numpy as jnp
import numpy as np
from jax import lax
from jax.experimental import pallas as pl
from jax.experimental.pallas import tpu as pltpu

f32, bf16, u32, i32 = jnp.float32, jnp.bfloat16, jnp.uint32, jnp.int32

S, D, H, DH = 2048, 640, 32, 20
NSEG, L = 4, 512
T = 128
NC = D // T
NB = S // T
NQ = L // T
NG = 8
GW = 4 * DH
NFV = 16
LOG2E = 1.4426950408889634
NEG = -1e30
MIX_PER_ITER = 7

def _env(name, default):
    return type(default)(os.environ.get(name, default))
WA, WP, WO, WM = _env("WA", 1.0), _env("WP", 1.0), _env("WO", 1.0), _env("WM", 1.0)
SLACK = _env("SLACK", 0.97)
LEAD = _env("LEAD", 400)
STAG = _env("STAG", 30)
PF32 = _env("PF32", 0)
PLAN0 = _env("PLAN0",
    "Qa0 Pa0 Qa1 Pa1 Qa2 Pa2 Qa3 Pa3 Qa4 Va0 Pa4 Qa5 Va1 Qa6 Va2 Qa7 Va3 Qa8 Va4 Qa9 Va5 Qb0 Va6 Qb1 Va7 "
    "Qb2 Va8 Qb3 Va9 Qb4 Vb0 Pb0 Qb5 Vb1 Pb1 Qb6 Vb2 Qb7 Vb3 Pb2 Qb8 Vb4 Qb9 Vb5 Pb3 Vb6 Pb4 Vb7 Vb8 Vb9").split()
PLAN1 = _env("PLAN1",
    "Ua Qa0 Pa0 Qa1 Pa1 Qa2 Pa2 Qa3 Pa3 Qa4 Va0 Pa4 Qa5 Va1 Oa0 Qa6 Va2 Oa1 Qa7 Va3 Oa2 Qa8 Va4 Oa3 Qa9 Va5 "
    "Oa4 Ub Qb0 Va6 Ra Qb1 Va7 Qb2 Va8 Qb3 Va9 Qb4 Vb0 Pb0 Qb5 Vb1 Pb1 Qb6 Vb2 Qb7 Vb3 Pb2 Qb8 Vb4 Qb9 Vb5 "
    "Pb3 Vb6 Pb4 Vb7 Rb Vb8 Vb9").split()
ORDER = [int(v) for v in _env("ORDER", "3,2,1,0").split(",")]

NN = (((1,), (0,)), ((), ()))
NT = (((1,), (1,)), ((), ()))


def _dft_tables():
    freq = np.concatenate([np.arange(0, T, 2), np.arange(1, T, 2)])
    theta = 2.0 * np.pi * (freq[:, None] + 0.5) * np.arange(T)[None, :] / (2 * T)
    re, im = np.cos(theta), -np.sin(theta)
    fwd = np.stack([re.reshape(NFV, 8, T), im.reshape(NFV, 8, T)], axis=1).reshape(2 * T, T)
    inv = fwd.T / T
    inv = np.stack([inv[:, :T], inv[:, T:]])
    return fwd.astype(np.float32).astype(bf16), inv.astype(np.float32).astype(bf16)


_FWD, _INV = _dft_tables()


def _as_bf16(words):
    return pltpu.bitcast(words, bf16)


def _as_words(x):
    return pltpu.bitcast(x.astype(bf16), u32)


def _dot(a, b):
    return jnp.dot(a, b, preferred_element_type=f32)


def _dot_nt(a, b):
    return lax.dot_general(a, b, NT, preferred_element_type=f32)


def _phi(t):
    return jnp.where(t > 0, t + 1.0, jnp.exp(t))


def _ds(start, size, align):
    if isinstance(start, int):
        return pl.ds(start, size)
    return pl.ds(pl.multiple_of(start, align), size)


class _Pacer:
    def __init__(self, never, side=None, rate=0.0):
        self.never, self.side, self.rate = never, side, rate
        self.credit, self.clock, self.history = 0.0, 0.0, []
        if side is not None:
            next(side)

    def issued(self, result, lane, weight=0.0):
        rows = result.shape[0]
        self.history.append((self.clock, result))
        if lane == 3:
            self.clock += rows
        self.credit += self.rate * rows / 4 * weight
        count = int(self.credit)
        self.credit -= count
        for i in range(count):
            if self.side is not None:
                v = min(rows // 8 - 1, int(rows // 8 * (lane + (i + 0.5) / count) / 4))
                try:
                    self.side.send(result[8 * v:8 * v + 8])
                except StopIteration:
                    self.side = None

    def hold(self, value, lead):
        target = self.clock - lead
        if target < 0 or self.never is None:
            return value
        for start, result in reversed(self.history):
            if start <= target:
                v = min(result.shape[0] // 8 - 1, int(target - start) // 8)
                return jnp.where(self.never, result[8 * v:8 * v + 8], value)
        return value


def _kernel(
    shift_ref, ssmd_ref, beta_ref, fwd_ref, inv_ref,
    q_hbm, k_hbm, v_hbm, ssm_hbm, x_hbm, wq_hbm, wk_hbm, wv_hbm, wo_hbm, out_hbm,
    xs, wraw, wt, wot, qa, ka, va, ssk, spec_buf, yf, outa, outb,
    fwd, inv, gate, qm, pq, kk, vt, pk_keep, vt_keep, ot, mz, sem_in, sem_out,
):
    def x_copies(s):
        return [
            pltpu.make_async_copy(
                x_hbm.at[0, pl.ds(s * L, L), pl.ds(c * T, T)],
                xs.at[c, pl.ds(s * L, L)], sem_in.at[s])
            for c in range(NC)
        ]

    def w_copies(i):
        src = (wq_hbm, wk_hbm, wv_hbm, wo_hbm)[i]
        return [
            pltpu.make_async_copy(src.at[:, pl.ds(n * T, T)], wraw.at[i, n], sem_in.at[4 + i])
            for n in range(NC)
        ]

    def conv_copies(c):
        cols = _ds(c * T, T, T)
        sem = sem_in.at[8 + c]
        return [
            pltpu.make_async_copy(k_hbm.at[0, :, cols], ka.at[c], sem),
            pltpu.make_async_copy(v_hbm.at[0, :, cols], va.at[c], sem),
            pltpu.make_async_copy(ssm_hbm.at[cols, :], ssk.at[c], sem),
        ]

    def q_copy(c):
        return pltpu.make_async_copy(q_hbm.at[0, :, _ds(c * T, T, T)], qa.at[c], sem_in.at[13 + c])

    def start(copies):
        for cp in copies:
            cp.start()

    def wait(copies):
        for cp in copies:
            cp.wait()

    for i in range(3):
        start(w_copies(i))
    start(x_copies(0))
    start(x_copies(1))
    for c in range(NC):
        start(conv_copies(c))
    start(w_copies(3))
    for s in range(2, NSEG):
        start(x_copies(s))
    start([q_copy(c) for c in range(NC)])

    fwd[...] = pltpu.bitcast(fwd_ref[...], u32)
    for half in range(2):
        inv[half] = pltpu.bitcast(inv_ref[half], u32)
    mz[...] = jnp.zeros(mz.shape, f32)
    beta = jnp.concatenate([beta_ref[...].astype(f32)[None, :], jnp.zeros((1, T - H), f32)], axis=1)
    gate[...] = jax.nn.sigmoid(jnp.broadcast_to(beta, (T, T)).T[:H])

    def transpose_weight(i):
        wait(w_copies(i))
        for n in range(NC):
            for c in range(NC):
                words = pltpu.bitcast(wraw[i, n, c * T:(c + 1) * T, :].T, u32)
                if i < 3:
                    wt[i, c, n * T // 2:(n + 1) * T // 2, :] = words
                else:
                    wot[c, n * T // 2:(n + 1) * T // 2, :] = words

    sub = lax.broadcasted_iota(i32, (8, T), 0)
    low = sub < 4

    def project(s, g, slot, pacer):
        rows = _ds(g * (GW // 2), GW // 2, 8)
        acc = [None] * NQ

        def store(n):
            q_t, k_t, v_t = acc[n][:GW], acc[n][GW:2 * GW], acc[n][2 * GW:]
            k_pad = jnp.concatenate([k_t.astype(bf16), jnp.zeros((T - GW, T), bf16)], axis=0)
            kk[slot, n] = pltpu.bitcast(k_pad.T, u32)
            qs = q_t * (DH ** -0.5 * LOG2E)
            r = [qs[8 * i:8 * i + 8] for i in range(10)]
            zero = jnp.zeros((8, T), f32)
            heads = [
                r[0], r[1], jnp.where(low, r[2], 0.0), zero,
                jnp.where(low, 0.0, r[2]), r[3], r[4], zero,
                zero, r[5], r[6], jnp.where(low, r[7], 0.0),
                zero, jnp.where(low, 0.0, r[7]), r[8], r[9],
            ]
            qm[slot, n] = _as_words(jnp.concatenate(heads, axis=0))
            pq[slot, n] = _as_words(_phi(q_t))
            pk_keep[s % 2, g, n] = _as_words(_phi(k_t))
            vt[slot, n] = v_t
            vt_keep[s % 2, g, n] = v_t

        def step(i):
            for lane in range(4):
                n, c = divmod(4 * i + lane, NC)
                w = _as_bf16(jnp.concatenate([wt[m, c, rows, :] for m in range(3)], axis=0))
                part = _dot_nt(w, xs[c, _ds(s * L + n * T, T, T), :])
                pacer.issued(part, lane, WP)
                acc[n] = part if c == 0 else acc[n] + part
                if c == NC - 1:
                    store(n)

        return step

    def attend(s, g, slot, pacer, memory):
        row = lax.broadcasted_iota(i32, (T, T), 0)
        col = lax.broadcasted_iota(i32, (T, T), 1)
        causal = row <= col
        tiles = [(qt, kt) for qt in ORDER for kt in range(qt + 1)]
        logits, run_max, col_max, acc, mem, done = {}, {}, {}, {}, {}, []
        gates = [jnp.broadcast_to(gate[pl.ds(4 * g + j, 1), :], (8, T)) for j in range(4)]

        def update(_):
            state = mz[g]
            for kt in range(NQ):
                v_one = jnp.concatenate(
                    [vt_keep[(s + 1) % 2, g, kt], jnp.ones((8, T), f32)], axis=0)
                pk_t = jnp.concatenate(
                    [_as_bf16(pk_keep[(s + 1) % 2, g, kt]), jnp.zeros((T - GW, T), bf16)], axis=0)
                part = _dot_nt(v_one, pk_t)
                pacer.issued(part, kt, WM)
                state = state + part
            mz[g] = state

        def read(_):
            def head_of(i):
                return (i >= DH).astype(i32) + (i >= 2 * DH).astype(i32) + (i >= 3 * DH).astype(i32)

            state = mz[g]
            row_m = lax.broadcasted_iota(i32, (GW, T), 0)
            col_m = lax.broadcasted_iota(i32, (GW, T), 1)
            weights = jnp.where(head_of(row_m) == head_of(col_m), state[:GW], 0.0)
            lane_head = head_of(lax.broadcasted_iota(i32, (8, T), 1))
            pair_of = sub // 2
            z_rows = jnp.where(lane_head == pair_of, state[GW:], 0.0)
            mem_w = jnp.concatenate([weights, z_rows], axis=0)[:, :GW]
            g_rows = jnp.where(low, jnp.where(sub < 2, gates[0], gates[1]),
                               jnp.where(sub < 6, gates[2], gates[3]))
            for qt in range(NQ):
                res = lax.dot_general(
                    mem_w, _as_bf16(pq[slot, qt]), NN, preferred_element_type=f32)
                pacer.issued(res, qt, WM)
                coef = g_rows / (res[GW:] + 1e-6)
                c0, c1, c2, c3 = (
                    jnp.broadcast_to(coef[2 * j:2 * j + 1], (8, T)) for j in range(4))
                cm = [c0, c0, jnp.where(low, c0, c1), c1, c1,
                      c2, c2, jnp.where(low, c2, c3), c3, c3]
                mem[qt] = [res[8 * i:8 * i + 8] * cm[i] for i in range(10)]
            finish()

        def scores(t):
            qt, kt = tiles[t]
            for j in range(4):
                window = _as_bf16(qm[slot, qt, 16 * j:16 * j + 16, :])
                rhs = window if j == 0 else jnp.concatenate(
                    [jnp.zeros((16 * j, T), bf16), window], axis=0)
                keys = _as_bf16(kk[slot, kt])[:, :16 * j + 32]
                sc = _dot(keys, rhs)
                pacer.issued(sc, j, WA)
                if kt == qt:
                    sc = jnp.where(causal, sc, NEG)
                m8 = jnp.max(sc.reshape(16, 8, T), axis=0)
                run_max[qt, j] = m8 if kt == 0 else jnp.maximum(run_max[qt, j], m8)
                if kt == qt:
                    col_max[qt, j] = jnp.broadcast_to(
                        jnp.max(run_max[qt, j], axis=0, keepdims=True), (8, T))
                logits[t, j] = sc

        def values(t):
            qt, kt = tiles[t]
            tops = [pacer.hold(col_max[qt, j], LEAD - STAG * j) for j in range(4)]
            for j in range(4):
                p = jnp.exp2(logits[t, j].reshape(16, 8, T) - tops[j][None])
                first = (0, 16, 40, 56)[j]
                v = [vt[slot, kt, first + 8 * i:first + 8 * i + 8, :] for i in range(3)]
                if j % 2 == 0:
                    v[2] = jnp.where(low, v[2], 1.0)
                else:
                    v[0] = jnp.where(low, 1.0, v[0])
                p = p.reshape(T, T)
                part = lax.dot_general(
                    jnp.concatenate(v, axis=0), p if PF32 else p.astype(bf16), NN,
                    preferred_element_type=f32)
                pacer.issued(part, j)
                acc[qt, j] = part if kt == 0 else acc[qt, j] + part
            if kt == qt:
                done.append(qt)
                finish()

        def finish():
            while done and (not memory or done[0] in mem):
                qt = done.pop(0)
                w = [[acc[qt, j][8 * i:8 * i + 8] for i in range(3)] for j in range(4)]
                c0, c1, c2, c3 = (
                    (1.0 - gates[j]) / jnp.broadcast_to(
                        w[j][0][0:1] if j % 2 else w[j][2][7:8], (8, T))
                    for j in range(4))
                o = [w[0][0] * c0, w[0][1] * c0,
                     jnp.where(low, w[0][2] * c0, w[1][0] * c1), w[1][1] * c1, w[1][2] * c1,
                     w[2][0] * c2, w[2][1] * c2,
                     jnp.where(low, w[2][2] * c2, w[3][0] * c3), w[3][1] * c3, w[3][2] * c3]
                if memory:
                    o = [mem[qt][i] + o[i] for i in range(10)]
                ot[s % 2, qt, _ds(g * (GW // 2), GW // 2, 8), :] = _as_words(
                    jnp.concatenate(o, axis=0))

        return {"Q": scores, "V": values, "U": update, "R": read}

    def out_project(s, n, pacer):
        acc = [None] * 4

        def step(c):
            rhs = _as_bf16(ot[s % 2, n, c * 64:(c + 1) * 64, :])
            for m in range(4):
                part = _dot(_as_bf16(wot[c, 80 * m:80 * (m + 1), :]), rhs)
                pacer.issued(part, m, WO)
                acc[m] = part if c == 0 else acc[m] + part
            if c == NC - 1:
                res = jnp.concatenate(acc, axis=0).astype(bf16)
                for i in range(NC):
                    outb[s, _ds(n * T, T, T), i * T:(i + 1) * T] = res[i * T:(i + 1) * T].T

        return step

    def outb_copy(s, n):
        return pltpu.make_async_copy(
            outb.at[s, _ds(n * T, T, T)],
            out_hbm.at[0, _ds(s * L + n * T, T, T), pl.ds(D, D)],
            sem_out.at[NC + s * NQ + n])

    def conv_forward(c, carry):
        wait(conv_copies(c))
        taps = shift_ref[:, _ds(c * T, T, T)].astype(f32)
        taps = [jnp.broadcast_to(taps[j:j + 1], (T, T)) for j in range(4)]
        skip = jnp.sum(
            jnp.where(lax.broadcasted_iota(i32, (NC, T), 0) == c, ssmd_ref[...].astype(f32), 0.0),
            axis=0, keepdims=True)
        fmat = _as_bf16(fwd[...])
        slices = pl.ds(c * NFV, NFV)
        prev = None
        ktail = jnp.zeros((8, T), f32)
        for b in range(NB):
            rows = slice(b * T, (b + 1) * T)
            k0 = ka[c, rows, :].astype(f32)
            ext = jnp.concatenate([ktail, k0], axis=0)
            ktail = k0[T - 8:]
            shifted = k0 * taps[0]
            for j in range(1, 4):
                shifted = shifted + ext[8 - j:8 + T - j] * taps[j]
            kv = (shifted * va[c, rows, :].astype(f32)).astype(bf16)
            spec = _dot_nt(fmat, ssk[c, :, rows]).reshape(NFV, 2, 8, T)
            spec_buf[slices, 0, b] = _dot(fmat, kv).reshape(NFV, 16, T)
            re, im = spec[:, 0], spec[:, 1]
            if prev is None:
                re2, im2 = re + skip[None], im
            else:
                half = NFV // 2
                pre, pim = prev
                re2 = jnp.concatenate([re[:half] - pim[:half], re[half:] + pim[half:]], axis=0)
                im2 = jnp.concatenate([im[:half] + pre[:half], im[half:] - pre[half:]], axis=0)
            prev = (re, im)
            spec_buf[slices, 1, b, 0:8, :] = re2
            spec_buf[slices, 1, b, 8:16, :] = im2
        return carry

    def conv_mix(first, never, blk=4):
        for item in range(MIX_PER_ITER):
            idx = jnp.minimum(first + item, NC * NFV - 1)

            def load(which, b):
                return spec_buf[idx, which, b, 0:8, :], spec_buf[idx, which, b, 8:16, :]

            for a0 in range(0, NB, blk):
                acc = [None] * blk
                kcache = {}
                for b in range(a0 + blk):
                    token = yield
                    ur, ui = load(0, b)
                    ur = jnp.where(never, token, ur)
                    ui = jnp.where(never, token, ui)
                    us = ur + ui
                    for a in range(max(a0, b), a0 + blk):
                        if a - b not in kcache:
                            kr, ki = load(1, a - b)
                            kcache[a - b] = (kr, ki - kr, kr + ki)
                        k1, k2, k3 = kcache[a - b]
                        terms = (us * k1, ur * k2, ui * k3)
                        old = acc[a - a0]
                        acc[a - a0] = terms if old is None else tuple(
                            o + t for o, t in zip(old, terms))
                for i in range(blk):
                    p1, p2, p3 = acc[i]
                    yf[idx, a0 + i] = _as_words(jnp.concatenate([p1 - p3, p1 + p2], axis=0))

    def outa_copy(c):
        return pltpu.make_async_copy(
            outa.at[c], out_hbm.at[0, :, _ds(c * T, T, T)], sem_out.at[c])

    def conv_inverse(c, carry):
        q_copy(c).wait()
        for a in range(NB):
            spec = _as_bf16(yf[pl.ds(c * NFV, NFV), a].reshape(T, T))
            y = _dot(_as_bf16(inv[0]), spec[:T]) + _dot(_as_bf16(inv[1]), spec[T:])
            rows = slice(a * T, (a + 1) * T)
            outa[c, rows, :] = (qa[c, rows, :].astype(f32) * y).astype(bf16)
        outa_copy(c).start()
        return carry

    def pair(s, p, first):
        never = sub > 100 + p
        if first:
            pacer = _Pacer(never)
        else:
            cycles = 2 * (1280 * WA + 1200 * WP + 176 * WM) + 800 * WO
            pacer = _Pacer(never, conv_mix(((s - 1) * 4 + p) * MIX_PER_ITER, never),
                           MIX_PER_ITER * 40 / (cycles * SLACK))
        steps = {"a": attend(s, 2 * p, 0, pacer, not first),
                 "b": attend(s, 2 * p + 1, 1, pacer, not first)}
        steps["a"]["P"] = project(s, 2 * p + 1, 1, pacer)
        steps["b"]["P"] = project(
            jnp.minimum(s + (p + 1) // 4, NSEG - 1), (2 * p + 2) % NG, 0, pacer)
        if not first:
            steps["a"]["O"] = out_project(s - 1, p, pacer)
        for item in (PLAN0 if first else PLAN1):
            steps[item[1]][item[0]](int(item[2:] or 0))
        assert pacer.side is None

    for i in range(3):
        transpose_weight(i)
    wait(x_copies(0))
    step = project(0, 0, 0, _Pacer(None))
    for i in range(NC):
        step(i)
    wait(x_copies(1))

    @pl.loop(0, 4)
    def _(p):
        pair(0, p, True)

    lax.fori_loop(0, NC, conv_forward, 0)
    transpose_weight(3)
    wait(x_copies(2))
    wait(x_copies(3))

    @pl.loop(4, 16)
    def _(i):
        s, p = i // 4, i % 4
        pair(s, p, False)
        outb_copy(s - 1, p).start()

    lax.fori_loop(0, NC, conv_inverse, 0)

    @pl.loop(0, NQ)
    def _(n):
        step = out_project(NSEG - 1, n, _Pacer(None))
        for c in range(NC):
            step(c)
        outb_copy(NSEG - 1, n).start()

    for s in range(NSEG):
        for n in range(NQ):
            outb_copy(s, n).wait()
    for c in range(NC):
        outa_copy(c).wait()


@jax.jit
def pallas_concat_heads__ssm_conv_h3__memory_aug_infini_attn__prompt_kernel(
    A_q: jax.Array,
    A_k: jax.Array,
    A_v: jax.Array,
    A_shift_k: jax.Array,
    A_ssm_k: jax.Array,
    A_ssm_D: jax.Array,
    B_x: jax.Array,
    B_wq: jax.Array,
    B_wk: jax.Array,
    B_wv: jax.Array,
    B_wo: jax.Array,
    B_beta: jax.Array,
):
    vmem = pl.BlockSpec(memory_space=pltpu.VMEM)
    hbm = pl.BlockSpec(memory_space=pl.ANY)
    scratch = [
        pltpu.VMEM((NC, S, T), bf16),
        pltpu.VMEM((4, NC, D, T), bf16),
        pltpu.VMEM((3, NC, D // 2, T), u32),
        pltpu.VMEM((NC, D // 2, T), u32),
        pltpu.VMEM((NC, S, T), bf16),
        pltpu.VMEM((NC, S, T), bf16),
        pltpu.VMEM((NC, S, T), bf16),
        pltpu.VMEM((NC, T, S), bf16),
        pltpu.VMEM((NC * NFV, 2, NB, 16, T), f32),
        pltpu.VMEM((NC * NFV, NB, 8, T), u32),
        pltpu.VMEM((NC, S, T), bf16),
        pltpu.VMEM((NSEG, L, D), bf16),
        pltpu.VMEM((T, T), u32),
        pltpu.VMEM((2, T // 2, T), u32),
        pltpu.VMEM((H, T), f32),
        pltpu.VMEM((2, NQ, 64, T), u32),
        pltpu.VMEM((2, NQ, GW // 2, T), u32),
        pltpu.VMEM((2, NQ, T // 2, T), u32),
        pltpu.VMEM((2, NQ, GW, T), f32),
        pltpu.VMEM((2, NG, NQ, GW // 2, T), u32),
        pltpu.VMEM((2, NG, NQ, GW, T), f32),
        pltpu.VMEM((2, NQ, D // 2, T), u32),
        pltpu.VMEM((NG, GW + 8, T), f32),
        pltpu.SemaphoreType.DMA((18,)),
        pltpu.SemaphoreType.DMA((NC + NSEG * NQ,)),
    ]
    return pl.pallas_call(
        _kernel,
        out_shape=jax.ShapeDtypeStruct((1, S, 2 * D), bf16),
        in_specs=[vmem] * 5 + [hbm] * 9,
        out_specs=hbm,
        scratch_shapes=scratch,
        compiler_params=pltpu.CompilerParams(vmem_limit_bytes=100 * 2**20),
    )(
        A_shift_k.T, A_ssm_D.reshape(NC, T), B_beta, _FWD, _INV,
        A_q, A_k, A_v, A_ssm_k, B_x, B_wq, B_wk, B_wv, B_wo,
    )
```

```python
import os
import jax
import jax.numpy as jnp
import numpy as np
from jax import lax
from jax.experimental import pallas as pl
from jax.experimental.pallas import tpu as pltpu

f32, bf16, u32, i32 = jnp.float32, jnp.bfloat16, jnp.uint32, jnp.int32

S, D, H, DH = 2048, 640, 32, 20
NSEG, L = 4, 512
T = 128
NC = D // T
NB = S // T
NQ = L // T
NG = 8
GW = 4 * DH
NFV = 16
LOG2E = 1.4426950408889634
NEG = -1e30
MIX_PER_ITER = 7

def _env(name, default):
    return type(default)(os.environ.get(name, default))
WA, WP, WO, WM = _env("WA", 1.0), _env("WP", 1.0), _env("WO", 1.0), _env("WM", 1.0)
SLACK = _env("SLACK", 0.97)
LEAD = _env("LEAD", 400)
STAG = _env("STAG", 40)
PF32 = _env("PF32", 0)
XB = _env("XB", 1)
FULLK = _env("FULLK", 1)
ONLY = _env("ONLY", "")
PLAN0 = _env("PLAN0",
    "Qa0 Da0 Pa0 Qa1 Pa1 Qa2 Pa2 Qa3 Pa3 Qa4 Va0 Pa4 Qa5 Va1 Qa6 Va2 Qa7 Da1 Va3 Qa8 Va4 Qa9 Va5 Qb0 Va6 Qb1 Db0 Va7 "
    "Qb2 Va8 Qb3 Va9 Qb4 Vb0 Pb0 Qb5 Vb1 Pb1 Qb6 Vb2 Qb7 Db1 Vb3 Pb2 Qb8 Vb4 Qb9 Vb5 Pb3 Vb6 Pb4 Vb7 Vb8 Vb9").split()
PLAN1 = _env("PLAN1",
    "Ua Qa0 Da0 Pa0 Qa1 Pa1 Qa2 Pa2 Qa3 Pa3 Qa4 Va0 Pa4 Qa5 Va1 Oa0 Qa6 Va2 Oa1 Qa7 Da1 Va3 Oa2 Qa8 Va4 Oa3 Qa9 Va5 "
    "Oa4 Ub Qb0 Va6 Ra Qb1 Db0 Va7 Qb2 Va8 Qb3 Va9 Qb4 Vb0 Pb0 Qb5 Vb1 Pb1 Qb6 Vb2 Qb7 Db1 Vb3 Pb2 Qb8 Vb4 Qb9 Vb5 "
    "Pb3 Vb6 Pb4 Vb7 Rb Vb8 Vb9 Cx").split()
WI = 1.0
PLAN_FIRST = _env("PLAN_FIRST",
    "Wx2 Qa0 Da0 Qa1 Tx1 Qa2 Qa3 Qa4 Va0 Qa5 Va1 Qa6 Va2 Pa0 Qa7 Da1 Va3 Pa1 Qa8 Va4 Pa2 Qa9 Va5 Pa3 Va6 Pa4 Va7 Wx3 Qb0 Db0 Va8 Tx2 "
    "Qb1 Va9 Qb2 Qb3 Tx3 Qb4 Vb0 Pb0 Qb5 Vb1 Pb1 Tx4 Qb6 Vb2 Qb7 Db1 Vb3 Pb2 Qb8 Vb4 Qb9 Vb5 Pb3 Vb6 Pb4 Vb7 Vb8 Vb9").split()
PLAN_LAST = _env("PLAN_LAST",
    "Ua Qa0 Da0 Pa0 Qa1 Pa1 Qa2 Pa2 Qa3 Pa3 Qa4 Va0 Pa4 Qa5 Va1 Oa0 Qa6 Va2 Oa1 Qa7 Da1 Va3 Oa2 Qa8 Va4 Oa3 Qa9 Va5 "
    "Oa4 Ub Qb0 Va6 Ra Ix0 Qb1 Db0 Va7 Ix1 Qb2 Va8 Ix2 Qb3 Va9 Ix3 Qb4 Vb0 Ix4 Qb5 Vb1 Ix5 Qb6 Vb2 Ix6 Qb7 Db1 Vb3 "
    "Ix7 Qb8 Vb4 Ix8 Qb9 Vb5 Ix9 Ix10 Rb Vb6 Ix11 Ix12 Vb7 Ix13 Vb8 Ix14 Vb9 Ix15 Cx Ax0 Ax1 Bx0 "
    + " ".join(f"Ix{i}" for i in range(16, 32)) + " Ax2 Ax3 Bx1 "
    + " ".join(f"Ex{i} Ix{32 + i}" for i in range(8)) + " Ax4 Fx0 Bx2 "
    + " ".join(f"Ex{i}" for i in range(8, 20)) + " Fx1 Fx2 Fx3 Bx3 Bx4").split()
ORDER = [int(v) for v in _env("ORDER", "3,2,1,0").split(",")]

NN = (((1,), (0,)), ((), ()))
NT = (((1,), (1,)), ((), ()))


def _dft_tables():
    freq = np.concatenate([np.arange(0, T, 2), np.arange(1, T, 2)])
    theta = 2.0 * np.pi * (freq[:, None] + 0.5) * np.arange(T)[None, :] / (2 * T)
    re, im = np.cos(theta), -np.sin(theta)
    fwd = np.stack([re.reshape(NFV, 8, T), im.reshape(NFV, 8, T)], axis=1).reshape(2 * T, T)
    inv = fwd.T / T
    inv = np.stack([inv[:, :T], inv[:, T:]])
    return fwd.astype(np.float32).astype(bf16), inv.astype(np.float32).astype(bf16)


_FWD, _INV = _dft_tables()


def _as_bf16(words):
    return pltpu.bitcast(words, bf16)


def _as_words(x):
    return pltpu.bitcast(x.astype(bf16), u32)


def _dot(a, b):
    return jnp.dot(a, b, preferred_element_type=f32)


def _dot_nt(a, b):
    return lax.dot_general(a, b, NT, preferred_element_type=f32)


def _phi(t):
    return jnp.maximum(t, 0.0) + jnp.exp(jnp.minimum(t, 0.0))


def _ds(start, size, align):
    if isinstance(start, int):
        return pl.ds(start, size)
    return pl.ds(pl.multiple_of(start, align), size)


class _Pacer:
    def __init__(self, never, side=None, rate=0.0):
        self.never, self.side, self.rate = never, side, rate
        self.credit, self.clock, self.history = 0.0, 0.0, []
        if side is not None:
            next(side)

    def issued(self, result, lane, weight=0.0):
        rows = result.shape[0]
        self.history.append((self.clock, result))
        if lane == 3:
            self.clock += rows
        self.credit += self.rate * rows / 4 * weight
        count = int(self.credit)
        self.credit -= count
        for i in range(count):
            if self.side is not None:
                v = min(rows // 8 - 1, int(rows // 8 * (lane + (i + 0.5) / count) / 4))
                try:
                    self.side.send(result[8 * v:8 * v + 8])
                except StopIteration:
                    self.side = None

    def hold(self, value, lead):
        target = self.clock - lead
        if target < 0 or self.never is None:
            return value
        for start, result in reversed(self.history):
            if start <= target:
                v = min(result.shape[0] // 8 - 1, int(target - start) // 8)
                return jnp.where(self.never, result[8 * v:8 * v + 8], value)
        return value


def _kernel(
    shift_hbm, ssmd_hbm, beta_hbm, fwd_hbm, inv_hbm,
    q_hbm, k_hbm, v_hbm, ssm_hbm, x_hbm, wq_hbm, wk_hbm, wv_hbm, wo_hbm, out_hbm,
    shift_ref, ssmd_ref, beta_ref, fwd_ref, inv_ref,
    xs, wraw, wt, wot, qa, ka, va, ssk, spec_buf, yf, outa, outb,
    fwd, inv, gate, bias, qm, qd, pq, kk, vt, pk_keep, vt_keep, ot, mz, sem_in, sem_out,
):
    def w_copies(n, sem):
        return [
            pltpu.make_async_copy(src.at[:, pl.ds(n * T, T)], wraw.at[i, n], sem)
            for i, src in enumerate((wq_hbm, wk_hbm, wv_hbm))
        ]

    def x_copies(lo, hi, sem):
        rows = pl.ds(lo * L, (hi - lo) * L)
        return [
            pltpu.make_async_copy(x_hbm.at[0, rows, pl.ds(c * T, T)], xs.at[c, rows], sem)
            for c in range(NC)
        ]

    loads = [
        w_copies(0, sem_in.at[0]),
        x_copies(0, 1, sem_in.at[1])
        + [pltpu.make_async_copy(beta_hbm, beta_ref, sem_in.at[1])],
        w_copies(1, sem_in.at[2]),
        sum((w_copies(n, sem_in.at[3]) for n in range(2, NC)), []),
        x_copies(1, 2, sem_in.at[4]),
        [pltpu.make_async_copy(src, dst, sem_in.at[5]) for src, dst in (
            (shift_hbm, shift_ref), (ssmd_hbm, ssmd_ref), (fwd_hbm, fwd_ref), (inv_hbm, inv_ref),
            (k_hbm.at[0], ka), (v_hbm.at[0], va), (ssm_hbm, ssk))]
        + [pltpu.make_async_copy(wo_hbm.at[:, pl.ds(n * T, T)], wraw.at[3, n], sem_in.at[5])
           for n in range(NC)],
        x_copies(2, NSEG, sem_in.at[6]),
        [pltpu.make_async_copy(q_hbm.at[0], qa, sem_in.at[7])],
    ]
    for copies in loads:
        for cp in copies:
            cp.start()

    def wait(i):
        for cp in loads[i]:
            cp.wait()

    mz[...] = jnp.zeros(mz.shape, f32)
    row = lax.broadcasted_iota(i32, (T // 2, T), 0)
    col = lax.broadcasted_iota(i32, (T // 2, T), 1)
    bias[0] = jnp.where(row <= col, 0.0, NEG)
    bias[1] = jnp.where(row <= col % (T // 2), 0.0, NEG)

    def setup_gate():
        beta = jnp.concatenate(
            [beta_ref[...].astype(f32)[None, :], jnp.zeros((1, T - H), f32)], axis=1)
        gate[...] = jax.nn.sigmoid(jnp.broadcast_to(beta, (T, T)).T[:H])

    def transpose_qkv(n):
        for i in range(3):
            for c in range(NC):
                wt[i, c, n * T // 2:(n + 1) * T // 2, :] = pltpu.bitcast(
                    wraw[i, n, c * T:(c + 1) * T, :].T, u32)

    def transpose_wo(n):
        for c in range(NC):
            wot[c, n * T // 2:(n + 1) * T // 2, :] = pltpu.bitcast(
                wraw[3, n, c * T:(c + 1) * T, :].T, u32)

    sub = lax.broadcasted_iota(i32, (8, T), 0)
    low = sub < 4
    left = lax.broadcasted_iota(i32, (8, T), 1) < T // 2

    def project(s, g, slot, pacer):
        rows = _ds(g * (GW // 2), GW // 2, 8)
        acc = [None] * NQ

        def store(n):
            q_t, k_t, v_t = acc[n][:GW], acc[n][GW:2 * GW], acc[n][2 * GW:]
            k_pad = jnp.concatenate([k_t.astype(bf16), jnp.zeros((T - GW, T), bf16)], axis=0)
            kk[slot, n] = pltpu.bitcast(k_pad.T, u32)
            qs = q_t * (DH ** -0.5 * LOG2E)
            r = [qs[8 * i:8 * i + 8] for i in range(10)]
            zero = jnp.zeros((8, T), f32)
            heads = [
                r[0], r[1], jnp.where(low, r[2], 0.0), zero,
                jnp.where(low, 0.0, r[2]), r[3], r[4], zero,
                zero, r[5], r[6], jnp.where(low, r[7], 0.0),
                zero, jnp.where(low, 0.0, r[7]), r[8], r[9],
            ]
            qm[slot, n] = _as_words(jnp.concatenate(heads, axis=0))
            e = {i: jnp.where(left, pltpu.roll(r[i], 64, 1), 0.0) for i in (0, 1, 2, 5, 6, 7)}
            o = {i: jnp.where(left, 0.0, r[i]) for i in (2, 3, 4, 7, 8, 9)}
            pairs = [
                e[0], e[1], jnp.where(low, e[2], o[2]), o[3], o[4], zero,
                zero, e[5], e[6], jnp.where(low, e[7], o[7]), o[8], o[9],
            ]
            qd[slot, n] = _as_words(jnp.concatenate(pairs, axis=0))
            pq[slot, n] = _as_words(_phi(q_t))
            pk_keep[s % 2, g, n] = _as_words(_phi(k_t))
            vt[slot, n] = v_t
            vt_keep[s % 2, g, n] = v_t

        def step(i):
            for lane in range(4):
                n, c = divmod(4 * i + lane, NC)
                w = _as_bf16(jnp.concatenate([wt[m, c, rows, :] for m in range(3)], axis=0))
                if XB:
                    xt = _as_bf16(xs.bitcast(u32)[c, _ds((s * L + n * T) // 2, T // 2, T // 2), :])
                else:
                    xt = xs[c, _ds(s * L + n * T, T, T), :]
                part = _dot_nt(w, xt)
                pacer.issued(part, lane, WP)
                acc[n] = part if c == 0 else acc[n] + part
                if c == NC - 1:
                    store(n)

        return step

    def masked_dot(key_words, window, first):
        end = first + window.shape[0]
        parts = [jnp.zeros((first, T), bf16), window, jnp.zeros((T - end if FULLK else 0, T), bf16)]
        rhs = jnp.concatenate([p for p in parts if p.shape[0]], axis=0)
        return _dot(_as_bf16(key_words)[:, :rhs.shape[0]], rhs)

    def attend(s, g, slot, pacer, memory):
        tiles = [(qt, kt) for qt in ORDER for kt in range(qt + 1)]
        logits, run_max, col_max, acc, mem, done = {}, {}, {}, {}, {}, []
        corner, corner_max, corner_p = {}, {}, {}
        gates = [jnp.broadcast_to(gate[pl.ds(4 * g + j, 1), :], (8, T)) for j in range(4)]

        low_pair = sub % 4 < 2
        rest_rows = 1.0 - jnp.where(low, jnp.where(low_pair, gates[1], gates[3]),
                                    jnp.where(low_pair, gates[0], gates[2]))

        def update(_):
            state = mz[g]
            for kt in range(NQ):
                v_one = jnp.concatenate(
                    [vt_keep[(s + 1) % 2, g, kt], jnp.ones((8, T), f32)], axis=0)
                pk_t = jnp.concatenate(
                    [_as_bf16(pk_keep[(s + 1) % 2, g, kt]), jnp.zeros((T - GW, T), bf16)], axis=0)
                part = _dot_nt(v_one, pk_t)
                pacer.issued(part, kt, WM)
                state = state + part
            mz[g] = state

        def read(_):
            def head_of(i):
                return (i >= DH).astype(i32) + (i >= 2 * DH).astype(i32) + (i >= 3 * DH).astype(i32)

            state = mz[g]
            row_m = lax.broadcasted_iota(i32, (GW, T), 0)
            col_m = lax.broadcasted_iota(i32, (GW, T), 1)
            weights = jnp.where(head_of(row_m) == head_of(col_m), state[:GW], 0.0)
            lane_head = head_of(lax.broadcasted_iota(i32, (8, T), 1))
            pair_of = sub // 2
            z_rows = jnp.where(lane_head == pair_of, state[GW:], 0.0)
            mem_w = jnp.concatenate([weights, z_rows], axis=0)
            g_rows = jnp.where(low, jnp.where(sub < 2, gates[0], gates[1]),
                               jnp.where(sub < 6, gates[2], gates[3]))
            for qt in range(NQ):
                rhs = _as_bf16(pq[slot, qt])
                if FULLK:
                    rhs = jnp.concatenate([rhs, jnp.zeros((T - GW, T), bf16)], axis=0)
                res = lax.dot_general(
                    mem_w[:, :rhs.shape[0]], rhs, NN, preferred_element_type=f32)
                pacer.issued(res, qt, WM)
                coef = g_rows / (res[GW:] + 1e-6)
                c0, c1, c2, c3 = (
                    jnp.broadcast_to(coef[2 * j:2 * j + 1], (8, T)) for j in range(4))
                cm = [c0, c0, jnp.where(low, c0, c1), c1, c1,
                      c2, c2, jnp.where(low, c2, c3), c3, c3]
                mem[qt] = [res[8 * i:8 * i + 8] * cm[i] for i in range(10)]
            finish()

        def corners(i):
            for lane in range(4):
                qt, pr = ORDER[2 * i + lane // 2], lane % 2
                window = _as_bf16(qd[slot, qt, 24 * pr:24 * pr + 24, :])
                sc = masked_dot(kk[slot, qt, T // 4:, :], window, 32 * pr)
                pacer.issued(sc, lane, WA)
                corner[qt, pr] = sc + bias[1]
                corner_max[qt, pr] = jnp.max(corner[qt, pr].reshape(8, 8, T), axis=0)

        def scores(t):
            qt, kt = tiles[t]
            for j in range(4):
                window = _as_bf16(qm[slot, qt, 16 * j:16 * j + 16, :])
                sc = masked_dot(
                    kk[slot, kt] if kt < qt else kk[slot, kt, :T // 4, :], window, 16 * j)
                pacer.issued(sc, j, WA)
                if kt == qt:
                    sc = sc + bias[0]
                m8 = jnp.max(sc.reshape(-1, 8, T), axis=0)
                run_max[qt, j] = m8 if kt == 0 else jnp.maximum(run_max[qt, j], m8)
                if kt == qt:
                    extra = corner_max[qt, j // 2]
                    if j % 2 == 0:
                        extra = pltpu.roll(extra, T // 2, 1)
                    top = jnp.maximum(run_max[qt, j], jnp.where(left, NEG, extra))
                    col_max[qt, j] = jnp.broadcast_to(
                        jnp.max(top, axis=0, keepdims=True), (8, T))
                logits[t, j] = sc
            if kt == qt:
                for pr in range(2):
                    top = jnp.where(left, pltpu.roll(col_max[qt, 2 * pr], T // 2, 1),
                                    col_max[qt, 2 * pr + 1])
                    words = _as_words(jnp.exp2(
                        corner[qt, pr].reshape(8, 8, T) - top[None]).reshape(T // 2, T))
                    for j, shifted in enumerate((pltpu.roll(words, T // 2, 1), words)):
                        corner_p[qt, 2 * pr + j] = _as_bf16(jnp.where(
                            left[None], jnp.uint32(0), shifted.reshape(4, 8, T)).reshape(32, T))

        def values(t):
            qt, kt = tiles[t]
            tops = [pacer.hold(col_max[qt, j], LEAD - STAG * j) for j in range(4)]
            for j in range(4):
                p = jnp.exp2(logits[t, j].reshape(-1, 8, T) - tops[j][None])
                p = p.reshape(-1, T).astype(bf16)
                if kt == qt:
                    p = jnp.concatenate([p, corner_p[qt, j]], axis=0)
                first = (0, 16, 40, 56)[j]
                v = [vt[slot, kt, first + 8 * i:first + 8 * i + 8, :] for i in range(3)]
                if j % 2 == 0:
                    v[2] = jnp.where(low, v[2], 1.0)
                else:
                    v[0] = jnp.where(low, 1.0, v[0])
                part = lax.dot_general(
                    jnp.concatenate(v, axis=0), p, NN, preferred_element_type=f32)
                pacer.issued(part, j)
                acc[qt, j] = part if kt == 0 else acc[qt, j] + part
            if kt == qt:
                done.append(qt)
                finish()

        def finish():
            while done and (not memory or done[0] in mem):
                qt = done.pop(0)
                w = [[acc[qt, j][8 * i:8 * i + 8] for i in range(3)] for j in range(4)]
                sums = jnp.where(
                    low_pair, jnp.where(low, w[1][0], w[0][2]),
                    pltpu.roll(jnp.where(low, w[3][0], w[2][2]), 2, 0))
                coef = rest_rows / sums
                c0, c1, c2, c3 = (
                    jnp.broadcast_to(coef[r:r + 1], (8, T)) for r in (4, 0, 6, 2))
                o = [w[0][0] * c0, w[0][1] * c0,
                     jnp.where(low, w[0][2] * c0, w[1][0] * c1), w[1][1] * c1, w[1][2] * c1,
                     w[2][0] * c2, w[2][1] * c2,
                     jnp.where(low, w[2][2] * c2, w[3][0] * c3), w[3][1] * c3, w[3][2] * c3]
                if memory:
                    o = [mem[qt][i] + o[i] for i in range(10)]
                ot[s % 2, qt, _ds(g * (GW // 2), GW // 2, 8), :] = _as_words(
                    jnp.concatenate(o, axis=0))

        return {"D": corners, "Q": scores, "V": values, "U": update, "R": read}

    def out_project(s, n, pacer):
        acc = [None] * 4

        def step(c):
            rhs = _as_bf16(ot[s % 2, n, c * 64:(c + 1) * 64, :])
            for m in range(4):
                part = _dot(_as_bf16(wot[c, 80 * m:80 * (m + 1), :]), rhs)
                pacer.issued(part, m, WO)
                acc[m] = part if c == 0 else acc[m] + part
            if c == NC - 1:
                res = jnp.concatenate(acc, axis=0).astype(bf16)
                for i in range(NC):
                    outb[s, _ds(n * T, T, T), i * T:(i + 1) * T] = res[i * T:(i + 1) * T].T

        return step

    def outb_copy(s, n):
        return pltpu.make_async_copy(
            outb.at[s, _ds(n * T, T, T)],
            out_hbm.at[0, _ds(s * L + n * T, T, T), pl.ds(D, D)],
            sem_out.at[NC])

    def conv_forward(c):
        cols = slice(c * T, (c + 1) * T)
        taps = shift_ref[:, cols].astype(f32)
        taps = [jnp.broadcast_to(taps[j:j + 1], (T, T)) for j in range(4)]
        skip = ssmd_ref[...].astype(f32)[c:c + 1]
        fmat = _as_bf16(fwd[...])
        slices = pl.ds(c * NFV, NFV)
        prev = None
        ktail = jnp.zeros((8, T), f32)
        for b in range(NB):
            rows = slice(b * T, (b + 1) * T)
            k0 = ka[rows, cols].astype(f32)
            ext = jnp.concatenate([ktail, k0], axis=0)
            ktail = k0[T - 8:]
            shifted = k0 * taps[0]
            for j in range(1, 4):
                shifted = shifted + ext[8 - j:8 + T - j] * taps[j]
            kv = (shifted * va[rows, cols].astype(f32)).astype(bf16)
            spec = _dot_nt(fmat, ssk[cols, rows]).reshape(NFV, 2, 8, T)
            spec_buf[slices, 0, b] = _dot(fmat, kv).reshape(NFV, 16, T)
            re, im = spec[:, 0], spec[:, 1]
            if prev is None:
                re2, im2 = re + skip[None], im
            else:
                half = NFV // 2
                pre, pim = prev
                re2 = jnp.concatenate([re[:half] - pim[:half], re[half:] + pim[half:]], axis=0)
                im2 = jnp.concatenate([im[:half] + pre[:half], im[half:] - pre[half:]], axis=0)
            prev = (re, im)
            spec_buf[slices, 1, b, 0:8, :] = re2
            spec_buf[slices, 1, b, 8:16, :] = im2

    def conv_mix(first, count, never, blk=4):
        for item in range(count):
            idx = first + item

            def load(which, b):
                return spec_buf[idx, which, b, 0:8, :], spec_buf[idx, which, b, 8:16, :]

            for a0 in range(0, NB, blk):
                acc = [None] * blk
                kcache = {}
                for b in range(a0 + blk):
                    token = yield
                    ur, ui = load(0, b)
                    ur = jnp.where(never, token, ur)
                    ui = jnp.where(never, token, ui)
                    us = ur + ui
                    for a in range(max(a0, b), a0 + blk):
                        if a - b not in kcache:
                            kr, ki = load(1, a - b)
                            kcache[a - b] = (kr, ki - kr, kr + ki)
                        k1, k2, k3 = kcache[a - b]
                        terms = (us * k1, ur * k2, ui * k3)
                        old = acc[a - a0]
                        acc[a - a0] = terms if old is None else tuple(
                            o + t for o, t in zip(old, terms))
                for i in range(blk):
                    p1, p2, p3 = acc[i]
                    yf[idx, a0 + i] = _as_words(jnp.concatenate([p1 - p3, p1 + p2], axis=0))

    def outa_copy(c):
        return pltpu.make_async_copy(
            outa.at[c], out_hbm.at[0, :, _ds(c * T, T, T)], sem_out.at[c])

    def conv_inverse(pacer):
        def step(i):
            c, a0 = divmod(2 * i, NB)
            for a in (a0, a0 + 1):
                spec = _as_bf16(yf[pl.ds(c * NFV, NFV), a].reshape(T, T))
                y = None
                for half in range(2):
                    part = _dot(_as_bf16(inv[half]), spec[half * T:(half + 1) * T])
                    pacer.issued(part, 2 * (a % 2) + half, WI)
                    y = part if y is None else y + part
                rows = slice(a * T, (a + 1) * T)
                outa[c, rows, :] = (qa[rows, c * T:(c + 1) * T].astype(f32) * y).astype(bf16)

        return step

    def pair(s, p, plan, mix=None):
        never = sub > 100 + p
        memory = "Ua" in plan
        if mix is None:
            pacer = _Pacer(never)
        else:
            first, count, cycles = mix
            pacer = _Pacer(never, conv_mix(first, count, never), count * 40 / cycles)
        steps = {"a": attend(s, 2 * p, 0, pacer, memory),
                 "b": attend(s, 2 * p + 1, 1, pacer, memory)}
        steps["a"]["P"] = project(s, 2 * p + 1, 1, pacer)
        steps["b"]["P"] = project(s + (p + 1) // 4, (2 * p + 2) % NG, 0, pacer)
        steps["a"]["O"] = out_project(s - 1, p, pacer)
        steps["x"] = {
            "T": transpose_qkv,
            "W": wait,
            "A": lambda c: outa_copy(c).start(),
            "B": lambda c: outa_copy(c).wait(),
            "I": conv_inverse(pacer),
            "C": lambda _: outb_copy(s - 1, p).start(),
        }
        last = {}

        def final(i):
            n, c = divmod(i, NC)
            if c == 0:
                last[n] = out_project(s, n, pacer)
            last[n](c)

        steps["x"]["E"] = final
        steps["x"]["F"] = lambda n: outb_copy(s, n).start()
        for item in plan:
            steps[item[1]][item[0]](int(item[2:] or 0))
        assert pacer.side is None

    if ONLY:
        for i in range(8):
            wait(i)
        setup_gate()
        if ONLY == "0":
            @pl.loop(1, 4)
            def _(p):
                pair(0, p, PLAN0)
        else:
            @pl.loop(0, 11)
            def _(i):
                cycles = 2 * (1152 * WA + 1200 * WP + 176 * WM) + 800 * WO
                pair(1 + i // 4, i % 4, PLAN1, (i * MIX_PER_ITER, MIX_PER_ITER, cycles * SLACK))
        outa[0, 0:16] = jnp.concatenate([mz[0, 0:8], pltpu.bitcast(ot[0, 0, 0:8] + yf[0, 0] + qm[0, 0, 0:8] + qd[0,0,0:8] + pq[0,0,0:8] + kk[0,0,0:8] + pk_keep[0,0,0,0:8], f32) + vt[0,0,0:8] + vt_keep[0,0,0,0:8]], axis=0).astype(bf16)
        outa_copy(0).start()
        outa_copy(0).wait()
        return

    wait(0)
    transpose_qkv(0)
    wait(1)
    setup_gate()
    step = project(0, 0, 0, _Pacer(None))
    for i in range(NC):
        step(i)
    pair(0, 0, PLAN_FIRST)
    wait(4)

    @pl.loop(1, 4)
    def _(p):
        pair(0, p, PLAN0)

    wait(5)
    fwd[...] = pltpu.bitcast(fwd_ref[...], u32)
    for half in range(2):
        inv[half] = pltpu.bitcast(inv_ref[half], u32)
    for c in range(NC):
        conv_forward(c)
        transpose_wo(c)
    wait(6)

    @pl.loop(0, 11)
    def _(i):
        cycles = 2 * (1152 * WA + 1200 * WP + 176 * WM) + 800 * WO
        pair(1 + i // 4, i % 4, PLAN1, (i * MIX_PER_ITER, MIX_PER_ITER, cycles * SLACK))

    wait(7)
    pair(NSEG - 1, 3, PLAN_LAST, (11 * MIX_PER_ITER, NC * NFV - 11 * MIX_PER_ITER, 4500))

    for s in range(NSEG):
        for n in range(NQ):
            outb_copy(s, n).wait()


@jax.jit
def pallas_concat_heads__ssm_conv_h3__memory_aug_infini_attn__prompt_kernel(
    A_q: jax.Array,
    A_k: jax.Array,
    A_v: jax.Array,
    A_shift_k: jax.Array,
    A_ssm_k: jax.Array,
    A_ssm_D: jax.Array,
    B_x: jax.Array,
    B_wq: jax.Array,
    B_wk: jax.Array,
    B_wv: jax.Array,
    B_wo: jax.Array,
    B_beta: jax.Array,
):
    hbm = pl.BlockSpec(memory_space=pl.ANY)
    scratch = [
        pltpu.VMEM((4, D), bf16),
        pltpu.VMEM((NC, T), bf16),
        pltpu.VMEM((H,), bf16),
        pltpu.VMEM((2 * T, T), bf16),
        pltpu.VMEM((2, T, T), bf16),
        pltpu.VMEM((NC, S, T), bf16),
        pltpu.VMEM((4, NC, D, T), bf16),
        pltpu.VMEM((3, NC, D // 2, T), u32),
        pltpu.VMEM((NC, D // 2, T), u32),
        pltpu.VMEM((S, D), bf16),
        pltpu.VMEM((S, D), bf16),
        pltpu.VMEM((S, D), bf16),
        pltpu.VMEM((D, S), bf16),
        pltpu.VMEM((NC * NFV, 2, NB, 16, T), f32),
        pltpu.VMEM((NC * NFV, NB, 8, T), u32),
        pltpu.VMEM((NC, S, T), bf16),
        pltpu.VMEM((NSEG, L, D), bf16),
        pltpu.VMEM((T, T), u32),
        pltpu.VMEM((2, T // 2, T), u32),
        pltpu.VMEM((H, T), f32),
        pltpu.VMEM((2, T // 2, T), f32),
        pltpu.VMEM((2, NQ, 64, T), u32),
        pltpu.VMEM((2, NQ, 48, T), u32),
        pltpu.VMEM((2, NQ, GW // 2, T), u32),
        pltpu.VMEM((2, NQ, T // 2, T), u32),
        pltpu.VMEM((2, NQ, GW, T), f32),
        pltpu.VMEM((2, NG, NQ, GW // 2, T), u32),
        pltpu.VMEM((2, NG, NQ, GW, T), f32),
        pltpu.VMEM((2, NQ, D // 2, T), u32),
        pltpu.VMEM((NG, GW + 8, T), f32),
        pltpu.SemaphoreType.DMA((8,)),
        pltpu.SemaphoreType.DMA((NC + 1,)),
    ]
    return pl.pallas_call(
        _kernel,
        out_shape=jax.ShapeDtypeStruct((1, S, 2 * D), bf16),
        in_specs=[hbm] * 14,
        out_specs=hbm,
        scratch_shapes=scratch,
        compiler_params=pltpu.CompilerParams(vmem_limit_bytes=100 * 2**20),
    )(
        A_shift_k.T, A_ssm_D.reshape(NC, T), B_beta, _FWD, _INV,
        A_q, A_k, A_v, A_ssm_k, B_x, B_wq, B_wk, B_wv, B_wo,
    )
```

```python
import os
import jax
import jax.numpy as jnp
import numpy as np
from jax import lax
from jax.experimental import pallas as pl
from jax.experimental.pallas import tpu as pltpu

f32, bf16, u32, i32 = jnp.float32, jnp.bfloat16, jnp.uint32, jnp.int32

S, D, H, DH = 2048, 640, 32, 20
NSEG, L = 4, 512
T = 128
NC = D // T
NB = S // (2 * T)
NQ = L // T
NG = 8
GW = 4 * DH
NFV = 16
LOG2E = 1.4426950408889634
NEG = -1e30
MIX_PER_ITER = 7

def _env(name, default):
    return type(default)(os.environ.get(name, default))
WA, WP, WO, WM = _env("WA", 1.0), _env("WP", 1.0), _env("WO", 1.0), _env("WM", 1.2)
SLACK = _env("SLACK", 0.965)
LEAD0, LEAD1 = _env("LEAD0", 400), _env("LEAD1", 400)
STAG0, STAG1 = _env("STAG0", 56), _env("STAG1", 32)
PF32 = _env("PF32", 0)
XB = _env("XB", 1)
FULLK = _env("FULLK", 1)
RHS32 = _env("RHS32", 1)
ONLY = _env("ONLY", "")
PLAN0 = _env("PLAN0",
    "Qa0 Da0 Pa0 Qa1 Pa1 Qa2 Qa3 Pa2 Pa3 Qa4 Va0 Va1 Qa5 Qa6 Pa4 Da1 Va2 Qa7 Va3 Qa8 Qa9 Va4 Qb0 Va5 "
    "Qb1 Va6 Db0 Va7 Qb2 Va8 Qb3 Va9 Qb4 Pb0 Qb5 Vb0 Vb1 Qb6 Vb2 Db1 Vb3 Qb7 Pb1 Pb2 Vb4 Qb8 Vb5 Qb9 "
    "Pb3 Pb4 Vb6 Vb7 Vb8 Vb9").split()
PLAN1 = _env("PLAN1",
    "Qa0 Da0 Pa0 Qa1 Pa1 Qa2 Pa2 Qa3 Pa3 Pa4 Qa4 Qa5 Va0 Va1 Oa0 Qa6 Va2 Qa7 Oa1 Da1 Va3 Oa2 Qa8 Oa3 "
    "Va4 Va5 Qa9 Oa4 Ra Ua Va6 Qb0 Va7 Qb1 Db0 Qb2 Va8 Qb3 Va9 Vb0 Pb0 Qb4 Pb1 Qb5 Qb6 Db1 Vb1 Vb2 "
    "Qb7 Vb3 Pb2 Qb8 Vb4 Vb5 Qb9 Pb3 Vb6 Pb4 Vb7 Rb Vb8 Vb9 Ub Cx").split()
WI = 1.0
PLAN_FIRST = _env("PLAN_FIRST",
    "Wx2 Qa0 Da0 Qa1 Tx1 Qa2 Qa3 Qa4 Va0 Qa5 Va1 Qa6 Va2 Pa0 Qa7 Da1 Va3 Pa1 Qa8 Va4 Pa2 Qa9 Va5 Pa3 Va6 Pa4 Va7 Wx3 Qb0 Db0 Va8 Tx2 "
    "Qb1 Va9 Qb2 Qb3 Tx3 Qb4 Vb0 Pb0 Qb5 Vb1 Pb1 Tx4 Qb6 Vb2 Qb7 Db1 Vb3 Pb2 Qb8 Vb4 Qb9 Vb5 Pb3 Vb6 Pb4 Vb7 Vb8 Vb9").split()
PLAN_LAST = _env("PLAN_LAST",
    "Qa0 Da0 Pa0 Qa1 Pa1 Qa2 Pa2 Qa3 Pa3 Qa4 Va0 Pa4 Qa5 Va1 Oa0 Qa6 Va2 Oa1 Qa7 Da1 Va3 Oa2 Qa8 Va4 Oa3 Qa9 Va5 "
    "Oa4 Ua Qb0 Va6 Ra Ix0 Qb1 Db0 Va7 Ix1 Qb2 Va8 Ix2 Qb3 Va9 Ix3 Qb4 Vb0 Ix4 Qb5 Vb1 Ix5 Qb6 Vb2 Ix6 Qb7 Db1 Vb3 "
    "Ix7 Qb8 Vb4 Ix8 Qb9 Vb5 Ix9 Ix10 Rb Vb6 Ix11 Ix12 Vb7 Ix13 Vb8 Ix14 Vb9 Ix15 Cx Ax0 Ax1 Bx0 "
    + " ".join(f"Ix{i}" for i in range(16, 32)) + " Ax2 Ax3 Bx1 "
    + " ".join(f"Ex{i} Ix{32 + i}" for i in range(8)) + " Ax4 Fx0 Bx2 "
    + " ".join(f"Ex{i}" for i in range(8, 20)) + " Fx1 Fx2 Fx3 Bx3 Bx4").split()
ORDER = [int(v) for v in _env("ORDER", "3,2,1,0").split(",")]

NN = (((1,), (0,)), ((), ()))
NT = (((1,), (1,)), ((), ()))


def _dft_tables():
    freq = np.concatenate([np.arange(0, T, 2), np.arange(1, T, 2)])
    fwd = []
    for parity in range(2):
        n = 2 * np.arange(T) + parity
        theta = 2.0 * np.pi * (freq[:, None] + 0.5) * n[None, :] / (4 * T)
        re, im = np.cos(theta), -np.sin(theta)
        fwd.append(np.stack(
            [re.reshape(NFV, 8, T), im.reshape(NFV, 8, T)], axis=1).reshape(2 * T, T))
    fwd = np.stack(fwd)
    inv = fwd.transpose(0, 2, 1) / (2 * T)
    inv = np.concatenate([inv[:, :, :T], inv[:, :, T:]], axis=1).reshape(4, T, T)
    return fwd.astype(np.float32).astype(bf16), inv.astype(np.float32).astype(bf16)


_FWD, _INV = _dft_tables()


def _as_bf16(words):
    return pltpu.bitcast(words, bf16)


def _as_words(x):
    return pltpu.bitcast(x.astype(bf16), u32)


def _even_rows(words):
    return pltpu.bitcast(words << 16, f32)


def _odd_rows(words):
    return pltpu.bitcast(words & np.uint32(0xFFFF0000), f32)


def _interleave(even, odd):
    even, odd = (pltpu.bitcast(x.astype(bf16).astype(f32), u32) for x in (even, odd))
    return pltpu.bitcast((even >> 16) | odd, bf16)


def _dot(a, b):
    return jnp.dot(a, b, preferred_element_type=f32)


def _dot_nt(a, b):
    return lax.dot_general(a, b, NT, preferred_element_type=f32)


def _phi(t):
    return jnp.maximum(t, 0.0) + jnp.exp(jnp.minimum(t, 0.0))


def _ds(start, size, align):
    if isinstance(start, int):
        return pl.ds(start, size)
    return pl.ds(pl.multiple_of(start, align), size)


class _Pacer:
    def __init__(self, never, side=None, rate=0.0):
        self.never, self.side, self.rate = never, side, rate
        self.credit, self.clock, self.history = 0.0, 0.0, []
        if side is not None:
            next(side)

    def issued(self, result, lane, weight=0.0):
        rows = result.shape[0]
        self.history.append((self.clock, result))
        if lane == 3:
            self.clock += rows
        self.credit += self.rate * rows / 4 * weight
        count = int(self.credit)
        self.credit -= count
        for i in range(count):
            if self.side is not None:
                v = min(rows // 8 - 1, int(rows // 8 * (lane + (i + 0.5) / count) / 4))
                try:
                    self.side.send(result[8 * v:8 * v + 8])
                except StopIteration:
                    self.side = None

    def hold(self, value, lead):
        target = self.clock - lead
        if target < 0 or self.never is None:
            return value
        for start, result in reversed(self.history):
            if start <= target:
                v = min(result.shape[0] // 8 - 1, int(target - start) // 8)
                return jnp.where(self.never, result[8 * v:8 * v + 8], value)
        return value


def _kernel(
    shift_hbm, ssmd_hbm, beta_hbm, fwd_hbm, inv_hbm,
    q_hbm, k_hbm, v_hbm, ssm_hbm, x_hbm, wq_hbm, wk_hbm, wv_hbm, wo_hbm, out_hbm,
    shift_ref, ssmd_ref, beta_ref, fwd_ref, inv_ref,
    xs, wraw, wt, wot, qa, ka, va, ssk, spec_buf, yf, outa, outb,
    fwd, inv, gate, bias, qm, qd, pq, kk, vt, pk_keep, vt_keep, ot, mz, sem_in, sem_out,
):
    def w_copies(n, sem):
        return [
            pltpu.make_async_copy(src.at[:, pl.ds(n * T, T)], wraw.at[i, n], sem)
            for i, src in enumerate((wq_hbm, wk_hbm, wv_hbm))
        ]

    def x_copies(lo, hi, sem):
        rows = pl.ds(lo * L, (hi - lo) * L)
        return [
            pltpu.make_async_copy(x_hbm.at[0, rows, pl.ds(c * T, T)], xs.at[c, rows], sem)
            for c in range(NC)
        ]

    loads = [
        w_copies(0, sem_in.at[0]),
        x_copies(0, 1, sem_in.at[1])
        + [pltpu.make_async_copy(beta_hbm, beta_ref, sem_in.at[1])],
        w_copies(1, sem_in.at[2]),
        sum((w_copies(n, sem_in.at[3]) for n in range(2, NC)), []),
        x_copies(1, 2, sem_in.at[4]),
        [pltpu.make_async_copy(src, dst, sem_in.at[5]) for src, dst in (
            (shift_hbm, shift_ref), (ssmd_hbm, ssmd_ref), (fwd_hbm, fwd_ref), (inv_hbm, inv_ref),
            (k_hbm.at[0], ka), (v_hbm.at[0], va), (ssm_hbm, ssk))]
        + [pltpu.make_async_copy(wo_hbm.at[:, pl.ds(n * T, T)], wraw.at[3, n], sem_in.at[5])
           for n in range(NC)],
        x_copies(2, NSEG, sem_in.at[6]),
        [pltpu.make_async_copy(q_hbm.at[0], qa, sem_in.at[7])],
    ]
    for copies in loads:
        for cp in copies:
            cp.start()

    def wait(i):
        for cp in loads[i]:
            cp.wait()

    mz[...] = jnp.zeros(mz.shape, f32)
    row = lax.broadcasted_iota(i32, (T // 2, T), 0)
    col = lax.broadcasted_iota(i32, (T // 2, T), 1)
    bias[0] = jnp.where(row <= col, 0.0, NEG)
    bias[1] = jnp.where(row <= col % (T // 2), 0.0, NEG)

    def setup_gate():
        beta = jnp.concatenate(
            [beta_ref[...].astype(f32)[None, :], jnp.zeros((1, T - H), f32)], axis=1)
        gate[...] = jax.nn.sigmoid(jnp.broadcast_to(beta, (T, T)).T[:H])

    def transpose_qkv(n):
        for i in range(3):
            for c in range(NC):
                wt[i, c, n * T // 2:(n + 1) * T // 2, :] = pltpu.bitcast(
                    wraw[i, n, c * T:(c + 1) * T, :].T, u32)

    def transpose_wo(n):
        for c in range(NC):
            wot[c, n * T // 2:(n + 1) * T // 2, :] = pltpu.bitcast(
                wraw[3, n, c * T:(c + 1) * T, :].T, u32)

    sub = lax.broadcasted_iota(i32, (8, T), 0)
    low = sub < 4
    left = lax.broadcasted_iota(i32, (8, T), 1) < T // 2

    def project(s, g, slot, pacer):
        rows = _ds(g * (GW // 2), GW // 2, 8)
        acc = [None] * NQ

        def store(n):
            q_t, k_t, v_t = acc[n][:GW], acc[n][GW:2 * GW], acc[n][2 * GW:]
            k_pad = jnp.concatenate([k_t.astype(bf16), jnp.zeros((T - GW, T), bf16)], axis=0)
            kk[slot, n] = pltpu.bitcast(k_pad.T, u32)
            qs = q_t * (DH ** -0.5 * LOG2E)
            r = [qs[8 * i:8 * i + 8] for i in range(10)]
            zero = jnp.zeros((8, T), f32)
            heads = [
                r[0], r[1], jnp.where(low, r[2], 0.0), zero,
                jnp.where(low, 0.0, r[2]), r[3], r[4], zero,
                zero, r[5], r[6], jnp.where(low, r[7], 0.0),
                zero, jnp.where(low, 0.0, r[7]), r[8], r[9],
            ]
            qm[slot, n] = _as_words(jnp.concatenate(heads, axis=0))
            e = {i: jnp.where(left, pltpu.roll(r[i], 64, 1), 0.0) for i in (0, 1, 2, 5, 6, 7)}
            o = {i: jnp.where(left, 0.0, r[i]) for i in (2, 3, 4, 7, 8, 9)}
            pairs = [
                e[0], e[1], jnp.where(low, e[2], o[2]), o[3], o[4], zero,
                zero, e[5], e[6], jnp.where(low, e[7], o[7]), o[8], o[9],
            ]
            qd[slot, n] = _as_words(jnp.concatenate(pairs, axis=0))
            pq[slot, n] = _as_words(_phi(q_t))
            pk_keep[s % 2, g, n] = _as_words(_phi(k_t))
            vt[slot, n] = v_t
            vt_keep[s % 2, g, n] = v_t

        def step(i):
            for lane in range(4):
                n, c = divmod(4 * i + lane, NC)
                w = _as_bf16(jnp.concatenate([wt[m, c, rows, :] for m in range(3)], axis=0))
                if XB:
                    xt = _as_bf16(xs.bitcast(u32)[c, _ds((s * L + n * T) // 2, T // 2, T // 2), :])
                else:
                    xt = xs[c, _ds(s * L + n * T, T, T), :]
                part = _dot_nt(w, xt)
                pacer.issued(part, lane, WP)
                acc[n] = part if c == 0 else acc[n] + part
                if c == NC - 1:
                    store(n)

        return step

    def masked_dot(key_words, window, first):
        end = first + window.shape[0]
        parts = [jnp.zeros((first, T), bf16), window, jnp.zeros((T - end if FULLK else 0, T), bf16)]
        rhs = jnp.concatenate([p for p in parts if p.shape[0]], axis=0)
        return _dot(_as_bf16(key_words)[:, :rhs.shape[0]], rhs)

    def update(s, g, pacer):
        state = mz[g]
        for kt in range(NQ):
            v_one = jnp.concatenate(
                [vt_keep[(s + 1) % 2, g, kt], jnp.ones((8, T), f32)], axis=0)
            pk_t = jnp.concatenate(
                [_as_bf16(pk_keep[(s + 1) % 2, g, kt]), jnp.zeros((T - GW, T), bf16)], axis=0)
            part = _dot_nt(v_one, pk_t)
            pacer.issued(part, kt, WM)
            state = state + part
        mz[g] = state

    def attend(s, g, slot, pacer, memory):
        lead, stagger = (LEAD1, STAG1) if memory else (LEAD0, STAG0)
        tiles = [(qt, kt) for qt in ORDER for kt in range(qt + 1)]
        logits, run_max, col_max, acc, mem, done = {}, {}, {}, {}, {}, []
        corner, corner_max, corner_p = {}, {}, {}
        gates = [jnp.broadcast_to(gate[pl.ds(4 * g + j, 1), :], (8, T)) for j in range(4)]

        low_pair = sub % 4 < 2
        rest_rows = 1.0 - jnp.where(low, jnp.where(low_pair, gates[1], gates[3]),
                                    jnp.where(low_pair, gates[0], gates[2]))

        def read(_):
            def head_of(i):
                return (i >= DH).astype(i32) + (i >= 2 * DH).astype(i32) + (i >= 3 * DH).astype(i32)

            state = mz[g]
            row_m = lax.broadcasted_iota(i32, (GW, T), 0)
            col_m = lax.broadcasted_iota(i32, (GW, T), 1)
            weights = jnp.where(head_of(row_m) == head_of(col_m), state[:GW], 0.0)
            lane_head = head_of(lax.broadcasted_iota(i32, (8, T), 1))
            pair_of = sub // 2
            z_rows = jnp.where(lane_head == pair_of, state[GW:], 0.0)
            mem_w = jnp.concatenate([weights, z_rows], axis=0)
            g_rows = jnp.where(low, jnp.where(sub < 2, gates[0], gates[1]),
                               jnp.where(sub < 6, gates[2], gates[3]))
            for qt in range(NQ):
                rhs = _as_bf16(pq[slot, qt])
                if FULLK:
                    rhs = jnp.concatenate([rhs, jnp.zeros((T - GW, T), bf16)], axis=0)
                res = lax.dot_general(
                    mem_w[:, :rhs.shape[0]], rhs, NN, preferred_element_type=f32)
                pacer.issued(res, qt, WM)
                coef = g_rows / (res[GW:] + 1e-6)
                c0, c1, c2, c3 = (
                    jnp.broadcast_to(coef[2 * j:2 * j + 1], (8, T)) for j in range(4))
                cm = [c0, c0, jnp.where(low, c0, c1), c1, c1,
                      c2, c2, jnp.where(low, c2, c3), c3, c3]
                mem[qt] = [res[8 * i:8 * i + 8] * cm[i] for i in range(10)]
            finish()

        def corners(i):
            for lane in range(4):
                qt, pr = ORDER[2 * i + lane // 2], lane % 2
                window = _as_bf16(qd[slot, qt, 24 * pr:24 * pr + 24, :])
                sc = masked_dot(kk[slot, qt, T // 4:, :], window, 32 * pr)
                pacer.issued(sc, lane, WA)
                corner[qt, pr] = sc + bias[1]
                corner_max[qt, pr] = jnp.max(corner[qt, pr].reshape(8, 8, T), axis=0)

        def scores(t):
            qt, kt = tiles[t]
            for j in range(4):
                window = _as_bf16(qm[slot, qt, 16 * j:16 * j + 16, :])
                sc = masked_dot(
                    kk[slot, kt] if kt < qt else kk[slot, kt, :T // 4, :], window, 16 * j)
                pacer.issued(sc, j, WA)
                if kt == qt:
                    sc = sc + bias[0]
                m8 = jnp.max(sc.reshape(-1, 8, T), axis=0)
                run_max[qt, j] = m8 if kt == 0 else jnp.maximum(run_max[qt, j], m8)
                if kt == qt:
                    extra = corner_max[qt, j // 2]
                    if j % 2 == 0:
                        extra = pltpu.roll(extra, T // 2, 1)
                    top = jnp.maximum(run_max[qt, j], jnp.where(left, NEG, extra))
                    col_max[qt, j] = jnp.broadcast_to(
                        jnp.max(top, axis=0, keepdims=True), (8, T))
                logits[t, j] = sc
            if kt == qt:
                for pr in range(2):
                    top = jnp.where(left, pltpu.roll(col_max[qt, 2 * pr], T // 2, 1),
                                    col_max[qt, 2 * pr + 1])
                    words = _as_words(jnp.exp2(
                        corner[qt, pr].reshape(8, 8, T) - top[None]).reshape(T // 2, T))
                    for j, shifted in enumerate((pltpu.roll(words, T // 2, 1), words)):
                        corner_p[qt, 2 * pr + j] = _as_bf16(jnp.where(
                            left[None], jnp.uint32(0), shifted.reshape(4, 8, T)).reshape(32, T))

        def values(t):
            qt, kt = tiles[t]
            tops = [pacer.hold(col_max[qt, j], lead - stagger * j) for j in range(4)]
            for j in range(4):
                p = jnp.exp2(logits[t, j].reshape(-1, 8, T) - tops[j][None])
                p = p.reshape(-1, T).astype(bf16)
                if kt == qt:
                    p = jnp.concatenate([p, corner_p[qt, j]], axis=0)
                first = (0, 16, 40, 56)[j]
                v = [vt[slot, kt, first + 8 * i:first + 8 * i + 8, :] for i in range(3)]
                if j % 2 == 0:
                    v[2] = jnp.where(low, v[2], 1.0)
                else:
                    v[0] = jnp.where(low, 1.0, v[0])
                part = lax.dot_general(
                    jnp.concatenate(v, axis=0), p, NN, preferred_element_type=f32)
                pacer.issued(part, j)
                acc[qt, j] = part if kt == 0 else acc[qt, j] + part
            if kt == qt:
                done.append(qt)
                finish()

        def finish():
            while done and (not memory or done[0] in mem):
                qt = done.pop(0)
                w = [[acc[qt, j][8 * i:8 * i + 8] for i in range(3)] for j in range(4)]
                sums = jnp.where(
                    low_pair, jnp.where(low, w[1][0], w[0][2]),
                    pltpu.roll(jnp.where(low, w[3][0], w[2][2]), 2, 0))
                coef = rest_rows / sums
                c0, c1, c2, c3 = (
                    jnp.broadcast_to(coef[r:r + 1], (8, T)) for r in (4, 0, 6, 2))
                o = [w[0][0] * c0, w[0][1] * c0,
                     jnp.where(low, w[0][2] * c0, w[1][0] * c1), w[1][1] * c1, w[1][2] * c1,
                     w[2][0] * c2, w[2][1] * c2,
                     jnp.where(low, w[2][2] * c2, w[3][0] * c3), w[3][1] * c3, w[3][2] * c3]
                if memory:
                    o = [mem[qt][i] + o[i] for i in range(10)]
                ot[s % 2, qt, _ds(g * (GW // 2), GW // 2, 8), :] = _as_words(
                    jnp.concatenate(o, axis=0))

        return {"D": corners, "Q": scores, "V": values, "R": read}

    def out_project(s, n, pacer):
        acc = [None] * 4

        def step(c):
            rhs = _as_bf16(ot[s % 2, n, c * 64:(c + 1) * 64, :])
            for m in range(4):
                part = _dot(_as_bf16(wot[c, 80 * m:80 * (m + 1), :]), rhs)
                pacer.issued(part, m, WO)
                acc[m] = part if c == 0 else acc[m] + part
            if c == NC - 1:
                res = jnp.concatenate(acc, axis=0).astype(bf16)
                for i in range(NC):
                    outb[s, _ds(n * T, T, T), i * T:(i + 1) * T] = res[i * T:(i + 1) * T].T

        return step

    def outb_copy(s, n):
        return pltpu.make_async_copy(
            outb.at[s, _ds(n * T, T, T)],
            out_hbm.at[0, _ds(s * L + n * T, T, T), pl.ds(D, D)],
            sem_out.at[NC])

    def conv_forward(c):
        cols = slice(c * T, (c + 1) * T)
        taps = shift_ref[:, cols].astype(f32)
        taps = [jnp.broadcast_to(taps[j:j + 1], (T, T)) for j in range(4)]
        skip = ssmd_ref[...].astype(f32)[c:c + 1]
        slices = pl.ds(c * NFV, NFV)

        def transform(even, odd):
            if not RHS32:
                even, odd = even.astype(bf16), odd.astype(bf16)
            e, o = (
                lax.dot_general(_as_bf16(fwd[i]), x, NN, preferred_element_type=f32)
                for i, x in enumerate((even, odd)))
            return [x.reshape(NFV, 2, 8, T) for x in (e + o, e - o)]

        tail = jnp.zeros((8, T), u32)
        prev = None
        for b in range(NB):
            rows = slice(2 * b * T, 2 * (b + 1) * T)
            taps_t = jnp.concatenate([
                pltpu.bitcast(ssk[cols, (2 * b + i) * T:(2 * b + i + 1) * T].T, u32)
                for i in range(2)], axis=0)
            filt = transform(_even_rows(taps_t), _odd_rows(taps_t))
            k0 = pltpu.bitcast(ka[rows, cols], u32)
            ext = jnp.concatenate([tail, k0], axis=0)
            tail = k0[T - 8:]
            k1, k2 = ext[7:7 + T], ext[6:6 + T]
            e0, o0, e1, o1, o2 = (
                _even_rows(k0), _odd_rows(k0), _even_rows(k1), _odd_rows(k1), _odd_rows(k2))
            v0 = pltpu.bitcast(va[rows, cols], u32)
            sig = transform(
                (e0 * taps[0] + o1 * taps[1] + e1 * taps[2] + o2 * taps[3]) * _even_rows(v0),
                (o0 * taps[0] + e0 * taps[1] + o1 * taps[2] + e1 * taps[3]) * _odd_rows(v0))
            for sign in range(2):
                spec_buf[slices, 0, sign, b] = sig[sign].reshape(NFV, 16, T)
                re, im = filt[sign][:, 0], filt[sign][:, 1]
                if prev is None:
                    re = re + skip[None]
                else:
                    half = NFV // 2
                    pre, pim = prev[sign][:, 0], prev[sign][:, 1]
                    re = jnp.concatenate([re[:half] - pim[:half], re[half:] + pim[half:]], axis=0)
                    im = jnp.concatenate([im[:half] + pre[:half], im[half:] - pre[half:]], axis=0)
                spec_buf[slices, 1, sign, b, 0:8, :] = re
                spec_buf[slices, 1, sign, b, 8:16, :] = im
            prev = filt

    def conv_mix(first, count, never, blk=4):
        for item in range(count):
            idx = first + item

            def load(which, sign, b):
                return spec_buf[idx, which, sign, b, 0:8, :], spec_buf[idx, which, sign, b, 8:16, :]

            for a0 in range(0, NB, blk):
                res = []
                for sign in range(2):
                    acc = [None] * blk
                    kcache = {}
                    for b in range(a0 + blk):
                        token = yield
                        ur, ui = load(0, sign, b)
                        ur = jnp.where(never, token, ur)
                        ui = jnp.where(never, token, ui)
                        us = ur + ui
                        for a in range(max(a0, b), a0 + blk):
                            if a - b not in kcache:
                                kr, ki = load(1, sign, a - b)
                                kcache[a - b] = (kr, ki - kr, kr + ki)
                            k1, k2, k3 = kcache[a - b]
                            terms = (us * k1, ur * k2, ui * k3)
                            old = acc[a - a0]
                            acc[a - a0] = terms if old is None else tuple(
                                o + t for o, t in zip(old, terms))
                    res.append([(p1 - p3, p1 + p2) for p1, p2, p3 in acc])
                for i in range(blk):
                    (pr, pi), (mr, mi) = res[0][i], res[1][i]
                    yf[idx, a0 + i, 0] = _as_words(jnp.concatenate([pr + mr, pi + mi], axis=0))
                    yf[idx, a0 + i, 1] = _as_words(jnp.concatenate([pr - mr, pi - mi], axis=0))

    def outa_copy(c):
        return pltpu.make_async_copy(
            outa.at[c], out_hbm.at[0, :, _ds(c * T, T, T)], sem_out.at[c])

    def conv_inverse(pacer):
        def step(i):
            c, a = divmod(i, NB)
            rows = slice(2 * a * T, 2 * (a + 1) * T)
            q_words = pltpu.bitcast(qa[rows, c * T:(c + 1) * T], u32)
            res = []
            for parity, q_rows in enumerate((_even_rows, _odd_rows)):
                spec = _as_bf16(yf[pl.ds(c * NFV, NFV), a, parity].reshape(T, T))
                y = None
                for half in range(2):
                    part = _dot(_as_bf16(inv[2 * parity + half]), spec[half * T:(half + 1) * T])
                    pacer.issued(part, 2 * parity + half, WI)
                    y = part if y is None else y + part
                res.append(q_rows(q_words) * y)
            outa[c, rows, :] = _interleave(*res)

        return step

    def pair(s, p, plan, mix=None):
        never = sub > 100 + p
        memory = "Ra" in plan
        if mix is None:
            pacer = _Pacer(never)
        else:
            first, count, cycles = mix
            pacer = _Pacer(never, conv_mix(first, count, never), count * 48 / cycles)
        steps = {"a": attend(s, 2 * p, 0, pacer, memory),
                 "b": attend(s, 2 * p + 1, 1, pacer, memory)}
        steps["a"]["P"] = project(s, 2 * p + 1, 1, pacer)
        next_s, next_g = s + (p + 1) // 4, (2 * p + 2) % NG
        steps["b"]["P"] = project(next_s, next_g, 0, pacer)
        steps["a"]["U"] = lambda _: update(s, 2 * p + 1, pacer)
        steps["b"]["U"] = lambda _: update(next_s, next_g, pacer)
        steps["a"]["O"] = out_project(s - 1, p, pacer)
        steps["x"] = {
            "T": transpose_qkv,
            "W": wait,
            "A": lambda c: outa_copy(c).start(),
            "B": lambda c: outa_copy(c).wait(),
            "I": conv_inverse(pacer),
            "C": lambda _: outb_copy(s - 1, p).start(),
        }
        last = {}

        def final(i):
            n, c = divmod(i, NC)
            if c == 0:
                last[n] = out_project(s, n, pacer)
            last[n](c)

        steps["x"]["E"] = final
        steps["x"]["F"] = lambda n: outb_copy(s, n).start()
        for item in plan:
            steps[item[1]][item[0]](int(item[2:] or 0))
        assert pacer.side is None

    if ONLY:
        for i in range(8):
            wait(i)
        setup_gate()
        if ONLY == "0":
            @pl.loop(1, 4)
            def _(p):
                pair(0, p, PLAN0)
        else:
            @pl.loop(0, 11)
            def _(i):
                cycles = 2 * (1152 * WA + 1200 * WP + 176 * WM) + 800 * WO
                pair(1 + i // 4, i % 4, PLAN1, (i * MIX_PER_ITER, MIX_PER_ITER, cycles * SLACK))
        outa[0, 0:16] = jnp.concatenate([mz[0, 0:8], pltpu.bitcast(ot[0, 0, 0:8] + yf[0, 0, 0] + qm[0, 0, 0:8] + qd[0,0,0:8] + pq[0,0,0:8] + kk[0,0,0:8] + pk_keep[0,0,0,0:8], f32) + vt[0,0,0:8] + vt_keep[0,0,0,0:8]], axis=0).astype(bf16)
        outa_copy(0).start()
        outa_copy(0).wait()
        return

    wait(0)
    transpose_qkv(0)
    wait(1)
    setup_gate()
    step = project(0, 0, 0, _Pacer(None))
    for i in range(NC):
        step(i)
    pair(0, 0, PLAN_FIRST)
    wait(4)

    @pl.loop(1, 4)
    def _(p):
        pair(0, p, PLAN0)

    wait(5)
    for i in range(2):
        fwd[i] = pltpu.bitcast(fwd_ref[i], u32)
    for i in range(4):
        inv[i] = pltpu.bitcast(inv_ref[i], u32)
    for c in range(NC):
        conv_forward(c)
        transpose_wo(c)
    update(1, 0, _Pacer(None))
    wait(6)

    @pl.loop(0, 11)
    def _(i):
        cycles = 2 * (1152 * WA + 1200 * WP + 176 * WM) + 800 * WO
        pair(1 + i // 4, i % 4, PLAN1, (i * MIX_PER_ITER, MIX_PER_ITER, cycles * SLACK))

    wait(7)
    pair(NSEG - 1, 3, PLAN_LAST, (11 * MIX_PER_ITER, NC * NFV - 11 * MIX_PER_ITER, 4500))

    for s in range(NSEG):
        for n in range(NQ):
            outb_copy(s, n).wait()


@jax.jit
def pallas_concat_heads__ssm_conv_h3__memory_aug_infini_attn__prompt_kernel(
    A_q: jax.Array,
    A_k: jax.Array,
    A_v: jax.Array,
    A_shift_k: jax.Array,
    A_ssm_k: jax.Array,
    A_ssm_D: jax.Array,
    B_x: jax.Array,
    B_wq: jax.Array,
    B_wk: jax.Array,
    B_wv: jax.Array,
    B_wo: jax.Array,
    B_beta: jax.Array,
):
    hbm = pl.BlockSpec(memory_space=pl.ANY)
    scratch = [
        pltpu.VMEM((4, D), bf16),
        pltpu.VMEM((NC, T), bf16),
        pltpu.VMEM((H,), bf16),
        pltpu.VMEM((2, 2 * T, T), bf16),
        pltpu.VMEM((4, T, T), bf16),
        pltpu.VMEM((NC, S, T), bf16),
        pltpu.VMEM((4, NC, D, T), bf16),
        pltpu.VMEM((3, NC, D // 2, T), u32),
        pltpu.VMEM((NC, D // 2, T), u32),
        pltpu.VMEM((S, D), bf16),
        pltpu.VMEM((S, D), bf16),
        pltpu.VMEM((S, D), bf16),
        pltpu.VMEM((D, S), bf16),
        pltpu.VMEM((NC * NFV, 2, 2, NB, 16, T), f32),
        pltpu.VMEM((NC * NFV, NB, 2, 8, T), u32),
        pltpu.VMEM((NC, S, T), bf16),
        pltpu.VMEM((NSEG, L, D), bf16),
        pltpu.VMEM((2, T, T), u32),
        pltpu.VMEM((4, T // 2, T), u32),
        pltpu.VMEM((H, T), f32),
        pltpu.VMEM((2, T // 2, T), f32),
        pltpu.VMEM((2, NQ, 64, T), u32),
        pltpu.VMEM((2, NQ, 48, T), u32),
        pltpu.VMEM((2, NQ, GW // 2, T), u32),
        pltpu.VMEM((2, NQ, T // 2, T), u32),
        pltpu.VMEM((2, NQ, GW, T), f32),
        pltpu.VMEM((2, NG, NQ, GW // 2, T), u32),
        pltpu.VMEM((2, NG, NQ, GW, T), f32),
        pltpu.VMEM((2, NQ, D // 2, T), u32),
        pltpu.VMEM((NG, GW + 8, T), f32),
        pltpu.SemaphoreType.DMA((8,)),
        pltpu.SemaphoreType.DMA((NC + 1,)),
    ]
    return pl.pallas_call(
        _kernel,
        out_shape=jax.ShapeDtypeStruct((1, S, 2 * D), bf16),
        in_specs=[hbm] * 14,
        out_specs=hbm,
        scratch_shapes=scratch,
        compiler_params=pltpu.CompilerParams(vmem_limit_bytes=100 * 2**20),
    )(
        A_shift_k.T, A_ssm_D.reshape(NC, T), B_beta, _FWD, _INV,
        A_q, A_k, A_v, A_ssm_k, B_x, B_wq, B_wk, B_wv, B_wo,
    )
```

```python
import os
import jax
import jax.numpy as jnp
import numpy as np
from jax import lax
from jax.experimental import pallas as pl
from jax.experimental.pallas import tpu as pltpu

f32, bf16, u32, i32 = jnp.float32, jnp.bfloat16, jnp.uint32, jnp.int32

S, D, H, DH = 2048, 640, 32, 20
NSEG, L = 4, 512
T = 128
NC = D // T
NB = S // (2 * T)
NQ = L // T
NG = 8
GW = 4 * DH
NFV = 16
LOG2E = 1.4426950408889634
NEG = -1e30
MIX_PER_ITER = 7

def _env(name, default):
    return type(default)(os.environ.get(name, default))
WA, WP, WO, WM = _env("WA", 1.0), _env("WP", 1.0), _env("WO", 1.0), _env("WM", 1.2)
SLACK = _env("SLACK", 0.965)
LEAD0, LEAD1 = _env("LEAD0", 400), _env("LEAD1", 400)
STAG0, STAG1 = _env("STAG0", 56), _env("STAG1", 32)
PF32 = _env("PF32", 0)
XB = _env("XB", 1)
FULLK = _env("FULLK", 1)
DMA0, DMA1 = _env("DMA0", 3), _env("DMA1", 4)
RHS32 = _env("RHS32", 1)
ONLY = _env("ONLY", "")
PLAN0 = _env("PLAN0",
    "Qa0 Da0 Pa0 Qa1 Pa1 Qa2 Qa3 Pa2 Pa3 Qa4 Va0 Va1 Qa5 Qa6 Pa4 Da1 Va2 Qa7 Va3 Qa8 Qa9 Va4 Qb0 Va5 "
    "Qb1 Va6 Db0 Va7 Qb2 Va8 Qb3 Va9 Qb4 Pb0 Qb5 Vb0 Vb1 Qb6 Vb2 Db1 Vb3 Qb7 Pb1 Pb2 Vb4 Qb8 Vb5 Qb9 "
    "Pb3 Pb4 Vb6 Vb7 Vb8 Vb9").split()
PLAN1 = _env("PLAN1",
    "Qa0 Da0 Pa0 Qa1 Pa1 Qa2 Pa2 Qa3 Pa3 Pa4 Qa4 Qa5 Va0 Va1 Oa0 Qa6 Va2 Qa7 Oa1 Da1 Va3 Oa2 Qa8 Oa3 "
    "Va4 Va5 Qa9 Oa4 Ra Ua Va6 Qb0 Va7 Qb1 Db0 Qb2 Va8 Qb3 Va9 Vb0 Pb0 Qb4 Pb1 Qb5 Qb6 Db1 Vb1 Vb2 "
    "Qb7 Vb3 Pb2 Qb8 Vb4 Vb5 Qb9 Pb3 Vb6 Pb4 Vb7 Rb Vb8 Vb9 Ub Cx").split()
WI = 1.0
PLAN_FIRST = _env("PLAN_FIRST",
    "Wx2 Qa0 Da0 Tx1 Qa1 Qa2 Qa3 Pa0 Qa4 Pa1 Va0 Pa2 Va1 Qa5 Pa3 Qa6 Pa4 Da1 Va2 Qa7 Va3 Qa8 Qa9 Va4 Qb0 Va5 Qb1 Va6 "
    "Db0 Va7 Qb2 Wx3 Tx2 Va8 Qb3 Vb0 Va9 Qb4 Pb0 Tx3 Qb5 Vb1 Qb6 Vb2 Db1 Vb3 Qb7 Tx4 Pb1 Pb2 Vb4 Qb8 Vb5 Qb9 Pb3 Pb4 "
    "Vb6 Vb7 Vb8 Vb9").split()
PLAN_LAST = _env("PLAN_LAST",
    "Qa0 Da0 Pa0 Qa1 Pa1 Qa2 Pa2 Qa3 Pa3 Pa4 Qa4 Qa5 Va0 Va1 Oa0 Qa6 Va2 Qa7 Oa1 Da1 Va3 Oa2 Qa8 Oa3 Va4 Va5 Qa9 Oa4 "
    "Ra Ua Va6 Ix0 Cx Qb0 Va7 Ix1 Qb1 Db0 Ix2 Qb2 Va8 Ix3 Qb3 Vb0 Va9 Ix4 Qb4 Ix5 Qb5 Ix6 Qb6 Db1 Vb1 Ix7 Vb2 Qb7 Ix8 "
    "Ax0 Vb3 Ix9 Qb8 Vb4 Ix10 Vb5 Qb9 Ix11 Ix12 Vb6 Ix13 Vb7 Rb Ix14 Vb8 Ix15 Vb9 Ix16 Ax1 Ix17 Lx3 Ix18 Lx2 Ix19 Lx1 Ix20 "
    "Lx0 Ix21 Ix22 Ix23 Ix24 Ax2 Ix25 Ix26 Ix27 Ix28 Ix29 Ix30 Ix31 Ix32 Ax3 Ix33 Ix34 Ix35 Ix36 Ix37 Ix38 Ex0 Ix39 Ex1 Jx "
    "Ax4 Ex2 Ex3 Ex4 Ex5 Ex6 Gx0 Fx0 Ex7 Ex8 Ex9 Ex10 Ex11 Ex12 Gx1 Fx1 Ex13 Ex14 Ex15 Ex16 Ex17 Ex18 Gx2 Fx2 Ex19 Ex20 "
    "Ex21 Ex22 Gx3 Ex23 Ex24 Gx4").split()
ORDER = [int(v) for v in _env("ORDER", "3,2,1,0").split(",")]

NN = (((1,), (0,)), ((), ()))
NT = (((1,), (1,)), ((), ()))


def _dft_tables():
    freq = np.concatenate([np.arange(0, T, 2), np.arange(1, T, 2)])
    fwd = []
    for parity in range(2):
        n = 2 * np.arange(T) + parity
        theta = 2.0 * np.pi * (freq[:, None] + 0.5) * n[None, :] / (4 * T)
        re, im = np.cos(theta), -np.sin(theta)
        fwd.append(np.stack(
            [re.reshape(NFV, 8, T), im.reshape(NFV, 8, T)], axis=1).reshape(2 * T, T))
    fwd = np.stack(fwd)
    inv = fwd.transpose(0, 2, 1) / (2 * T)
    inv = np.concatenate([inv[:, :, :T], inv[:, :, T:]], axis=1).reshape(4, T, T)
    return fwd.astype(np.float32).astype(bf16), inv.astype(np.float32).astype(bf16)


_FWD, _INV = _dft_tables()


def _as_bf16(words):
    return pltpu.bitcast(words, bf16)


def _as_words(x):
    return pltpu.bitcast(x.astype(bf16), u32)


def _even_rows(words):
    return pltpu.bitcast(words << 16, f32)


def _odd_rows(words):
    return pltpu.bitcast(words & np.uint32(0xFFFF0000), f32)


def _interleave(even, odd):
    even, odd = (pltpu.bitcast(x.astype(bf16).astype(f32), u32) for x in (even, odd))
    return pltpu.bitcast((even >> 16) | odd, bf16)


def _dot(a, b):
    return jnp.dot(a, b, preferred_element_type=f32)


def _dot_nt(a, b):
    return lax.dot_general(a, b, NT, preferred_element_type=f32)


def _phi(t):
    return jnp.maximum(t, 0.0) + jnp.exp(jnp.minimum(t, 0.0))


def _ds(start, size, align):
    if isinstance(start, int):
        return pl.ds(start, size)
    return pl.ds(pl.multiple_of(start, align), size)


class _Pacer:
    def __init__(self, never, side=None, rate=0.0):
        self.never, self.side, self.rate = never, side, rate
        self.credit, self.clock, self.history = 0.0, 0.0, []
        if side is not None:
            next(side)

    def issued(self, result, lane, weight=0.0):
        rows = result.shape[0]
        self.history.append((self.clock, result))
        if lane == 3:
            self.clock += rows
        self.credit += self.rate * rows / 4 * weight
        count = int(self.credit)
        self.credit -= count
        for i in range(count):
            if self.side is not None:
                v = min(rows // 8 - 1, int(rows // 8 * (lane + (i + 0.5) / count) / 4))
                try:
                    self.side.send(result[8 * v:8 * v + 8])
                except StopIteration:
                    self.side = None

    def hold(self, value, lead):
        target = self.clock - lead
        if target < 0 or self.never is None:
            return value
        for start, result in reversed(self.history):
            if start <= target:
                v = min(result.shape[0] // 8 - 1, int(target - start) // 8)
                return jnp.where(self.never, result[8 * v:8 * v + 8], value)
        return value


def _kernel(
    shift_hbm, ssmd_hbm, beta_hbm, fwd_hbm, inv_hbm,
    q_hbm, k_hbm, v_hbm, ssm_hbm, x_hbm, wq_hbm, wk_hbm, wv_hbm, wo_hbm, out_hbm,
    shift_ref, ssmd_ref, beta_ref, fwd_ref, inv_ref,
    xs, wraw, wt, wot, qa, ka, va, ssk, spec_buf, yf, outa, outb,
    fwd, inv, gate, bias, qm, qd, pq, kk, vt, pk_keep, vt_keep, ot, mz, sem_in, sem_out,
):
    def w_copies(n, sem):
        return [
            pltpu.make_async_copy(src.at[:, pl.ds(n * T, T)], wraw.at[i, n], sem)
            for i, src in enumerate((wq_hbm, wk_hbm, wv_hbm))
        ]

    def x_copies(lo, hi, sem):
        rows = pl.ds(lo * L, (hi - lo) * L)
        return [
            pltpu.make_async_copy(x_hbm.at[0, rows, pl.ds(c * T, T)], xs.at[c, rows], sem)
            for c in range(NC)
        ]

    loads = [
        w_copies(0, sem_in.at[0]),
        x_copies(0, 1, sem_in.at[1])
        + [pltpu.make_async_copy(beta_hbm, beta_ref, sem_in.at[1])],
        w_copies(1, sem_in.at[2]),
        sum((w_copies(n, sem_in.at[3]) for n in range(2, NC)), []),
        x_copies(1, 2, sem_in.at[4]),
        [pltpu.make_async_copy(src, dst, sem_in.at[5]) for src, dst in (
            (shift_hbm, shift_ref), (ssmd_hbm, ssmd_ref), (fwd_hbm, fwd_ref), (inv_hbm, inv_ref),
            (k_hbm.at[0], ka), (v_hbm.at[0], va), (ssm_hbm, ssk))]
        + [pltpu.make_async_copy(wo_hbm.at[:, pl.ds(n * T, T)], wraw.at[3, n], sem_in.at[5])
           for n in range(NC)],
        x_copies(2, NSEG, sem_in.at[6]),
        [pltpu.make_async_copy(q_hbm.at[0], qa, sem_in.at[7])],
    ]
    def start(lo, hi):
        for copies in loads[lo:hi]:
            for cp in copies:
                cp.start()

    start(0, DMA0)

    def wait(i):
        for cp in loads[i]:
            cp.wait()

    mz[...] = jnp.zeros(mz.shape, f32)
    row = lax.broadcasted_iota(i32, (T // 2, T), 0)
    col = lax.broadcasted_iota(i32, (T // 2, T), 1)
    bias[0] = jnp.where(row <= col, 0.0, NEG)
    bias[1] = jnp.where(row <= col % (T // 2), 0.0, NEG)

    def setup_gate():
        beta = jnp.concatenate(
            [beta_ref[...].astype(f32)[None, :], jnp.zeros((1, T - H), f32)], axis=1)
        gate[...] = jax.nn.sigmoid(jnp.broadcast_to(beta, (T, T)).T[:H])

    def transpose_qkv(n):
        for i in range(3):
            for c in range(NC):
                wt[i, c, n * T // 2:(n + 1) * T // 2, :] = pltpu.bitcast(
                    wraw[i, n, c * T:(c + 1) * T, :].T, u32)

    def transpose_wo(n):
        for c in range(NC):
            wot[c, n * T // 2:(n + 1) * T // 2, :] = pltpu.bitcast(
                wraw[3, n, c * T:(c + 1) * T, :].T, u32)

    sub = lax.broadcasted_iota(i32, (8, T), 0)
    low = sub < 4
    left = lax.broadcasted_iota(i32, (8, T), 1) < T // 2

    def project(s, g, slot, pacer):
        rows = _ds(g * (GW // 2), GW // 2, 8)
        acc = [None] * NQ

        def store(n):
            q_t, k_t, v_t = acc[n][:GW], acc[n][GW:2 * GW], acc[n][2 * GW:]
            k_pad = jnp.concatenate([k_t.astype(bf16), jnp.zeros((T - GW, T), bf16)], axis=0)
            kk[slot, n] = pltpu.bitcast(k_pad.T, u32)
            qs = q_t * (DH ** -0.5 * LOG2E)
            r = [qs[8 * i:8 * i + 8] for i in range(10)]
            zero = jnp.zeros((8, T), f32)
            heads = [
                r[0], r[1], jnp.where(low, r[2], 0.0), zero,
                jnp.where(low, 0.0, r[2]), r[3], r[4], zero,
                zero, r[5], r[6], jnp.where(low, r[7], 0.0),
                zero, jnp.where(low, 0.0, r[7]), r[8], r[9],
            ]
            qm[slot, n] = _as_words(jnp.concatenate(heads, axis=0))
            e = {i: jnp.where(left, pltpu.roll(r[i], 64, 1), 0.0) for i in (0, 1, 2, 5, 6, 7)}
            o = {i: jnp.where(left, 0.0, r[i]) for i in (2, 3, 4, 7, 8, 9)}
            pairs = [
                e[0], e[1], jnp.where(low, e[2], o[2]), o[3], o[4], zero,
                zero, e[5], e[6], jnp.where(low, e[7], o[7]), o[8], o[9],
            ]
            qd[slot, n] = _as_words(jnp.concatenate(pairs, axis=0))
            pq[slot, n] = _as_words(_phi(q_t))
            pk_keep[s % 2, g, n] = _as_words(_phi(k_t))
            vt[slot, n] = v_t
            vt_keep[s % 2, g, n] = v_t

        def step(i):
            for lane in range(4):
                n, c = divmod(4 * i + lane, NC)
                w = _as_bf16(jnp.concatenate([wt[m, c, rows, :] for m in range(3)], axis=0))
                if XB:
                    xt = _as_bf16(xs.bitcast(u32)[c, _ds((s * L + n * T) // 2, T // 2, T // 2), :])
                else:
                    xt = xs[c, _ds(s * L + n * T, T, T), :]
                part = _dot_nt(w, xt)
                pacer.issued(part, lane, WP)
                acc[n] = part if c == 0 else acc[n] + part
                if c == NC - 1:
                    store(n)

        return step

    def masked_dot(key_words, window, first):
        end = first + window.shape[0]
        parts = [jnp.zeros((first, T), bf16), window, jnp.zeros((T - end if FULLK else 0, T), bf16)]
        rhs = jnp.concatenate([p for p in parts if p.shape[0]], axis=0)
        return _dot(_as_bf16(key_words)[:, :rhs.shape[0]], rhs)

    def update(s, g, pacer):
        state = mz[g]
        for kt in range(NQ):
            v_one = jnp.concatenate(
                [vt_keep[(s + 1) % 2, g, kt], jnp.ones((8, T), f32)], axis=0)
            pk_t = jnp.concatenate(
                [_as_bf16(pk_keep[(s + 1) % 2, g, kt]), jnp.zeros((T - GW, T), bf16)], axis=0)
            part = _dot_nt(v_one, pk_t)
            pacer.issued(part, kt, WM)
            state = state + part
        mz[g] = state

    def attend(s, g, slot, pacer, memory):
        lead, stagger = (LEAD1, STAG1) if memory else (LEAD0, STAG0)
        tiles = [(qt, kt) for qt in ORDER for kt in range(qt + 1)]
        logits, run_max, col_max, acc, mem, done = {}, {}, {}, {}, {}, []
        corner, corner_max, corner_p = {}, {}, {}
        gates = [jnp.broadcast_to(gate[pl.ds(4 * g + j, 1), :], (8, T)) for j in range(4)]

        low_pair = sub % 4 < 2
        rest_rows = 1.0 - jnp.where(low, jnp.where(low_pair, gates[1], gates[3]),
                                    jnp.where(low_pair, gates[0], gates[2]))

        def read(_):
            def head_of(i):
                return (i >= DH).astype(i32) + (i >= 2 * DH).astype(i32) + (i >= 3 * DH).astype(i32)

            state = mz[g]
            row_m = lax.broadcasted_iota(i32, (GW, T), 0)
            col_m = lax.broadcasted_iota(i32, (GW, T), 1)
            weights = jnp.where(head_of(row_m) == head_of(col_m), state[:GW], 0.0)
            lane_head = head_of(lax.broadcasted_iota(i32, (8, T), 1))
            pair_of = sub // 2
            z_rows = jnp.where(lane_head == pair_of, state[GW:], 0.0)
            mem_w = jnp.concatenate([weights, z_rows], axis=0)
            g_rows = jnp.where(low, jnp.where(sub < 2, gates[0], gates[1]),
                               jnp.where(sub < 6, gates[2], gates[3]))
            for qt in range(NQ):
                rhs = _as_bf16(pq[slot, qt])
                if FULLK:
                    rhs = jnp.concatenate([rhs, jnp.zeros((T - GW, T), bf16)], axis=0)
                res = lax.dot_general(
                    mem_w[:, :rhs.shape[0]], rhs, NN, preferred_element_type=f32)
                pacer.issued(res, qt, WM)
                coef = g_rows / (res[GW:] + 1e-6)
                c0, c1, c2, c3 = (
                    jnp.broadcast_to(coef[2 * j:2 * j + 1], (8, T)) for j in range(4))
                cm = [c0, c0, jnp.where(low, c0, c1), c1, c1,
                      c2, c2, jnp.where(low, c2, c3), c3, c3]
                mem[qt] = [res[8 * i:8 * i + 8] * cm[i] for i in range(10)]
            finish()

        def corners(i):
            for lane in range(4):
                qt, pr = ORDER[2 * i + lane // 2], lane % 2
                window = _as_bf16(qd[slot, qt, 24 * pr:24 * pr + 24, :])
                sc = masked_dot(kk[slot, qt, T // 4:, :], window, 32 * pr)
                pacer.issued(sc, lane, WA)
                corner[qt, pr] = sc + bias[1]
                corner_max[qt, pr] = jnp.max(corner[qt, pr].reshape(8, 8, T), axis=0)

        def scores(t):
            qt, kt = tiles[t]
            for j in range(4):
                window = _as_bf16(qm[slot, qt, 16 * j:16 * j + 16, :])
                sc = masked_dot(
                    kk[slot, kt] if kt < qt else kk[slot, kt, :T // 4, :], window, 16 * j)
                pacer.issued(sc, j, WA)
                if kt == qt:
                    sc = sc + bias[0]
                m8 = jnp.max(sc.reshape(-1, 8, T), axis=0)
                run_max[qt, j] = m8 if kt == 0 else jnp.maximum(run_max[qt, j], m8)
                if kt == qt:
                    extra = corner_max[qt, j // 2]
                    if j % 2 == 0:
                        extra = pltpu.roll(extra, T // 2, 1)
                    top = jnp.maximum(run_max[qt, j], jnp.where(left, NEG, extra))
                    col_max[qt, j] = jnp.broadcast_to(
                        jnp.max(top, axis=0, keepdims=True), (8, T))
                logits[t, j] = sc
            if kt == qt:
                for pr in range(2):
                    top = jnp.where(left, pltpu.roll(col_max[qt, 2 * pr], T // 2, 1),
                                    col_max[qt, 2 * pr + 1])
                    words = _as_words(jnp.exp2(
                        corner[qt, pr].reshape(8, 8, T) - top[None]).reshape(T // 2, T))
                    for j, shifted in enumerate((pltpu.roll(words, T // 2, 1), words)):
                        corner_p[qt, 2 * pr + j] = _as_bf16(jnp.where(
                            left[None], jnp.uint32(0), shifted.reshape(4, 8, T)).reshape(32, T))

        def values(t):
            qt, kt = tiles[t]
            tops = [pacer.hold(col_max[qt, j], lead - stagger * j) for j in range(4)]
            for j in range(4):
                p = jnp.exp2(logits[t, j].reshape(-1, 8, T) - tops[j][None])
                p = p.reshape(-1, T).astype(bf16)
                if kt == qt:
                    p = jnp.concatenate([p, corner_p[qt, j]], axis=0)
                first = (0, 16, 40, 56)[j]
                v = [vt[slot, kt, first + 8 * i:first + 8 * i + 8, :] for i in range(3)]
                if j % 2 == 0:
                    v[2] = jnp.where(low, v[2], 1.0)
                else:
                    v[0] = jnp.where(low, 1.0, v[0])
                part = lax.dot_general(
                    jnp.concatenate(v, axis=0), p, NN, preferred_element_type=f32)
                pacer.issued(part, j)
                acc[qt, j] = part if kt == 0 else acc[qt, j] + part
            if kt == qt:
                done.append(qt)
                finish()

        def finish():
            while done and (not memory or done[0] in mem):
                qt = done.pop(0)
                w = [[acc[qt, j][8 * i:8 * i + 8] for i in range(3)] for j in range(4)]
                sums = jnp.where(
                    low_pair, jnp.where(low, w[1][0], w[0][2]),
                    pltpu.roll(jnp.where(low, w[3][0], w[2][2]), 2, 0))
                coef = rest_rows / sums
                c0, c1, c2, c3 = (
                    jnp.broadcast_to(coef[r:r + 1], (8, T)) for r in (4, 0, 6, 2))
                o = [w[0][0] * c0, w[0][1] * c0,
                     jnp.where(low, w[0][2] * c0, w[1][0] * c1), w[1][1] * c1, w[1][2] * c1,
                     w[2][0] * c2, w[2][1] * c2,
                     jnp.where(low, w[2][2] * c2, w[3][0] * c3), w[3][1] * c3, w[3][2] * c3]
                if memory:
                    o = [mem[qt][i] + o[i] for i in range(10)]
                ot[s % 2, qt, _ds(g * (GW // 2), GW // 2, 8), :] = _as_words(
                    jnp.concatenate(o, axis=0))

        return {"D": corners, "Q": scores, "V": values, "R": read}

    def out_project(s, n, pacer):
        acc = [None] * 4

        def step(c):
            rhs = _as_bf16(ot[s % 2, n, c * 64:(c + 1) * 64, :])
            for m in range(4):
                part = _dot(_as_bf16(wot[c, 80 * m:80 * (m + 1), :]), rhs)
                pacer.issued(part, m, WO)
                acc[m] = part if c == 0 else acc[m] + part
            if c == NC - 1:
                res = jnp.concatenate(acc, axis=0).astype(bf16)
                for i in range(NC):
                    outb[s, _ds(n * T, T, T), i * T:(i + 1) * T] = res[i * T:(i + 1) * T].T

        return step

    def outb_copy(s, n):
        return pltpu.make_async_copy(
            outb.at[s, _ds(n * T, T, T)],
            out_hbm.at[0, _ds(s * L + n * T, T, T), pl.ds(D, D)],
            sem_out.at[0])

    def conv_forward(c):
        cols = slice(c * T, (c + 1) * T)
        taps = shift_ref[:, cols].astype(f32)
        taps = [jnp.broadcast_to(taps[j:j + 1], (T, T)) for j in range(4)]
        skip = ssmd_ref[...].astype(f32)[c:c + 1]
        slices = pl.ds(c * NFV, NFV)

        def transform(even, odd):
            if not RHS32:
                even, odd = even.astype(bf16), odd.astype(bf16)
            e, o = (
                lax.dot_general(_as_bf16(fwd[i]), x, NN, preferred_element_type=f32)
                for i, x in enumerate((even, odd)))
            return [x.reshape(NFV, 2, 8, T) for x in (e + o, e - o)]

        tail = jnp.zeros((8, T), u32)
        prev = None
        for b in range(NB):
            rows = slice(2 * b * T, 2 * (b + 1) * T)
            taps_t = jnp.concatenate([
                pltpu.bitcast(ssk[cols, (2 * b + i) * T:(2 * b + i + 1) * T].T, u32)
                for i in range(2)], axis=0)
            filt = transform(_even_rows(taps_t), _odd_rows(taps_t))
            k0 = pltpu.bitcast(ka[rows, cols], u32)
            ext = jnp.concatenate([tail, k0], axis=0)
            tail = k0[T - 8:]
            k1, k2 = ext[7:7 + T], ext[6:6 + T]
            e0, o0, e1, o1, o2 = (
                _even_rows(k0), _odd_rows(k0), _even_rows(k1), _odd_rows(k1), _odd_rows(k2))
            v0 = pltpu.bitcast(va[rows, cols], u32)
            sig = transform(
                (e0 * taps[0] + o1 * taps[1] + e1 * taps[2] + o2 * taps[3]) * _even_rows(v0),
                (o0 * taps[0] + e0 * taps[1] + o1 * taps[2] + e1 * taps[3]) * _odd_rows(v0))
            for sign in range(2):
                spec_buf[slices, 0, sign, b] = sig[sign].reshape(NFV, 16, T)
                re, im = filt[sign][:, 0], filt[sign][:, 1]
                if prev is None:
                    re = re + skip[None]
                else:
                    half = NFV // 2
                    pre, pim = prev[sign][:, 0], prev[sign][:, 1]
                    re = jnp.concatenate([re[:half] - pim[:half], re[half:] + pim[half:]], axis=0)
                    im = jnp.concatenate([im[:half] + pre[:half], im[half:] - pre[half:]], axis=0)
                spec_buf[slices, 1, sign, b, 0:8, :] = re
                spec_buf[slices, 1, sign, b, 8:16, :] = im
            prev = filt

    def conv_mix(first, count, never, blk=4):
        for item in range(count):
            idx = first + item

            def load(which, sign, b):
                return spec_buf[idx, which, sign, b, 0:8, :], spec_buf[idx, which, sign, b, 8:16, :]

            for a0 in range(0, NB, blk):
                res = []
                for sign in range(2):
                    acc = [None] * blk
                    kcache = {}
                    for b in range(a0 + blk):
                        token = yield
                        ur, ui = load(0, sign, b)
                        ur = jnp.where(never, token, ur)
                        ui = jnp.where(never, token, ui)
                        us = ur + ui
                        for a in range(max(a0, b), a0 + blk):
                            if a - b not in kcache:
                                kr, ki = load(1, sign, a - b)
                                kcache[a - b] = (kr, ki - kr, kr + ki)
                            k1, k2, k3 = kcache[a - b]
                            terms = (us * k1, ur * k2, ui * k3)
                            old = acc[a - a0]
                            acc[a - a0] = terms if old is None else tuple(
                                o + t for o, t in zip(old, terms))
                    res.append([(p1 - p3, p1 + p2) for p1, p2, p3 in acc])
                for i in range(blk):
                    (pr, pi), (mr, mi) = res[0][i], res[1][i]
                    yf[idx, a0 + i, 0] = _as_words(jnp.concatenate([pr + mr, pi + mi], axis=0))
                    yf[idx, a0 + i, 1] = _as_words(jnp.concatenate([pr - mr, pi - mi], axis=0))

    def outa_copy(c):
        return pltpu.make_async_copy(
            outa.at[c], out_hbm.at[0, :, _ds(c * T, T, T)], sem_out.at[0])

    def conv_inverse(pacer, zero):
        pending, pin = [], []

        def send(c):
            outa_copy(c).start()
            pin.append(True)

        def flush(_=0):
            while pending:
                c, rows, (even, odd) = pending.pop(0)
                q_words = pltpu.bitcast(qa[rows, c * T:(c + 1) * T], u32)
                tile = c + zero if pin else c
                pin.clear()
                outa[tile, rows, :] = _interleave(
                    _even_rows(q_words) * even, _odd_rows(q_words) * odd)

        def step(i):
            c, a = divmod(i, NB)
            res = []
            for parity in range(2):
                spec = _as_bf16(yf[pl.ds(c * NFV, NFV), a, parity].reshape(T, T))
                y = None
                for half in range(2):
                    part = _dot(_as_bf16(inv[2 * parity + half]), spec[half * T:(half + 1) * T])
                    pacer.issued(part, 2 * parity + half, WI)
                    y = part if y is None else y + part
                res.append(y)
            flush()
            pending.append((c, slice(2 * a * T, 2 * (a + 1) * T), res))

        return step, flush, send

    def out_project_last(pacer, zero):
        s = NSEG - 1
        o_rows, acc = {}, {}

        def transpose(n):
            for c in range(NC):
                o_rows[n, c] = _as_bf16(ot[s % 2, n, c * 64:(c + 1) * 64, :]).T

        def step(i):
            for lane in range(4):
                tile, c = divmod(4 * i + lane, NC)
                n, m = divmod(tile, NC)
                part = _dot(o_rows[n, c], wraw[3, m, c * T:(c + 1) * T, :])
                pacer.issued(part, lane)
                acc[tile] = part if c == 0 else acc[tile] + part

        def store(part):
            n = min(part, NQ - 1)
            for m in range(NC) if part < NQ - 1 else ((0, 1, 2), (3, 4))[part - n]:
                seg = s + zero if m == 0 else s
                outb[seg, n * T:(n + 1) * T, m * T:(m + 1) * T] = acc[n * NC + m].astype(bf16)

        return transpose, step, store

    def pair(s, p, plan, mix=None):
        never = gate[0:8, :] > 2.0
        memory = "Ra" in plan
        if mix is None:
            pacer = _Pacer(never)
        else:
            first, count, cycles = mix
            pacer = _Pacer(never, conv_mix(first, count, never), count * 48 / cycles)
        steps = {"a": attend(s, 2 * p, 0, pacer, memory),
                 "b": attend(s, 2 * p + 1, 1, pacer, memory)}
        steps["a"]["P"] = project(s, 2 * p + 1, 1, pacer)
        next_s, next_g = s + (p + 1) // 4, (2 * p + 2) % NG
        steps["b"]["P"] = project(next_s, next_g, 0, pacer)
        steps["a"]["U"] = lambda _: update(s, 2 * p + 1, pacer)
        steps["b"]["U"] = lambda _: update(next_s, next_g, pacer)
        steps["a"]["O"] = out_project(s - 1, p, pacer)
        steps["x"] = {
            "T": transpose_qkv,
            "W": wait,

            "C": lambda _: outb_copy(s - 1, p).start(),
        }
        if "Jx" in plan:
            zero = never.astype(i32)[0, 0]
            steps["x"]["I"], steps["x"]["J"], steps["x"]["A"] = conv_inverse(pacer, zero)
            steps["x"]["L"], steps["x"]["E"], steps["x"]["G"] = out_project_last(pacer, zero)
        steps["x"]["F"] = lambda n: outb_copy(s, n).start()
        for item in plan:
            steps[item[1]][item[0]](int(item[2:] or 0))
        assert pacer.side is None

    if ONLY:
        start(DMA0, len(loads))
        for i in range(8):
            wait(i)
        setup_gate()
        if ONLY == "0":
            @pl.loop(1, 4)
            def _(p):
                pair(0, p, PLAN0)
        else:
            @pl.loop(0, 11)
            def _(i):
                cycles = 2 * (1152 * WA + 1200 * WP + 176 * WM) + 800 * WO
                pair(1 + i // 4, i % 4, PLAN1, (i * MIX_PER_ITER, MIX_PER_ITER, cycles * SLACK))
        outa[0, 0:16] = jnp.concatenate([mz[0, 0:8], pltpu.bitcast(ot[0, 0, 0:8] + yf[0, 0, 0] + qm[0, 0, 0:8] + qd[0,0,0:8] + pq[0,0,0:8] + kk[0,0,0:8] + pk_keep[0,0,0,0:8], f32) + vt[0,0,0:8] + vt_keep[0,0,0,0:8]], axis=0).astype(bf16)
        outa_copy(0).start()
        outa_copy(0).wait()
        return

    wait(0)
    start(DMA0, DMA1)
    transpose_qkv(0)
    wait(1)
    start(DMA1, len(loads))
    setup_gate()
    step = project(0, 0, 0, _Pacer(None))
    for i in range(NC):
        step(i)
    pair(0, 0, PLAN_FIRST)
    wait(4)

    @pl.loop(1, 4)
    def _(p):
        pair(0, p, PLAN0)

    wait(5)
    for i in range(2):
        fwd[i] = pltpu.bitcast(fwd_ref[i], u32)
    for i in range(4):
        inv[i] = pltpu.bitcast(inv_ref[i], u32)
    for c in range(NC):
        conv_forward(c)
        transpose_wo(c)
    update(1, 0, _Pacer(None))
    wait(6)

    @pl.loop(0, 11)
    def _(i):
        cycles = 2 * (1152 * WA + 1200 * WP + 176 * WM) + 800 * WO
        pair(1 + i // 4, i % 4, PLAN1, (i * MIX_PER_ITER, MIX_PER_ITER, cycles * SLACK))

    wait(7)
    pair(NSEG - 1, 3, PLAN_LAST, (11 * MIX_PER_ITER, NC * NFV - 11 * MIX_PER_ITER, 4500))

    outb_copy(NSEG - 1, NQ - 1).start()
    for c in range(NC):
        outa_copy(c).wait()
    for s in range(NSEG):
        for n in range(NQ):
            outb_copy(s, n).wait()


@jax.jit
def pallas_concat_heads__ssm_conv_h3__memory_aug_infini_attn__prompt_kernel(
    A_q: jax.Array,
    A_k: jax.Array,
    A_v: jax.Array,
    A_shift_k: jax.Array,
    A_ssm_k: jax.Array,
    A_ssm_D: jax.Array,
    B_x: jax.Array,
    B_wq: jax.Array,
    B_wk: jax.Array,
    B_wv: jax.Array,
    B_wo: jax.Array,
    B_beta: jax.Array,
):
    hbm = pl.BlockSpec(memory_space=pl.ANY)
    scratch = [
        pltpu.VMEM((4, D), bf16),
        pltpu.VMEM((NC, T), bf16),
        pltpu.VMEM((H,), bf16),
        pltpu.VMEM((2, 2 * T, T), bf16),
        pltpu.VMEM((4, T, T), bf16),
        pltpu.VMEM((NC, S, T), bf16),
        pltpu.VMEM((4, NC, D, T), bf16),
        pltpu.VMEM((3, NC, D // 2, T), u32),
        pltpu.VMEM((NC, D // 2, T), u32),
        pltpu.VMEM((S, D), bf16),
        pltpu.VMEM((S, D), bf16),
        pltpu.VMEM((S, D), bf16),
        pltpu.VMEM((D, S), bf16),
        pltpu.VMEM((NC * NFV, 2, 2, NB, 16, T), f32),
        pltpu.VMEM((NC * NFV, NB, 2, 8, T), u32),
        pltpu.VMEM((NC, S, T), bf16),
        pltpu.VMEM((NSEG, L, D), bf16),
        pltpu.VMEM((2, T, T), u32),
        pltpu.VMEM((4, T // 2, T), u32),
        pltpu.VMEM((H, T), f32),
        pltpu.VMEM((2, T // 2, T), f32),
        pltpu.VMEM((2, NQ, 64, T), u32),
        pltpu.VMEM((2, NQ, 48, T), u32),
        pltpu.VMEM((2, NQ, GW // 2, T), u32),
        pltpu.VMEM((2, NQ, T // 2, T), u32),
        pltpu.VMEM((2, NQ, GW, T), f32),
        pltpu.VMEM((2, NG, NQ, GW // 2, T), u32),
        pltpu.VMEM((2, NG, NQ, GW, T), f32),
        pltpu.VMEM((2, NQ, D // 2, T), u32),
        pltpu.VMEM((NG, GW + 8, T), f32),
        pltpu.SemaphoreType.DMA((8,)),
        pltpu.SemaphoreType.DMA((1,)),
    ]
    return pl.pallas_call(
        _kernel,
        out_shape=jax.ShapeDtypeStruct((1, S, 2 * D), bf16),
        in_specs=[hbm] * 14,
        out_specs=hbm,
        scratch_shapes=scratch,
        compiler_params=pltpu.CompilerParams(vmem_limit_bytes=100 * 2**20),
    )(
        A_shift_k.T, A_ssm_D.reshape(NC, T), B_beta, _FWD, _INV,
        A_q, A_k, A_v, A_ssm_k, B_x, B_wq, B_wk, B_wv, B_wo,
    )
```

```python
import os
import jax
import jax.numpy as jnp
import numpy as np
from jax import lax
from jax.experimental import pallas as pl
from jax.experimental.pallas import tpu as pltpu

f32, bf16, u32, i32 = jnp.float32, jnp.bfloat16, jnp.uint32, jnp.int32

S, D, H, DH = 2048, 640, 32, 20
NSEG, L = 4, 512
T = 128
NC = D // T
NB = S // (2 * T)
NQ = L // T
NG = 8
GW = 4 * DH
NFV = 16
LOG2E = 1.4426950408889634
NEG = -1e30
MIX_PER_ITER = 4

def _env(name, default):
    return type(default)(os.environ.get(name, default))
WA, WP, WO, WM = _env("WA", 1.0), _env("WP", 1.0), _env("WO", 1.0), _env("WM", 1.0)
SLACK = _env("SLACK", 0.965)
LEAD0, LEAD1 = _env("LEAD0", 400), _env("LEAD1", 400)
STAG0, STAG1 = _env("STAG0", 56), _env("STAG1", 32)
PF32 = _env("PF32", 0)
XB = _env("XB", 1)
FULLK = _env("FULLK", 1)
CTOP = _env("CTOP", 0)
XSPLIT = _env("XSPLIT", 1.0)
GATE2 = _env("GATE2", 0)
TLEAD = _env("TLEAD", 250)
DMA0, DMA1 = _env("DMA0", 3), _env("DMA1", 4)
RHS32 = _env("RHS32", 1)
ONLY = _env("ONLY", "")
PLAN0 = _env("PLAN0",
    "Qa0 Da0 Pa0 Qa1 Pa1 Qa2 Qa3 Pa2 Pa3 Qa4 Va0 Va1 Qa5 Qa6 Pa4 Da1 Va2 Qa7 Va3 Qa8 Qa9 Va4 Qb0 Va5 "
    "Qb1 Va6 Db0 Va7 Qb2 Va8 Qb3 Va9 Qb4 Pb0 Qb5 Vb0 Vb1 Qb6 Vb2 Db1 Vb3 Qb7 Pb1 Pb2 Vb4 Qb8 Vb5 Qb9 "
    "Pb3 Pb4 Vb6 Vb7 Vb8 Vb9").split()
PLAN1 = _env("PLAN1",
    "Qa0 Da0 Pa0 Pa1 Qa1 Qa2 Qa3 Pa2 Pa3 Pa4 Qa4 Qa5 Va0 Va1 Qa6 Oa0 Va2 Qa7 Da1 Va3 Oa1 Oa2 Qa8 Va4 "
    "Oa3 Oa4 Va5 Qa9 Ra Ua Va6 Qb0 Va7 Qb1 Db0 Qb2 Va8 Qb3 Pb0 Vb0 Va9 Qb4 Pb1 Qb5 Vb1 Qb6 Db1 Vb2 "
    "Qb7 Vb3 Pb2 Qb8 Vb4 Vb5 Qb9 Pb3 Vb6 Pb4 Rb Vb7 Vb8 Vb9 Cx Ub").split()
if _env("CTOP", 0):
    PLAN1 = [item for item in PLAN1 if item != "Cx"]
WI = 1.0
PLAN_FIRST = _env("PLAN_FIRST",
    "Wx2 Qa0 Da0 Tx3 Tx4 Tx5 Qa1 Qa2 Qa3 Pa0 Qa4 Pa1 Va0 Pa2 Va1 Qa5 Pa3 Qa6 Pa4 Da1 Va2 Qa7 Va3 Qa8 Qa9 Va4 "
    "Qb0 Va5 Qb1 Va6 Db0 Va7 Qb2 Wx3 Tx6 Tx7 Tx8 Va8 Qb3 Vb0 Va9 Qb4 Pb0 Tx9 Tx10 Tx11 Qb5 Vb1 Qb6 Vb2 Db1 "
    "Vb3 Qb7 Tx12 Tx13 Tx14 Pb1 Pb2 Vb4 Qb8 Vb5 Qb9 Pb3 Pb4 Vb6 Vb7 Vb8 Vb9").split()
PLAN_LAST = _env("PLAN_LAST",
    "Qa0 Da0 Pa0 Pa1 Qa1 Qa2 Qa3 Pa2 Pa3 Pa4 Qa4 Ix0 Qa5 Ix1 Va0 Ix2 Va1 Qa6 Ix3 Oa0 Va2 Qa7 Ix4 Da1 Va3 Oa1 Ix5 Oa2 "
    "Qa8 Ix6 Va4 Oa3 Ix7 Oa4 Va5 Qa9 Ix8 Cx Ax0 Ra Ua Va6 Ix9 Qb0 Ix10 Va7 Qb1 Ix11 Db0 Ix12 Qb2 Va8 Ix13 Qb3 Ix14 "
    "Vb0 Va9 Ix15 Qb4 Ix16 Ax1 Qb5 Ix17 Vb1 Qb6 Ix18 Db1 Ix19 Vb2 Qb7 Ix20 Vb3 Ix21 Qb8 Ix22 Vb4 Ix23 Vb5 Qb9 Ix24 Ax2 "
    "Ix25 Ix26 Vb6 Ix27 Rb Ix28 Vb7 Ix29 Ix30 Vb8 Ix31 Ix32 Ax3 Vb9 Ix33 Lx3 Ix34 Lx2 Ix35 Ix36 Lx1 Ix37 Ix38 Lx0 Ix39 "
    "Ex0 Jx Ax4 Ex1 Ex2 Ex3 Ex4 Ex5 Ex6 Gx0 Fx0 Ex7 Ex8 Ex9 Ex10 Ex11 Ex12 Gx1 Fx1 Ex13 Ex14 Ex15 Ex16 Ex17 Ex18 Gx2 Fx2 "
    "Ex19 Ex20 Ex21 Ex22 Gx3 Ex23 Ex24 Gx4").split()
ORDER = [int(v) for v in _env("ORDER", "3,2,1,0").split(",")]

NN = (((1,), (0,)), ((), ()))
NT = (((1,), (1,)), ((), ()))


def _dft_tables():
    freq = np.concatenate([np.arange(0, T, 2), T - 1 - np.arange(0, T, 2)])

    def table(freq, n):
        theta = 2.0 * np.pi * (freq[:, None] + 0.5) * n[None, :] / (4 * T)
        parts = [f(theta).reshape(-1, 8, len(n)) for f in (np.cos, lambda t: -np.sin(t))]
        return np.stack(parts, axis=1).reshape(-1, len(n))

    fwd = np.stack([table(freq, 2 * np.arange(T) + r) for r in range(2)])
    inv = np.stack([table(freq[:T // 2], 4 * np.arange(T // 2) + r).T / (2 * T) for r in range(4)])
    return fwd.astype(np.float32).astype(bf16), inv.astype(np.float32).astype(bf16)


_FWD, _INV = _dft_tables()


def _as_bf16(words):
    return pltpu.bitcast(words, bf16)


def _as_words(x):
    return pltpu.bitcast(x.astype(bf16), u32)


def _even_rows(words):
    return pltpu.bitcast(words << 16, f32)


def _odd_rows(words):
    return pltpu.bitcast(words & np.uint32(0xFFFF0000), f32)


def _interleave(even, odd):
    even, odd = (pltpu.bitcast(x.astype(bf16).astype(f32), u32) for x in (even, odd))
    return (even >> 16) | odd


def _dot(a, b):
    return jnp.dot(a, b, preferred_element_type=f32)


def _dot_nt(a, b):
    return lax.dot_general(a, b, NT, preferred_element_type=f32)


def _phi(t):
    return jnp.maximum(t, 0.0) + jnp.exp(jnp.minimum(t, 0.0))


def _ds(start, size, align):
    if isinstance(start, int):
        return pl.ds(start, size)
    return pl.ds(pl.multiple_of(start, align), size)


class _Pacer:
    def __init__(self, never):
        self.never, self.side, self.rate = never, None, 0.0
        self.credit, self.clock, self.history = 0.0, 0.0, []

    def attach(self, side, rate):
        self.side, self.rate, self.credit = side, rate, 0.0
        next(side)

    def issued(self, result, lane, weight=0.0):
        rows = result.shape[0]
        self.history.append((self.clock, result))
        if lane == 3:
            self.clock += rows
        self.credit += self.rate * rows / 4 * weight
        count = int(self.credit)
        self.credit -= count
        for i in range(count):
            if self.side is not None:
                v = min(rows // 8 - 1, int(rows // 8 * (lane + (i + 0.5) / count) / 4))
                try:
                    self.side.send(result[8 * v:8 * v + 8])
                except StopIteration:
                    self.side = None

    def hold(self, value, lead):
        target = self.clock - lead
        if target < 0 or self.never is None:
            return value
        for start, result in reversed(self.history):
            if start <= target:
                v = min(result.shape[0] // 8 - 1, int(target - start) // 8)
                return jnp.where(self.never, result[8 * v:8 * v + 8], value)
        return value


def _kernel(
    shift_hbm, ssmd_hbm, beta_hbm, fwd_hbm, inv_hbm,
    q_hbm, k_hbm, v_hbm, ssm_hbm, x_hbm, wq_hbm, wk_hbm, wv_hbm, wo_hbm, out_hbm,
    shift_ref, ssmd_ref, beta_ref, fwd_ref, inv_ref,
    xs, wraw, wt, wot, qa, ka, va, ssk, spec_buf, yf, outa, outb,
    gate, bias, qm, qd, pq, kk, vt, pk_keep, vt_keep, ot, mz, sem_in, sem_out,
):
    def w_copies(n, sem):
        return [
            pltpu.make_async_copy(src.at[:, pl.ds(n * T, T)], wraw.at[i, n], sem)
            for i, src in enumerate((wq_hbm, wk_hbm, wv_hbm))
        ]

    def x_copies(lo, hi, sem):
        rows = pl.ds(int(lo * L), int((hi - lo) * L))
        return [
            pltpu.make_async_copy(x_hbm.at[0, rows, pl.ds(c * T, T)], xs.at[c, rows], sem)
            for c in range(NC)
        ]

    def column_tiles(src, dst, sem):
        return [
            pltpu.make_async_copy(src.at[0, :, pl.ds(c * T, T)], dst.at[c], sem)
            for c in range(NC)
        ]

    loads = [
        w_copies(0, sem_in.at[0]),
        x_copies(0, XSPLIT, sem_in.at[1])
        + [pltpu.make_async_copy(beta_hbm, beta_ref, sem_in.at[1])],
        w_copies(1, sem_in.at[2]),
        sum((w_copies(n, sem_in.at[3]) for n in range(2, NC)), x_copies(1, 2, sem_in.at[3])),
        x_copies(XSPLIT, 1, sem_in.at[4]) if XSPLIT < 1 else [],
        [pltpu.make_async_copy(src, dst, sem_in.at[5]) for src, dst in (
            (shift_hbm, shift_ref), (ssmd_hbm, ssmd_ref), (fwd_hbm, fwd_ref), (inv_hbm, inv_ref),
            (ssm_hbm, ssk))]
        + column_tiles(k_hbm, ka, sem_in.at[5]) + column_tiles(v_hbm, va, sem_in.at[5])
        + [pltpu.make_async_copy(wo_hbm.at[:, pl.ds(n * T, T)], wraw.at[3, n], sem_in.at[5])
           for n in range(NC)],
        x_copies(2, NSEG, sem_in.at[6]),
        column_tiles(q_hbm, qa, sem_in.at[7]),
    ]
    def start(lo, hi):
        for copies in loads[lo:hi]:
            for cp in copies:
                cp.start()

    start(0, 2)
    start(4, 5)
    start(2, DMA0)

    def wait(i):
        for cp in loads[i]:
            cp.wait()

    mz[...] = jnp.zeros(mz.shape, f32)
    row = lax.broadcasted_iota(i32, (T // 2, T), 0)
    col = lax.broadcasted_iota(i32, (T // 2, T), 1)
    bias[0] = jnp.where(row <= col, 0.0, NEG)
    bias[1] = jnp.where(row <= col % (T // 2), 0.0, NEG)

    def setup_gate():
        beta = jnp.concatenate(
            [beta_ref[...].astype(f32)[None, :], jnp.zeros((1, T - H), f32)], axis=1)
        gate[...] = jax.nn.sigmoid(jnp.broadcast_to(beta, (T, T)).T[:H])

    def transpose_qkv(part):
        n, i = divmod(part, 3)
        for c in range(NC):
            tile = _as_bf16(wraw.bitcast(u32)[i, n, c * 64:(c + 1) * 64, :])
            wt[i, c, n * T // 2:(n + 1) * T // 2, :] = pltpu.bitcast(tile.T, u32)

    def transpose_wo(n):
        for c in range(NC):
            words = wraw.bitcast(u32)[3, n, c * 64:(c + 1) * 64, :]
            wot[c, n * T // 2:(n + 1) * T // 2, :] = pltpu.bitcast(_as_bf16(words).T, u32)

    sub = lax.broadcasted_iota(i32, (8, T), 0)
    low = sub < 4
    left = lax.broadcasted_iota(i32, (8, T), 1) < T // 2

    def project(s, g, slot, pacer):
        rows = _ds(g * (GW // 2), GW // 2, 8)
        acc = [None] * NQ

        def store(n):
            q_t, k_t, v_t = acc[n][:GW], acc[n][GW:2 * GW], acc[n][2 * GW:]
            k_pad = jnp.concatenate([k_t.astype(bf16), jnp.zeros((T - GW, T), bf16)], axis=0)
            kk[slot, n] = pltpu.bitcast(k_pad.T, u32)
            qs = q_t * (DH ** -0.5 * LOG2E)
            r = [qs[8 * i:8 * i + 8] for i in range(10)]
            zero = jnp.zeros((8, T), f32)
            heads = [
                r[0], r[1], jnp.where(low, r[2], 0.0), zero,
                jnp.where(low, 0.0, r[2]), r[3], r[4], zero,
                zero, r[5], r[6], jnp.where(low, r[7], 0.0),
                zero, jnp.where(low, 0.0, r[7]), r[8], r[9],
            ]
            qm[slot, n] = _as_words(jnp.concatenate(heads, axis=0))
            e = {i: jnp.where(left, pltpu.roll(r[i], 64, 1), 0.0) for i in (0, 1, 2, 5, 6, 7)}
            o = {i: jnp.where(left, 0.0, r[i]) for i in (2, 3, 4, 7, 8, 9)}
            pairs = [
                e[0], e[1], jnp.where(low, e[2], o[2]), o[3], o[4], zero,
                zero, e[5], e[6], jnp.where(low, e[7], o[7]), o[8], o[9],
            ]
            qd[slot, n] = _as_words(jnp.concatenate(pairs, axis=0))
            pq[slot, n] = _as_words(_phi(q_t))
            pk_keep[s % 2, g, n] = _as_words(_phi(k_t))
            vt[slot, n] = v_t
            vt_keep[s % 2, g, n] = v_t

        def step(i):
            for lane in range(4):
                n, c = divmod(4 * i + lane, NC)
                w = _as_bf16(jnp.concatenate([wt[m, c, rows, :] for m in range(3)], axis=0))
                if XB:
                    xt = _as_bf16(xs.bitcast(u32)[c, _ds(s * (L // 2) + n * (T // 2), T // 2, T // 2), :])
                else:
                    xt = xs[c, _ds(s * L + n * T, T, T), :]
                part = _dot_nt(w, xt)
                pacer.issued(part, lane, WP)
                acc[n] = part if c == 0 else acc[n] + part
                if c == NC - 1:
                    store(n)

        return step

    def masked_dot(key_words, window, first):
        end = first + window.shape[0]
        parts = [jnp.zeros((first, T), bf16), window, jnp.zeros((T - end if FULLK else 0, T), bf16)]
        rhs = jnp.concatenate([p for p in parts if p.shape[0]], axis=0)
        return _dot(_as_bf16(key_words)[:, :rhs.shape[0]], rhs)

    def update(s, g, pacer):
        state = mz[g]
        for kt in range(NQ):
            v_one = jnp.concatenate(
                [vt_keep[(s + 1) % 2, g, kt], jnp.ones((8, T), f32)], axis=0)
            pk_t = jnp.concatenate(
                [_as_bf16(pk_keep[(s + 1) % 2, g, kt]), jnp.zeros((T - GW, T), bf16)], axis=0)
            part = _dot_nt(v_one, pk_t)
            pacer.issued(part, kt, WM)
            state = state + part
        mz[g] = state

    def attend(s, g, slot, pacer, memory):
        lead, stagger = (LEAD1, STAG1) if memory else (LEAD0, STAG0)
        tiles = [(qt, kt) for qt in ORDER for kt in range(qt + 1)]
        logits, run_max, col_max, acc, mem, done = {}, {}, {}, {}, {}, []
        corner, corner_max, corner_p = {}, {}, {}
        gates = [jnp.broadcast_to(gate[pl.ds(4 * g + j, 1), :], (8, T)) for j in range(4)]

        low_pair = sub % 4 < 2
        rest_rows = 1.0 - jnp.where(low, jnp.where(low_pair, gates[1], gates[3]),
                                    jnp.where(low_pair, gates[0], gates[2]))

        def read(_):
            def head_of(i):
                return (i >= DH).astype(i32) + (i >= 2 * DH).astype(i32) + (i >= 3 * DH).astype(i32)

            state = mz[g]
            row_m = lax.broadcasted_iota(i32, (GW, T), 0)
            col_m = lax.broadcasted_iota(i32, (GW, T), 1)
            weights = jnp.where(head_of(row_m) == head_of(col_m), state[:GW], 0.0)
            lane_head = head_of(lax.broadcasted_iota(i32, (8, T), 1))
            pair_of = sub // 2
            z_rows = jnp.where(lane_head == pair_of, state[GW:], 0.0)
            mem_w = jnp.concatenate([weights, z_rows], axis=0)
            g_rows = jnp.where(low, jnp.where(sub < 2, gates[0], gates[1]),
                               jnp.where(sub < 6, gates[2], gates[3]))
            for qt in range(NQ):
                rhs = _as_bf16(pq[slot, qt])
                if FULLK:
                    rhs = jnp.concatenate([rhs, jnp.zeros((T - GW, T), bf16)], axis=0)
                res = lax.dot_general(
                    mem_w[:, :rhs.shape[0]], rhs, NN, preferred_element_type=f32)
                pacer.issued(res, qt, WM)
                coef = g_rows / (res[GW:] + 1e-6)
                c0, c1, c2, c3 = (
                    jnp.broadcast_to(coef[2 * j:2 * j + 1], (8, T)) for j in range(4))
                cm = [c0, c0, jnp.where(low, c0, c1), c1, c1,
                      c2, c2, jnp.where(low, c2, c3), c3, c3]
                mem[qt] = [res[8 * i:8 * i + 8] * cm[i] for i in range(10)]
            finish()

        def corners(i):
            for lane in range(4):
                qt, pr = ORDER[2 * i + lane // 2], lane % 2
                window = _as_bf16(qd[slot, qt, 24 * pr:24 * pr + 24, :])
                sc = masked_dot(kk[slot, qt, T // 4:, :], window, 32 * pr)
                pacer.issued(sc, lane, WA)
                corner[qt, pr] = sc + bias[1]
                corner_max[qt, pr] = jnp.max(corner[qt, pr].reshape(8, 8, T), axis=0)

        def scores(t):
            qt, kt = tiles[t]
            for j in range(4):
                window = _as_bf16(qm[slot, qt, 16 * j:16 * j + 16, :])
                sc = masked_dot(
                    kk[slot, kt] if kt < qt else kk[slot, kt, :T // 4, :], window, 16 * j)
                pacer.issued(sc, j, WA)
                if kt == qt:
                    sc = sc + bias[0]
                m8 = jnp.max(sc.reshape(-1, 8, T), axis=0)
                run_max[qt, j] = m8 if kt == 0 else jnp.maximum(run_max[qt, j], m8)
                if kt == qt:
                    extra = corner_max[qt, j // 2]
                    if j % 2 == 0:
                        extra = pltpu.roll(extra, T // 2, 1)
                    top = jnp.maximum(run_max[qt, j], jnp.where(left, NEG, extra))
                    col_max[qt, j] = jnp.broadcast_to(
                        jnp.max(top, axis=0, keepdims=True), (8, T))
                logits[t, j] = sc
            if kt == qt:
                for pr in range(2):
                    top = jnp.where(left, pltpu.roll(col_max[qt, 2 * pr], T // 2, 1),
                                    col_max[qt, 2 * pr + 1])
                    words = _as_words(jnp.exp2(
                        corner[qt, pr].reshape(8, 8, T) - top[None]).reshape(T // 2, T))
                    for j, shifted in enumerate((pltpu.roll(words, T // 2, 1), words)):
                        corner_p[qt, 2 * pr + j] = _as_bf16(jnp.where(
                            left[None], jnp.uint32(0), shifted.reshape(4, 8, T)).reshape(32, T))

        def values(t):
            qt, kt = tiles[t]
            tops = [pacer.hold(col_max[qt, j], lead - stagger * j) for j in range(4)]
            for j in range(4):
                p = jnp.exp2(logits[t, j].reshape(-1, 8, T) - tops[j][None])
                p = p.reshape(-1, T).astype(bf16)
                if kt == qt:
                    p = jnp.concatenate([p, corner_p[qt, j]], axis=0)
                first = (0, 16, 40, 56)[j]
                v = [vt[slot, kt, first + 8 * i:first + 8 * i + 8, :] for i in range(3)]
                if j % 2 == 0:
                    v[2] = jnp.where(low, v[2], 1.0)
                else:
                    v[0] = jnp.where(low, 1.0, v[0])
                part = lax.dot_general(
                    jnp.concatenate(v, axis=0), p, NN, preferred_element_type=f32)
                pacer.issued(part, j)
                acc[qt, j] = part if kt == 0 else acc[qt, j] + part
            if kt == qt:
                done.append(qt)
                finish()

        def finish():
            while done and (not memory or done[0] in mem):
                qt = done.pop(0)
                w = [[acc[qt, j][8 * i:8 * i + 8] for i in range(3)] for j in range(4)]
                sums = jnp.where(
                    low_pair, jnp.where(low, w[1][0], w[0][2]),
                    pltpu.roll(jnp.where(low, w[3][0], w[2][2]), 2, 0))
                coef = rest_rows / sums
                c0, c1, c2, c3 = (
                    jnp.broadcast_to(coef[r:r + 1], (8, T)) for r in (4, 0, 6, 2))
                o = [w[0][0] * c0, w[0][1] * c0,
                     jnp.where(low, w[0][2] * c0, w[1][0] * c1), w[1][1] * c1, w[1][2] * c1,
                     w[2][0] * c2, w[2][1] * c2,
                     jnp.where(low, w[2][2] * c2, w[3][0] * c3), w[3][1] * c3, w[3][2] * c3]
                if memory:
                    o = [mem[qt][i] + o[i] for i in range(10)]
                ot[s % 2, qt, _ds(g * (GW // 2), GW // 2, 8), :] = _as_words(
                    jnp.concatenate(o, axis=0))

        return {"D": corners, "Q": scores, "V": values, "R": read}

    def wo_tile(c, m):
        return _as_bf16(wraw.bitcast(u32)[3, m, c * 64:(c + 1) * 64, :])

    def out_project(s, n, pacer):
        acc, done = [None] * 4, []

        def step(i):
            for lane in range(4):
                m, c = divmod(4 * i + lane, NC)
                part = _dot(_as_bf16(wot[c, 80 * m:80 * (m + 1), :]),
                            _as_bf16(ot[s % 2, n, c * 64:(c + 1) * 64, :]))
                pacer.issued(part, lane, WO)
                acc[m] = part if c == 0 else acc[m] + part
                if c == NC - 1:
                    acc[m] = acc[m].astype(bf16)
                    while T * (len(done) + 1) <= 160 * (m + 1):
                        i0 = T * len(done)
                        pieces = [acc[k][max(i0 - 160 * k, 0):min(i0 + T - 160 * k, 160)]
                                  for k in range(i0 // 160, (i0 + T - 1) // 160 + 1)]
                        tile = jnp.concatenate(pieces, axis=0).T
                        outb.bitcast(u32)[s, n, len(done)] = pltpu.bitcast(tile, u32)
                        done.append(True)

        return step

    def outb_copies(s, n):
        rows = _ds(s * L + n * T, T, T)
        return [
            pltpu.make_async_copy(
                outb.at[s, n, m], out_hbm.at[0, rows, pl.ds(D + m * T, T)], sem_out.at[0])
            for m in range(NC)
        ]

    def send_outb(s, n):
        for cp in outb_copies(s, n):
            cp.start()

    def conv_forward(c):
        cols = slice(c * T, (c + 1) * T)
        taps = shift_ref[:, cols].astype(f32)
        taps = [jnp.broadcast_to(taps[j:j + 1], (T, T)) for j in range(4)]
        skip = ssmd_ref[...].astype(f32)[c:c + 1]
        slices = pl.ds(c * NFV, NFV)

        def transform(even, odd):
            if not RHS32:
                even, odd = even.astype(bf16), odd.astype(bf16)
            e, o = (
                lax.dot_general(_as_bf16(fwd_ref.bitcast(u32)[i]), x, NN, preferred_element_type=f32)
                for i, x in enumerate((even, odd)))
            return [x.reshape(NFV, 2, 8, T) for x in (e + o, e - o)]

        tail = jnp.zeros((8, T), u32)
        prev = None
        for b in range(NB):
            taps_t = jnp.concatenate([
                pltpu.bitcast(ssk[cols, (2 * b + i) * T:(2 * b + i + 1) * T].T, u32)
                for i in range(2)], axis=0)
            filt = transform(_even_rows(taps_t), _odd_rows(taps_t))
            k0 = ka.bitcast(u32)[c, b * T:(b + 1) * T, :]
            ext = jnp.concatenate([tail, k0], axis=0)
            tail = k0[T - 8:]
            k1, k2 = ext[7:7 + T], ext[6:6 + T]
            e0, o0, e1, o1, o2 = (
                _even_rows(k0), _odd_rows(k0), _even_rows(k1), _odd_rows(k1), _odd_rows(k2))
            v0 = va.bitcast(u32)[c, b * T:(b + 1) * T, :]
            sig = transform(
                (e0 * taps[0] + o1 * taps[1] + e1 * taps[2] + o2 * taps[3]) * _even_rows(v0),
                (o0 * taps[0] + e0 * taps[1] + o1 * taps[2] + e1 * taps[3]) * _odd_rows(v0))
            for sign in range(2):
                spec_buf[slices, 0, sign, b] = sig[sign].reshape(NFV, 16, T)
                re, im = filt[sign][:, 0], filt[sign][:, 1]
                if prev is None:
                    re = re + skip[None]
                else:
                    half = NFV // 2
                    pre, pim = prev[sign][:, 0], prev[sign][:, 1]
                    re = jnp.concatenate([re[:half] - pim[:half], re[half:] + pim[half:]], axis=0)
                    im = jnp.concatenate([im[:half] + pre[:half], im[half:] - pre[half:]], axis=0)
                spec_buf[slices, 1, sign, b, 0:8, :] = re
                spec_buf[slices, 1, sign, b, 8:16, :] = im
            prev = filt

    def conv_mix(first, count, never, blk=4):
        half = NFV // 2
        for item in range(count):
            idx = jnp.minimum(first + item, NC * half - 1)
            base = idx // half * NFV + idx % half

            def products(fv, sign, a0):
                def load(which, b):
                    return (spec_buf[fv, which, sign, b, 0:8, :],
                            spec_buf[fv, which, sign, b, 8:16, :])

                acc, kcache = [None] * blk, {}
                for b in range(a0 + blk):
                    token = yield
                    ur, ui = load(0, b)
                    ur = jnp.where(never, token, ur)
                    if GATE2:
                        ui = jnp.where(never, token, ui)
                    us = ur + ui
                    for a in range(max(a0, b), a0 + blk):
                        if a - b not in kcache:
                            kr, ki = load(1, a - b)
                            kcache[a - b] = (kr, ki - kr, kr + ki)
                        k1, k2, k3 = kcache[a - b]
                        terms = (us * k1, ur * k2, ui * k3)
                        old = acc[a - a0]
                        acc[a - a0] = terms if old is None else tuple(
                            o + t for o, t in zip(old, terms))
                return [(p1 - p3, p1 + p2) for p1, p2, p3 in acc]

            for a0 in range(0, NB, blk):
                parity = []
                for fv in (base, base + half):
                    plus = yield from products(fv, 0, a0)
                    minus = yield from products(fv, 1, a0)
                    parity.append((
                        [(pr + mr, pi + mi) for (pr, pi), (mr, mi) in zip(plus, minus)],
                        [(pr - mr, pi - mi) for (pr, pi), (mr, mi) in zip(plus, minus)]))
                for i in range(blk):
                    (ar, ai), (br, bi) = parity[0][0][i], parity[1][0][i]
                    (cr, ci), (dr, di) = parity[0][1][i], parity[1][1][i]
                    folded = ((ar + br, ai - bi), (cr - di, ci - dr),
                              (ar - br, ai + bi), (cr + di, ci + dr))
                    for r in range(4):
                        yf[idx, a0 + i, r] = _as_words(jnp.concatenate(folded[r], axis=0))

    def outa_copy(c):
        return pltpu.make_async_copy(
            outa.at[c], out_hbm.at[0, :, _ds(c * T, T, T)], sem_out.at[0])

    def conv_inverse(pacer, zero):
        pending, pin, hold = [], [], []

        def send(c):
            outa_copy(c).start()
            pin.append(True)

        def flush(_=0):
            while pending:
                c, a, y = pending.pop(0)
                tile = c + zero if pin else c
                for i in range(2):
                    rows = pl.ds(a * T + i, T // 2, stride=2)
                    q_words = qa.bitcast(u32)[c, rows, :]
                    outa.bitcast(u32)[tile, rows, :] = _interleave(
                        _even_rows(q_words) * y[2 * i], _odd_rows(q_words) * y[2 * i + 1])
                if pin:
                    hold.append(outa.bitcast(u32)[tile, a * T:a * T + 8, :])
                    pin.clear()

        def step(i):
            c, a = divmod(i, NB)
            res = []
            for r in range(4):
                words = yf[pl.ds(c * NFV // 2, NFV // 2), a, r].reshape(T // 2, T)
                if hold:
                    words = jnp.concatenate(
                        [jnp.where(pacer.never, hold.pop(), words[:8]), words[8:]], axis=0)
                res.append(_dot(
                    _as_bf16(inv_ref.bitcast(u32)[r]), _as_bf16(words)))
                pacer.issued(res[-1], r, WI)
            flush()
            pending.append((c, a, res))

        return step, flush, send

    def out_project_last(pacer, zero):
        s = NSEG - 1
        o_rows, acc = {}, {}

        def transpose(n):
            for c in range(NC):
                o_rows[n, c] = _as_bf16(ot[s % 2, n, c * 64:(c + 1) * 64, :]).T

        def step(i):
            for lane in range(4):
                tile, c = divmod(4 * i + lane, NC)
                n, m = divmod(tile, NC)
                part = _dot(o_rows[n, c], wo_tile(c, m))
                pacer.issued(part, lane)
                acc[tile] = part if c == 0 else acc[tile] + part

        def store(part):
            n = min(part, NQ - 1)
            for m in range(NC) if part < NQ - 1 else ((0, 1, 2), (3, 4))[part - n]:
                seg = s + zero if m == 0 else s
                outb.bitcast(u32)[seg, n, m] = _as_words(acc[n * NC + m])

        return transpose, step, store

    def new_pacer():
        return _Pacer(gate[0:8, :] > 2.0)

    def pair(s, p, plan, pacer, mix=None):
        memory = "Ra" in plan
        if mix is not None:
            first, count, cycles = mix
            pacer.attach(conv_mix(first, count, pacer.never), count * 96 / cycles)
        steps = {"a": attend(s, 2 * p, 0, pacer, memory),
                 "b": attend(s, 2 * p + 1, 1, pacer, memory)}
        steps["a"]["P"] = project(s, 2 * p + 1, 1, pacer)
        next_s, next_g = s + (p + 1) // 4, (2 * p + 2) % NG
        steps["b"]["P"] = project(next_s, next_g, 0, pacer)
        steps["a"]["U"] = lambda _: update(s, 2 * p + 1, pacer)
        steps["b"]["U"] = lambda _: update(next_s, next_g, pacer)
        steps["a"]["O"] = out_project(s - 1, p, pacer)
        steps["x"] = {
            "T": transpose_qkv,
            "W": wait,

            "C": lambda _: send_outb(s - 1, p),
        }
        if "Jx" in plan:
            zero = pacer.never.astype(i32)[0, 0]
            steps["x"]["I"], steps["x"]["J"], steps["x"]["A"] = conv_inverse(pacer, zero)
            steps["x"]["L"], steps["x"]["E"], steps["x"]["G"] = out_project_last(pacer, zero)
        steps["x"]["F"] = lambda n: send_outb(s, n)
        for item in plan:
            steps[item[1]][item[0]](int(item[2:] or 0))
        assert pacer.side is None

    mix_cycles = (2 * (1152 * WA + 1200 * WP + 176 * WM) + 800 * WO) * SLACK

    def memory_pair(i):
        pair(1 + i // 4, i % 4, PLAN1, new_pacer(), (i * MIX_PER_ITER, MIX_PER_ITER, mix_cycles))

    if ONLY:
        start(DMA0, 4)
        start(5, len(loads))
        for i in range(8):
            wait(i)
        setup_gate()
        if ONLY == "0":
            @pl.loop(1, 4)
            def _(p):
                pair(0, p, PLAN0, new_pacer())
        else:
            @pl.loop(0, 11)
            def _(i):
                memory_pair(i)
        outa[0, 0:16] = jnp.concatenate([mz[0, 0:8], pltpu.bitcast(ot[0, 0, 0:8] + yf[0, 0, 0] + qm[0, 0, 0:8] + qd[0,0,0:8] + pq[0,0,0:8] + kk[0,0,0:8] + pk_keep[0,0,0,0:8] + outb.bitcast(u32)[0,0,0,0:8], f32) + vt[0,0,0:8] + vt_keep[0,0,0,0:8]], axis=0).astype(bf16)
        outa_copy(0).start()
        outa_copy(0).wait()
        return

    wait(0)
    start(DMA0, DMA1)
    for part in range(3):
        transpose_qkv(part)
    wait(1)
    start(5, len(loads))
    setup_gate()
    step = project(0, 0, 0, _Pacer(None))
    for i in range(NC):
        if i == int(XSPLIT * NC):
            wait(4)
        step(i)
    pair(0, 0, PLAN_FIRST, new_pacer())

    @pl.loop(1, 4)
    def _(p):
        pair(0, p, PLAN0, new_pacer())

    wait(5)
    for c in range(NC):
        conv_forward(c)
        transpose_wo(c)
    update(1, 0, _Pacer(None))
    wait(6)
    wait(7)

    @pl.loop(0, 11)
    def _(i):
        if CTOP:
            @pl.when(i > 0)
            def _():
                send_outb((i - 1) // 4, (i - 1) % 4)

        memory_pair(i)

    if CTOP:
        send_outb(2, 2)
    pair(NSEG - 1, 3, PLAN_LAST, new_pacer())

    send_outb(NSEG - 1, NQ - 1)
    for c in range(NC):
        outa_copy(c).wait()
    for s in range(NSEG):
        for n in range(NQ):
            for cp in outb_copies(s, n):
                cp.wait()


@jax.jit
def pallas_concat_heads__ssm_conv_h3__memory_aug_infini_attn__prompt_kernel(
    A_q: jax.Array,
    A_k: jax.Array,
    A_v: jax.Array,
    A_shift_k: jax.Array,
    A_ssm_k: jax.Array,
    A_ssm_D: jax.Array,
    B_x: jax.Array,
    B_wq: jax.Array,
    B_wk: jax.Array,
    B_wv: jax.Array,
    B_wo: jax.Array,
    B_beta: jax.Array,
):
    hbm = pl.BlockSpec(memory_space=pl.ANY)
    scratch = [
        pltpu.VMEM((4, D), bf16),
        pltpu.VMEM((NC, T), bf16),
        pltpu.VMEM((H,), bf16),
        pltpu.VMEM((2, 2 * T, T), bf16),
        pltpu.VMEM((4, T // 2, T), bf16),
        pltpu.VMEM((NC, S, T), bf16),
        pltpu.VMEM((4, NC, D, T), bf16),
        pltpu.VMEM((3, NC, D // 2, T), u32),
        pltpu.VMEM((NC, D // 2, T), u32),
        pltpu.VMEM((NC, S, T), bf16),
        pltpu.VMEM((NC, S, T), bf16),
        pltpu.VMEM((NC, S, T), bf16),
        pltpu.VMEM((D, S), bf16),
        pltpu.VMEM((NC * NFV, 2, 2, NB, 16, T), f32),
        pltpu.VMEM((NC * NFV // 2, NB, 4, 8, T), u32),
        pltpu.VMEM((NC, S, T), bf16),
        pltpu.VMEM((NSEG, NQ, NC, T, T), bf16),
        pltpu.VMEM((H, T), f32),
        pltpu.VMEM((2, T // 2, T), f32),
        pltpu.VMEM((2, NQ, 64, T), u32),
        pltpu.VMEM((2, NQ, 48, T), u32),
        pltpu.VMEM((2, NQ, GW // 2, T), u32),
        pltpu.VMEM((2, NQ, T // 2, T), u32),
        pltpu.VMEM((2, NQ, GW, T), f32),
        pltpu.VMEM((2, NG, NQ, GW // 2, T), u32),
        pltpu.VMEM((2, NG, NQ, GW, T), f32),
        pltpu.VMEM((2, NQ, D // 2, T), u32),
        pltpu.VMEM((NG, GW + 8, T), f32),
        pltpu.SemaphoreType.DMA((8,)),
        pltpu.SemaphoreType.DMA((1,)),
    ]
    return pl.pallas_call(
        _kernel,
        out_shape=jax.ShapeDtypeStruct((1, S, 2 * D), bf16),
        in_specs=[hbm] * 14,
        out_specs=hbm,
        scratch_shapes=scratch,
        compiler_params=pltpu.CompilerParams(vmem_limit_bytes=100 * 2**20),
    )(
        A_shift_k.T, A_ssm_D.reshape(NC, T), B_beta, _FWD, _INV,
        A_q, A_k, A_v, A_ssm_k, B_x, B_wq, B_wk, B_wv, B_wo,
    )
```

```python
import os
import jax
import jax.numpy as jnp
import numpy as np
from jax import lax
from jax.experimental import pallas as pl
from jax.experimental.pallas import tpu as pltpu

f32, bf16, u32, i32 = jnp.float32, jnp.bfloat16, jnp.uint32, jnp.int32

S, D, H, DH = 2048, 640, 32, 20
NSEG, L = 4, 512
T = 128
NC = D // T
NB = S // (2 * T)
NQ = L // T
NG = 8
GW = 4 * DH
NFV = 16
LOG2E = 1.4426950408889634
NEG = -1e30
MIX_PER_ITER = 4

def _env(name, default):
    return type(default)(os.environ.get(name, default))
WA, WP, WO, WM = _env("WA", 1.2), _env("WP", 1.0), _env("WO", 1.0), _env("WM", 1.2)
SLACK = _env("SLACK", 0.965)
LEAD0, LEAD1 = _env("LEAD0", 400), _env("LEAD1", 400)
STAG0, STAG1 = _env("STAG0", 56), _env("STAG1", 24)
PF32 = _env("PF32", 0)
XB = _env("XB", 1)
FULLK = _env("FULLK", 1)
MIXBLK = _env("MIXBLK", 4)
XSPLIT = _env("XSPLIT", 1.0)
GATE2 = _env("GATE2", 0)
TLEAD = _env("TLEAD", 250)
DMA0, DMA1 = _env("DMA0", 3), _env("DMA1", 4)
RHS32 = _env("RHS32", 1)
ONLY = _env("ONLY", "")
PLAN0 = _env("PLAN0",
    "Qa0 Da0 Pa0 Qa1 Pa1 Qa2 Qa3 Pa2 Pa3 Qa4 Va0 Va1 Qa5 Qa6 Pa4 Da1 Va2 Qa7 Va3 Qa8 Qa9 Va4 Qb0 Va5 "
    "Qb1 Va6 Db0 Va7 Qb2 Va8 Qb3 Va9 Qb4 Pb0 Qb5 Vb0 Vb1 Qb6 Vb2 Db1 Vb3 Qb7 Pb1 Pb2 Vb4 Qb8 Vb5 Qb9 "
    "Pb3 Pb4 Vb6 Vb7 Vb8 Vb9").split()
PLAN1 = _env("PLAN1",
    "Qa0 Da0 Pa0 Pa1 Qa1 Qa2 Qa3 Pa2 Pa3 Va0 Pa4 Qa4 Qa5 Va1 Qa6 Oa0 Va2 Qa7 Va3 Da1 Oa1 Oa2 Qa8 Va4 "
    "Oa3 Oa4 Va5 Qa9 Ua Ra Va6 Qb0 Va7 Qb1 Db0 Qb2 Va8 Qb3 Pb0 Vb0 Va9 Pb1 Qb4 Qb5 Qb6 Vb1 Db1 Vb2 "
    "Qb7 Vb3 Pb2 Qb8 Vb4 Vb5 Qb9 Pb3 Vb6 Cx Pb4 Rb Vb7 Vb8 Vb9 Ub").split()
WI = 1.0
PLAN_FIRST = _env("PLAN_FIRST",
    "Wx2 Qa0 Da0 Tx3 Tx4 Tx5 Qa1 Qa2 Qa3 Pa0 Qa4 Pa1 Va0 Pa2 Va1 Qa5 Pa3 Qa6 Pa4 Da1 Va2 Qa7 Va3 Qa8 Qa9 Va4 "
    "Qb0 Va5 Qb1 Va6 Db0 Va7 Qb2 Wx3 Tx6 Tx7 Tx8 Va8 Qb3 Vb0 Va9 Qb4 Pb0 Tx9 Tx10 Tx11 Qb5 Vb1 Qb6 Vb2 Db1 "
    "Vb3 Qb7 Tx12 Tx13 Tx14 Pb1 Pb2 Vb4 Qb8 Vb5 Qb9 Pb3 Pb4 Vb6 Vb7 Vb8 Vb9").split()
PLAN_LAST = _env("PLAN_LAST",
    "Qa0 Da0 Pa0 Pa1 Qa1 Qa2 Qa3 Pa2 Pa3 Pa4 Qa4 Ix0 Qa5 Ix1 Va0 Ix2 Va1 Qa6 Ix3 Oa0 Va2 Qa7 Ix4 Da1 Va3 Oa1 Ix5 Oa2 "
    "Qa8 Ix6 Va4 Oa3 Ix7 Oa4 Va5 Qa9 Ix8 Cx Ax0 Ra Ua Va6 Ix9 Qb0 Ix10 Va7 Qb1 Ix11 Db0 Ix12 Qb2 Va8 Ix13 Qb3 Ix14 "
    "Vb0 Va9 Ix15 Qb4 Ix16 Ax1 Qb5 Ix17 Vb1 Qb6 Ix18 Db1 Ix19 Vb2 Qb7 Ix20 Vb3 Ix21 Qb8 Ix22 Vb4 Ix23 Vb5 Qb9 Ix24 Ax2 "
    "Ix25 Ix26 Vb6 Ix27 Rb Ix28 Vb7 Ix29 Ix30 Vb8 Ix31 Ix32 Ax3 Vb9 Ix33 Lx3 Ix34 Lx2 Ix35 Ix36 Lx1 Ix37 Ix38 Lx0 Ix39 "
    "Ex0 Jx Ax4 Ex1 Ex2 Ex3 Ex4 Ex5 Ex6 Gx0 Fx0 Ex7 Ex8 Ex9 Ex10 Ex11 Ex12 Gx1 Fx1 Ex13 Ex14 Ex15 Ex16 Ex17 Ex18 Gx2 Fx2 "
    "Ex19 Ex20 Ex21 Ex22 Gx3 Ex23 Ex24 Gx4").split()
ORDER = [int(v) for v in _env("ORDER", "3,2,1,0").split(",")]

NN = (((1,), (0,)), ((), ()))
NT = (((1,), (1,)), ((), ()))


def _dft_tables():
    freq = np.concatenate([np.arange(0, T, 2), T - 1 - np.arange(0, T, 2)])

    def table(freq, n):
        theta = 2.0 * np.pi * (freq[:, None] + 0.5) * n[None, :] / (4 * T)
        parts = [f(theta).reshape(-1, 8, len(n)) for f in (np.cos, lambda t: -np.sin(t))]
        return np.stack(parts, axis=1).reshape(-1, len(n))

    fwd = np.stack([table(freq, 2 * np.arange(T) + r) for r in range(2)])
    inv = np.stack([table(freq[:T // 2], 4 * np.arange(T // 2) + r).T / (2 * T) for r in range(4)])
    return fwd.astype(np.float32).astype(bf16), inv.astype(np.float32).astype(bf16)


_FWD, _INV = _dft_tables()


def _as_bf16(words):
    return pltpu.bitcast(words, bf16)


def _as_words(x):
    return pltpu.bitcast(x.astype(bf16), u32)


def _even_rows(words):
    return pltpu.bitcast(words << 16, f32)


def _odd_rows(words):
    return pltpu.bitcast(words & np.uint32(0xFFFF0000), f32)


def _interleave(even, odd):
    even, odd = (pltpu.bitcast(x.astype(bf16).astype(f32), u32) for x in (even, odd))
    return (even >> 16) | odd


def _dot(a, b):
    return jnp.dot(a, b, preferred_element_type=f32)


def _dot_nt(a, b):
    return lax.dot_general(a, b, NT, preferred_element_type=f32)


def _phi(t):
    return jnp.maximum(t, 0.0) + jnp.exp(jnp.minimum(t, 0.0))


def _ds(start, size, align):
    if isinstance(start, int):
        return pl.ds(start, size)
    return pl.ds(pl.multiple_of(start, align), size)


class _Pacer:
    def __init__(self, never):
        self.never, self.side, self.rate = never, None, 0.0
        self.credit, self.clock, self.history = 0.0, 0.0, []

    def attach(self, side, rate):
        self.side, self.rate, self.credit = side, rate, 0.0
        next(side)

    def issued(self, result, lane, weight=0.0):
        rows = result.shape[0]
        self.history.append((self.clock, result))
        if lane == 3:
            self.clock += rows
        self.credit += self.rate * rows / 4 * weight
        count = int(self.credit)
        self.credit -= count
        for i in range(count):
            if self.side is not None:
                v = min(rows // 8 - 1, int(rows // 8 * (lane + (i + 0.5) / count) / 4))
                try:
                    self.side.send(result[8 * v:8 * v + 8])
                except StopIteration:
                    self.side = None

    def hold(self, value, lead):
        target = self.clock - lead
        if target < 0 or self.never is None:
            return value
        for start, result in reversed(self.history):
            if start <= target:
                v = min(result.shape[0] // 8 - 1, int(target - start) // 8)
                return jnp.where(self.never, result[8 * v:8 * v + 8], value)
        return value


def _kernel(
    shift_hbm, ssmd_hbm, beta_hbm, fwd_hbm, inv_hbm,
    q_hbm, k_hbm, v_hbm, ssm_hbm, x_hbm, wq_hbm, wk_hbm, wv_hbm, wo_hbm, out_hbm,
    shift_ref, ssmd_ref, beta_ref, fwd_ref, inv_ref,
    xs, wraw, wt, wot, qa, ka, va, ssk, spec_buf, yf, outa, outb,
    gate, bias, qm, qd, pq, kk, vt, pk_keep, vt_keep, ot, mz, sem_in, sem_out,
):
    def w_copies(n, sem):
        return [
            pltpu.make_async_copy(src.at[:, pl.ds(n * T, T)], wraw.at[i, n], sem)
            for i, src in enumerate((wq_hbm, wk_hbm, wv_hbm))
        ]

    def x_copies(lo, hi, sem):
        rows = pl.ds(int(lo * L), int((hi - lo) * L))
        return [
            pltpu.make_async_copy(x_hbm.at[0, rows, pl.ds(c * T, T)], xs.at[c, rows], sem)
            for c in range(NC)
        ]

    def column_tiles(src, dst, sem):
        return [
            pltpu.make_async_copy(src.at[0, :, pl.ds(c * T, T)], dst.at[c], sem)
            for c in range(NC)
        ]

    loads = [
        w_copies(0, sem_in.at[0]),
        x_copies(0, XSPLIT, sem_in.at[1])
        + [pltpu.make_async_copy(beta_hbm, beta_ref, sem_in.at[1])],
        w_copies(1, sem_in.at[2]),
        sum((w_copies(n, sem_in.at[3]) for n in range(2, NC)), x_copies(1, 2, sem_in.at[3])),
        x_copies(XSPLIT, 1, sem_in.at[4]) if XSPLIT < 1 else [],
        [pltpu.make_async_copy(src, dst, sem_in.at[5]) for src, dst in (
            (shift_hbm, shift_ref), (ssmd_hbm, ssmd_ref), (fwd_hbm, fwd_ref), (inv_hbm, inv_ref),
            (ssm_hbm, ssk))]
        + column_tiles(k_hbm, ka, sem_in.at[5]) + column_tiles(v_hbm, va, sem_in.at[5])
        + [pltpu.make_async_copy(wo_hbm.at[:, pl.ds(n * T, T)], wraw.at[3, n], sem_in.at[5])
           for n in range(NC)],
        x_copies(2, NSEG, sem_in.at[6]),
        column_tiles(q_hbm, qa, sem_in.at[7]),
    ]
    def start(lo, hi):
        for copies in loads[lo:hi]:
            for cp in copies:
                cp.start()

    start(0, 2)
    start(4, 5)
    start(2, DMA0)

    def wait(i):
        for cp in loads[i]:
            cp.wait()

    mz[...] = jnp.zeros(mz.shape, f32)
    row = lax.broadcasted_iota(i32, (T // 2, T), 0)
    col = lax.broadcasted_iota(i32, (T // 2, T), 1)
    bias[0] = jnp.where(row <= col, 0.0, NEG)
    bias[1] = jnp.where(row <= col % (T // 2), 0.0, NEG)

    def setup_gate():
        beta = jnp.concatenate(
            [beta_ref[...].astype(f32)[None, :], jnp.zeros((1, T - H), f32)], axis=1)
        gate[...] = jax.nn.sigmoid(jnp.broadcast_to(beta, (T, T)).T[:H])

    def transpose_qkv(part):
        n, i = divmod(part, 3)
        for c in range(NC):
            tile = _as_bf16(wraw.bitcast(u32)[i, n, c * 64:(c + 1) * 64, :])
            wt[i, c, n * T // 2:(n + 1) * T // 2, :] = pltpu.bitcast(tile.T, u32)

    def transpose_wo(n):
        for c in range(NC):
            words = wraw.bitcast(u32)[3, n, c * 64:(c + 1) * 64, :]
            wot[c, n * T // 2:(n + 1) * T // 2, :] = pltpu.bitcast(_as_bf16(words).T, u32)

    sub = lax.broadcasted_iota(i32, (8, T), 0)
    low = sub < 4
    left = lax.broadcasted_iota(i32, (8, T), 1) < T // 2

    def project(s, g, slot, pacer):
        rows = _ds(g * (GW // 2), GW // 2, 8)
        acc = [None] * NQ

        def store(n):
            q_t, k_t, v_t = acc[n][:GW], acc[n][GW:2 * GW], acc[n][2 * GW:]
            k_pad = jnp.concatenate([k_t.astype(bf16), jnp.zeros((T - GW, T), bf16)], axis=0)
            kk[slot, n] = pltpu.bitcast(k_pad.T, u32)
            qs = q_t * (DH ** -0.5 * LOG2E)
            r = [qs[8 * i:8 * i + 8] for i in range(10)]
            zero = jnp.zeros((8, T), f32)
            heads = [
                r[0], r[1], jnp.where(low, r[2], 0.0), zero,
                jnp.where(low, 0.0, r[2]), r[3], r[4], zero,
                zero, r[5], r[6], jnp.where(low, r[7], 0.0),
                zero, jnp.where(low, 0.0, r[7]), r[8], r[9],
            ]
            qm[slot, n] = _as_words(jnp.concatenate(heads, axis=0))
            e = {i: jnp.where(left, pltpu.roll(r[i], 64, 1), 0.0) for i in (0, 1, 2, 5, 6, 7)}
            o = {i: jnp.where(left, 0.0, r[i]) for i in (2, 3, 4, 7, 8, 9)}
            pairs = [
                e[0], e[1], jnp.where(low, e[2], o[2]), o[3], o[4], zero,
                zero, e[5], e[6], jnp.where(low, e[7], o[7]), o[8], o[9],
            ]
            qd[slot, n] = _as_words(jnp.concatenate(pairs, axis=0))
            pq[slot, n] = _as_words(_phi(q_t))
            pk_keep[s % 2, g, n] = _as_words(_phi(k_t))
            vt[slot, n] = v_t
            vt_keep[s % 2, g, n] = v_t

        def step(i):
            for lane in range(4):
                n, c = divmod(4 * i + lane, NC)
                w = _as_bf16(jnp.concatenate([wt[m, c, rows, :] for m in range(3)], axis=0))
                if XB:
                    xt = _as_bf16(xs.bitcast(u32)[c, _ds(s * (L // 2) + n * (T // 2), T // 2, T // 2), :])
                else:
                    xt = xs[c, _ds(s * L + n * T, T, T), :]
                part = _dot_nt(w, xt)
                pacer.issued(part, lane, WP)
                acc[n] = part if c == 0 else acc[n] + part
                if c == NC - 1:
                    store(n)

        return step

    def masked_dot(key_words, window, first):
        end = first + window.shape[0]
        parts = [window, jnp.zeros((T - end, T), bf16)]
        if first:
            parts.insert(0, jnp.zeros((first, T), bf16))
        return _dot(_as_bf16(key_words), jnp.concatenate(parts, axis=0))

    def update(s, g, pacer):
        state = mz[g]
        for kt in range(NQ):
            v_one = jnp.concatenate(
                [vt_keep[(s + 1) % 2, g, kt], jnp.ones((8, T), f32)], axis=0)
            pk_t = jnp.concatenate(
                [_as_bf16(pk_keep[(s + 1) % 2, g, kt]), jnp.zeros((T - GW, T), bf16)], axis=0)
            part = _dot_nt(v_one, pk_t)
            pacer.issued(part, kt, WM)
            state = state + part
        mz[g] = state

    def attend(s, g, slot, pacer, memory):
        lead, stagger = (LEAD1, STAG1) if memory else (LEAD0, STAG0)
        tiles = [(qt, kt) for qt in ORDER for kt in range(qt + 1)]
        logits, run_max, col_max, acc, mem, done = {}, {}, {}, {}, {}, []
        corner, corner_max, corner_p = {}, {}, {}
        gates = [jnp.broadcast_to(gate[pl.ds(4 * g + j, 1), :], (8, T)) for j in range(4)]

        low_pair = sub % 4 < 2
        rest_rows = 1.0 - jnp.where(low, jnp.where(low_pair, gates[1], gates[3]),
                                    jnp.where(low_pair, gates[0], gates[2]))

        def read(_):
            def head_of(i):
                return (i >= DH).astype(i32) + (i >= 2 * DH).astype(i32) + (i >= 3 * DH).astype(i32)

            state = mz[g]
            row_m = lax.broadcasted_iota(i32, (GW, T), 0)
            col_m = lax.broadcasted_iota(i32, (GW, T), 1)
            weights = jnp.where(head_of(row_m) == head_of(col_m), state[:GW], 0.0)
            lane_head = head_of(lax.broadcasted_iota(i32, (8, T), 1))
            pair_of = sub // 2
            z_rows = jnp.where(lane_head == pair_of, state[GW:], 0.0)
            mem_w = jnp.concatenate([weights, z_rows], axis=0)
            g_rows = jnp.where(low, jnp.where(sub < 2, gates[0], gates[1]),
                               jnp.where(sub < 6, gates[2], gates[3]))
            for qt in range(NQ):
                rhs = _as_bf16(pq[slot, qt])
                if FULLK:
                    rhs = jnp.concatenate([rhs, jnp.zeros((T - GW, T), bf16)], axis=0)
                res = lax.dot_general(
                    mem_w[:, :rhs.shape[0]], rhs, NN, preferred_element_type=f32)
                pacer.issued(res, qt, WM)
                coef = g_rows / (res[GW:] + 1e-6)
                c0, c1, c2, c3 = (
                    jnp.broadcast_to(coef[2 * j:2 * j + 1], (8, T)) for j in range(4))
                cm = [c0, c0, jnp.where(low, c0, c1), c1, c1,
                      c2, c2, jnp.where(low, c2, c3), c3, c3]
                mem[qt] = [res[8 * i:8 * i + 8] * cm[i] for i in range(10)]
            finish()

        def corners(i):
            for lane in range(4):
                qt, pr = ORDER[2 * i + lane // 2], lane % 2
                window = _as_bf16(qd[slot, qt, 24 * pr:24 * pr + 24, :])
                sc = masked_dot(kk[slot, qt, T // 4:, :], window, 32 * pr)
                pacer.issued(sc, lane, WA)
                corner[qt, pr] = sc + bias[1]
                corner_max[qt, pr] = jnp.max(corner[qt, pr].reshape(8, 8, T), axis=0)

        def scores(t):
            qt, kt = tiles[t]
            for j in range(4):
                window = _as_bf16(qm[slot, qt, 16 * j:16 * j + 16, :])
                sc = masked_dot(
                    kk[slot, kt] if kt < qt else kk[slot, kt, :T // 4, :], window, 16 * j)
                pacer.issued(sc, j, WA)
                if kt == qt:
                    sc = sc + bias[0]
                m8 = jnp.max(sc.reshape(-1, 8, T), axis=0)
                run_max[qt, j] = m8 if kt == 0 else jnp.maximum(run_max[qt, j], m8)
                if kt == qt:
                    extra = corner_max[qt, j // 2]
                    if j % 2 == 0:
                        extra = pltpu.roll(extra, T // 2, 1)
                    top = jnp.maximum(run_max[qt, j], jnp.where(left, NEG, extra))
                    col_max[qt, j] = jnp.broadcast_to(
                        jnp.max(top, axis=0, keepdims=True), (8, T))
                logits[t, j] = sc
            if kt == qt:
                for pr in range(2):
                    top = jnp.where(left, pltpu.roll(col_max[qt, 2 * pr], T // 2, 1),
                                    col_max[qt, 2 * pr + 1])
                    words = _as_words(jnp.exp2(
                        corner[qt, pr].reshape(8, 8, T) - top[None]).reshape(T // 2, T))
                    for j, shifted in enumerate((pltpu.roll(words, T // 2, 1), words)):
                        corner_p[qt, 2 * pr + j] = _as_bf16(jnp.where(
                            left[None], jnp.uint32(0), shifted.reshape(4, 8, T)).reshape(32, T))

        def values(t):
            qt, kt = tiles[t]
            tops = [pacer.hold(col_max[qt, j], lead - stagger * j) for j in range(4)]
            for j in range(4):
                p = jnp.exp2(logits[t, j].reshape(-1, 8, T) - tops[j][None])
                p = p.reshape(-1, T).astype(bf16)
                if kt == qt:
                    p = jnp.concatenate([p, corner_p[qt, j]], axis=0)
                first = (0, 16, 40, 56)[j]
                v = [vt[slot, kt, first + 8 * i:first + 8 * i + 8, :] for i in range(3)]
                if j % 2 == 0:
                    v[2] = jnp.where(low, v[2], 1.0)
                else:
                    v[0] = jnp.where(low, 1.0, v[0])
                part = lax.dot_general(
                    jnp.concatenate(v, axis=0), p, NN, preferred_element_type=f32)
                pacer.issued(part, j)
                acc[qt, j] = part if kt == 0 else acc[qt, j] + part
            if kt == qt:
                done.append(qt)
                finish()

        def finish():
            while done and (not memory or done[0] in mem):
                qt = done.pop(0)
                w = [[acc[qt, j][8 * i:8 * i + 8] for i in range(3)] for j in range(4)]
                sums = jnp.where(
                    low_pair, jnp.where(low, w[1][0], w[0][2]),
                    pltpu.roll(jnp.where(low, w[3][0], w[2][2]), 2, 0))
                coef = rest_rows / sums
                c0, c1, c2, c3 = (
                    jnp.broadcast_to(coef[r:r + 1], (8, T)) for r in (4, 0, 6, 2))
                o = [w[0][0] * c0, w[0][1] * c0,
                     jnp.where(low, w[0][2] * c0, w[1][0] * c1), w[1][1] * c1, w[1][2] * c1,
                     w[2][0] * c2, w[2][1] * c2,
                     jnp.where(low, w[2][2] * c2, w[3][0] * c3), w[3][1] * c3, w[3][2] * c3]
                if memory:
                    o = [mem[qt][i] + o[i] for i in range(10)]
                ot[s % 2, qt, _ds(g * (GW // 2), GW // 2, 8), :] = _as_words(
                    jnp.concatenate(o, axis=0))

        return {"D": corners, "Q": scores, "V": values, "R": read}

    def wo_tile(c, m):
        return _as_bf16(wraw.bitcast(u32)[3, m, c * 64:(c + 1) * 64, :])

    def out_project(s, n, pacer):
        acc, done = [None] * 4, []

        def step(i):
            for lane in range(4):
                m, c = divmod(4 * i + lane, NC)
                part = _dot(_as_bf16(wot[c, 80 * m:80 * (m + 1), :]),
                            _as_bf16(ot[s % 2, n, c * 64:(c + 1) * 64, :]))
                pacer.issued(part, lane, WO)
                acc[m] = part if c == 0 else acc[m] + part
                if c == NC - 1:
                    acc[m] = acc[m].astype(bf16)
                    while T * (len(done) + 1) <= 160 * (m + 1):
                        i0 = T * len(done)
                        pieces = [acc[k][max(i0 - 160 * k, 0):min(i0 + T - 160 * k, 160)]
                                  for k in range(i0 // 160, (i0 + T - 1) // 160 + 1)]
                        tile = jnp.concatenate(pieces, axis=0).T
                        outb.bitcast(u32)[s, _ds(n * 64, 64, 64), i0:i0 + T] = pltpu.bitcast(tile, u32)
                        done.append(True)

        return step

    def outb_copy(s, n):
        return pltpu.make_async_copy(
            outb.at[s, _ds(n * T, T, T)],
            out_hbm.at[0, _ds(s * L + n * T, T, T), pl.ds(D, D)], sem_out.at[0])

    def conv_forward(c):
        cols = slice(c * T, (c + 1) * T)
        taps = shift_ref[:, cols].astype(f32)
        taps = [jnp.broadcast_to(taps[j:j + 1], (T, T)) for j in range(4)]
        skip = ssmd_ref[...].astype(f32)[c:c + 1]
        slices = pl.ds(c * NFV, NFV)

        def transform(even, odd):
            if not RHS32:
                even, odd = even.astype(bf16), odd.astype(bf16)
            e, o = (
                lax.dot_general(_as_bf16(fwd_ref.bitcast(u32)[i]), x, NN, preferred_element_type=f32)
                for i, x in enumerate((even, odd)))
            return [x.reshape(NFV, 2, 8, T) for x in (e + o, e - o)]

        tail = jnp.zeros((8, T), u32)
        prev = None
        for b in range(NB):
            k0 = ka.bitcast(u32)[c, b * T:(b + 1) * T, :]
            ext = jnp.concatenate([tail, k0], axis=0)
            tail = k0[T - 8:]
            k1, k2 = ext[7:7 + T], ext[6:6 + T]
            e0, o0, e1, o1, o2 = (
                _even_rows(k0), _odd_rows(k0), _even_rows(k1), _odd_rows(k1), _odd_rows(k2))
            v0 = va.bitcast(u32)[c, b * T:(b + 1) * T, :]
            sig = transform(
                (e0 * taps[0] + o1 * taps[1] + e1 * taps[2] + o2 * taps[3]) * _even_rows(v0),
                (o0 * taps[0] + e0 * taps[1] + o1 * taps[2] + e1 * taps[3]) * _odd_rows(v0))
            taps_t = jnp.concatenate([
                pltpu.bitcast(ssk[cols, (2 * b + i) * T:(2 * b + i + 1) * T].T, u32)
                for i in range(2)], axis=0)
            filt = transform(_even_rows(taps_t), _odd_rows(taps_t))
            for sign in range(2):
                spec_buf[slices, 0, sign, b] = sig[sign].reshape(NFV, 16, T)
                re, im = filt[sign][:, 0], filt[sign][:, 1]
                if prev is None:
                    re = re + skip[None]
                else:
                    half = NFV // 2
                    pre, pim = prev[sign][:, 0], prev[sign][:, 1]
                    re = jnp.concatenate([re[:half] - pim[:half], re[half:] + pim[half:]], axis=0)
                    im = jnp.concatenate([im[:half] + pre[:half], im[half:] - pre[half:]], axis=0)
                spec_buf[slices, 1, sign, b, 0:8, :] = re
                spec_buf[slices, 1, sign, b, 8:16, :] = im
            prev = filt

    def conv_mix(first, count, never, blk=MIXBLK):
        half = NFV // 2
        for item in range(count):
            idx = jnp.minimum(first + item, NC * half - 1)
            base = idx // half * NFV + idx % half

            def products(fv, sign, a0):
                def load(which, b):
                    return (spec_buf[fv, which, sign, b, 0:8, :],
                            spec_buf[fv, which, sign, b, 8:16, :])

                acc, kcache = [None] * blk, {}
                for b in range(a0 + blk):
                    token = yield
                    ur, ui = load(0, b)
                    ur = jnp.where(never, token, ur)
                    if GATE2:
                        ui = jnp.where(never, token, ui)
                    us = ur + ui
                    for a in range(max(a0, b), a0 + blk):
                        if a - b not in kcache:
                            kr, ki = load(1, a - b)
                            kcache[a - b] = (kr, ki - kr, kr + ki)
                        k1, k2, k3 = kcache[a - b]
                        terms = (us * k1, ur * k2, ui * k3)
                        old = acc[a - a0]
                        acc[a - a0] = terms if old is None else tuple(
                            o + t for o, t in zip(old, terms))
                return [(p1 - p3, p1 + p2) for p1, p2, p3 in acc]

            for a0 in range(0, NB, blk):
                parity = []
                for fv in (base, base + half):
                    plus = yield from products(fv, 0, a0)
                    minus = yield from products(fv, 1, a0)
                    parity.append((
                        [(pr + mr, pi + mi) for (pr, pi), (mr, mi) in zip(plus, minus)],
                        [(pr - mr, pi - mi) for (pr, pi), (mr, mi) in zip(plus, minus)]))
                for i in range(blk):
                    (ar, ai), (br, bi) = parity[0][0][i], parity[1][0][i]
                    (cr, ci), (dr, di) = parity[0][1][i], parity[1][1][i]
                    folded = ((ar + br, ai - bi), (cr - di, ci - dr),
                              (ar - br, ai + bi), (cr + di, ci + dr))
                    for r in range(4):
                        yf[idx, a0 + i, r] = _as_words(jnp.concatenate(folded[r], axis=0))

    def outa_copy(c):
        return pltpu.make_async_copy(
            outa.at[c], out_hbm.at[0, :, _ds(c * T, T, T)], sem_out.at[0])

    def conv_inverse(pacer, zero):
        pending, pin, hold = [], [], []

        def send(c):
            outa_copy(c).start()
            pin.append(True)

        def flush(_=0):
            while pending:
                c, a, y = pending.pop(0)
                tile = c + zero if pin else c
                for i in range(2):
                    rows = pl.ds(a * T + i, T // 2, stride=2)
                    q_words = qa.bitcast(u32)[c, rows, :]
                    outa.bitcast(u32)[tile, rows, :] = _interleave(
                        _even_rows(q_words) * y[2 * i], _odd_rows(q_words) * y[2 * i + 1])
                if pin:
                    hold.append(outa.bitcast(u32)[tile, a * T:a * T + 8, :])
                    pin.clear()

        def step(i):
            c, a = divmod(i, NB)
            res = []
            for r in range(4):
                words = yf[pl.ds(c * NFV // 2, NFV // 2), a, r].reshape(T // 2, T)
                if hold:
                    words = jnp.concatenate(
                        [jnp.where(pacer.never, hold.pop(), words[:8]), words[8:]], axis=0)
                res.append(_dot(
                    _as_bf16(inv_ref.bitcast(u32)[r]), _as_bf16(words)))
                pacer.issued(res[-1], r, WI)
            flush()
            pending.append((c, a, res))

        return step, flush, send

    def out_project_last(pacer, zero):
        s = NSEG - 1
        o_rows, acc = {}, {}

        def transpose(n):
            for c in range(NC):
                o_rows[n, c] = _as_bf16(ot[s % 2, n, c * 64:(c + 1) * 64, :]).T

        def step(i):
            for lane in range(4):
                tile, c = divmod(4 * i + lane, NC)
                n, m = divmod(tile, NC)
                part = _dot(o_rows[n, c], wo_tile(c, m))
                pacer.issued(part, lane)
                acc[tile] = part if c == 0 else acc[tile] + part

        def store(part):
            n = min(part, NQ - 1)
            for m in range(NC) if part < NQ - 1 else ((0, 1, 2), (3, 4))[part - n]:
                seg = s + zero if m == 0 else s
                outb.bitcast(u32)[seg, n * 64:(n + 1) * 64, m * T:(m + 1) * T] = _as_words(
                    acc[n * NC + m])

        return transpose, step, store

    def new_pacer():
        return _Pacer(gate[0:8, :] > 2.0)

    def pair(s, p, plan, pacer, mix=None):
        memory = "Ra" in plan
        if mix is not None:
            first, count, cycles = mix
            pacer.attach(conv_mix(first, count, pacer.never), count * {2: 80, 4: 48, 8: 32}[MIXBLK] * 2 / cycles)
        steps = {"a": attend(s, 2 * p, 0, pacer, memory),
                 "b": attend(s, 2 * p + 1, 1, pacer, memory)}
        steps["a"]["P"] = project(s, 2 * p + 1, 1, pacer)
        next_s, next_g = s + (p + 1) // 4, (2 * p + 2) % NG
        steps["b"]["P"] = project(next_s, next_g, 0, pacer)
        steps["a"]["U"] = lambda _: update(s, 2 * p + 1, pacer)
        steps["b"]["U"] = lambda _: update(next_s, next_g, pacer)
        steps["a"]["O"] = out_project(s - 1, p, pacer)
        steps["x"] = {
            "T": transpose_qkv,
            "W": wait,

            "C": lambda _: outb_copy(s - 1, p).start(),
        }
        if "Jx" in plan:
            zero = pacer.never.astype(i32)[0, 0]
            steps["x"]["I"], steps["x"]["J"], steps["x"]["A"] = conv_inverse(pacer, zero)
            steps["x"]["L"], steps["x"]["E"], steps["x"]["G"] = out_project_last(pacer, zero)
        steps["x"]["F"] = lambda n: outb_copy(s, n).start()
        for item in plan:
            steps[item[1]][item[0]](int(item[2:] or 0))
        assert pacer.side is None

    mix_cycles = (2 * (1152 * WA + 1200 * WP + 176 * WM) + 800 * WO) * SLACK

    def memory_pair(s, p):
        first = ((s - 1) * 4 + p) * MIX_PER_ITER
        pair(s, p, PLAN1, new_pacer(), (first, MIX_PER_ITER, mix_cycles))

    if ONLY:
        start(DMA0, 4)
        start(5, len(loads))
        for i in range(8):
            wait(i)
        setup_gate()
        if ONLY == "0":
            @pl.loop(1, 4)
            def _(p):
                pair(0, p, PLAN0, new_pacer())
        else:
            @pl.loop(0, 11)
            def _(i):
                memory_pair(1 + i // 4, i % 4)
        outa[0, 0:16] = jnp.concatenate([mz[0, 0:8], pltpu.bitcast(ot[0, 0, 0:8] + yf[0, 0, 0] + qm[0, 0, 0:8] + qd[0,0,0:8] + pq[0,0,0:8] + kk[0,0,0:8] + pk_keep[0,0,0,0:8] + outb.bitcast(u32)[0,0:8,0:128], f32) + vt[0,0,0:8] + vt_keep[0,0,0,0:8]], axis=0).astype(bf16)
        outa_copy(0).start()
        outa_copy(0).wait()
        return

    wait(0)
    start(DMA0, DMA1)
    for part in range(3):
        transpose_qkv(part)
    wait(1)
    start(5, len(loads))
    setup_gate()
    step = project(0, 0, 0, _Pacer(None))
    for i in range(NC):
        if i == int(XSPLIT * NC):
            wait(4)
        step(i)
    pair(0, 0, PLAN_FIRST, new_pacer())

    @pl.loop(1, 4)
    def _(p):
        pair(0, p, PLAN0, new_pacer())

    wait(5)
    update(1, 0, _Pacer(None))
    for c in range(NC):
        conv_forward(c)
        transpose_wo(c)
    wait(6)
    wait(7)

    @pl.loop(0, 11)
    def _(i):
        memory_pair(1 + i // 4, i % 4)

    pair(NSEG - 1, 3, PLAN_LAST, new_pacer())

    outb_copy(NSEG - 1, NQ - 1).start()
    for c in range(NC):
        outa_copy(c).wait()
    for s in range(NSEG):
        for n in range(NQ):
            outb_copy(s, n).wait()


@jax.jit
def pallas_concat_heads__ssm_conv_h3__memory_aug_infini_attn__prompt_kernel(
    A_q: jax.Array,
    A_k: jax.Array,
    A_v: jax.Array,
    A_shift_k: jax.Array,
    A_ssm_k: jax.Array,
    A_ssm_D: jax.Array,
    B_x: jax.Array,
    B_wq: jax.Array,
    B_wk: jax.Array,
    B_wv: jax.Array,
    B_wo: jax.Array,
    B_beta: jax.Array,
):
    hbm = pl.BlockSpec(memory_space=pl.ANY)
    scratch = [
        pltpu.VMEM((4, D), bf16),
        pltpu.VMEM((NC, T), bf16),
        pltpu.VMEM((H,), bf16),
        pltpu.VMEM((2, 2 * T, T), bf16),
        pltpu.VMEM((4, T // 2, T), bf16),
        pltpu.VMEM((NC, S, T), bf16),
        pltpu.VMEM((4, NC, D, T), bf16),
        pltpu.VMEM((3, NC, D // 2, T), u32),
        pltpu.VMEM((NC, D // 2, T), u32),
        pltpu.VMEM((NC, S, T), bf16),
        pltpu.VMEM((NC, S, T), bf16),
        pltpu.VMEM((NC, S, T), bf16),
        pltpu.VMEM((D, S), bf16),
        pltpu.VMEM((NC * NFV, 2, 2, NB, 16, T), f32),
        pltpu.VMEM((NC * NFV // 2, NB, 4, 8, T), u32),
        pltpu.VMEM((NC, S, T), bf16),
        pltpu.VMEM((NSEG, L, D), bf16),
        pltpu.VMEM((H, T), f32),
        pltpu.VMEM((2, T // 2, T), f32),
        pltpu.VMEM((2, NQ, 64, T), u32),
        pltpu.VMEM((2, NQ, 48, T), u32),
        pltpu.VMEM((2, NQ, GW // 2, T), u32),
        pltpu.VMEM((2, NQ, T // 2, T), u32),
        pltpu.VMEM((2, NQ, GW, T), f32),
        pltpu.VMEM((2, NG, NQ, GW // 2, T), u32),
        pltpu.VMEM((2, NG, NQ, GW, T), f32),
        pltpu.VMEM((2, NQ, D // 2, T), u32),
        pltpu.VMEM((NG, GW + 8, T), f32),
        pltpu.SemaphoreType.DMA((8,)),
        pltpu.SemaphoreType.DMA((1,)),
    ]
    return pl.pallas_call(
        _kernel,
        out_shape=jax.ShapeDtypeStruct((1, S, 2 * D), bf16),
        in_specs=[hbm] * 14,
        out_specs=hbm,
        scratch_shapes=scratch,
        compiler_params=pltpu.CompilerParams(
            vmem_limit_bytes=100 * 2**20,
            flags={_env("FLAG", ""): _env("FLAGV", 0) or True} if _env("FLAG", "") else None),
    )(
        A_shift_k.T, A_ssm_D.reshape(NC, T), B_beta, _FWD, _INV,
        A_q, A_k, A_v, A_ssm_k, B_x, B_wq, B_wk, B_wv, B_wo,
    )
```

```python
import jax
import jax.numpy as jnp
import numpy as np
from jax import lax
from jax.experimental import pallas as pl
from jax.experimental.pallas import tpu as pltpu

f32, bf16, u32, i32 = jnp.float32, jnp.bfloat16, jnp.uint32, jnp.int32

S, D, H, DH = 2048, 640, 32, 20
NSEG, L = 4, 512
T = 128
NC = D // T
NB = S // (2 * T)
NQ = L // T
NG = 8
GW = 4 * DH
NFV = 16
LOG2E = 1.4426950408889634
NEG = -1e30
MIX_PER_ITER = 4

PLAN_FIRST = (
    "Wx2 Qa0 Da0 Tx3 Tx4 Tx5 Qa1 Qa2 Qa3 Pa0 Qa4 Pa1 Va0 Pa2 Va1 Qa5 Pa3 Qa6 Pa4 Da1 Va2 Qa7 Va3 "
    "Qa8 Qa9 Va4 Qb0 Va5 Qb1 Va6 Db0 Va7 Qb2 Wx3 Tx6 Tx7 Tx8 Va8 Qb3 Vb0 Va9 Qb4 Pb0 Tx9 Tx10 "
    "Tx11 Qb5 Vb1 Qb6 Vb2 Db1 Vb3 Qb7 Tx12 Tx13 Tx14 Pb1 Pb2 Vb4 Qb8 Vb5 Qb9 Pb3 Pb4 Vb6 Vb7 Vb8 "
    "Vb9"
).split()
PLAN0 = (
    "Qa0 Da0 Pa0 Qa1 Pa1 Qa2 Qa3 Pa2 Pa3 Qa4 Va0 Va1 Qa5 Qa6 Pa4 Da1 Va2 Qa7 Va3 Qa8 Qa9 Va4 Qb0 "
    "Va5 Qb1 Va6 Db0 Va7 Qb2 Va8 Qb3 Va9 Qb4 Pb0 Qb5 Vb0 Vb1 Qb6 Vb2 Db1 Vb3 Qb7 Pb1 Pb2 Vb4 Qb8 "
    "Vb5 Qb9 Pb3 Pb4 Vb6 Vb7 Vb8 Vb9"
).split()
PLAN1 = (
    "Qa0 Da0 Pa0 Pa1 Qa1 Qa2 Qa3 Pa2 Pa3 Va0 Pa4 Qa4 Qa5 Va1 Qa6 Oa0 Va2 Qa7 Va3 Da1 Oa1 Oa2 Qa8 "
    "Va4 Oa3 Oa4 Va5 Qa9 Ua Ra Va6 Qb0 Va7 Qb1 Db0 Qb2 Va8 Qb3 Pb0 Vb0 Va9 Pb1 Qb4 Qb5 Qb6 Vb1 "
    "Db1 Vb2 Qb7 Vb3 Pb2 Qb8 Vb4 Vb5 Qb9 Pb3 Vb6 Cx Pb4 Rb Vb7 Vb8 Vb9 Ub"
).split()
PLAN_LAST = (
    "Qa0 Da0 Pa0 Pa1 Qa1 Qa2 Qa3 Pa2 Pa3 Pa4 Qa4 Ix0 Qa5 Ix1 Va0 Ix2 Va1 Qa6 Ix3 Oa0 Va2 Qa7 Ix4 "
    "Da1 Va3 Oa1 Ix5 Oa2 Qa8 Ix6 Va4 Oa3 Ix7 Oa4 Va5 Qa9 Ix8 Cx Ax0 Ra Ua Va6 Ix9 Qb0 Ix10 Va7 "
    "Qb1 Ix11 Db0 Ix12 Qb2 Va8 Ix13 Qb3 Ix14 Vb0 Va9 Ix15 Qb4 Ix16 Ax1 Qb5 Ix17 Vb1 Qb6 Ix18 Db1 "
    "Ix19 Vb2 Qb7 Ix20 Vb3 Ix21 Qb8 Ix22 Vb4 Ix23 Vb5 Qb9 Ix24 Ax2 Ix25 Ix26 Vb6 Ix27 Rb Ix28 Vb7 "
    "Ix29 Ix30 Vb8 Ix31 Ix32 Ax3 Vb9 Ix33 Lx3 Ix34 Lx2 Ix35 Ix36 Lx1 Ix37 Ix38 Lx0 Ix39 Ex0 Jx "
    "Ax4 Ex1 Ex2 Ex3 Ex4 Ex5 Ex6 Gx0 Fx0 Ex7 Ex8 Ex9 Ex10 Ex11 Ex12 Gx1 Fx1 Ex13 Ex14 Ex15 Ex16 "
    "Ex17 Ex18 Gx2 Fx2 Ex19 Ex20 Ex21 Ex22 Gx3 Ex23 Ex24 Gx4"
).split()
ORDER = (3, 2, 1, 0)
LEAD = {False: (400, 56), True: (400, 24)}
WA, WP, WO, WM = 1.2, 1.0, 1.0, 1.2
MIX_CYCLES = (2 * (1152 * WA + 1200 * WP + 176 * WM) + 800 * WO) * 0.965

NN = (((1,), (0,)), ((), ()))
NT = (((1,), (1,)), ((), ()))


def _dft_tables():
    freq = np.concatenate([np.arange(0, T, 2), T - 1 - np.arange(0, T, 2)])

    def table(freq, n):
        theta = 2.0 * np.pi * (freq[:, None] + 0.5) * n[None, :] / (4 * T)
        parts = [f(theta).reshape(-1, 8, len(n)) for f in (np.cos, lambda t: -np.sin(t))]
        return np.stack(parts, axis=1).reshape(-1, len(n))

    fwd = np.stack([table(freq, 2 * np.arange(T) + r) for r in range(2)])
    inv = np.stack([table(freq[:T // 2], 4 * np.arange(T // 2) + r).T / (2 * T) for r in range(4)])
    return fwd.astype(np.float32).astype(bf16), inv.astype(np.float32).astype(bf16)


_FWD, _INV = _dft_tables()


def _as_bf16(words):
    return pltpu.bitcast(words, bf16)


def _as_words(x):
    return pltpu.bitcast(x.astype(bf16), u32)


def _even_rows(words):
    return pltpu.bitcast(words << 16, f32)


def _odd_rows(words):
    return pltpu.bitcast(words & np.uint32(0xFFFF0000), f32)


def _interleave(even, odd):
    even, odd = (pltpu.bitcast(x.astype(bf16).astype(f32), u32) for x in (even, odd))
    return (even >> 16) | odd


def _dot(a, b):
    return lax.dot_general(a, b, NN, preferred_element_type=f32)


def _dot_nt(a, b):
    return lax.dot_general(a, b, NT, preferred_element_type=f32)


def _phi(t):
    return jnp.maximum(t, 0.0) + jnp.exp(jnp.minimum(t, 0.0))


def _ds(start, size, align):
    if isinstance(start, int):
        return pl.ds(start, size)
    return pl.ds(pl.multiple_of(start, align), size)


class _Pacer:
    def __init__(self, never):
        self.never, self.side, self.rate = never, None, 0.0
        self.credit, self.clock, self.history = 0.0, 0.0, []

    def attach(self, side, rate):
        self.side, self.rate, self.credit = side, rate, 0.0
        next(side)

    def issued(self, result, lane, weight=0.0):
        rows = result.shape[0]
        self.history.append((self.clock, result))
        if lane == 3:
            self.clock += rows
        self.credit += self.rate * rows / 4 * weight
        count = int(self.credit)
        self.credit -= count
        for i in range(count):
            if self.side is not None:
                v = min(rows // 8 - 1, int(rows // 8 * (lane + (i + 0.5) / count) / 4))
                try:
                    self.side.send(result[8 * v:8 * v + 8])
                except StopIteration:
                    self.side = None

    def hold(self, value, lead):
        target = self.clock - lead
        if target < 0 or self.never is None:
            return value
        for start, result in reversed(self.history):
            if start <= target:
                v = min(result.shape[0] // 8 - 1, int(target - start) // 8)
                return jnp.where(self.never, result[8 * v:8 * v + 8], value)
        return value


def _kernel(
    shift_hbm, ssmd_hbm, beta_hbm, fwd_hbm, inv_hbm,
    q_hbm, k_hbm, v_hbm, ssm_hbm, x_hbm, wq_hbm, wk_hbm, wv_hbm, wo_hbm, out_hbm,
    shift_ref, ssmd_ref, beta_ref, fwd_ref, inv_ref,
    xs, wraw, wt, wot, qa, ka, va, ssk, spec_buf, yf, outa, outb,
    gate, bias, qm, qd, pq, kk, vt, pk_keep, vt_keep, ot, mz, sem_in, sem_out,
):
    def w_copies(n, sem):
        return [
            pltpu.make_async_copy(src.at[:, pl.ds(n * T, T)], wraw.at[i, n], sem)
            for i, src in enumerate((wq_hbm, wk_hbm, wv_hbm))
        ]

    def x_copies(lo, hi, sem):
        rows = pl.ds(lo * L, (hi - lo) * L)
        return [
            pltpu.make_async_copy(x_hbm.at[0, rows, pl.ds(c * T, T)], xs.at[c, rows], sem)
            for c in range(NC)
        ]

    def column_tiles(src, dst, sem):
        return [
            pltpu.make_async_copy(src.at[0, :, pl.ds(c * T, T)], dst.at[c, pl.ds(0, S)], sem)
            for c in range(NC)
        ]

    loads = [
        w_copies(0, sem_in.at[0]),
        x_copies(0, 1, sem_in.at[1])
        + [pltpu.make_async_copy(beta_hbm, beta_ref, sem_in.at[1])],
        w_copies(1, sem_in.at[2]),
        sum((w_copies(n, sem_in.at[3]) for n in range(2, NC)), x_copies(1, 2, sem_in.at[3])),
        [pltpu.make_async_copy(src, dst, sem_in.at[4]) for src, dst in (
            (shift_hbm, shift_ref), (ssmd_hbm, ssmd_ref), (fwd_hbm, fwd_ref), (inv_hbm, inv_ref),
            (ssm_hbm, ssk))]
        + column_tiles(k_hbm, ka, sem_in.at[4]) + column_tiles(v_hbm, va, sem_in.at[4])
        + [pltpu.make_async_copy(wo_hbm.at[:, pl.ds(n * T, T)], wraw.at[3, n], sem_in.at[4])
           for n in range(NC)],
        x_copies(2, NSEG, sem_in.at[5]),
        column_tiles(q_hbm, qa, sem_in.at[6]),
    ]
    def start(lo, hi):
        for copies in loads[lo:hi]:
            for cp in copies:
                cp.start()

    start(0, 3)

    def wait(i):
        for cp in loads[i]:
            cp.wait()

    mz[...] = jnp.zeros(mz.shape, f32)
    row = lax.broadcasted_iota(i32, (T // 2, T), 0)
    col = lax.broadcasted_iota(i32, (T // 2, T), 1)
    bias[0] = jnp.where(row <= col, 0.0, NEG)
    bias[1] = jnp.where(row <= col % (T // 2), 0.0, NEG)

    def setup_gate():
        beta = jnp.concatenate(
            [beta_ref[...].astype(f32)[None, :], jnp.zeros((1, T - H), f32)], axis=1)
        gate[...] = jax.nn.sigmoid(jnp.broadcast_to(beta, (T, T)).T[:H])

    def transpose_qkv(part):
        n, i = divmod(part, 3)
        for c in range(NC):
            tile = _as_bf16(wraw.bitcast(u32)[i, n, c * 64:(c + 1) * 64, :])
            wt[i, c, n * T // 2:(n + 1) * T // 2, :] = pltpu.bitcast(tile.T, u32)

    def transpose_wo(n):
        for c in range(NC):
            words = wraw.bitcast(u32)[3, n, c * 64:(c + 1) * 64, :]
            wot[c, n * T // 2:(n + 1) * T // 2, :] = pltpu.bitcast(_as_bf16(words).T, u32)

    sub = lax.broadcasted_iota(i32, (8, T), 0)
    low = sub < 4
    left = lax.broadcasted_iota(i32, (8, T), 1) < T // 2

    def project(s, g, slot, pacer):
        rows = _ds(g * (GW // 2), GW // 2, 8)
        acc = [None] * NQ

        def store(n):
            q_t, k_t, v_t = acc[n][:GW], acc[n][GW:2 * GW], acc[n][2 * GW:]
            k_pad = jnp.concatenate([k_t.astype(bf16), jnp.zeros((T - GW, T), bf16)], axis=0)
            kk[slot, n] = pltpu.bitcast(k_pad.T, u32)
            qs = q_t * (DH ** -0.5 * LOG2E)
            r = [qs[8 * i:8 * i + 8] for i in range(10)]
            zero = jnp.zeros((8, T), f32)
            heads = [
                r[0], r[1], jnp.where(low, r[2], 0.0), zero,
                jnp.where(low, 0.0, r[2]), r[3], r[4], zero,
                zero, r[5], r[6], jnp.where(low, r[7], 0.0),
                zero, jnp.where(low, 0.0, r[7]), r[8], r[9],
            ]
            qm[slot, n] = _as_words(jnp.concatenate(heads, axis=0))
            e = {i: jnp.where(left, pltpu.roll(r[i], 64, 1), 0.0) for i in (0, 1, 2, 5, 6, 7)}
            o = {i: jnp.where(left, 0.0, r[i]) for i in (2, 3, 4, 7, 8, 9)}
            pairs = [
                e[0], e[1], jnp.where(low, e[2], o[2]), o[3], o[4], zero,
                zero, e[5], e[6], jnp.where(low, e[7], o[7]), o[8], o[9],
            ]
            qd[slot, n] = _as_words(jnp.concatenate(pairs, axis=0))
            pq[slot, n] = _as_words(_phi(q_t))
            pk_keep[s % 2, g, n] = _as_words(_phi(k_t))
            vt[slot, n] = v_t
            vt_keep[s % 2, g, n] = v_t

        def step(i):
            for lane in range(4):
                n, c = divmod(4 * i + lane, NC)
                w = _as_bf16(jnp.concatenate([wt[m, c, rows, :] for m in range(3)], axis=0))
                times = _ds(s * (L // 2) + n * (T // 2), T // 2, T // 2)
                part = _dot_nt(w, _as_bf16(xs.bitcast(u32)[c, times, :]))
                pacer.issued(part, lane, WP)
                acc[n] = part if c == 0 else acc[n] + part
                if c == NC - 1:
                    store(n)

        return step

    def masked_dot(key_words, window, first):
        end = first + window.shape[0]
        parts = [window, jnp.zeros((T - end, T), bf16)]
        if first:
            parts.insert(0, jnp.zeros((first, T), bf16))
        return _dot(_as_bf16(key_words), jnp.concatenate(parts, axis=0))

    def update(s, g, pacer):
        state = mz[g]
        for kt in range(NQ):
            v_one = jnp.concatenate(
                [vt_keep[(s + 1) % 2, g, kt], jnp.ones((8, T), f32)], axis=0)
            pk_t = jnp.concatenate(
                [_as_bf16(pk_keep[(s + 1) % 2, g, kt]), jnp.zeros((T - GW, T), bf16)], axis=0)
            part = _dot_nt(v_one, pk_t)
            pacer.issued(part, kt, WM)
            state = state + part
        mz[g] = state

    def attend(s, g, slot, pacer, memory):
        lead, stagger = LEAD[memory]
        tiles = [(qt, kt) for qt in ORDER for kt in range(qt + 1)]
        logits, run_max, col_max, acc, mem, done = {}, {}, {}, {}, {}, []
        corner, corner_max, corner_p = {}, {}, {}
        gates = [jnp.broadcast_to(gate[pl.ds(4 * g + j, 1), :], (8, T)) for j in range(4)]

        low_pair = sub % 4 < 2
        rest_rows = 1.0 - jnp.where(low, jnp.where(low_pair, gates[1], gates[3]),
                                    jnp.where(low_pair, gates[0], gates[2]))

        def read(_):
            def head_of(i):
                return (i >= DH).astype(i32) + (i >= 2 * DH).astype(i32) + (i >= 3 * DH).astype(i32)

            state = mz[g]
            row_m = lax.broadcasted_iota(i32, (GW, T), 0)
            col_m = lax.broadcasted_iota(i32, (GW, T), 1)
            weights = jnp.where(head_of(row_m) == head_of(col_m), state[:GW], 0.0)
            lane_head = head_of(lax.broadcasted_iota(i32, (8, T), 1))
            pair_of = sub // 2
            z_rows = jnp.where(lane_head == pair_of, state[GW:], 0.0)
            mem_w = jnp.concatenate([weights, z_rows], axis=0)
            g_rows = jnp.where(low, jnp.where(sub < 2, gates[0], gates[1]),
                               jnp.where(sub < 6, gates[2], gates[3]))
            for qt in range(NQ):
                res = _dot(mem_w, jnp.concatenate(
                    [_as_bf16(pq[slot, qt]), jnp.zeros((T - GW, T), bf16)], axis=0))
                pacer.issued(res, qt, WM)
                coef = g_rows / (res[GW:] + 1e-6)
                c0, c1, c2, c3 = (
                    jnp.broadcast_to(coef[2 * j:2 * j + 1], (8, T)) for j in range(4))
                cm = [c0, c0, jnp.where(low, c0, c1), c1, c1,
                      c2, c2, jnp.where(low, c2, c3), c3, c3]
                mem[qt] = [res[8 * i:8 * i + 8] * cm[i] for i in range(10)]
            finish()

        def corners(i):
            for lane in range(4):
                qt, pr = ORDER[2 * i + lane // 2], lane % 2
                window = _as_bf16(qd[slot, qt, 24 * pr:24 * pr + 24, :])
                sc = masked_dot(kk[slot, qt, T // 4:, :], window, 32 * pr)
                pacer.issued(sc, lane, WA)
                corner[qt, pr] = sc + bias[1]
                corner_max[qt, pr] = jnp.max(corner[qt, pr].reshape(8, 8, T), axis=0)

        def scores(t):
            qt, kt = tiles[t]
            for j in range(4):
                window = _as_bf16(qm[slot, qt, 16 * j:16 * j + 16, :])
                sc = masked_dot(
                    kk[slot, kt] if kt < qt else kk[slot, kt, :T // 4, :], window, 16 * j)
                pacer.issued(sc, j, WA)
                if kt == qt:
                    sc = sc + bias[0]
                m8 = jnp.max(sc.reshape(-1, 8, T), axis=0)
                run_max[qt, j] = m8 if kt == 0 else jnp.maximum(run_max[qt, j], m8)
                if kt == qt:
                    extra = corner_max[qt, j // 2]
                    if j % 2 == 0:
                        extra = pltpu.roll(extra, T // 2, 1)
                    top = jnp.maximum(run_max[qt, j], jnp.where(left, NEG, extra))
                    col_max[qt, j] = jnp.broadcast_to(
                        jnp.max(top, axis=0, keepdims=True), (8, T))
                logits[t, j] = sc
            if kt == qt:
                for pr in range(2):
                    top = jnp.where(left, pltpu.roll(col_max[qt, 2 * pr], T // 2, 1),
                                    col_max[qt, 2 * pr + 1])
                    words = _as_words(jnp.exp2(
                        corner[qt, pr].reshape(8, 8, T) - top[None]).reshape(T // 2, T))
                    for j, shifted in enumerate((pltpu.roll(words, T // 2, 1), words)):
                        corner_p[qt, 2 * pr + j] = _as_bf16(jnp.where(
                            left[None], jnp.uint32(0), shifted.reshape(4, 8, T)).reshape(32, T))

        def values(t):
            qt, kt = tiles[t]
            tops = [pacer.hold(col_max[qt, j], lead - stagger * j) for j in range(4)]
            for j in range(4):
                p = jnp.exp2(logits[t, j].reshape(-1, 8, T) - tops[j][None])
                p = p.reshape(-1, T).astype(bf16)
                if kt == qt:
                    p = jnp.concatenate([p, corner_p[qt, j]], axis=0)
                first = (0, 16, 40, 56)[j]
                v = [vt[slot, kt, first + 8 * i:first + 8 * i + 8, :] for i in range(3)]
                if j % 2 == 0:
                    v[2] = jnp.where(low, v[2], 1.0)
                else:
                    v[0] = jnp.where(low, 1.0, v[0])
                part = _dot(jnp.concatenate(v, axis=0), p)
                pacer.issued(part, j)
                acc[qt, j] = part if kt == 0 else acc[qt, j] + part
            if kt == qt:
                done.append(qt)
                finish()

        def finish():
            while done and (not memory or done[0] in mem):
                qt = done.pop(0)
                w = [[acc[qt, j][8 * i:8 * i + 8] for i in range(3)] for j in range(4)]
                sums = jnp.where(
                    low_pair, jnp.where(low, w[1][0], w[0][2]),
                    pltpu.roll(jnp.where(low, w[3][0], w[2][2]), 2, 0))
                coef = rest_rows / sums
                c0, c1, c2, c3 = (
                    jnp.broadcast_to(coef[r:r + 1], (8, T)) for r in (4, 0, 6, 2))
                o = [w[0][0] * c0, w[0][1] * c0,
                     jnp.where(low, w[0][2] * c0, w[1][0] * c1), w[1][1] * c1, w[1][2] * c1,
                     w[2][0] * c2, w[2][1] * c2,
                     jnp.where(low, w[2][2] * c2, w[3][0] * c3), w[3][1] * c3, w[3][2] * c3]
                if memory:
                    o = [mem[qt][i] + o[i] for i in range(10)]
                ot[s % 2, qt, _ds(g * (GW // 2), GW // 2, 8), :] = _as_words(
                    jnp.concatenate(o, axis=0))

        return {"D": corners, "Q": scores, "V": values, "R": read}

    def wo_tile(c, m):
        return _as_bf16(wraw.bitcast(u32)[3, m, c * 64:(c + 1) * 64, :])

    def out_project(s, n, pacer):
        acc, done = [None] * 4, []

        def step(i):
            for lane in range(4):
                m, c = divmod(4 * i + lane, NC)
                part = _dot(_as_bf16(wot[c, 80 * m:80 * (m + 1), :]),
                            _as_bf16(ot[s % 2, n, c * 64:(c + 1) * 64, :]))
                pacer.issued(part, lane, WO)
                acc[m] = part if c == 0 else acc[m] + part
                if c == NC - 1:
                    acc[m] = acc[m].astype(bf16)
                    while T * (len(done) + 1) <= 160 * (m + 1):
                        i0 = T * len(done)
                        pieces = [acc[k][max(i0 - 160 * k, 0):min(i0 + T - 160 * k, 160)]
                                  for k in range(i0 // 160, (i0 + T - 1) // 160 + 1)]
                        tile = jnp.concatenate(pieces, axis=0).T
                        outb.bitcast(u32)[s, _ds(n * 64, 64, 64), i0:i0 + T] = pltpu.bitcast(tile, u32)
                        done.append(True)

        return step

    def outb_copy(s, n):
        return pltpu.make_async_copy(
            outb.at[s, _ds(n * T, T, T)],
            out_hbm.at[0, _ds(s * L + n * T, T, T), pl.ds(D, D)], sem_out.at[0])

    def conv_forward(c):
        cols = slice(c * T, (c + 1) * T)
        taps = shift_ref[:, cols].astype(f32)
        taps = [jnp.broadcast_to(taps[j:j + 1], (T, T)) for j in range(4)]
        skip = ssmd_ref[...].astype(f32)[c:c + 1]
        slices = pl.ds(c * NFV, NFV)

        def transform(even, odd):
            e, o = (_dot(_as_bf16(fwd_ref.bitcast(u32)[i]), x) for i, x in enumerate((even, odd)))
            return [x.reshape(NFV, 2, 8, T) for x in (e + o, e - o)]

        tail = jnp.zeros((8, T), u32)
        prev = None
        for b in range(NB):
            k0 = ka.bitcast(u32)[c, b * T:(b + 1) * T, :]
            ext = jnp.concatenate([tail, k0], axis=0)
            tail = k0[T - 8:]
            k1, k2 = ext[7:7 + T], ext[6:6 + T]
            e0, o0, e1, o1, o2 = (
                _even_rows(k0), _odd_rows(k0), _even_rows(k1), _odd_rows(k1), _odd_rows(k2))
            v0 = va.bitcast(u32)[c, b * T:(b + 1) * T, :]
            sig = transform(
                (e0 * taps[0] + o1 * taps[1] + e1 * taps[2] + o2 * taps[3]) * _even_rows(v0),
                (o0 * taps[0] + e0 * taps[1] + o1 * taps[2] + e1 * taps[3]) * _odd_rows(v0))
            taps_t = jnp.concatenate([
                pltpu.bitcast(ssk[cols, (2 * b + i) * T:(2 * b + i + 1) * T].T, u32)
                for i in range(2)], axis=0)
            filt = transform(_even_rows(taps_t), _odd_rows(taps_t))
            for sign in range(2):
                spec_buf[slices, 0, sign, b] = sig[sign].reshape(NFV, 16, T)
                re, im = filt[sign][:, 0], filt[sign][:, 1]
                if prev is None:
                    re = re + skip[None]
                else:
                    half = NFV // 2
                    pre, pim = prev[sign][:, 0], prev[sign][:, 1]
                    re = jnp.concatenate([re[:half] - pim[:half], re[half:] + pim[half:]], axis=0)
                    im = jnp.concatenate([im[:half] + pre[:half], im[half:] - pre[half:]], axis=0)
                spec_buf[slices, 1, sign, b, 0:8, :] = re
                spec_buf[slices, 1, sign, b, 8:16, :] = im
            prev = filt

    def conv_mix(first, count, never, blk=4):
        half = NFV // 2
        for item in range(count):
            idx = jnp.minimum(first + item, NC * half - 1)
            base = idx // half * NFV + idx % half

            def products(fv, sign, a0):
                def load(which, b):
                    return (spec_buf[fv, which, sign, b, 0:8, :],
                            spec_buf[fv, which, sign, b, 8:16, :])

                acc, kcache = [None] * blk, {}
                for b in range(a0 + blk):
                    token = yield
                    ur, ui = load(0, b)
                    ur = jnp.where(never, token, ur)
                    us = ur + ui
                    for a in range(max(a0, b), a0 + blk):
                        if a - b not in kcache:
                            kr, ki = load(1, a - b)
                            kcache[a - b] = (kr, ki - kr, kr + ki)
                        k1, k2, k3 = kcache[a - b]
                        terms = (us * k1, ur * k2, ui * k3)
                        old = acc[a - a0]
                        acc[a - a0] = terms if old is None else tuple(
                            o + t for o, t in zip(old, terms))
                return [(p1 - p3, p1 + p2) for p1, p2, p3 in acc]

            for a0 in range(0, NB, blk):
                parity = []
                for fv in (base, base + half):
                    plus = yield from products(fv, 0, a0)
                    minus = yield from products(fv, 1, a0)
                    parity.append((
                        [(pr + mr, pi + mi) for (pr, pi), (mr, mi) in zip(plus, minus)],
                        [(pr - mr, pi - mi) for (pr, pi), (mr, mi) in zip(plus, minus)]))
                for i in range(blk):
                    (ar, ai), (br, bi) = parity[0][0][i], parity[1][0][i]
                    (cr, ci), (dr, di) = parity[0][1][i], parity[1][1][i]
                    folded = ((ar + br, ai - bi), (cr - di, ci - dr),
                              (ar - br, ai + bi), (cr + di, ci + dr))
                    for r in range(4):
                        yf[idx, a0 + i, r] = _as_words(jnp.concatenate(folded[r], axis=0))

    def outa_copy(c):
        return pltpu.make_async_copy(
            outa.at[c, pl.ds(0, S)], out_hbm.at[0, :, pl.ds(c * T, T)], sem_out.at[0])

    def conv_inverse(pacer, zero):
        pending, pin, hold = [], [], []

        def send(c):
            outa_copy(c).start()
            pin.append(True)

        def flush(_=0):
            while pending:
                c, a, y = pending.pop(0)
                tile = c + zero if pin else c
                for i in range(2):
                    rows = pl.ds(a * T + i, T // 2, stride=2)
                    q_words = qa.bitcast(u32)[c, rows, :]
                    outa.bitcast(u32)[tile, rows, :] = _interleave(
                        _even_rows(q_words) * y[2 * i], _odd_rows(q_words) * y[2 * i + 1])
                if pin:
                    hold.append(outa.bitcast(u32)[tile, a * T:a * T + 8, :])
                    pin.clear()

        def step(i):
            c, a = divmod(i, NB)
            res = []
            for r in range(4):
                words = yf[pl.ds(c * NFV // 2, NFV // 2), a, r].reshape(T // 2, T)
                if hold:
                    words = jnp.concatenate(
                        [jnp.where(pacer.never, hold.pop(), words[:8]), words[8:]], axis=0)
                res.append(_dot(
                    _as_bf16(inv_ref.bitcast(u32)[r]), _as_bf16(words)))
                pacer.issued(res[-1], r)
            flush()
            pending.append((c, a, res))

        return step, flush, send

    def out_project_last(pacer, zero):
        s = NSEG - 1
        o_rows, acc = {}, {}

        def transpose(n):
            for c in range(NC):
                o_rows[n, c] = _as_bf16(ot[s % 2, n, c * 64:(c + 1) * 64, :]).T

        def step(i):
            for lane in range(4):
                tile, c = divmod(4 * i + lane, NC)
                n, m = divmod(tile, NC)
                part = _dot(o_rows[n, c], wo_tile(c, m))
                pacer.issued(part, lane)
                acc[tile] = part if c == 0 else acc[tile] + part

        def store(part):
            n = min(part, NQ - 1)
            for m in range(NC) if part < NQ - 1 else ((0, 1, 2), (3, 4))[part - n]:
                seg = s + zero if m == 0 else s
                outb.bitcast(u32)[seg, n * 64:(n + 1) * 64, m * T:(m + 1) * T] = _as_words(
                    acc[n * NC + m])

        return transpose, step, store

    def new_pacer():
        return _Pacer(gate[0:8, :] > 2.0)

    def pair(s, p, plan, pacer, mix=None):
        memory = "Ra" in plan
        if mix is not None:
            first, count, cycles = mix
            pacer.attach(conv_mix(first, count, pacer.never), count * 96 / cycles)
        steps = {"a": attend(s, 2 * p, 0, pacer, memory),
                 "b": attend(s, 2 * p + 1, 1, pacer, memory)}
        steps["a"]["P"] = project(s, 2 * p + 1, 1, pacer)
        next_s, next_g = s + (p + 1) // 4, (2 * p + 2) % NG
        steps["b"]["P"] = project(next_s, next_g, 0, pacer)
        steps["a"]["U"] = lambda _: update(s, 2 * p + 1, pacer)
        steps["b"]["U"] = lambda _: update(next_s, next_g, pacer)
        steps["a"]["O"] = out_project(s - 1, p, pacer)
        steps["x"] = {
            "T": transpose_qkv,
            "W": wait,

            "C": lambda _: outb_copy(s - 1, p).start(),
        }
        if "Jx" in plan:
            zero = pacer.never.astype(i32)[0, 0]
            steps["x"]["I"], steps["x"]["J"], steps["x"]["A"] = conv_inverse(pacer, zero)
            steps["x"]["L"], steps["x"]["E"], steps["x"]["G"] = out_project_last(pacer, zero)
        steps["x"]["F"] = lambda n: outb_copy(s, n).start()
        for item in plan:
            steps[item[1]][item[0]](int(item[2:] or 0))
        assert pacer.side is None

    def memory_pair(s, p):
        first = ((s - 1) * 4 + p) * MIX_PER_ITER
        pair(s, p, PLAN1, new_pacer(), (first, MIX_PER_ITER, MIX_CYCLES))

    wait(0)
    start(3, 4)
    for part in range(3):
        transpose_qkv(part)
    wait(1)
    start(4, len(loads))
    setup_gate()
    step = project(0, 0, 0, _Pacer(None))
    for i in range(NC):
        step(i)
    pair(0, 0, PLAN_FIRST, new_pacer())

    @pl.loop(1, 4)
    def _(p):
        pair(0, p, PLAN0, new_pacer())

    wait(4)
    update(1, 0, _Pacer(None))
    for c in range(NC):
        conv_forward(c)
        transpose_wo(c)
    wait(5)
    wait(6)

    @pl.loop(0, 11)
    def _(i):
        memory_pair(1 + i // 4, i % 4)

    pair(NSEG - 1, 3, PLAN_LAST, new_pacer())

    outb_copy(NSEG - 1, NQ - 1).start()
    for c in range(NC):
        outa_copy(c).wait()
    for s in range(NSEG):
        for n in range(NQ):
            outb_copy(s, n).wait()


@jax.jit
def pallas_concat_heads__ssm_conv_h3__memory_aug_infini_attn__prompt_kernel(
    A_q: jax.Array,
    A_k: jax.Array,
    A_v: jax.Array,
    A_shift_k: jax.Array,
    A_ssm_k: jax.Array,
    A_ssm_D: jax.Array,
    B_x: jax.Array,
    B_wq: jax.Array,
    B_wk: jax.Array,
    B_wv: jax.Array,
    B_wo: jax.Array,
    B_beta: jax.Array,
):
    hbm = pl.BlockSpec(memory_space=pl.ANY)
    scratch = [
        pltpu.VMEM((4, D), bf16),
        pltpu.VMEM((NC, T), bf16),
        pltpu.VMEM((H,), bf16),
        pltpu.VMEM((2, 2 * T, T), bf16),
        pltpu.VMEM((4, T // 2, T), bf16),
        pltpu.VMEM((NC, S, T), bf16),
        pltpu.VMEM((4, NC, D, T), bf16),
        pltpu.VMEM((3, NC, D // 2, T), u32),
        pltpu.VMEM((NC, D // 2, T), u32),
        pltpu.VMEM((NC, S + 16, T), bf16),
        pltpu.VMEM((NC, S, T), bf16),
        pltpu.VMEM((NC, S, T), bf16),
        pltpu.VMEM((D, S), bf16),
        pltpu.VMEM((NC * NFV, 2, 2, NB, 16, T), f32),
        pltpu.VMEM((NC * NFV // 2, NB, 4, 8, T), u32),
        pltpu.VMEM((NC, S + 16, T), bf16),
        pltpu.VMEM((NSEG, L, D), bf16),
        pltpu.VMEM((H, T), f32),
        pltpu.VMEM((2, T // 2, T), f32),
        pltpu.VMEM((2, NQ, 64, T), u32),
        pltpu.VMEM((2, NQ, 48, T), u32),
        pltpu.VMEM((2, NQ, GW // 2, T), u32),
        pltpu.VMEM((2, NQ, T // 2, T), u32),
        pltpu.VMEM((2, NQ, GW, T), f32),
        pltpu.VMEM((2, NG, NQ, GW // 2, T), u32),
        pltpu.VMEM((2, NG, NQ, GW, T), f32),
        pltpu.VMEM((2, NQ, D // 2, T), u32),
        pltpu.VMEM((NG, GW + 8, T), f32),
        pltpu.SemaphoreType.DMA((7,)),
        pltpu.SemaphoreType.DMA((1,)),
    ]
    return pl.pallas_call(
        _kernel,
        out_shape=jax.ShapeDtypeStruct((1, S, 2 * D), bf16),
        in_specs=[hbm] * 14,
        out_specs=hbm,
        scratch_shapes=scratch,
        compiler_params=pltpu.CompilerParams(vmem_limit_bytes=100 * 2**20),
    )(
        A_shift_k.T, A_ssm_D.reshape(NC, T), B_beta, _FWD, _INV,
        A_q, A_k, A_v, A_ssm_k, B_x, B_wq, B_wk, B_wv, B_wo,
    )
```

```python
import jax
import jax.numpy as jnp
import numpy as np
from jax import lax
from jax.experimental import pallas as pl
from jax.experimental.pallas import tpu as pltpu

f32, bf16, u32, i32 = jnp.float32, jnp.bfloat16, jnp.uint32, jnp.int32

S, D, H, DH = 2048, 640, 32, 20
NSEG, L = 4, 512
T = 128
NC = D // T
NB = S // (2 * T)
NQ = L // T
NG = 8
GW = 4 * DH
APARTS = 2
NFV = 16
LOG2E = 1.4426950408889634
NEG = -1e30
MIX_PER_ITER = 4

PLAN_FIRST = (
    "Wx2 Qa0 Da0 Tx3 Tx4 Tx5 Qa1 Qa2 Qa3 Pa0 Qa4 Pa1 Va0 Pa2 Va1 Qa5 Pa3 Qa6 Pa4 Da1 Va2 Qa7 Va3 "
    "Qa8 Qa9 Va4 Qb0 Va5 Qb1 Va6 Db0 Va7 Qb2 Wx3 Tx6 Tx7 Tx8 Va8 Qb3 Vb0 Va9 Qb4 Pb0 Tx9 Tx10 "
    "Tx11 Qb5 Vb1 Qb6 Vb2 Db1 Vb3 Qb7 Tx12 Tx13 Tx14 Pb1 Kx Pb2 Vb4 Qb8 Vb5 Qb9 Pb3 Pb4 Vb6 Vb7 "
    "Vb8 Vb9"
).split()
PLAN0 = (
    "Qa0 Da0 Pa0 Qa1 Pa1 Qa2 Qa3 Pa2 Pa3 Qa4 Va0 Va1 Qa5 Qa6 Pa4 Da1 Va2 Qa7 Va3 Qa8 Qa9 Va4 Qb0 "
    "Va5 Qb1 Va6 Db0 Va7 Qb2 Va8 Qb3 Va9 Qb4 Pb0 Qb5 Vb0 Vb1 Qb6 Vb2 Db1 Vb3 Qb7 Pb1 Pb2 Vb4 Qb8 "
    "Vb5 Qb9 Pb3 Pb4 Vb6 Vb7 Vb8 Vb9"
).split()
PLAN1 = (
    "Qa0 Da0 Pa0 Pa1 Qa1 Qa2 Pa2 Qa3 Pa3 Va0 Pa4 Qa4 Qa5 Va1 Qa6 Oa0 Va2 Va3 Qa7 Oa1 Da1 Va4 Oa2 "
    "Qa8 Oa3 Oa4 Qa9 Ua Ra Va5 Va6 Qb0 Va7 Qb1 Db0 Qb2 Va8 Qb3 Pb0 Vb0 Va9 Pb1 Qb4 Qb5 Qb6 Vb1 "
    "Db1 Vb2 Qb7 Vb3 Pb2 Qb8 Vb4 Cx Vb5 Qb9 Pb3 Vb6 Pb4 Rb Vb7 Vb8 Vb9 Ub"
).split()
PLAN_LAST = (
    "Qa0 Da0 Pa0 Pa1 Qa1 Qa2 Qa3 Pa2 Pa3 Pa4 Qa4 Ix0 Qa5 Ix1 Va0 Ix2 Va1 Qa6 Ix3 Oa0 Va2 Qa7 Ix4 "
    "Da1 Va3 Oa1 Ix5 Ax0 Oa2 Qa8 Ix6 Va4 Oa3 Ix7 Oa4 Va5 Qa9 Ix8 Ra Ua Va6 Ix9 Ax1 Cx Qb0 Ix10 "
    "Va7 Qb1 Ix11 Db0 Ix12 Qb2 Va8 Ix13 Ax2 Qb3 Ix14 Vb0 Va9 Ix15 Qb4 Ix16 Qb5 Ix17 Ax3 Vb1 Qb6 "
    "Ix18 Db1 Ix19 Vb2 Qb7 Ix20 Vb3 Ix21 Ax4 Qb8 Ix22 Vb4 Ix23 Vb5 Qb9 Ix24 Ix25 Ax5 Ix26 Vb6 "
    "Ix27 Rb Ix28 Vb7 Ix29 Ax6 Ix30 Vb8 Ix31 Ix32 Vb9 Ix33 Ax7 Lx3 Ix34 Lx2 Ix35 Ix36 Lx1 Ix37 "
    "Ax8 Ix38 Lx0 Ix39 Ex0 Jx Ex1 Jx Ax9 Ex2 Ex3 Ex4 Ex5 Ex6 Gx0 Fx0 Ex7 Ex8 Ex9 Ex10 Ex11 Ex12 "
    "Gx1 Fx1 Ex13 Ex14 Ex15 Ex16 Ex17 Ex18 Gx2 Fx2 Ex19 Ex20 Ex21 Ex22 Gx3 Ex23 Ex24 Gx4"
).split()
ORDER = (3, 2, 1, 0)
LEAD = {False: (400, 56), True: (400, 24)}
WA, WP, WO, WM = 1.2, 1.0, 1.0, 1.4
MIX_CYCLES = (2 * (1152 * WA + 1200 * WP + 176 * WM) + 800 * WO) * 0.965

NN = (((1,), (0,)), ((), ()))
NT = (((1,), (1,)), ((), ()))


def _dft_tables():
    freq = np.concatenate([np.arange(0, T, 2), T - 1 - np.arange(0, T, 2)])

    def table(freq, n):
        theta = 2.0 * np.pi * (freq[:, None] + 0.5) * n[None, :] / (4 * T)
        parts = [f(theta).reshape(-1, 8, len(n)) for f in (np.cos, lambda t: -np.sin(t))]
        return np.stack(parts, axis=1).reshape(-1, len(n))

    fwd = np.stack([table(freq, 2 * np.arange(T) + r) for r in range(2)])
    inv = np.stack([table(freq[:T // 2], 4 * np.arange(T // 2) + r).T / (2 * T) for r in range(4)])
    return fwd.astype(np.float32).astype(bf16), inv.astype(np.float32).astype(bf16)


_FWD, _INV = _dft_tables()


def _as_bf16(words):
    return pltpu.bitcast(words, bf16)


def _as_words(x):
    return pltpu.bitcast(x.astype(bf16), u32)


def _even_rows(words):
    return pltpu.bitcast(words << 16, f32)


def _odd_rows(words):
    return pltpu.bitcast(words & np.uint32(0xFFFF0000), f32)


def _interleave(even, odd):
    even, odd = (pltpu.bitcast(x.astype(bf16).astype(f32), u32) for x in (even, odd))
    return (even >> 16) | odd


def _dot(a, b):
    return lax.dot_general(a, b, NN, preferred_element_type=f32)


def _dot_nt(a, b):
    return lax.dot_general(a, b, NT, preferred_element_type=f32)


def _phi(t):
    return jnp.maximum(t, 0.0) + jnp.exp(jnp.minimum(t, 0.0))


def _ds(start, size, align):
    if isinstance(start, int):
        return pl.ds(start, size)
    return pl.ds(pl.multiple_of(start, align), size)


class _Pacer:
    def __init__(self, never):
        self.never, self.side, self.rate = never, None, 0.0
        self.credit, self.clock, self.history = 0.0, 0.0, []

    def attach(self, side, rate):
        self.side, self.rate, self.credit = side, rate, 0.0
        next(side)

    def issued(self, result, lane, weight=0.0):
        rows = result.shape[0]
        self.history.append((self.clock, result))
        if lane == 3:
            self.clock += rows
        self.credit += self.rate * rows / 4 * weight
        count = int(self.credit)
        self.credit -= count
        for i in range(count):
            if self.side is not None:
                v = min(rows // 8 - 1, int(rows // 8 * (lane + (i + 0.5) / count) / 4))
                try:
                    self.side.send(result[8 * v:8 * v + 8])
                except StopIteration:
                    self.side = None

    def hold(self, value, lead):
        target = self.clock - lead
        if target < 0 or self.never is None:
            return value
        for start, result in reversed(self.history):
            if start <= target:
                v = min(result.shape[0] // 8 - 1, int(target - start) // 8)
                return jnp.where(self.never, result[8 * v:8 * v + 8], value)
        return value


def _kernel(
    shift_hbm, ssmd_hbm, beta_hbm, fwd_hbm, inv_hbm,
    q_hbm, k_hbm, v_hbm, ssm_hbm, x_hbm, wq_hbm, wk_hbm, wv_hbm, wo_hbm, out_hbm,
    shift_ref, ssmd_ref, beta_ref, fwd_ref, inv_ref,
    xs, wraw, wt, wot, qa, ka, va, ssk, spec_buf, yf, outa, outb,
    fwd, inv, ystage, gate, bias, qm, qd, pq, kk, vt, pk_keep, vt_keep, ot, mz, sem_in, sem_out,
):
    def w_copies(n, sem):
        return [
            pltpu.make_async_copy(src.at[:, pl.ds(n * T, T)], wraw.at[i, n], sem)
            for i, src in enumerate((wq_hbm, wk_hbm, wv_hbm))
        ]

    def x_copies(lo, hi, sem):
        rows = pl.ds(lo * L, (hi - lo) * L)
        return [
            pltpu.make_async_copy(x_hbm.at[0, rows, pl.ds(c * T, T)], xs.at[c, rows], sem)
            for c in range(NC)
        ]

    def column_tiles(src, dst, sem):
        return [
            pltpu.make_async_copy(src.at[0, :, pl.ds(c * T, T)], dst.at[c], sem)
            for c in range(NC)
        ]

    loads = [
        w_copies(0, sem_in.at[0]),
        x_copies(0, 1, sem_in.at[1])
        + [pltpu.make_async_copy(beta_hbm, beta_ref, sem_in.at[1])],
        w_copies(1, sem_in.at[2]),
        sum((w_copies(n, sem_in.at[3]) for n in range(2, NC)), [
            pltpu.make_async_copy(fwd_hbm, fwd_ref, sem_in.at[3]),
            pltpu.make_async_copy(inv_hbm, inv_ref, sem_in.at[3])]),
        x_copies(1, 2, sem_in.at[4]),
        [pltpu.make_async_copy(src, dst, sem_in.at[5]) for src, dst in (
            (shift_hbm, shift_ref), (ssmd_hbm, ssmd_ref),
            (ssm_hbm, ssk))]
        + column_tiles(k_hbm, ka, sem_in.at[5]) + column_tiles(v_hbm, va, sem_in.at[5])
        + [pltpu.make_async_copy(wo_hbm.at[:, pl.ds(n * T, T)], wraw.at[3, n], sem_in.at[5])
           for n in range(NC)],
        x_copies(2, NSEG, sem_in.at[6]),
        column_tiles(q_hbm, qa, sem_in.at[7]),
    ]
    def start(lo, hi):
        for copies in loads[lo:hi]:
            for cp in copies:
                cp.start()

    start(0, 3)

    def wait(i):
        for cp in loads[i]:
            cp.wait()

    mz[...] = jnp.zeros(mz.shape, f32)
    row = lax.broadcasted_iota(i32, (T // 2, T), 0)
    col = lax.broadcasted_iota(i32, (T // 2, T), 1)
    bias[0] = jnp.where(row <= col, 0.0, NEG)
    bias[1] = jnp.where(row <= col % (T // 2), 0.0, NEG)

    def setup_gate():
        beta = jnp.concatenate(
            [beta_ref[...].astype(f32)[None, :], jnp.zeros((1, T - H), f32)], axis=1)
        gate[...] = jax.nn.sigmoid(jnp.broadcast_to(beta, (T, T)).T[:H])

    def transpose_qkv(part):
        n, i = divmod(part, 3)
        for c in range(NC):
            tile = wraw[i, n, c * T:(c + 1) * T, :]
            wt[i, c, n * T // 2:(n + 1) * T // 2, :] = pltpu.bitcast(tile.T, u32)

    def repack_tables(_):
        for i in range(2):
            fwd[i] = pltpu.bitcast(fwd_ref[i], u32)
        for i in range(4):
            inv[i] = pltpu.bitcast(inv_ref[i], u32)

    def transpose_wo(n):
        for c in range(NC):
            wot[c, n * T // 2:(n + 1) * T // 2, :] = pltpu.bitcast(wo_tile(c, n).T, u32)

    sub = lax.broadcasted_iota(i32, (8, T), 0)
    low = sub < 4
    left = lax.broadcasted_iota(i32, (8, T), 1) < T // 2

    def project(s, g, slot, pacer):
        rows = _ds(g * (GW // 2), GW // 2, 8)
        acc = [None] * NQ

        def store(n):
            q_t, k_t, v_t = acc[n][:GW], acc[n][GW:2 * GW], acc[n][2 * GW:]
            k_pad = jnp.concatenate([k_t.astype(bf16), jnp.zeros((T - GW, T), bf16)], axis=0)
            kk[slot, n] = pltpu.bitcast(k_pad.T, u32)
            qs = q_t * (DH ** -0.5 * LOG2E)
            r = [qs[8 * i:8 * i + 8] for i in range(10)]
            zero = jnp.zeros((8, T), f32)
            heads = [
                r[0], r[1], jnp.where(low, r[2], 0.0), zero,
                jnp.where(low, 0.0, r[2]), r[3], r[4], zero,
                zero, r[5], r[6], jnp.where(low, r[7], 0.0),
                zero, jnp.where(low, 0.0, r[7]), r[8], r[9],
            ]
            qm[slot, n] = _as_words(jnp.concatenate(heads, axis=0))
            e = {i: jnp.where(left, pltpu.roll(r[i], 64, 1), 0.0) for i in (0, 1, 2, 5, 6, 7)}
            o = {i: jnp.where(left, 0.0, r[i]) for i in (2, 3, 4, 7, 8, 9)}
            pairs = [
                e[0], e[1], jnp.where(low, e[2], o[2]), o[3], o[4], zero,
                zero, e[5], e[6], jnp.where(low, e[7], o[7]), o[8], o[9],
            ]
            qd[slot, n] = _as_words(jnp.concatenate(pairs, axis=0))
            pq[slot, n] = _as_words(_phi(q_t))
            pk_keep[s % 2, g, n] = _as_words(_phi(k_t))
            vt[slot, n] = v_t
            vt_keep[s % 2, g, n] = v_t

        def step(i):
            for lane in range(4):
                n, c = divmod(4 * i + lane, NC)
                w = _as_bf16(jnp.concatenate([wt[m, c, rows, :] for m in range(3)], axis=0))
                part = _dot_nt(w, xs[c, _ds(s * L + n * T, T, T), :])
                pacer.issued(part, lane, WP)
                acc[n] = part if c == 0 else acc[n] + part
                if c == NC - 1:
                    store(n)

        return step

    def masked_dot(key_words, window, first):
        end = first + window.shape[0]
        parts = [window, jnp.zeros((T - end, T), bf16)]
        if first:
            parts.insert(0, jnp.zeros((first, T), bf16))
        return _dot(_as_bf16(key_words), jnp.concatenate(parts, axis=0))

    def update(s, g, pacer):
        state = mz[g]
        for kt in range(NQ):
            v_one = jnp.concatenate(
                [vt_keep[(s + 1) % 2, g, kt], jnp.ones((8, T), f32)], axis=0)
            pk_t = jnp.concatenate(
                [_as_bf16(pk_keep[(s + 1) % 2, g, kt]), jnp.zeros((T - GW, T), bf16)], axis=0)
            part = _dot_nt(v_one, pk_t)
            pacer.issued(part, kt, WM)
            state = state + part
        mz[g] = state

    def attend(s, g, slot, pacer, memory):
        lead, stagger = LEAD[memory]
        tiles = [(qt, kt) for qt in ORDER for kt in range(qt + 1)]
        logits, run_max, col_max, acc, mem, done = {}, {}, {}, {}, {}, []
        corner, corner_max, corner_p = {}, {}, {}
        gates = [jnp.broadcast_to(gate[pl.ds(4 * g + j, 1), :], (8, T)) for j in range(4)]

        low_pair = sub % 4 < 2
        rest_rows = 1.0 - jnp.where(low, jnp.where(low_pair, gates[1], gates[3]),
                                    jnp.where(low_pair, gates[0], gates[2]))

        def read(_):
            def head_of(i):
                return (i >= DH).astype(i32) + (i >= 2 * DH).astype(i32) + (i >= 3 * DH).astype(i32)

            state = mz[g]
            row_m = lax.broadcasted_iota(i32, (GW, T), 0)
            col_m = lax.broadcasted_iota(i32, (GW, T), 1)
            weights = jnp.where(head_of(row_m) == head_of(col_m), state[:GW], 0.0)
            lane_head = head_of(lax.broadcasted_iota(i32, (8, T), 1))
            pair_of = sub // 2
            z_rows = jnp.where(lane_head == pair_of, state[GW:], 0.0)
            mem_w = jnp.concatenate([weights, z_rows], axis=0)
            g_rows = jnp.where(low, jnp.where(sub < 2, gates[0], gates[1]),
                               jnp.where(sub < 6, gates[2], gates[3]))
            for qt in range(NQ):
                res = _dot(mem_w, jnp.concatenate(
                    [_as_bf16(pq[slot, qt]), jnp.zeros((T - GW, T), bf16)], axis=0))
                pacer.issued(res, qt, WM)
                coef = g_rows / (res[GW:] + 1e-6)
                c0, c1, c2, c3 = (
                    jnp.broadcast_to(coef[2 * j:2 * j + 1], (8, T)) for j in range(4))
                cm = [c0, c0, jnp.where(low, c0, c1), c1, c1,
                      c2, c2, jnp.where(low, c2, c3), c3, c3]
                mem[qt] = [res[8 * i:8 * i + 8] * cm[i] for i in range(10)]
            finish()

        def corners(i):
            for lane in range(4):
                qt, pr = ORDER[2 * i + lane // 2], lane % 2
                window = _as_bf16(qd[slot, qt, 24 * pr:24 * pr + 24, :])
                sc = masked_dot(kk[slot, qt, T // 4:, :], window, 32 * pr)
                pacer.issued(sc, lane, WA)
                corner[qt, pr] = sc + bias[1]
                corner_max[qt, pr] = jnp.max(corner[qt, pr].reshape(8, 8, T), axis=0)

        def scores(t):
            qt, kt = tiles[t]
            for j in range(4):
                window = _as_bf16(qm[slot, qt, 16 * j:16 * j + 16, :])
                sc = masked_dot(
                    kk[slot, kt] if kt < qt else kk[slot, kt, :T // 4, :], window, 16 * j)
                pacer.issued(sc, j, WA)
                if kt == qt:
                    sc = sc + bias[0]
                m8 = jnp.max(sc.reshape(-1, 8, T), axis=0)
                run_max[qt, j] = m8 if kt == 0 else jnp.maximum(run_max[qt, j], m8)
                if kt == qt:
                    extra = corner_max[qt, j // 2]
                    if j % 2 == 0:
                        extra = pltpu.roll(extra, T // 2, 1)
                    top = jnp.maximum(run_max[qt, j], jnp.where(left, NEG, extra))
                    col_max[qt, j] = jnp.broadcast_to(
                        jnp.max(top, axis=0, keepdims=True), (8, T))
                logits[t, j] = sc
            if kt == qt:
                for pr in range(2):
                    top = jnp.where(left, pltpu.roll(col_max[qt, 2 * pr], T // 2, 1),
                                    col_max[qt, 2 * pr + 1])
                    words = _as_words(jnp.exp2(
                        corner[qt, pr].reshape(8, 8, T) - top[None]).reshape(T // 2, T))
                    for j, shifted in enumerate((pltpu.roll(words, T // 2, 1), words)):
                        corner_p[qt, 2 * pr + j] = _as_bf16(jnp.where(
                            left[None], jnp.uint32(0), shifted.reshape(4, 8, T)).reshape(32, T))

        def values(t):
            qt, kt = tiles[t]
            tops = [pacer.hold(col_max[qt, j], lead - stagger * j) for j in range(4)]
            for j in range(4):
                p = jnp.exp2(logits[t, j].reshape(-1, 8, T) - tops[j][None])
                p = p.reshape(-1, T).astype(bf16)
                if kt == qt:
                    p = jnp.concatenate([p, corner_p[qt, j]], axis=0)
                first = (0, 16, 40, 56)[j]
                v = [vt[slot, kt, first + 8 * i:first + 8 * i + 8, :] for i in range(3)]
                if j % 2 == 0:
                    v[2] = jnp.where(low, v[2], 1.0)
                else:
                    v[0] = jnp.where(low, 1.0, v[0])
                part = _dot(jnp.concatenate(v, axis=0), p)
                pacer.issued(part, j)
                acc[qt, j] = part if kt == 0 else acc[qt, j] + part
            if kt == qt:
                done.append(qt)
                finish()

        def finish():
            while done and (not memory or done[0] in mem):
                qt = done.pop(0)
                w = [[acc[qt, j][8 * i:8 * i + 8] for i in range(3)] for j in range(4)]
                sums = jnp.where(
                    low_pair, jnp.where(low, w[1][0], w[0][2]),
                    pltpu.roll(jnp.where(low, w[3][0], w[2][2]), 2, 0))
                coef = rest_rows / sums
                c0, c1, c2, c3 = (
                    jnp.broadcast_to(coef[r:r + 1], (8, T)) for r in (4, 0, 6, 2))
                o = [w[0][0] * c0, w[0][1] * c0,
                     jnp.where(low, w[0][2] * c0, w[1][0] * c1), w[1][1] * c1, w[1][2] * c1,
                     w[2][0] * c2, w[2][1] * c2,
                     jnp.where(low, w[2][2] * c2, w[3][0] * c3), w[3][1] * c3, w[3][2] * c3]
                if memory:
                    o = [mem[qt][i] + o[i] for i in range(10)]
                ot[s % 2, qt, _ds(g * (GW // 2), GW // 2, 8), :] = _as_words(
                    jnp.concatenate(o, axis=0))

        return {"D": corners, "Q": scores, "V": values, "R": read}

    def wo_tile(c, m):
        return wraw[3, m, c * T:(c + 1) * T, :]

    def out_project(s, n, pacer):
        acc, done = [None] * 4, []

        def step(i):
            for lane in range(4):
                m, c = divmod(4 * i + lane, NC)
                part = _dot(_as_bf16(wot[c, 80 * m:80 * (m + 1), :]),
                            _as_bf16(ot[s % 2, n, c * 64:(c + 1) * 64, :]))
                pacer.issued(part, lane, WO)
                acc[m] = part if c == 0 else acc[m] + part
                if c == NC - 1:
                    acc[m] = acc[m].astype(bf16)
                    while T * (len(done) + 1) <= 160 * (m + 1):
                        i0 = T * len(done)
                        pieces = [acc[k][max(i0 - 160 * k, 0):min(i0 + T - 160 * k, 160)]
                                  for k in range(i0 // 160, (i0 + T - 1) // 160 + 1)]
                        tile = jnp.concatenate(pieces, axis=0).T
                        outb[s, _ds(n * T, T, T), i0:i0 + T] = tile
                        done.append(True)

        return step

    def outb_copy(s, n):
        return pltpu.make_async_copy(
            outb.at[s, _ds(n * T, T, T)],
            out_hbm.at[0, _ds(s * L + n * T, T, T), pl.ds(D, D)], sem_out.at[0])

    def conv_forward(c):
        cols = slice(c * T, (c + 1) * T)
        taps = shift_ref[:, cols].astype(f32)
        taps = [jnp.broadcast_to(taps[j:j + 1], (T, T)) for j in range(4)]
        skip = ssmd_ref[...].astype(f32)[c:c + 1]
        slices = pl.ds(c * NFV, NFV)

        def transform(even, odd):
            e, o = (_dot(_as_bf16(fwd[i]), x) for i, x in enumerate((even, odd)))
            return [x.reshape(NFV, 2, 8, T) for x in (e + o, e - o)]

        tail = jnp.zeros((8, T), u32)
        prev = None
        for b in range(NB):
            k0 = pltpu.bitcast(ka[c, 2 * b * T:2 * (b + 1) * T, :], u32)
            ext = jnp.concatenate([tail, k0], axis=0)
            tail = k0[T - 8:]
            k1, k2 = ext[7:7 + T], ext[6:6 + T]
            e0, o0, e1, o1, o2 = (
                _even_rows(k0), _odd_rows(k0), _even_rows(k1), _odd_rows(k1), _odd_rows(k2))
            v0 = pltpu.bitcast(va[c, 2 * b * T:2 * (b + 1) * T, :], u32)
            sig = transform(
                (e0 * taps[0] + o1 * taps[1] + e1 * taps[2] + o2 * taps[3]) * _even_rows(v0),
                (o0 * taps[0] + e0 * taps[1] + o1 * taps[2] + e1 * taps[3]) * _odd_rows(v0))
            taps_t = jnp.concatenate([
                pltpu.bitcast(ssk[cols, (2 * b + i) * T:(2 * b + i + 1) * T].T, u32)
                for i in range(2)], axis=0)
            filt = transform(_even_rows(taps_t), _odd_rows(taps_t))
            for sign in range(2):
                spec_buf[slices, 0, sign, b] = sig[sign].reshape(NFV, 16, T)
                re, im = filt[sign][:, 0], filt[sign][:, 1]
                if prev is None:
                    re = re + skip[None]
                else:
                    half = NFV // 2
                    pre, pim = prev[sign][:, 0], prev[sign][:, 1]
                    re = jnp.concatenate([re[:half] - pim[:half], re[half:] + pim[half:]], axis=0)
                    im = jnp.concatenate([im[:half] + pre[:half], im[half:] - pre[half:]], axis=0)
                spec_buf[slices, 1, sign, b, 0:8, :] = re
                spec_buf[slices, 1, sign, b, 8:16, :] = im
            prev = filt

    def conv_mix(first, count, never, blk=4):
        half = NFV // 2
        for item in range(count):
            idx = jnp.minimum(first + item, NC * half - 1)
            base = idx // half * NFV + idx % half

            def products(fv, sign, a0):
                def load(which, b):
                    return (spec_buf[fv, which, sign, b, 0:8, :],
                            spec_buf[fv, which, sign, b, 8:16, :])

                acc, kcache = [None] * blk, {}
                for b in range(a0 + blk):
                    token = yield
                    ur, ui = load(0, b)
                    ur = jnp.where(never, token, ur)
                    us = ur + ui
                    for a in range(max(a0, b), a0 + blk):
                        if a - b not in kcache:
                            kr, ki = load(1, a - b)
                            kcache[a - b] = (kr, ki - kr, kr + ki)
                        k1, k2, k3 = kcache[a - b]
                        terms = (us * k1, ur * k2, ui * k3)
                        old = acc[a - a0]
                        acc[a - a0] = terms if old is None else tuple(
                            o + t for o, t in zip(old, terms))
                return [(p1 - p3, p1 + p2) for p1, p2, p3 in acc]

            for a0 in range(0, NB, blk):
                parity = []
                for fv in (base, base + half):
                    plus = yield from products(fv, 0, a0)
                    minus = yield from products(fv, 1, a0)
                    parity.append((
                        [(pr + mr, pi + mi) for (pr, pi), (mr, mi) in zip(plus, minus)],
                        [(pr - mr, pi - mi) for (pr, pi), (mr, mi) in zip(plus, minus)]))
                for i in range(blk):
                    (ar, ai), (br, bi) = parity[0][0][i], parity[1][0][i]
                    (cr, ci), (dr, di) = parity[0][1][i], parity[1][1][i]
                    folded = ((ar + br, ai - bi), (cr - di, ci - dr),
                              (ar - br, ai + bi), (cr + di, ci + dr))
                    for r in range(4):
                        yf[idx, a0 + i, r] = _as_words(jnp.concatenate(folded[r], axis=0))

    def outa_copy(k):
        c, part = divmod(k, APARTS)
        rows = pl.ds(part * (S // APARTS), S // APARTS)
        return pltpu.make_async_copy(
            outa.at[c, rows], out_hbm.at[0, rows, pl.ds(c * T, T)], sem_out.at[0])

    def conv_inverse(pacer, zero):
        pending, staged, pin, hold = [], [], [], []

        def send(c):
            outa_copy(c).start()
            pin.append(True)

        def gate_blocks():
            while staged:
                c, a = staged.pop(0)
                tile = c + zero if pin else c
                rows = slice(2 * a * T, 2 * (a + 1) * T)
                conv = _as_bf16(ystage[a % 4, :T, :]).astype(f32)
                outa[tile, rows, :] = (qa[c, rows, :].astype(f32) * conv).astype(bf16)
                if pin:
                    hold.append(pltpu.bitcast(outa[tile, rows.start:rows.start + 16, :], u32))
                    pin.clear()

        def stage_blocks():
            while pending:
                c, a, y = pending.pop(0)
                for h in range(2):
                    ystage[a % 4, pl.ds(h, T // 2, stride=2), :] = _interleave(
                        y[2 * h], y[2 * h + 1])
                staged.append((c, a))

        def flush(_):
            gate_blocks()
            stage_blocks()

        def step(i):
            c, a = divmod(i, NB)
            res = []
            for r in range(4):
                words = yf[pl.ds(c * NFV // 2, NFV // 2), a, r].reshape(T // 2, T)
                if hold:
                    words = jnp.concatenate(
                        [jnp.where(pacer.never, hold.pop(), words[:8]), words[8:]], axis=0)
                res.append(_dot(
                    _as_bf16(inv[r]), _as_bf16(words)))
                pacer.issued(res[-1], r)
            flush(0)
            pending.append((c, a, res))

        return step, flush, send

    def out_project_last(pacer, zero):
        s = NSEG - 1
        o_rows, acc = {}, {}

        def transpose(n):
            for c in range(NC):
                o_rows[n, c] = _as_bf16(ot[s % 2, n, c * 64:(c + 1) * 64, :]).T

        def step(i):
            for lane in range(4):
                tile, c = divmod(4 * i + lane, NC)
                n, m = divmod(tile, NC)
                part = _dot(o_rows[n, c], wo_tile(c, m))
                pacer.issued(part, lane)
                acc[tile] = part if c == 0 else acc[tile] + part

        def store(part):
            n = min(part, NQ - 1)
            for m in range(NC) if part < NQ - 1 else ((0, 1, 2), (3, 4))[part - n]:
                seg = s + zero if m == 0 else s
                outb[seg, n * T:(n + 1) * T, m * T:(m + 1) * T] = acc[n * NC + m].astype(bf16)

        return transpose, step, store

    def new_pacer():
        return _Pacer(gate[0:8, :] > 2.0)

    def pair(s, p, plan, pacer, mix=None):
        memory = "Ra" in plan
        if mix is not None:
            first, count, cycles = mix
            pacer.attach(conv_mix(first, count, pacer.never), count * 96 / cycles)
        steps = {"a": attend(s, 2 * p, 0, pacer, memory),
                 "b": attend(s, 2 * p + 1, 1, pacer, memory)}
        steps["a"]["P"] = project(s, 2 * p + 1, 1, pacer)
        next_s, next_g = s + (p + 1) // 4, (2 * p + 2) % NG
        steps["b"]["P"] = project(next_s, next_g, 0, pacer)
        steps["a"]["U"] = lambda _: update(s, 2 * p + 1, pacer)
        steps["b"]["U"] = lambda _: update(next_s, next_g, pacer)
        steps["a"]["O"] = out_project(s - 1, p, pacer)
        steps["x"] = {
            "T": transpose_qkv,
            "K": repack_tables,
            "W": wait,

            "C": lambda _: outb_copy(s - 1, p).start(),
        }
        if "Jx" in plan:
            zero = pacer.never.astype(i32)[0, 0]
            steps["x"]["I"], steps["x"]["J"], steps["x"]["A"] = conv_inverse(pacer, zero)
            steps["x"]["L"], steps["x"]["E"], steps["x"]["G"] = out_project_last(pacer, zero)
        steps["x"]["F"] = lambda n: outb_copy(s, n).start()
        for item in plan:
            steps[item[1]][item[0]](int(item[2:] or 0))
        assert pacer.side is None

    def memory_pair(s, p):
        first = ((s - 1) * 4 + p) * MIX_PER_ITER
        pair(s, p, PLAN1, new_pacer(), (first, MIX_PER_ITER, MIX_CYCLES))

    wait(0)
    start(3, 4)
    for part in range(3):
        transpose_qkv(part)
    wait(1)
    start(4, len(loads))
    setup_gate()
    step = project(0, 0, 0, _Pacer(None))
    for i in range(NC):
        step(i)
    pair(0, 0, PLAN_FIRST, new_pacer())
    wait(4)

    @pl.loop(1, 4)
    def _(p):
        pair(0, p, PLAN0, new_pacer())

    wait(5)
    update(1, 0, _Pacer(None))
    for c in range(NC):
        conv_forward(c)
        transpose_wo(c)
    wait(6)
    wait(7)

    @pl.loop(0, 11)
    def _(i):
        memory_pair(1 + i // 4, i % 4)

    pair(NSEG - 1, 3, PLAN_LAST, new_pacer())

    outb_copy(NSEG - 1, NQ - 1).start()
    for k in range(NC * APARTS):
        outa_copy(k).wait()
    for s in range(NSEG):
        for n in range(NQ):
            outb_copy(s, n).wait()


@jax.jit
def pallas_concat_heads__ssm_conv_h3__memory_aug_infini_attn__prompt_kernel(
    A_q: jax.Array,
    A_k: jax.Array,
    A_v: jax.Array,
    A_shift_k: jax.Array,
    A_ssm_k: jax.Array,
    A_ssm_D: jax.Array,
    B_x: jax.Array,
    B_wq: jax.Array,
    B_wk: jax.Array,
    B_wv: jax.Array,
    B_wo: jax.Array,
    B_beta: jax.Array,
):
    hbm = pl.BlockSpec(memory_space=pl.ANY)
    scratch = [
        pltpu.VMEM((4, D), bf16),
        pltpu.VMEM((NC, T), bf16),
        pltpu.VMEM((H,), bf16),
        pltpu.VMEM((2, 2 * T, T), bf16),
        pltpu.VMEM((4, T // 2, T), bf16),
        pltpu.VMEM((NC, S, T), bf16),
        pltpu.VMEM((4, NC, D, T), bf16),
        pltpu.VMEM((3, NC, D // 2, T), u32),
        pltpu.VMEM((NC, D // 2, T), u32),
        pltpu.VMEM((NC, S, T), bf16),
        pltpu.VMEM((NC, S, T), bf16),
        pltpu.VMEM((NC, S, T), bf16),
        pltpu.VMEM((D, S), bf16),
        pltpu.VMEM((NC * NFV, 2, 2, NB, 16, T), f32),
        pltpu.VMEM((NC * NFV // 2, NB, 4, 8, T), u32),
        pltpu.VMEM((NC, S, T), bf16),
        pltpu.VMEM((NSEG, L, D), bf16),
        pltpu.VMEM((2, T, T), u32),
        pltpu.VMEM((4, T // 4, T), u32),
        pltpu.VMEM((4, T + 8, T), u32),
        pltpu.VMEM((H, T), f32),
        pltpu.VMEM((2, T // 2, T), f32),
        pltpu.VMEM((2, NQ, 64, T), u32),
        pltpu.VMEM((2, NQ, 48, T), u32),
        pltpu.VMEM((2, NQ, GW // 2, T), u32),
        pltpu.VMEM((2, NQ, T // 2, T), u32),
        pltpu.VMEM((2, NQ, GW, T), f32),
        pltpu.VMEM((2, NG, NQ, GW // 2, T), u32),
        pltpu.VMEM((2, NG, NQ, GW, T), f32),
        pltpu.VMEM((2, NQ, D // 2, T), u32),
        pltpu.VMEM((NG, GW + 8, T), f32),
        pltpu.SemaphoreType.DMA((8,)),
        pltpu.SemaphoreType.DMA((1,)),
    ]
    return pl.pallas_call(
        _kernel,
        out_shape=jax.ShapeDtypeStruct((1, S, 2 * D), bf16),
        in_specs=[hbm] * 14,
        out_specs=hbm,
        scratch_shapes=scratch,
        compiler_params=pltpu.CompilerParams(vmem_limit_bytes=100 * 2**20),
    )(
        A_shift_k.T, A_ssm_D.reshape(NC, T), B_beta, _FWD, _INV,
        A_q, A_k, A_v, A_ssm_k, B_x, B_wq, B_wk, B_wv, B_wo,
    )
```

```python
import jax
import jax.numpy as jnp
import numpy as np
from jax import lax
from jax.experimental import pallas as pl
from jax.experimental.pallas import tpu as pltpu

f32, bf16, u32, i32 = jnp.float32, jnp.bfloat16, jnp.uint32, jnp.int32

S, D, H, DH = 2048, 640, 32, 20
NSEG, L = 4, 512
T = 128
NC = D // T
NB = S // (2 * T)
NQ = L // T
NG = 8
GW = 4 * DH
APARTS = 2
NFV = 16
LOG2E = 1.4426950408889634
NEG = -1e30
MIX_PER_ITER = 4

PLAN_FIRST = (
    "Wx2 Qa0 Da0 Tx3 Tx4 Tx5 Qa1 Qa2 Qa3 Pa0 Qa4 Pa1 Va0 Pa2 Va1 Qa5 Pa3 Qa6 Pa4 Da1 Va2 Qa7 Va3 "
    "Qa8 Qa9 Va4 Qb0 Va5 Qb1 Va6 Db0 Va7 Qb2 Wx3 Tx6 Tx7 Tx8 Va8 Qb3 Vb0 Va9 Qb4 Pb0 Tx9 Tx10 "
    "Tx11 Qb5 Vb1 Qb6 Vb2 Db1 Vb3 Qb7 Tx12 Tx13 Tx14 Pb1 Kx Pb2 Vb4 Qb8 Vb5 Qb9 Pb3 Pb4 Vb6 Vb7 "
    "Vb8 Vb9"
).split()
PLAN0 = (
    "Qa0 Da0 Pa0 Qa1 Pa1 Qa2 Qa3 Pa2 Pa3 Qa4 Va0 Va1 Qa5 Qa6 Pa4 Da1 Va2 Qa7 Va3 Qa8 Qa9 Va4 Qb0 "
    "Va5 Qb1 Va6 Db0 Va7 Qb2 Va8 Qb3 Va9 Qb4 Pb0 Qb5 Vb0 Vb1 Qb6 Vb2 Db1 Vb3 Qb7 Pb1 Pb2 Vb4 Qb8 "
    "Vb5 Qb9 Pb3 Pb4 Vb6 Vb7 Vb8 Vb9"
).split()
PLAN1 = (
    "Qa0 Da0 Pa0 Pa1 Qa1 Qa2 Pa2 Qa3 Pa3 Va0 Pa4 Qa4 Qa5 Va1 Qa6 Oa0 Va2 Va3 Qa7 Oa1 Da1 Va4 Oa2 "
    "Qa8 Oa3 Oa4 Qa9 Ua Ra Va5 Va6 Qb0 Va7 Qb1 Db0 Qb2 Va8 Qb3 Pb0 Vb0 Va9 Pb1 Qb4 Qb5 Qb6 Vb1 "
    "Db1 Vb2 Qb7 Vb3 Pb2 Qb8 Vb4 Cx Vb5 Qb9 Pb3 Vb6 Pb4 Rb Vb7 Vb8 Vb9 Ub"
).split()
PLAN_LAST = (
    "Qa0 Da0 Pa0 Pa1 Qa1 Qa2 Qa3 Pa2 Pa3 Pa4 Qa4 Ix0 Qa5 Ix1 Va0 Ix2 Va1 Qa6 Ix3 Oa0 Va2 Qa7 Ix4 "
    "Ax0 Da1 Va3 Oa1 Ix5 Oa2 Qa8 Ix6 Va4 Oa3 Ix7 Oa4 Va5 Qa9 Ix8 Ax1 Ra Ua Va6 Ix9 Cx Qb0 Ix10 "
    "Va7 Qb1 Ix11 Db0 Ix12 Ax2 Qb2 Va8 Ix13 Qb3 Ix14 Vb0 Va9 Ix15 Qb4 Ix16 Ax3 Qb5 Ix17 Vb1 Qb6 "
    "Ix18 Db1 Ix19 Vb2 Qb7 Ix20 Ax4 Vb3 Ix21 Qb8 Ix22 Vb4 Ix23 Vb5 Qb9 Ix24 Ax5 Ix25 Ix26 Vb6 "
    "Ix27 Rb Ix28 Ax6 Vb7 Ix29 Ix30 Vb8 Ix31 Ix32 Ax7 Vb9 Ix33 Lx3 Ix34 Lx2 Ix35 Ix36 Ax8 Lx1 "
    "Ix37 Ix38 Lx0 Ix39 Ex0 Jx Ax9 Ex1 Ex2 Ex3 Ex4 Ex5 Ex6 Gx0 Fx0 Ex7 Ex8 Ex9 Ex10 Ex11 Ex12 Gx1 "
    "Fx1 Ex13 Ex14 Ex15 Ex16 Ex17 Ex18 Gx2 Fx2 Ex19 Ex20 Ex21 Ex22 Gx3 Ex23 Ex24 Gx4"
).split()
ORDER = (3, 2, 1, 0)
LEAD = {False: (400, 56), True: (400, 24)}
WA, WP, WO, WM = 1.2, 1.0, 1.0, 1.4
MIX_CYCLES = (2 * (1152 * WA + 1200 * WP + 176 * WM) + 800 * WO) * 0.965

NN = (((1,), (0,)), ((), ()))
NT = (((1,), (1,)), ((), ()))


def _dft_tables():
    freq = np.concatenate([np.arange(0, T, 2), T - 1 - np.arange(0, T, 2)])

    def table(freq, n):
        theta = 2.0 * np.pi * (freq[:, None] + 0.5) * n[None, :] / (4 * T)
        parts = [f(theta).reshape(-1, 8, len(n)) for f in (np.cos, lambda t: -np.sin(t))]
        return np.stack(parts, axis=1).reshape(-1, len(n))

    fwd = np.stack([table(freq, 2 * np.arange(T) + r) for r in range(2)])
    inv = np.stack([table(freq[:T // 2], 4 * np.arange(T // 2) + r).T / (2 * T) for r in range(4)])
    return fwd.astype(np.float32).astype(bf16), inv.astype(np.float32).astype(bf16)


_FWD, _INV = _dft_tables()


def _as_bf16(words):
    return pltpu.bitcast(words, bf16)


def _as_words(x):
    return pltpu.bitcast(x.astype(bf16), u32)


def _even_rows(words):
    return pltpu.bitcast(words << 16, f32)


def _odd_rows(words):
    return pltpu.bitcast(words & np.uint32(0xFFFF0000), f32)


def _interleave(even, odd):
    even, odd = (pltpu.bitcast(x.astype(bf16).astype(f32), u32) for x in (even, odd))
    return (even >> 16) | odd


def _dot(a, b):
    return lax.dot_general(a, b, NN, preferred_element_type=f32)


def _dot_nt(a, b):
    return lax.dot_general(a, b, NT, preferred_element_type=f32)


def _phi(t):
    return jnp.maximum(t, 0.0) + jnp.exp(jnp.minimum(t, 0.0))


def _ds(start, size, align):
    if isinstance(start, int):
        return pl.ds(start, size)
    return pl.ds(pl.multiple_of(start, align), size)


class _Pacer:
    def __init__(self, never):
        self.never, self.side, self.rate = never, None, 0.0
        self.credit, self.clock, self.history = 0.0, 0.0, []

    def attach(self, side, rate):
        self.side, self.rate, self.credit = side, rate, 0.0
        next(side)

    def issued(self, result, lane, weight=0.0):
        rows = result.shape[0]
        self.history.append((self.clock, result))
        if lane == 3:
            self.clock += rows
        self.credit += self.rate * rows / 4 * weight
        count = int(self.credit)
        self.credit -= count
        for i in range(count):
            if self.side is not None:
                v = min(rows // 8 - 1, int(rows // 8 * (lane + (i + 0.5) / count) / 4))
                try:
                    self.side.send(result[8 * v:8 * v + 8])
                except StopIteration:
                    self.side = None

    def hold(self, value, lead):
        target = self.clock - lead
        if target < 0 or self.never is None:
            return value
        for start, result in reversed(self.history):
            if start <= target:
                v = min(result.shape[0] // 8 - 1, int(target - start) // 8)
                return jnp.where(self.never, result[8 * v:8 * v + 8], value)
        return value


def _kernel(
    shift_hbm, ssmd_hbm, beta_hbm, fwd_hbm, inv_hbm,
    q_hbm, k_hbm, v_hbm, ssm_hbm, x_hbm, wq_hbm, wk_hbm, wv_hbm, wo_hbm, out_hbm,
    shift_ref, ssmd_ref, beta_ref, fwd_ref, inv_ref,
    xs, wraw, wt, wot, qa, ka, va, ssk, spec_buf, yf, outa, outb,
    fwd, inv, gate, bias, qm, qd, pq, kk, vt, pk_keep, vt_keep, ot, mz, sem_in, sem_out,
):
    def w_copies(n, sem):
        return [
            pltpu.make_async_copy(src.at[:, pl.ds(n * T, T)], wraw.at[i, n], sem)
            for i, src in enumerate((wq_hbm, wk_hbm, wv_hbm))
        ]

    def x_copies(lo, hi, sem):
        rows = pl.ds(lo * L, (hi - lo) * L)
        return [
            pltpu.make_async_copy(x_hbm.at[0, rows, pl.ds(c * T, T)], xs.at[c, rows], sem)
            for c in range(NC)
        ]

    def column_tiles(src, dst, sem):
        return [
            pltpu.make_async_copy(src.at[0, :, pl.ds(c * T, T)], dst.at[c], sem)
            for c in range(NC)
        ]

    loads = [
        w_copies(0, sem_in.at[0]),
        x_copies(0, 1, sem_in.at[1])
        + [pltpu.make_async_copy(beta_hbm, beta_ref, sem_in.at[1])],
        w_copies(1, sem_in.at[2]),
        sum((w_copies(n, sem_in.at[3]) for n in range(2, NC)), [
            pltpu.make_async_copy(fwd_hbm, fwd_ref, sem_in.at[3]),
            pltpu.make_async_copy(inv_hbm, inv_ref, sem_in.at[3])]),
        x_copies(1, 2, sem_in.at[4]),
        [pltpu.make_async_copy(src, dst, sem_in.at[5]) for src, dst in (
            (shift_hbm, shift_ref), (ssmd_hbm, ssmd_ref),
            (ssm_hbm, ssk))]
        + column_tiles(k_hbm, ka, sem_in.at[5]) + column_tiles(v_hbm, va, sem_in.at[5])
        + [pltpu.make_async_copy(wo_hbm.at[:, pl.ds(n * T, T)], wraw.at[3, n], sem_in.at[5])
           for n in range(NC)],
        x_copies(2, NSEG, sem_in.at[6]),
        column_tiles(q_hbm, qa, sem_in.at[7]),
    ]
    def start(lo, hi):
        for copies in loads[lo:hi]:
            for cp in copies:
                cp.start()

    start(0, 3)

    def wait(i):
        for cp in loads[i]:
            cp.wait()

    mz[...] = jnp.zeros(mz.shape, f32)
    row = lax.broadcasted_iota(i32, (T // 2, T), 0)
    col = lax.broadcasted_iota(i32, (T // 2, T), 1)
    bias[0] = jnp.where(row <= col, 0.0, NEG)
    bias[1] = jnp.where(row <= col % (T // 2), 0.0, NEG)

    def setup_gate():
        beta = jnp.concatenate(
            [beta_ref[...].astype(f32)[None, :], jnp.zeros((1, T - H), f32)], axis=1)
        gate[...] = jax.nn.sigmoid(jnp.broadcast_to(beta, (T, T)).T[:H])

    def transpose_qkv(part):
        n, i = divmod(part, 3)
        for c in range(NC):
            tile = wraw[i, n, c * T:(c + 1) * T, :]
            wt[i, c, n * T // 2:(n + 1) * T // 2, :] = pltpu.bitcast(tile.T, u32)

    def repack_tables(_):
        for i in range(2):
            fwd[i] = pltpu.bitcast(fwd_ref[i], u32)
        for i in range(4):
            inv[i] = pltpu.bitcast(inv_ref[i], u32)

    def transpose_wo(n):
        for c in range(NC):
            wot[c, n * T // 2:(n + 1) * T // 2, :] = pltpu.bitcast(wo_tile(c, n).T, u32)

    sub = lax.broadcasted_iota(i32, (8, T), 0)
    low = sub < 4
    left = lax.broadcasted_iota(i32, (8, T), 1) < T // 2

    def project(s, g, slot, pacer):
        rows = _ds(g * (GW // 2), GW // 2, 8)
        acc = [None] * NQ

        def store(n):
            q_t, k_t, v_t = acc[n][:GW], acc[n][GW:2 * GW], acc[n][2 * GW:]
            k_pad = jnp.concatenate([k_t.astype(bf16), jnp.zeros((T - GW, T), bf16)], axis=0)
            kk[slot, n] = pltpu.bitcast(k_pad.T, u32)
            qs = q_t * (DH ** -0.5 * LOG2E)
            r = [qs[8 * i:8 * i + 8] for i in range(10)]
            zero = jnp.zeros((8, T), f32)
            heads = [
                r[0], r[1], jnp.where(low, r[2], 0.0), zero,
                jnp.where(low, 0.0, r[2]), r[3], r[4], zero,
                zero, r[5], r[6], jnp.where(low, r[7], 0.0),
                zero, jnp.where(low, 0.0, r[7]), r[8], r[9],
            ]
            qm[slot, n] = _as_words(jnp.concatenate(heads, axis=0))
            e = {i: jnp.where(left, pltpu.roll(r[i], 64, 1), 0.0) for i in (0, 1, 2, 5, 6, 7)}
            o = {i: jnp.where(left, 0.0, r[i]) for i in (2, 3, 4, 7, 8, 9)}
            pairs = [
                e[0], e[1], jnp.where(low, e[2], o[2]), o[3], o[4], zero,
                zero, e[5], e[6], jnp.where(low, e[7], o[7]), o[8], o[9],
            ]
            qd[slot, n] = _as_words(jnp.concatenate(pairs, axis=0))
            pq[slot, n] = _as_words(_phi(q_t))
            pk_keep[s % 2, g, n] = _as_words(_phi(k_t))
            vt[slot, n] = v_t
            vt_keep[s % 2, g, n] = v_t

        def step(i):
            for lane in range(4):
                n, c = divmod(4 * i + lane, NC)
                w = _as_bf16(jnp.concatenate([wt[m, c, rows, :] for m in range(3)], axis=0))
                part = _dot_nt(w, xs[c, _ds(s * L + n * T, T, T), :])
                pacer.issued(part, lane, WP)
                acc[n] = part if c == 0 else acc[n] + part
                if c == NC - 1:
                    store(n)

        return step

    def masked_dot(key_words, window, first):
        end = first + window.shape[0]
        parts = [window, jnp.zeros((T - end, T), bf16)]
        if first:
            parts.insert(0, jnp.zeros((first, T), bf16))
        return _dot(_as_bf16(key_words), jnp.concatenate(parts, axis=0))

    def update(s, g, pacer):
        state = mz[g]
        for kt in range(NQ):
            v_one = jnp.concatenate(
                [vt_keep[(s + 1) % 2, g, kt], jnp.ones((8, T), f32)], axis=0)
            pk_t = jnp.concatenate(
                [_as_bf16(pk_keep[(s + 1) % 2, g, kt]), jnp.zeros((T - GW, T), bf16)], axis=0)
            part = _dot_nt(v_one, pk_t)
            pacer.issued(part, kt, WM)
            state = state + part
        mz[g] = state

    def attend(s, g, slot, pacer, memory):
        lead, stagger = LEAD[memory]
        tiles = [(qt, kt) for qt in ORDER for kt in range(qt + 1)]
        logits, run_max, col_max, acc, mem, done = {}, {}, {}, {}, {}, []
        corner, corner_max, corner_p = {}, {}, {}
        gates = [jnp.broadcast_to(gate[pl.ds(4 * g + j, 1), :], (8, T)) for j in range(4)]

        low_pair = sub % 4 < 2
        rest_rows = 1.0 - jnp.where(low, jnp.where(low_pair, gates[1], gates[3]),
                                    jnp.where(low_pair, gates[0], gates[2]))

        def read(_):
            def head_of(i):
                return (i >= DH).astype(i32) + (i >= 2 * DH).astype(i32) + (i >= 3 * DH).astype(i32)

            state = mz[g]
            row_m = lax.broadcasted_iota(i32, (GW, T), 0)
            col_m = lax.broadcasted_iota(i32, (GW, T), 1)
            weights = jnp.where(head_of(row_m) == head_of(col_m), state[:GW], 0.0)
            lane_head = head_of(lax.broadcasted_iota(i32, (8, T), 1))
            pair_of = sub // 2
            z_rows = jnp.where(lane_head == pair_of, state[GW:], 0.0)
            mem_w = jnp.concatenate([weights, z_rows], axis=0)
            g_rows = jnp.where(low, jnp.where(sub < 2, gates[0], gates[1]),
                               jnp.where(sub < 6, gates[2], gates[3]))
            for qt in range(NQ):
                res = _dot(mem_w, jnp.concatenate(
                    [_as_bf16(pq[slot, qt]), jnp.zeros((T - GW, T), bf16)], axis=0))
                pacer.issued(res, qt, WM)
                coef = g_rows / (res[GW:] + 1e-6)
                c0, c1, c2, c3 = (
                    jnp.broadcast_to(coef[2 * j:2 * j + 1], (8, T)) for j in range(4))
                cm = [c0, c0, jnp.where(low, c0, c1), c1, c1,
                      c2, c2, jnp.where(low, c2, c3), c3, c3]
                mem[qt] = [res[8 * i:8 * i + 8] * cm[i] for i in range(10)]
            finish()

        def corners(i):
            for lane in range(4):
                qt, pr = ORDER[2 * i + lane // 2], lane % 2
                window = _as_bf16(qd[slot, qt, 24 * pr:24 * pr + 24, :])
                sc = masked_dot(kk[slot, qt, T // 4:, :], window, 32 * pr)
                pacer.issued(sc, lane, WA)
                corner[qt, pr] = sc + bias[1]
                corner_max[qt, pr] = jnp.max(corner[qt, pr].reshape(8, 8, T), axis=0)

        def scores(t):
            qt, kt = tiles[t]
            for j in range(4):
                window = _as_bf16(qm[slot, qt, 16 * j:16 * j + 16, :])
                sc = masked_dot(
                    kk[slot, kt] if kt < qt else kk[slot, kt, :T // 4, :], window, 16 * j)
                pacer.issued(sc, j, WA)
                if kt == qt:
                    sc = sc + bias[0]
                m8 = jnp.max(sc.reshape(-1, 8, T), axis=0)
                run_max[qt, j] = m8 if kt == 0 else jnp.maximum(run_max[qt, j], m8)
                if kt == qt:
                    extra = corner_max[qt, j // 2]
                    if j % 2 == 0:
                        extra = pltpu.roll(extra, T // 2, 1)
                    top = jnp.maximum(run_max[qt, j], jnp.where(left, NEG, extra))
                    col_max[qt, j] = jnp.broadcast_to(
                        jnp.max(top, axis=0, keepdims=True), (8, T))
                logits[t, j] = sc
            if kt == qt:
                for pr in range(2):
                    top = jnp.where(left, pltpu.roll(col_max[qt, 2 * pr], T // 2, 1),
                                    col_max[qt, 2 * pr + 1])
                    words = _as_words(jnp.exp2(
                        corner[qt, pr].reshape(8, 8, T) - top[None]).reshape(T // 2, T))
                    for j, shifted in enumerate((pltpu.roll(words, T // 2, 1), words)):
                        corner_p[qt, 2 * pr + j] = _as_bf16(jnp.where(
                            left[None], jnp.uint32(0), shifted.reshape(4, 8, T)).reshape(32, T))

        def values(t):
            qt, kt = tiles[t]
            tops = [pacer.hold(col_max[qt, j], lead - stagger * j) for j in range(4)]
            for j in range(4):
                p = jnp.exp2(logits[t, j].reshape(-1, 8, T) - tops[j][None])
                p = p.reshape(-1, T).astype(bf16)
                if kt == qt:
                    p = jnp.concatenate([p, corner_p[qt, j]], axis=0)
                first = (0, 16, 40, 56)[j]
                v = [vt[slot, kt, first + 8 * i:first + 8 * i + 8, :] for i in range(3)]
                if j % 2 == 0:
                    v[2] = jnp.where(low, v[2], 1.0)
                else:
                    v[0] = jnp.where(low, 1.0, v[0])
                part = _dot(jnp.concatenate(v, axis=0), p)
                pacer.issued(part, j)
                acc[qt, j] = part if kt == 0 else acc[qt, j] + part
            if kt == qt:
                done.append(qt)
                finish()

        def finish():
            while done and (not memory or done[0] in mem):
                qt = done.pop(0)
                w = [[acc[qt, j][8 * i:8 * i + 8] for i in range(3)] for j in range(4)]
                sums = jnp.where(
                    low_pair, jnp.where(low, w[1][0], w[0][2]),
                    pltpu.roll(jnp.where(low, w[3][0], w[2][2]), 2, 0))
                coef = rest_rows / sums
                c0, c1, c2, c3 = (
                    jnp.broadcast_to(coef[r:r + 1], (8, T)) for r in (4, 0, 6, 2))
                o = [w[0][0] * c0, w[0][1] * c0,
                     jnp.where(low, w[0][2] * c0, w[1][0] * c1), w[1][1] * c1, w[1][2] * c1,
                     w[2][0] * c2, w[2][1] * c2,
                     jnp.where(low, w[2][2] * c2, w[3][0] * c3), w[3][1] * c3, w[3][2] * c3]
                if memory:
                    o = [mem[qt][i] + o[i] for i in range(10)]
                ot[s % 2, qt, _ds(g * (GW // 2), GW // 2, 8), :] = _as_words(
                    jnp.concatenate(o, axis=0))

        return {"D": corners, "Q": scores, "V": values, "R": read}

    def wo_tile(c, m):
        return wraw[3, m, c * T:(c + 1) * T, :]

    def out_project(s, n, pacer):
        acc, done = [None] * 4, []

        def step(i):
            for lane in range(4):
                m, c = divmod(4 * i + lane, NC)
                part = _dot(_as_bf16(wot[c, 80 * m:80 * (m + 1), :]),
                            _as_bf16(ot[s % 2, n, c * 64:(c + 1) * 64, :]))
                pacer.issued(part, lane, WO)
                acc[m] = part if c == 0 else acc[m] + part
                if c == NC - 1:
                    acc[m] = acc[m].astype(bf16)
                    while T * (len(done) + 1) <= 160 * (m + 1):
                        i0 = T * len(done)
                        pieces = [acc[k][max(i0 - 160 * k, 0):min(i0 + T - 160 * k, 160)]
                                  for k in range(i0 // 160, (i0 + T - 1) // 160 + 1)]
                        tile = jnp.concatenate(pieces, axis=0).T
                        outb[s, _ds(n * T, T, T), i0:i0 + T] = tile
                        done.append(True)

        return step

    def outb_copy(s, n):
        return pltpu.make_async_copy(
            outb.at[s, _ds(n * T, T, T)],
            out_hbm.at[0, _ds(s * L + n * T, T, T), pl.ds(D, D)], sem_out.at[0])

    def conv_forward(c):
        cols = slice(c * T, (c + 1) * T)
        taps = shift_ref[:, cols].astype(f32)
        taps = [jnp.broadcast_to(taps[j:j + 1], (T, T)) for j in range(4)]
        skip = ssmd_ref[...].astype(f32)[c:c + 1]
        slices = pl.ds(c * NFV, NFV)

        def transform(even, odd):
            e, o = (_dot(_as_bf16(fwd[i]), x) for i, x in enumerate((even, odd)))
            return [x.reshape(NFV, 2, 8, T) for x in (e + o, e - o)]

        tail = jnp.zeros((8, T), u32)
        prev = None
        for b in range(NB):
            k0 = pltpu.bitcast(ka[c, 2 * b * T:2 * (b + 1) * T, :], u32)
            ext = jnp.concatenate([tail, k0], axis=0)
            tail = k0[T - 8:]
            k1, k2 = ext[7:7 + T], ext[6:6 + T]
            e0, o0, e1, o1, o2 = (
                _even_rows(k0), _odd_rows(k0), _even_rows(k1), _odd_rows(k1), _odd_rows(k2))
            v0 = pltpu.bitcast(va[c, 2 * b * T:2 * (b + 1) * T, :], u32)
            sig = transform(
                (e0 * taps[0] + o1 * taps[1] + e1 * taps[2] + o2 * taps[3]) * _even_rows(v0),
                (o0 * taps[0] + e0 * taps[1] + o1 * taps[2] + e1 * taps[3]) * _odd_rows(v0))
            taps_t = jnp.concatenate([
                pltpu.bitcast(ssk[cols, (2 * b + i) * T:(2 * b + i + 1) * T].T, u32)
                for i in range(2)], axis=0)
            filt = transform(_even_rows(taps_t), _odd_rows(taps_t))
            for sign in range(2):
                spec_buf[slices, 0, sign, b] = sig[sign].reshape(NFV, 16, T)
                re, im = filt[sign][:, 0], filt[sign][:, 1]
                if prev is None:
                    re = re + skip[None]
                else:
                    half = NFV // 2
                    pre, pim = prev[sign][:, 0], prev[sign][:, 1]
                    re = jnp.concatenate([re[:half] - pim[:half], re[half:] + pim[half:]], axis=0)
                    im = jnp.concatenate([im[:half] + pre[:half], im[half:] - pre[half:]], axis=0)
                spec_buf[slices, 1, sign, b, 0:8, :] = re
                spec_buf[slices, 1, sign, b, 8:16, :] = im
            prev = filt

    def conv_mix(first, count, never, blk=4):
        half = NFV // 2
        for item in range(count):
            idx = jnp.minimum(first + item, NC * half - 1)
            base = idx // half * NFV + idx % half

            def products(fv, sign, a0):
                def load(which, b):
                    return (spec_buf[fv, which, sign, b, 0:8, :],
                            spec_buf[fv, which, sign, b, 8:16, :])

                acc, kcache = [None] * blk, {}
                for b in range(a0 + blk):
                    token = yield
                    ur, ui = load(0, b)
                    ur = jnp.where(never, token, ur)
                    us = ur + ui
                    for a in range(max(a0, b), a0 + blk):
                        if a - b not in kcache:
                            kr, ki = load(1, a - b)
                            kcache[a - b] = (kr, ki - kr, kr + ki)
                        k1, k2, k3 = kcache[a - b]
                        terms = (us * k1, ur * k2, ui * k3)
                        old = acc[a - a0]
                        acc[a - a0] = terms if old is None else tuple(
                            o + t for o, t in zip(old, terms))
                return [(p1 - p3, p1 + p2) for p1, p2, p3 in acc]

            for a0 in range(0, NB, blk):
                parity = []
                for fv in (base, base + half):
                    plus = yield from products(fv, 0, a0)
                    minus = yield from products(fv, 1, a0)
                    parity.append((
                        [(pr + mr, pi + mi) for (pr, pi), (mr, mi) in zip(plus, minus)],
                        [(pr - mr, pi - mi) for (pr, pi), (mr, mi) in zip(plus, minus)]))
                for i in range(blk):
                    (ar, ai), (br, bi) = parity[0][0][i], parity[1][0][i]
                    (cr, ci), (dr, di) = parity[0][1][i], parity[1][1][i]
                    folded = ((ar + br, ai - bi), (cr - di, ci - dr),
                              (ar - br, ai + bi), (cr + di, ci + dr))
                    for r in range(4):
                        yf[idx, a0 + i, r] = _as_words(jnp.concatenate(folded[r], axis=0))

    def outa_copy(k):
        c, part = divmod(k, APARTS)
        rows = pl.ds(part * (S // APARTS), S // APARTS)
        return pltpu.make_async_copy(
            outa.at[c, rows], out_hbm.at[0, rows, pl.ds(c * T, T)], sem_out.at[0])

    def conv_inverse(pacer, zero):
        pending, pin, hold = [], [], []

        def send(c):
            outa_copy(c).start()
            pin.append(True)

        def flush(_):
            while pending:
                c, a, y = pending.pop(0)
                tile = c + zero if pin else c
                rows = slice(2 * a * T, 2 * (a + 1) * T)
                w01, w23 = _interleave(y[0], y[1]), _interleave(y[2], y[3])
                words = jnp.concatenate([
                    jnp.where(sub % 2 == 0, *(
                        jnp.take_along_axis(w[8 * v:8 * v + 8], sub // 2 + 4 * h, axis=0)
                        for w in (w01, w23)))
                    for v in range(8) for h in range(2)], axis=0)
                conv = _as_bf16(words).astype(f32)
                outa[tile, rows, :] = (qa[c, rows, :].astype(f32) * conv).astype(bf16)
                if pin:
                    hold.append(pltpu.bitcast(outa[tile, rows.start:rows.start + 16, :], u32))
                    pin.clear()

        def step(i):
            c, a = divmod(i, NB)
            res = []
            for r in range(4):
                words = yf[pl.ds(c * NFV // 2, NFV // 2), a, r].reshape(T // 2, T)
                if hold:
                    words = jnp.concatenate(
                        [jnp.where(pacer.never, hold.pop(), words[:8]), words[8:]], axis=0)
                res.append(_dot(
                    _as_bf16(inv[r]), _as_bf16(words)))
                pacer.issued(res[-1], r)
            flush(0)
            pending.append((c, a, res))

        return step, flush, send

    def out_project_last(pacer, zero):
        s = NSEG - 1
        o_rows, acc = {}, {}

        def transpose(n):
            for c in range(NC):
                o_rows[n, c] = _as_bf16(ot[s % 2, n, c * 64:(c + 1) * 64, :]).T

        def step(i):
            for lane in range(4):
                tile, c = divmod(4 * i + lane, NC)
                n, m = divmod(tile, NC)
                part = _dot(o_rows[n, c], wo_tile(c, m))
                pacer.issued(part, lane)
                acc[tile] = part if c == 0 else acc[tile] + part

        def store(part):
            n = min(part, NQ - 1)
            for m in range(NC) if part < NQ - 1 else ((0, 1, 2), (3, 4))[part - n]:
                seg = s + zero if m == 0 else s
                outb[seg, n * T:(n + 1) * T, m * T:(m + 1) * T] = acc[n * NC + m].astype(bf16)

        return transpose, step, store

    def new_pacer():
        return _Pacer(gate[0:8, :] > 2.0)

    def pair(s, p, plan, pacer, mix=None):
        memory = "Ra" in plan
        if mix is not None:
            first, count, cycles = mix
            pacer.attach(conv_mix(first, count, pacer.never), count * 96 / cycles)
        steps = {"a": attend(s, 2 * p, 0, pacer, memory),
                 "b": attend(s, 2 * p + 1, 1, pacer, memory)}
        steps["a"]["P"] = project(s, 2 * p + 1, 1, pacer)
        next_s, next_g = s + (p + 1) // 4, (2 * p + 2) % NG
        steps["b"]["P"] = project(next_s, next_g, 0, pacer)
        steps["a"]["U"] = lambda _: update(s, 2 * p + 1, pacer)
        steps["b"]["U"] = lambda _: update(next_s, next_g, pacer)
        steps["a"]["O"] = out_project(s - 1, p, pacer)
        steps["x"] = {
            "T": transpose_qkv,
            "K": repack_tables,
            "W": wait,

            "C": lambda _: outb_copy(s - 1, p).start(),
        }
        if "Jx" in plan:
            zero = pacer.never.astype(i32)[0, 0]
            steps["x"]["I"], steps["x"]["J"], steps["x"]["A"] = conv_inverse(pacer, zero)
            steps["x"]["L"], steps["x"]["E"], steps["x"]["G"] = out_project_last(pacer, zero)
        steps["x"]["F"] = lambda n: outb_copy(s, n).start()
        for item in plan:
            steps[item[1]][item[0]](int(item[2:] or 0))
        assert pacer.side is None

    def memory_pair(s, p):
        first = ((s - 1) * 4 + p) * MIX_PER_ITER
        pair(s, p, PLAN1, new_pacer(), (first, MIX_PER_ITER, MIX_CYCLES))

    wait(0)
    start(3, 4)
    for part in range(3):
        transpose_qkv(part)
    wait(1)
    start(4, len(loads))
    setup_gate()
    step = project(0, 0, 0, _Pacer(None))
    for i in range(NC):
        step(i)
    pair(0, 0, PLAN_FIRST, new_pacer())
    wait(4)

    @pl.loop(1, 4)
    def _(p):
        pair(0, p, PLAN0, new_pacer())

    wait(5)
    update(1, 0, _Pacer(None))
    for c in range(NC):
        conv_forward(c)
        transpose_wo(c)
    wait(6)
    wait(7)

    @pl.loop(0, 11)
    def _(i):
        memory_pair(1 + i // 4, i % 4)

    pair(NSEG - 1, 3, PLAN_LAST, new_pacer())

    outb_copy(NSEG - 1, NQ - 1).start()
    for k in range(NC * APARTS):
        outa_copy(k).wait()
    for s in range(NSEG):
        for n in range(NQ):
            outb_copy(s, n).wait()


@jax.jit
def pallas_concat_heads__ssm_conv_h3__memory_aug_infini_attn__prompt_kernel(
    A_q: jax.Array,
    A_k: jax.Array,
    A_v: jax.Array,
    A_shift_k: jax.Array,
    A_ssm_k: jax.Array,
    A_ssm_D: jax.Array,
    B_x: jax.Array,
    B_wq: jax.Array,
    B_wk: jax.Array,
    B_wv: jax.Array,
    B_wo: jax.Array,
    B_beta: jax.Array,
):
    hbm = pl.BlockSpec(memory_space=pl.ANY)
    scratch = [
        pltpu.VMEM((4, D), bf16),
        pltpu.VMEM((NC, T), bf16),
        pltpu.VMEM((H,), bf16),
        pltpu.VMEM((2, 2 * T, T), bf16),
        pltpu.VMEM((4, T // 2, T), bf16),
        pltpu.VMEM((NC, S, T), bf16),
        pltpu.VMEM((4, NC, D, T), bf16),
        pltpu.VMEM((3, NC, D // 2, T), u32),
        pltpu.VMEM((NC, D // 2, T), u32),
        pltpu.VMEM((NC, S, T), bf16),
        pltpu.VMEM((NC, S, T), bf16),
        pltpu.VMEM((NC, S, T), bf16),
        pltpu.VMEM((D, S), bf16),
        pltpu.VMEM((NC * NFV, 2, 2, NB, 16, T), f32),
        pltpu.VMEM((NC * NFV // 2, NB, 4, 8, T), u32),
        pltpu.VMEM((NC, S, T), bf16),
        pltpu.VMEM((NSEG, L, D), bf16),
        pltpu.VMEM((2, T, T), u32),
        pltpu.VMEM((4, T // 4, T), u32),
        pltpu.VMEM((H, T), f32),
        pltpu.VMEM((2, T // 2, T), f32),
        pltpu.VMEM((2, NQ, 64, T), u32),
        pltpu.VMEM((2, NQ, 48, T), u32),
        pltpu.VMEM((2, NQ, GW // 2, T), u32),
        pltpu.VMEM((2, NQ, T // 2, T), u32),
        pltpu.VMEM((2, NQ, GW, T), f32),
        pltpu.VMEM((2, NG, NQ, GW // 2, T), u32),
        pltpu.VMEM((2, NG, NQ, GW, T), f32),
        pltpu.VMEM((2, NQ, D // 2, T), u32),
        pltpu.VMEM((NG, GW + 8, T), f32),
        pltpu.SemaphoreType.DMA((8,)),
        pltpu.SemaphoreType.DMA((1,)),
    ]
    return pl.pallas_call(
        _kernel,
        out_shape=jax.ShapeDtypeStruct((1, S, 2 * D), bf16),
        in_specs=[hbm] * 14,
        out_specs=hbm,
        scratch_shapes=scratch,
        compiler_params=pltpu.CompilerParams(vmem_limit_bytes=100 * 2**20),
    )(
        A_shift_k.T, A_ssm_D.reshape(NC, T), B_beta, _FWD, _INV,
        A_q, A_k, A_v, A_ssm_k, B_x, B_wq, B_wk, B_wv, B_wo,
    )
```

```python
import jax
import jax.numpy as jnp
import numpy as np
from jax import lax
from jax.experimental import pallas as pl
from jax.experimental.pallas import tpu as pltpu

f32, bf16, u32, i32 = jnp.float32, jnp.bfloat16, jnp.uint32, jnp.int32

S, D, H, DH = 2048, 640, 32, 20
NSEG, L = 4, 512
T = 128
NC = D // T
NB = S // (2 * T)
NQ = L // T
NG = 8
GW = 4 * DH
APARTS = 2
NFV = 16
LOG2E = 1.4426950408889634
NEG = -1e30
MIX_PER_ITER = 4

PLAN_FIRST = (
    "Wx2 Qa0 Da0 Tx3 Tx4 Tx5 Qa1 Qa2 Qa3 Pa0 Qa4 Pa1 Va0 Pa2 Va1 Qa5 Pa3 Qa6 Pa4 Da1 Va2 Qa7 Va3 "
    "Qa8 Qa9 Va4 Qb0 Va5 Qb1 Va6 Db0 Va7 Qb2 Wx3 Tx6 Tx7 Tx8 Va8 Qb3 Vb0 Va9 Qb4 Pb0 Tx9 Tx10 "
    "Tx11 Qb5 Vb1 Qb6 Vb2 Db1 Vb3 Qb7 Tx12 Tx13 Tx14 Pb1 Kx Pb2 Vb4 Qb8 Vb5 Qb9 Pb3 Pb4 Vb6 Vb7 "
    "Vb8 Vb9"
).split()
PLAN0 = (
    "Qa0 Da0 Pa0 Qa1 Pa1 Qa2 Qa3 Pa2 Pa3 Qa4 Va0 Va1 Qa5 Qa6 Pa4 Da1 Va2 Qa7 Va3 Qa8 Qa9 Va4 Qb0 "
    "Va5 Qb1 Va6 Db0 Va7 Qb2 Va8 Qb3 Va9 Qb4 Pb0 Qb5 Vb0 Vb1 Qb6 Vb2 Db1 Vb3 Qb7 Pb1 Pb2 Vb4 Qb8 "
    "Vb5 Qb9 Pb3 Pb4 Vb6 Vb7 Vb8 Vb9"
).split()
PLAN1 = (
    "Qa0 Pa0 Da0 Pa1 Qa1 Qa2 Qa3 Pa2 Pa3 Pa4 Oa0 Qa4 Qa5 Qa6 Va0 Va1 Qa7 Va2 Oa1 Da1 Va3 Qa8 Qb0 "
    "Oa2 Ua Oa3 Oa4 Qa9 Va4 Ra Va5 Qb1 Va6 Va7 Db0 Qb2 Qb3 Va8 Qb4 Pb0 Qb5 Va9 Pb1 Qb6 Vb0 Vb1 "
    "Db1 Vb2 Qb7 Vb3 Pb2 Qb8 Vb4 Vb5 Qb9 Pb3 Vb6 Cx Pb4 Rb Vb7 Vb8 Vb9 Ub"
).split()
PLAN_LAST = (
    "Qa0 Da0 Pa0 Pa1 Qa1 Qa2 Qa3 Pa2 Pa3 Pa4 Qa4 Ix0 Qa5 Ix1 Va0 Ix2 Va1 Qa6 Ix3 Oa0 Va2 Qa7 Ix4 "
    "Ax0 Da1 Va3 Oa1 Ix5 Oa2 Qa8 Ix6 Va4 Oa3 Ix7 Oa4 Va5 Qa9 Ix8 Ax1 Ra Ua Va6 Ix9 Cx Qb0 Ix10 "
    "Va7 Qb1 Ix11 Db0 Ix12 Ax2 Qb2 Va8 Ix13 Qb3 Ix14 Vb0 Va9 Ix15 Qb4 Ix16 Ax3 Qb5 Ix17 Vb1 Qb6 "
    "Ix18 Db1 Ix19 Vb2 Qb7 Ix20 Ax4 Vb3 Ix21 Qb8 Ix22 Vb4 Ix23 Vb5 Qb9 Ix24 Ax5 Ix25 Ix26 Vb6 "
    "Ix27 Rb Ix28 Ax6 Vb7 Ix29 Ix30 Vb8 Ix31 Ix32 Ax7 Vb9 Ix33 Lx3 Ix34 Lx2 Ix35 Ix36 Ax8 Lx1 "
    "Ix37 Ix38 Lx0 Ix39 Ex0 Jx Ax9 Ex1 Ex2 Ex3 Ex4 Ex5 Ex6 Gx0 Fx0 Ex7 Ex8 Ex9 Ex10 Ex11 Ex12 Gx1 "
    "Fx1 Ex13 Ex14 Ex15 Ex16 Ex17 Ex18 Gx2 Fx2 Ex19 Ex20 Ex21 Ex22 Gx3 Ex23 Ex24 Gx4"
).split()
ORDER = (3, 2, 1, 0)
LEAD = {False: (400, 56), True: (380, 32)}
WA, WP, WO, WM = 1.2, 1.0, 1.2, 1.6
MIX_CYCLES = (2 * (1152 * WA + 1200 * WP + 176 * WM) + 800 * WO) * 0.965

NN = (((1,), (0,)), ((), ()))
NT = (((1,), (1,)), ((), ()))


def _dft_tables():
    freq = np.concatenate([np.arange(0, T, 2), T - 1 - np.arange(0, T, 2)])

    def table(freq, n):
        theta = 2.0 * np.pi * (freq[:, None] + 0.5) * n[None, :] / (4 * T)
        parts = [f(theta).reshape(-1, 8, len(n)) for f in (np.cos, lambda t: -np.sin(t))]
        return np.stack(parts, axis=1).reshape(-1, len(n))

    fwd = np.stack([table(freq, 2 * np.arange(T) + r) for r in range(2)])
    inv = np.stack([table(freq[:T // 2], 4 * np.arange(T // 2) + r).T / (2 * T) for r in range(4)])
    return fwd.astype(np.float32).astype(bf16), inv.astype(np.float32).astype(bf16)


_FWD, _INV = _dft_tables()


def _as_bf16(words):
    return pltpu.bitcast(words, bf16)


def _as_words(x):
    return pltpu.bitcast(x.astype(bf16), u32)


def _even_rows(words):
    return pltpu.bitcast(words << 16, f32)


def _odd_rows(words):
    return pltpu.bitcast(words & np.uint32(0xFFFF0000), f32)


def _interleave(even, odd):
    even, odd = (pltpu.bitcast(x.astype(bf16).astype(f32), u32) for x in (even, odd))
    return (even >> 16) | odd


def _dot(a, b):
    return lax.dot_general(a, b, NN, preferred_element_type=f32)


def _dot_nt(a, b):
    return lax.dot_general(a, b, NT, preferred_element_type=f32)


def _phi(t):
    return jnp.maximum(t, 0.0) + jnp.exp(jnp.minimum(t, 0.0))


def _ds(start, size, align):
    if isinstance(start, int):
        return pl.ds(start, size)
    return pl.ds(pl.multiple_of(start, align), size)


class _Pacer:
    def __init__(self, never):
        self.never, self.side, self.rate = never, None, 0.0
        self.credit, self.clock, self.history = 0.0, 0.0, []

    def attach(self, side, rate):
        self.side, self.rate, self.credit = side, rate, 0.0
        next(side)

    def issued(self, result, lane, weight=0.0):
        rows = result.shape[0]
        self.history.append((self.clock, result))
        if lane == 3:
            self.clock += rows
        self.credit += self.rate * rows / 4 * weight
        count = int(self.credit)
        self.credit -= count
        for i in range(count):
            if self.side is not None:
                v = min(rows // 8 - 1, int(rows // 8 * (lane + (i + 0.5) / count) / 4))
                try:
                    self.side.send(result[8 * v:8 * v + 8])
                except StopIteration:
                    self.side = None

    def hold(self, value, lead):
        target = self.clock - lead
        if target < 0 or self.never is None:
            return value
        for start, result in reversed(self.history):
            if start <= target:
                v = min(result.shape[0] // 8 - 1, int(target - start) // 8)
                return jnp.where(self.never, result[8 * v:8 * v + 8], value)
        return value


def _kernel(
    shift_hbm, ssmd_hbm, beta_hbm, fwd_hbm, inv_hbm,
    q_hbm, k_hbm, v_hbm, ssm_hbm, x_hbm, wq_hbm, wk_hbm, wv_hbm, wo_hbm, out_hbm,
    shift_ref, ssmd_ref, beta_ref, fwd_ref, inv_ref,
    xs, wraw, wt, wot, qa, ka, va, ssk, spec_buf, yf, outa, outb,
    fwd, inv, gate, bias, qm, qd, pq, kk, vt, pk_keep, vt_keep, ot, mz, sem_in, sem_out,
):
    def w_copies(n, sem):
        return [
            pltpu.make_async_copy(src.at[:, pl.ds(n * T, T)], wraw.at[i, n], sem)
            for i, src in enumerate((wq_hbm, wk_hbm, wv_hbm))
        ]

    def x_copies(lo, hi, sem):
        rows = pl.ds(lo * L, (hi - lo) * L)
        return [
            pltpu.make_async_copy(x_hbm.at[0, rows, pl.ds(c * T, T)], xs.at[c, rows], sem)
            for c in range(NC)
        ]

    def column_tiles(src, dst, sem):
        return [
            pltpu.make_async_copy(src.at[0, :, pl.ds(c * T, T)], dst.at[c], sem)
            for c in range(NC)
        ]

    loads = [
        w_copies(0, sem_in.at[0]),
        x_copies(0, 1, sem_in.at[1])
        + [pltpu.make_async_copy(beta_hbm, beta_ref, sem_in.at[1])],
        w_copies(1, sem_in.at[2]),
        sum((w_copies(n, sem_in.at[3]) for n in range(2, NC)), [
            pltpu.make_async_copy(fwd_hbm, fwd_ref, sem_in.at[3]),
            pltpu.make_async_copy(inv_hbm, inv_ref, sem_in.at[3])]),
        x_copies(1, 2, sem_in.at[4]),
        [pltpu.make_async_copy(src, dst, sem_in.at[5]) for src, dst in (
            (shift_hbm, shift_ref), (ssmd_hbm, ssmd_ref),
            (ssm_hbm, ssk))]
        + column_tiles(k_hbm, ka, sem_in.at[5]) + column_tiles(v_hbm, va, sem_in.at[5])
        + [pltpu.make_async_copy(wo_hbm.at[:, pl.ds(n * T, T)], wraw.at[3, n], sem_in.at[5])
           for n in range(NC)],
        x_copies(2, NSEG, sem_in.at[6]),
        column_tiles(q_hbm, qa, sem_in.at[7]),
    ]

    def start(lo, hi):
        for copies in loads[lo:hi]:
            for cp in copies:
                cp.start()

    start(0, 3)

    def wait(i):
        for cp in loads[i]:
            cp.wait()

    mz[...] = jnp.zeros(mz.shape, f32)
    row = lax.broadcasted_iota(i32, (T // 2, T), 0)
    col = lax.broadcasted_iota(i32, (T // 2, T), 1)
    bias[0] = jnp.where(row <= col, 0.0, NEG)
    bias[1] = jnp.where(row <= col % (T // 2), 0.0, NEG)

    def setup_gate():
        beta = jnp.concatenate(
            [beta_ref[...].astype(f32)[None, :], jnp.zeros((1, T - H), f32)], axis=1)
        gate[...] = jax.nn.sigmoid(jnp.broadcast_to(beta, (T, T)).T[:H])

    def transpose_qkv(part):
        n, i = divmod(part, 3)
        for c in range(NC):
            tile = wraw[i, n, c * T:(c + 1) * T, :]
            wt[i, c, n * T // 2:(n + 1) * T // 2, :] = pltpu.bitcast(tile.T, u32)

    def repack_tables(_):
        for i in range(2):
            fwd[i] = pltpu.bitcast(fwd_ref[i], u32)
        for i in range(4):
            inv[i] = pltpu.bitcast(inv_ref[i], u32)

    def transpose_wo(n):
        for c in range(NC):
            wot[c, n * T // 2:(n + 1) * T // 2, :] = pltpu.bitcast(wo_tile(c, n).T, u32)

    sub = lax.broadcasted_iota(i32, (8, T), 0)
    low = sub < 4
    left = lax.broadcasted_iota(i32, (8, T), 1) < T // 2

    def project(s, g, slot, pacer):
        rows = _ds(g * (GW // 2), GW // 2, 8)
        acc = [None] * NQ

        def store(n):
            q_t, k_t, v_t = acc[n][:GW], acc[n][GW:2 * GW], acc[n][2 * GW:]
            k_pad = jnp.concatenate([k_t.astype(bf16), jnp.zeros((T - GW, T), bf16)], axis=0)
            kk[slot, n] = pltpu.bitcast(k_pad.T, u32)
            qs = q_t * (DH ** -0.5 * LOG2E)
            r = [qs[8 * i:8 * i + 8] for i in range(10)]
            zero = jnp.zeros((8, T), f32)
            heads = [
                r[0], r[1], jnp.where(low, r[2], 0.0), zero,
                jnp.where(low, 0.0, r[2]), r[3], r[4], zero,
                zero, r[5], r[6], jnp.where(low, r[7], 0.0),
                zero, jnp.where(low, 0.0, r[7]), r[8], r[9],
            ]
            qm[slot, n] = _as_words(jnp.concatenate(heads, axis=0))
            e = {i: jnp.where(left, pltpu.roll(r[i], 64, 1), 0.0) for i in (0, 1, 2, 5, 6, 7)}
            o = {i: jnp.where(left, 0.0, r[i]) for i in (2, 3, 4, 7, 8, 9)}
            pairs = [
                e[0], e[1], jnp.where(low, e[2], o[2]), o[3], o[4], zero,
                zero, e[5], e[6], jnp.where(low, e[7], o[7]), o[8], o[9],
            ]
            qd[slot, n] = _as_words(jnp.concatenate(pairs, axis=0))
            pq[slot, n] = _as_words(_phi(q_t))
            pk_keep[s % 2, g, n] = _as_words(_phi(k_t))
            vt[slot, n] = v_t
            vt_keep[s % 2, g, n] = v_t

        def step(i):
            for lane in range(4):
                n, c = divmod(4 * i + lane, NC)
                w = _as_bf16(jnp.concatenate([wt[m, c, rows, :] for m in range(3)], axis=0))
                part = _dot_nt(w, xs[c, _ds(s * L + n * T, T, T), :])
                pacer.issued(part, lane, WP)
                acc[n] = part if c == 0 else acc[n] + part
                if c == NC - 1:
                    store(n)

        return step

    def masked_dot(key_words, window, first):
        end = first + window.shape[0]
        parts = [window, jnp.zeros((T - end, T), bf16)]
        if first:
            parts.insert(0, jnp.zeros((first, T), bf16))
        return _dot(_as_bf16(key_words), jnp.concatenate(parts, axis=0))

    def update(s, g, pacer):
        state = mz[g]
        for kt in range(NQ):
            v_one = jnp.concatenate(
                [vt_keep[(s + 1) % 2, g, kt], jnp.ones((8, T), f32)], axis=0)
            pk_t = jnp.concatenate(
                [_as_bf16(pk_keep[(s + 1) % 2, g, kt]), jnp.zeros((T - GW, T), bf16)], axis=0)
            part = _dot_nt(v_one, pk_t)
            pacer.issued(part, kt, WM)
            state = state + part
        mz[g] = state

    def attend(s, g, slot, pacer, memory):
        lead, stagger = LEAD[memory]
        tiles = [(qt, kt) for qt in ORDER for kt in range(qt + 1)]
        logits, run_max, col_max, acc, mem, done = {}, {}, {}, {}, {}, []
        corner, corner_max, corner_p = {}, {}, {}
        gates = [jnp.broadcast_to(gate[pl.ds(4 * g + j, 1), :], (8, T)) for j in range(4)]
        low_pair = sub % 4 < 2
        rest_rows = 1.0 - jnp.where(low, jnp.where(low_pair, gates[1], gates[3]),
                                    jnp.where(low_pair, gates[0], gates[2]))

        def read(_):
            def head_of(i):
                return (i >= DH).astype(i32) + (i >= 2 * DH).astype(i32) + (i >= 3 * DH).astype(i32)

            state = mz[g]
            row_m = lax.broadcasted_iota(i32, (GW, T), 0)
            col_m = lax.broadcasted_iota(i32, (GW, T), 1)
            weights = jnp.where(head_of(row_m) == head_of(col_m), state[:GW], 0.0)
            lane_head = head_of(lax.broadcasted_iota(i32, (8, T), 1))
            pair_of = sub // 2
            z_rows = jnp.where(lane_head == pair_of, state[GW:], 0.0)
            mem_w = jnp.concatenate([weights, z_rows], axis=0)
            g_rows = jnp.where(low, jnp.where(sub < 2, gates[0], gates[1]),
                               jnp.where(sub < 6, gates[2], gates[3]))
            for qt in range(NQ):
                res = _dot(mem_w, jnp.concatenate(
                    [_as_bf16(pq[slot, qt]), jnp.zeros((T - GW, T), bf16)], axis=0))
                pacer.issued(res, qt, WM)
                coef = g_rows / (res[GW:] + 1e-6)
                c0, c1, c2, c3 = (
                    jnp.broadcast_to(coef[2 * j:2 * j + 1], (8, T)) for j in range(4))
                cm = [c0, c0, jnp.where(low, c0, c1), c1, c1,
                      c2, c2, jnp.where(low, c2, c3), c3, c3]
                mem[qt] = [res[8 * i:8 * i + 8] * cm[i] for i in range(10)]
            finish()

        def corners(i):
            for lane in range(4):
                qt, pr = ORDER[2 * i + lane // 2], lane % 2
                window = _as_bf16(qd[slot, qt, 24 * pr:24 * pr + 24, :])
                sc = masked_dot(kk[slot, qt, T // 4:, :], window, 32 * pr)
                pacer.issued(sc, lane, WA)
                corner[qt, pr] = sc + bias[1]
                corner_max[qt, pr] = jnp.max(corner[qt, pr].reshape(8, 8, T), axis=0)

        def scores(t):
            qt, kt = tiles[t]
            for j in range(4):
                window = _as_bf16(qm[slot, qt, 16 * j:16 * j + 16, :])
                sc = masked_dot(
                    kk[slot, kt] if kt < qt else kk[slot, kt, :T // 4, :], window, 16 * j)
                pacer.issued(sc, j, WA)
                if kt == qt:
                    sc = sc + bias[0]
                m8 = jnp.max(sc.reshape(-1, 8, T), axis=0)
                run_max[qt, j] = m8 if kt == 0 else jnp.maximum(run_max[qt, j], m8)
                if kt == qt:
                    extra = corner_max[qt, j // 2]
                    if j % 2 == 0:
                        extra = pltpu.roll(extra, T // 2, 1)
                    top = jnp.maximum(run_max[qt, j], jnp.where(left, NEG, extra))
                    col_max[qt, j] = jnp.broadcast_to(
                        jnp.max(top, axis=0, keepdims=True), (8, T))
                logits[t, j] = sc
            if kt == qt:
                for pr in range(2):
                    top = jnp.where(left, pltpu.roll(col_max[qt, 2 * pr], T // 2, 1),
                                    col_max[qt, 2 * pr + 1])
                    words = _as_words(jnp.exp2(
                        corner[qt, pr].reshape(8, 8, T) - top[None]).reshape(T // 2, T))
                    for j, shifted in enumerate((pltpu.roll(words, T // 2, 1), words)):
                        corner_p[qt, 2 * pr + j] = _as_bf16(jnp.where(
                            left[None], jnp.uint32(0), shifted.reshape(4, 8, T)).reshape(32, T))

        def values(t):
            qt, kt = tiles[t]
            tops = [pacer.hold(col_max[qt, j], lead - stagger * j) for j in range(4)]
            for j in range(4):
                p = jnp.exp2(logits[t, j].reshape(-1, 8, T) - tops[j][None])
                p = p.reshape(-1, T).astype(bf16)
                if kt == qt:
                    p = jnp.concatenate([p, corner_p[qt, j]], axis=0)
                first = (0, 16, 40, 56)[j]
                v = [vt[slot, kt, first + 8 * i:first + 8 * i + 8, :] for i in range(3)]
                if j % 2 == 0:
                    v[2] = jnp.where(low, v[2], 1.0)
                else:
                    v[0] = jnp.where(low, 1.0, v[0])
                part = _dot(jnp.concatenate(v, axis=0), p)
                pacer.issued(part, j)
                acc[qt, j] = part if kt == 0 else acc[qt, j] + part
            if kt == qt:
                done.append(qt)
                finish()

        def finish():
            while done and (not memory or done[0] in mem):
                qt = done.pop(0)
                w = [[acc[qt, j][8 * i:8 * i + 8] for i in range(3)] for j in range(4)]
                sums = jnp.where(
                    low_pair, jnp.where(low, w[1][0], w[0][2]),
                    pltpu.roll(jnp.where(low, w[3][0], w[2][2]), 2, 0))
                coef = rest_rows / sums
                c0, c1, c2, c3 = (
                    jnp.broadcast_to(coef[r:r + 1], (8, T)) for r in (4, 0, 6, 2))
                o = [w[0][0] * c0, w[0][1] * c0,
                     jnp.where(low, w[0][2] * c0, w[1][0] * c1), w[1][1] * c1, w[1][2] * c1,
                     w[2][0] * c2, w[2][1] * c2,
                     jnp.where(low, w[2][2] * c2, w[3][0] * c3), w[3][1] * c3, w[3][2] * c3]
                if memory:
                    o = [mem[qt][i] + o[i] for i in range(10)]
                ot[s % 2, qt, _ds(g * (GW // 2), GW // 2, 8), :] = _as_words(
                    jnp.concatenate(o, axis=0))

        return {"D": corners, "Q": scores, "V": values, "R": read}

    def wo_tile(c, m):
        return wraw[3, m, c * T:(c + 1) * T, :]

    def out_project(s, n, pacer):
        acc, done = [None] * 4, []

        def step(i):
            for lane in range(4):
                m, c = divmod(4 * i + lane, NC)
                part = _dot(_as_bf16(wot[c, 80 * m:80 * (m + 1), :]),
                            _as_bf16(ot[s % 2, n, c * 64:(c + 1) * 64, :]))
                pacer.issued(part, lane, WO)
                acc[m] = part if c == 0 else acc[m] + part
                if c == NC - 1:
                    acc[m] = acc[m].astype(bf16)
                    while T * (len(done) + 1) <= 160 * (m + 1):
                        i0 = T * len(done)
                        pieces = [acc[k][max(i0 - 160 * k, 0):min(i0 + T - 160 * k, 160)]
                                  for k in range(i0 // 160, (i0 + T - 1) // 160 + 1)]
                        tile = jnp.concatenate(pieces, axis=0).T
                        outb[s, _ds(n * T, T, T), i0:i0 + T] = tile
                        done.append(True)

        return step

    def outb_copy(s, n):
        return pltpu.make_async_copy(
            outb.at[s, _ds(n * T, T, T)],
            out_hbm.at[0, _ds(s * L + n * T, T, T), pl.ds(D, D)], sem_out.at[0])

    def conv_forward(c):
        cols = slice(c * T, (c + 1) * T)
        taps = shift_ref[:, cols].astype(f32)
        taps = [jnp.broadcast_to(taps[j:j + 1], (T, T)) for j in range(4)]
        skip = ssmd_ref[...].astype(f32)[c:c + 1]
        slices = pl.ds(c * NFV, NFV)

        def transform(even, odd):
            e, o = (_dot(_as_bf16(fwd[i]), x) for i, x in enumerate((even, odd)))
            return [x.reshape(NFV, 2, 8, T) for x in (e + o, e - o)]

        tail = jnp.zeros((8, T), u32)
        prev = None
        for b in range(NB):
            k0 = pltpu.bitcast(ka[c, 2 * b * T:2 * (b + 1) * T, :], u32)
            ext = jnp.concatenate([tail, k0], axis=0)
            tail = k0[T - 8:]
            k1, k2 = ext[7:7 + T], ext[6:6 + T]
            e0, o0, e1, o1, o2 = (
                _even_rows(k0), _odd_rows(k0), _even_rows(k1), _odd_rows(k1), _odd_rows(k2))
            v0 = pltpu.bitcast(va[c, 2 * b * T:2 * (b + 1) * T, :], u32)
            sig = transform(
                (e0 * taps[0] + o1 * taps[1] + e1 * taps[2] + o2 * taps[3]) * _even_rows(v0),
                (o0 * taps[0] + e0 * taps[1] + o1 * taps[2] + e1 * taps[3]) * _odd_rows(v0))
            taps_t = jnp.concatenate([
                pltpu.bitcast(ssk[cols, (2 * b + i) * T:(2 * b + i + 1) * T].T, u32)
                for i in range(2)], axis=0)
            filt = transform(_even_rows(taps_t), _odd_rows(taps_t))
            for sign in range(2):
                spec_buf[slices, 0, sign, b] = sig[sign].reshape(NFV, 16, T)
                re, im = filt[sign][:, 0], filt[sign][:, 1]
                if prev is None:
                    re = re + skip[None]
                else:
                    half = NFV // 2
                    pre, pim = prev[sign][:, 0], prev[sign][:, 1]
                    re = jnp.concatenate([re[:half] - pim[:half], re[half:] + pim[half:]], axis=0)
                    im = jnp.concatenate([im[:half] + pre[:half], im[half:] - pre[half:]], axis=0)
                spec_buf[slices, 1, sign, b, 0:8, :] = re
                spec_buf[slices, 1, sign, b, 8:16, :] = im
            prev = filt

    def conv_mix(first, count, never, blk=4):
        half = NFV // 2
        for item in range(count):
            idx = jnp.minimum(first + item, NC * half - 1)
            base = idx // half * NFV + idx % half

            def products(fv, sign, a0):
                def load(which, b):
                    return (spec_buf[fv, which, sign, b, 0:8, :],
                            spec_buf[fv, which, sign, b, 8:16, :])

                acc, kcache = [None] * blk, {}
                for b in range(a0 + blk):
                    token = yield
                    ur, ui = load(0, b)
                    ur = jnp.where(never, token, ur)
                    us = ur + ui
                    for a in range(max(a0, b), a0 + blk):
                        if a - b not in kcache:
                            kr, ki = load(1, a - b)
                            kcache[a - b] = (kr, ki - kr, kr + ki)
                        k1, k2, k3 = kcache[a - b]
                        terms = (us * k1, ur * k2, ui * k3)
                        old = acc[a - a0]
                        acc[a - a0] = terms if old is None else tuple(
                            o + t for o, t in zip(old, terms))
                return [(p1 - p3, p1 + p2) for p1, p2, p3 in acc]

            for a0 in range(0, NB, blk):
                parity = []
                for fv in (base, base + half):
                    plus = yield from products(fv, 0, a0)
                    minus = yield from products(fv, 1, a0)
                    parity.append((
                        [(pr + mr, pi + mi) for (pr, pi), (mr, mi) in zip(plus, minus)],
                        [(pr - mr, pi - mi) for (pr, pi), (mr, mi) in zip(plus, minus)]))
                for i in range(blk):
                    (ar, ai), (br, bi) = parity[0][0][i], parity[1][0][i]
                    (cr, ci), (dr, di) = parity[0][1][i], parity[1][1][i]
                    folded = ((ar + br, ai - bi), (cr - di, ci - dr),
                              (ar - br, ai + bi), (cr + di, ci + dr))
                    for r in range(4):
                        yf[idx, a0 + i, r] = _as_words(jnp.concatenate(folded[r], axis=0))

    def outa_copy(k):
        c, part = divmod(k, APARTS)
        rows = pl.ds(part * (S // APARTS), S // APARTS)
        return pltpu.make_async_copy(
            outa.at[c, rows], out_hbm.at[0, rows, pl.ds(c * T, T)], sem_out.at[0])

    def conv_inverse(pacer, zero):
        pending, pin, hold = [], [], []

        def send(c):
            outa_copy(c).start()
            pin.append(True)

        def flush(_):
            while pending:
                c, a, y = pending.pop(0)
                tile = c + zero if pin else c
                rows = slice(2 * a * T, 2 * (a + 1) * T)
                w01, w23 = _interleave(y[0], y[1]), _interleave(y[2], y[3])
                words = jnp.concatenate([
                    jnp.where(sub % 2 == 0, *(
                        jnp.take_along_axis(w[8 * v:8 * v + 8], sub // 2 + 4 * h, axis=0)
                        for w in (w01, w23)))
                    for v in range(8) for h in range(2)], axis=0)
                conv = _as_bf16(words).astype(f32)
                outa[tile, rows, :] = (qa[c, rows, :].astype(f32) * conv).astype(bf16)
                if pin:
                    hold.append(pltpu.bitcast(outa[tile, rows.start:rows.start + 16, :], u32))
                    pin.clear()

        def step(i):
            c, a = divmod(i, NB)
            res = []
            for r in range(4):
                words = yf[pl.ds(c * NFV // 2, NFV // 2), a, r].reshape(T // 2, T)
                if hold:
                    words = jnp.concatenate(
                        [jnp.where(pacer.never, hold.pop(), words[:8]), words[8:]], axis=0)
                res.append(_dot(
                    _as_bf16(inv[r]), _as_bf16(words)))
                pacer.issued(res[-1], r)
            flush(0)
            pending.append((c, a, res))

        return step, flush, send

    def out_project_last(pacer, zero):
        s = NSEG - 1
        o_rows, acc = {}, {}

        def transpose(n):
            for c in range(NC):
                o_rows[n, c] = _as_bf16(ot[s % 2, n, c * 64:(c + 1) * 64, :]).T

        def step(i):
            for lane in range(4):
                tile, c = divmod(4 * i + lane, NC)
                n, m = divmod(tile, NC)
                part = _dot(o_rows[n, c], wo_tile(c, m))
                pacer.issued(part, lane)
                acc[tile] = part if c == 0 else acc[tile] + part

        def store(part):
            n = min(part, NQ - 1)
            for m in range(NC) if part < NQ - 1 else ((0, 1, 2), (3, 4))[part - n]:
                seg = s + zero if m == 0 else s
                outb[seg, n * T:(n + 1) * T, m * T:(m + 1) * T] = acc[n * NC + m].astype(bf16)

        return transpose, step, store

    def new_pacer():
        return _Pacer(gate[0:8, :] > 2.0)

    def pair(s, p, plan, pacer, mix=None):
        memory = "Ra" in plan
        if mix is not None:
            first, count, cycles = mix
            pacer.attach(conv_mix(first, count, pacer.never), count * 96 / cycles)
        steps = {"a": attend(s, 2 * p, 0, pacer, memory),
                 "b": attend(s, 2 * p + 1, 1, pacer, memory)}
        steps["a"]["P"] = project(s, 2 * p + 1, 1, pacer)
        next_s, next_g = s + (p + 1) // 4, (2 * p + 2) % NG
        steps["b"]["P"] = project(next_s, next_g, 0, pacer)
        steps["a"]["U"] = lambda _: update(s, 2 * p + 1, pacer)
        steps["b"]["U"] = lambda _: update(next_s, next_g, pacer)
        steps["a"]["O"] = out_project(s - 1, p, pacer)
        steps["x"] = {
            "T": transpose_qkv,
            "K": repack_tables,
            "W": wait,
            "C": lambda _: outb_copy(s - 1, p).start(),
        }
        if "Jx" in plan:
            zero = pacer.never.astype(i32)[0, 0]
            steps["x"]["I"], steps["x"]["J"], steps["x"]["A"] = conv_inverse(pacer, zero)
            steps["x"]["L"], steps["x"]["E"], steps["x"]["G"] = out_project_last(pacer, zero)
        steps["x"]["F"] = lambda n: outb_copy(s, n).start()
        for item in plan:
            steps[item[1]][item[0]](int(item[2:] or 0))
        assert pacer.side is None

    def memory_pair(s, p):
        first = ((s - 1) * 4 + p) * MIX_PER_ITER
        pair(s, p, PLAN1, new_pacer(), (first, MIX_PER_ITER, MIX_CYCLES))

    wait(0)
    start(3, 4)
    for part in range(3):
        transpose_qkv(part)
    wait(1)
    start(4, len(loads))
    setup_gate()
    step = project(0, 0, 0, _Pacer(None))
    for i in range(NC):
        step(i)
    pacer = new_pacer()
    pair(0, 0, PLAN_FIRST, pacer)
    for p in range(1, 4):
        plan = ["Pa0"] + [item for item in PLAN0 if item != "Pa0"]
        if p == 1:
            plan.insert(plan.index("Qa5") + 1, "Wx4")
        pair(0, p, plan, pacer)

    wait(5)
    update(1, 0, _Pacer(None))
    for c in range(NC):
        conv_forward(c)
        transpose_wo(c)
    wait(6)

    @pl.loop(0, 11)
    def _(i):
        memory_pair(1 + i // 4, i % 4)

    wait(7)
    pair(NSEG - 1, 3, PLAN_LAST, new_pacer())

    outb_copy(NSEG - 1, NQ - 1).start()
    for k in range(NC * APARTS):
        outa_copy(k).wait()
    for s in range(NSEG):
        for n in range(NQ):
            outb_copy(s, n).wait()


@jax.jit
def pallas_concat_heads__ssm_conv_h3__memory_aug_infini_attn__prompt_kernel(
    A_q: jax.Array,
    A_k: jax.Array,
    A_v: jax.Array,
    A_shift_k: jax.Array,
    A_ssm_k: jax.Array,
    A_ssm_D: jax.Array,
    B_x: jax.Array,
    B_wq: jax.Array,
    B_wk: jax.Array,
    B_wv: jax.Array,
    B_wo: jax.Array,
    B_beta: jax.Array,
):
    hbm = pl.BlockSpec(memory_space=pl.ANY)
    scratch = [
        pltpu.VMEM((4, D), bf16),
        pltpu.VMEM((NC, T), bf16),
        pltpu.VMEM((H,), bf16),
        pltpu.VMEM((2, 2 * T, T), bf16),
        pltpu.VMEM((4, T // 2, T), bf16),
        pltpu.VMEM((NC, S, T), bf16),
        pltpu.VMEM((4, NC, D, T), bf16),
        pltpu.VMEM((3, NC, D // 2, T), u32),
        pltpu.VMEM((NC, D // 2, T), u32),
        pltpu.VMEM((NC, S, T), bf16),
        pltpu.VMEM((NC, S, T), bf16),
        pltpu.VMEM((NC, S, T), bf16),
        pltpu.VMEM((D, S), bf16),
        pltpu.VMEM((NC * NFV, 2, 2, NB, 16, T), f32),
        pltpu.VMEM((NC * NFV // 2, NB, 4, 8, T), u32),
        pltpu.VMEM((NC, S, T), bf16),
        pltpu.VMEM((NSEG, L, D), bf16),
        pltpu.VMEM((2, T, T), u32),
        pltpu.VMEM((4, T // 4, T), u32),
        pltpu.VMEM((H, T), f32),
        pltpu.VMEM((2, T // 2, T), f32),
        pltpu.VMEM((2, NQ, 64, T), u32),
        pltpu.VMEM((2, NQ, 48, T), u32),
        pltpu.VMEM((2, NQ, GW // 2, T), u32),
        pltpu.VMEM((2, NQ, T // 2, T), u32),
        pltpu.VMEM((2, NQ, GW, T), f32),
        pltpu.VMEM((2, NG, NQ, GW // 2, T), u32),
        pltpu.VMEM((2, NG, NQ, GW, T), f32),
        pltpu.VMEM((2, NQ, D // 2, T), u32),
        pltpu.VMEM((NG, GW + 8, T), f32),
        pltpu.SemaphoreType.DMA((8,)),
        pltpu.SemaphoreType.DMA((1,)),
    ]
    return pl.pallas_call(
        _kernel,
        out_shape=jax.ShapeDtypeStruct((1, S, 2 * D), bf16),
        in_specs=[hbm] * 14,
        out_specs=hbm,
        scratch_shapes=scratch,
        compiler_params=pltpu.CompilerParams(vmem_limit_bytes=100 * 2**20),
    )(
        A_shift_k.T, A_ssm_D.reshape(NC, T), B_beta, _FWD, _INV,
        A_q, A_k, A_v, A_ssm_k, B_x, B_wq, B_wk, B_wv, B_wo,
    )
```

```python
import jax
import jax.numpy as jnp
import numpy as np
from jax import lax
from jax.experimental import pallas as pl
from jax.experimental.pallas import tpu as pltpu

f32, bf16, u32, i32 = jnp.float32, jnp.bfloat16, jnp.uint32, jnp.int32

S, D, H, DH = 2048, 640, 32, 20
NSEG, L = 4, 512
T = 128
NC = D // T
NB = S // (2 * T)
NQ = L // T
NG = 8
GW = 4 * DH
APARTS = 2
NFV = 16
LOG2E = 1.4426950408889634
NEG = -1e30
MIX_PER_ITER = 4

PLAN_FIRST = (
    "Wx2 Qa0 Da0 Tx3 Tx4 Tx5 Qa1 Qa2 Qa3 Pa0 Qa4 Pa1 Va0 Pa2 Va1 Qa5 Pa3 Qa6 Pa4 Da1 Va2 Qa7 Va3 "
    "Qa8 Qa9 Va4 Qb0 Va5 Qb1 Va6 Db0 Va7 Qb2 Wx3 Tx6 Tx7 Tx8 Va8 Qb3 Vb0 Va9 Qb4 Pb0 Tx9 Tx10 "
    "Tx11 Qb5 Vb1 Qb6 Vb2 Db1 Vb3 Qb7 Tx12 Tx13 Tx14 Pb1 Kx Pb2 Vb4 Qb8 Vb5 Qb9 Pb3 Pb4 Vb6 Vb7 "
    "Vb8 Vb9"
).split()
PLAN0 = (
    "Qa0 Da0 Pa0 Qa1 Pa1 Qa2 Qa3 Pa2 Pa3 Qa4 Va0 Va1 Qa5 Qa6 Pa4 Da1 Va2 Qa7 Va3 Qa8 Qa9 Va4 Qb0 "
    "Va5 Qb1 Va6 Db0 Va7 Qb2 Va8 Qb3 Va9 Qb4 Pb0 Qb5 Vb0 Vb1 Qb6 Vb2 Db1 Vb3 Qb7 Pb1 Pb2 Vb4 Qb8 "
    "Vb5 Qb9 Pb3 Pb4 Vb6 Vb7 Vb8 Vb9"
).split()
PLAN1 = (
    "Qa0 Pa0 Da0 Pa1 Qa1 Qa2 Qa3 Pa2 Pa3 Pa4 Oa0 Qa4 Qa5 Qa6 Va0 Va1 Qa7 Va2 Oa1 Da1 Va3 Qa8 Qb0 "
    "Oa2 Ua Oa3 Oa4 Qa9 Va4 Ra Va5 Qb1 Va6 Va7 Db0 Qb2 Qb3 Va8 Qb4 Pb0 Qb5 Va9 Pb1 Qb6 Vb0 Vb1 "
    "Db1 Vb2 Qb7 Vb3 Pb2 Qb8 Vb4 Vb5 Qb9 Pb3 Vb6 Cx Pb4 Rb Vb7 Vb8 Vb9 Ub"
).split()
PLAN_LAST = (
    "Qa0 Da0 Pa0 Pa1 Qa1 Qa2 Qa3 Pa2 Pa3 Pa4 Qa4 Ix0 Qa5 Ix1 Va0 Ix2 Va1 Qa6 Ix3 Oa0 Va2 Qa7 Ix4 "
    "Ax0 Da1 Va3 Oa1 Ix5 Oa2 Qa8 Ix6 Va4 Oa3 Ix7 Oa4 Va5 Qa9 Ix8 Ax1 Ra Ua Va6 Ix9 Cx Qb0 Ix10 "
    "Va7 Qb1 Ix11 Db0 Ix12 Ax2 Qb2 Va8 Ix13 Qb3 Ix14 Vb0 Va9 Ix15 Qb4 Ix16 Ax3 Qb5 Ix17 Vb1 Qb6 "
    "Ix18 Db1 Ix19 Vb2 Qb7 Ix20 Ax4 Vb3 Ix21 Qb8 Ix22 Vb4 Ix23 Vb5 Qb9 Ix24 Ax5 Ix25 Ix26 Vb6 "
    "Ix27 Rb Ix28 Ax6 Vb7 Ix29 Ix30 Vb8 Ix31 Ix32 Ax7 Vb9 Ix33 Lx3 Ix34 Lx2 Ix35 Ix36 Ax8 Lx1 "
    "Ix37 Ix38 Lx0 Ix39 Ex0 Jx Ax9 Ex1 Ex2 Ex3 Ex4 Ex5 Ex6 Gx0 Fx0 Ex7 Ex8 Ex9 Ex10 Ex11 Ex12 Gx1 "
    "Fx1 Ex13 Ex14 Ex15 Ex16 Ex17 Ex18 Gx2 Fx2 Ex19 Ex20 Ex21 Ex22 Gx3 Ex23 Ex24 Gx4"
).split()
ORDER = (3, 2, 1, 0)
LEAD = {False: (400, 56), True: (380, 32)}
WA, WP, WO, WM = 1.2, 1.0, 1.2, 1.6
MIX_CYCLES = (2 * (1152 * WA + 1200 * WP + 176 * WM) + 800 * WO) * 0.965

NN = (((1,), (0,)), ((), ()))
NT = (((1,), (1,)), ((), ()))


def _dft_tables():
    freq = np.concatenate([np.arange(0, T, 2), T - 1 - np.arange(0, T, 2)])

    def table(freq, n):
        theta = 2.0 * np.pi * (freq[:, None] + 0.5) * n[None, :] / (4 * T)
        parts = [f(theta).reshape(-1, 8, len(n)) for f in (np.cos, lambda t: -np.sin(t))]
        return np.stack(parts, axis=1).reshape(-1, len(n))

    fwd = np.stack([table(freq, 2 * np.arange(T) + r) for r in range(2)])
    inv = np.stack([table(freq[:T // 2], 4 * np.arange(T // 2) + r).T / (2 * T) for r in range(4)])
    return fwd.astype(np.float32).astype(bf16), inv.astype(np.float32).astype(bf16)


_FWD, _INV = _dft_tables()


def _as_bf16(words):
    return pltpu.bitcast(words, bf16)


def _as_words(x):
    return pltpu.bitcast(x.astype(bf16), u32)


def _even_rows(words):
    return pltpu.bitcast(words << 16, f32)


def _odd_rows(words):
    return pltpu.bitcast(words & np.uint32(0xFFFF0000), f32)


def _interleave(even, odd):
    even, odd = (pltpu.bitcast(x.astype(bf16).astype(f32), u32) for x in (even, odd))
    return (even >> 16) | odd


def _dot(a, b):
    return lax.dot_general(a, b, NN, preferred_element_type=f32)


def _dot_nt(a, b):
    return lax.dot_general(a, b, NT, preferred_element_type=f32)


def _phi(t):
    return jnp.maximum(t, 0.0) + jnp.exp(jnp.minimum(t, 0.0))


def _ds(start, size, align):
    if isinstance(start, int):
        return pl.ds(start, size)
    return pl.ds(pl.multiple_of(start, align), size)


class _Pacer:
    def __init__(self, never):
        self.never, self.side, self.rate = never, None, 0.0
        self.credit, self.clock, self.history = 0.0, 0.0, []

    def attach(self, side, rate):
        self.side, self.rate, self.credit = side, rate, 0.0
        next(side)

    def issued(self, result, lane, weight=0.0):
        rows = result.shape[0]
        self.history.append((self.clock, result))
        if lane == 3:
            self.clock += rows
        self.credit += self.rate * rows / 4 * weight
        count = int(self.credit)
        self.credit -= count
        for i in range(count):
            if self.side is not None:
                v = min(rows // 8 - 1, int(rows // 8 * (lane + (i + 0.5) / count) / 4))
                try:
                    self.side.send(result[8 * v:8 * v + 8])
                except StopIteration:
                    self.side = None

    def hold(self, value, lead):
        target = self.clock - lead
        if target < 0 or self.never is None:
            return value
        for start, result in reversed(self.history):
            if start <= target:
                v = min(result.shape[0] // 8 - 1, int(target - start) // 8)
                return jnp.where(self.never, result[8 * v:8 * v + 8], value)
        return value


def _kernel(
    shift_hbm, ssmd_hbm, beta_hbm, fwd_hbm, inv_hbm,
    q_hbm, k_hbm, v_hbm, ssm_hbm, x_hbm, wq_hbm, wk_hbm, wv_hbm, wo_hbm, out_hbm,
    shift_ref, ssmd_ref, beta_ref, fwd_ref, inv_ref,
    xs, wraw, wt, wot, qa, ka, va, ssk, spec_buf, yf, outa, outb,
    fwd, inv, gate, bias, qm, qd, pq, kk, vt, pk_keep, vt_keep, ot, mz, sem_in, sem_out,
):
    def w_copies(n, sem):
        return [
            pltpu.make_async_copy(src.at[:, pl.ds(n * T, T)], wraw.at[i, n], sem)
            for i, src in enumerate((wq_hbm, wk_hbm, wv_hbm))
        ]

    def x_copies(lo, hi, sem):
        rows = pl.ds(lo * L, (hi - lo) * L)
        return [
            pltpu.make_async_copy(x_hbm.at[0, rows, pl.ds(c * T, T)], xs.at[c, rows], sem)
            for c in range(NC)
        ]

    def column_tiles(src, dst, sem):
        return [
            pltpu.make_async_copy(src.at[0, :, pl.ds(c * T, T)], dst.at[c], sem)
            for c in range(NC)
        ]

    loads = [
        w_copies(0, sem_in.at[0]),
        x_copies(0, 1, sem_in.at[1])
        + [pltpu.make_async_copy(beta_hbm, beta_ref, sem_in.at[1])],
        w_copies(1, sem_in.at[2]),
        sum((w_copies(n, sem_in.at[3]) for n in range(2, NC)), [
            pltpu.make_async_copy(fwd_hbm, fwd_ref, sem_in.at[3]),
            pltpu.make_async_copy(inv_hbm, inv_ref, sem_in.at[3])]),
        x_copies(1, 2, sem_in.at[4]),
        [pltpu.make_async_copy(src, dst, sem_in.at[5]) for src, dst in (
            (shift_hbm, shift_ref), (ssmd_hbm, ssmd_ref),
            (ssm_hbm, ssk))]
        + [pltpu.make_async_copy(k_hbm.at[0], ka, sem_in.at[5]), pltpu.make_async_copy(v_hbm.at[0], va, sem_in.at[5])]
        + [pltpu.make_async_copy(wo_hbm.at[:, pl.ds(n * T, T)], wraw.at[3, n], sem_in.at[5])
           for n in range(NC)],
        x_copies(2, NSEG, sem_in.at[6]),
        column_tiles(q_hbm, qa, sem_in.at[7]),
    ]

    def start(lo, hi):
        for copies in loads[lo:hi]:
            for cp in copies:
                cp.start()

    start(0, 3)

    def wait(i):
        for cp in loads[i]:
            cp.wait()

    mz[...] = jnp.zeros(mz.shape, f32)
    row = lax.broadcasted_iota(i32, (T // 2, T), 0)
    col = lax.broadcasted_iota(i32, (T // 2, T), 1)
    bias[0] = jnp.where(row <= col, 0.0, NEG)
    bias[1] = jnp.where(row <= col % (T // 2), 0.0, NEG)

    def setup_gate():
        beta = jnp.concatenate(
            [beta_ref[...].astype(f32)[None, :], jnp.zeros((1, T - H), f32)], axis=1)
        gate[...] = jax.nn.sigmoid(jnp.broadcast_to(beta, (T, T)).T[:H])

    def transpose_qkv(part):
        n, i = divmod(part, 3)
        for c in range(NC):
            tile = wraw[i, n, c * T:(c + 1) * T, :]
            wt[i, c, n * T // 2:(n + 1) * T // 2, :] = pltpu.bitcast(tile.T, u32)

    def repack_tables(_):
        for i in range(2):
            fwd[i] = pltpu.bitcast(fwd_ref[i], u32)
        for i in range(4):
            inv[i] = pltpu.bitcast(inv_ref[i], u32)

    def transpose_wo(n):
        for c in range(NC):
            wot[c, n * T // 2:(n + 1) * T // 2, :] = pltpu.bitcast(wo_tile(c, n).T, u32)

    sub = lax.broadcasted_iota(i32, (8, T), 0)
    low = sub < 4
    left = lax.broadcasted_iota(i32, (8, T), 1) < T // 2

    def project(s, g, slot, pacer):
        rows = _ds(g * (GW // 2), GW // 2, 8)
        acc = [None] * NQ

        def store(n):
            q_t, k_t, v_t = acc[n][:GW], acc[n][GW:2 * GW], acc[n][2 * GW:]
            k_pad = jnp.concatenate([k_t.astype(bf16), jnp.zeros((T - GW, T), bf16)], axis=0)
            kk[slot, n] = pltpu.bitcast(k_pad.T, u32)
            qs = q_t * (DH ** -0.5 * LOG2E)
            r = [qs[8 * i:8 * i + 8] for i in range(10)]
            zero = jnp.zeros((8, T), f32)
            heads = [
                r[0], r[1], jnp.where(low, r[2], 0.0), zero,
                jnp.where(low, 0.0, r[2]), r[3], r[4], zero,
                zero, r[5], r[6], jnp.where(low, r[7], 0.0),
                zero, jnp.where(low, 0.0, r[7]), r[8], r[9],
            ]
            qm[slot, n] = _as_words(jnp.concatenate(heads, axis=0))
            e = {i: jnp.where(left, pltpu.roll(r[i], 64, 1), 0.0) for i in (0, 1, 2, 5, 6, 7)}
            o = {i: jnp.where(left, 0.0, r[i]) for i in (2, 3, 4, 7, 8, 9)}
            pairs = [
                e[0], e[1], jnp.where(low, e[2], o[2]), o[3], o[4], zero,
                zero, e[5], e[6], jnp.where(low, e[7], o[7]), o[8], o[9],
            ]
            qd[slot, n] = _as_words(jnp.concatenate(pairs, axis=0))
            pq[slot, n] = _as_words(_phi(q_t))
            pk_keep[s % 2, g, n] = _as_words(_phi(k_t))
            vt[slot, n] = v_t
            vt_keep[s % 2, g, n] = v_t

        def step(i):
            for lane in range(4):
                n, c = divmod(4 * i + lane, NC)
                w = _as_bf16(jnp.concatenate([wt[m, c, rows, :] for m in range(3)], axis=0))
                part = _dot_nt(w, xs[c, _ds(s * L + n * T, T, T), :])
                pacer.issued(part, lane, WP)
                acc[n] = part if c == 0 else acc[n] + part
                if c == NC - 1:
                    store(n)

        return step

    def masked_dot(key_words, window, first):
        end = first + window.shape[0]
        parts = [window, jnp.zeros((T - end, T), bf16)]
        if first:
            parts.insert(0, jnp.zeros((first, T), bf16))
        return _dot(_as_bf16(key_words), jnp.concatenate(parts, axis=0))

    def update(s, g, pacer):
        state = mz[g]
        for kt in range(NQ):
            v_one = jnp.concatenate(
                [vt_keep[(s + 1) % 2, g, kt], jnp.ones((8, T), f32)], axis=0)
            pk_t = jnp.concatenate(
                [_as_bf16(pk_keep[(s + 1) % 2, g, kt]), jnp.zeros((T - GW, T), bf16)], axis=0)
            part = _dot_nt(v_one, pk_t)
            pacer.issued(part, kt, WM)
            state = state + part
        mz[g] = state

    def attend(s, g, slot, pacer, memory):
        lead, stagger = LEAD[memory]
        tiles = [(qt, kt) for qt in ORDER for kt in range(qt + 1)]
        logits, run_max, col_max, acc, mem, done = {}, {}, {}, {}, {}, []
        corner, corner_max, corner_p = {}, {}, {}
        gates = [jnp.broadcast_to(gate[pl.ds(4 * g + j, 1), :], (8, T)) for j in range(4)]
        low_pair = sub % 4 < 2
        rest_rows = 1.0 - jnp.where(low, jnp.where(low_pair, gates[1], gates[3]),
                                    jnp.where(low_pair, gates[0], gates[2]))

        def read(_):
            def head_of(i):
                return (i >= DH).astype(i32) + (i >= 2 * DH).astype(i32) + (i >= 3 * DH).astype(i32)

            state = mz[g]
            row_m = lax.broadcasted_iota(i32, (GW, T), 0)
            col_m = lax.broadcasted_iota(i32, (GW, T), 1)
            weights = jnp.where(head_of(row_m) == head_of(col_m), state[:GW], 0.0)
            lane_head = head_of(lax.broadcasted_iota(i32, (8, T), 1))
            pair_of = sub // 2
            z_rows = jnp.where(lane_head == pair_of, state[GW:], 0.0)
            mem_w = jnp.concatenate([weights, z_rows], axis=0)
            g_rows = jnp.where(low, jnp.where(sub < 2, gates[0], gates[1]),
                               jnp.where(sub < 6, gates[2], gates[3]))
            for qt in range(NQ):
                res = _dot(mem_w, jnp.concatenate(
                    [_as_bf16(pq[slot, qt]), jnp.zeros((T - GW, T), bf16)], axis=0))
                pacer.issued(res, qt, WM)
                coef = g_rows / (res[GW:] + 1e-6)
                c0, c1, c2, c3 = (
                    jnp.broadcast_to(coef[2 * j:2 * j + 1], (8, T)) for j in range(4))
                cm = [c0, c0, jnp.where(low, c0, c1), c1, c1,
                      c2, c2, jnp.where(low, c2, c3), c3, c3]
                mem[qt] = [res[8 * i:8 * i + 8] * cm[i] for i in range(10)]
            finish()

        def corners(i):
            for lane in range(4):
                qt, pr = ORDER[2 * i + lane // 2], lane % 2
                window = _as_bf16(qd[slot, qt, 24 * pr:24 * pr + 24, :])
                sc = masked_dot(kk[slot, qt, T // 4:, :], window, 32 * pr)
                pacer.issued(sc, lane, WA)
                corner[qt, pr] = sc + bias[1]
                corner_max[qt, pr] = jnp.max(corner[qt, pr].reshape(8, 8, T), axis=0)

        def scores(t):
            qt, kt = tiles[t]
            for j in range(4):
                window = _as_bf16(qm[slot, qt, 16 * j:16 * j + 16, :])
                sc = masked_dot(
                    kk[slot, kt] if kt < qt else kk[slot, kt, :T // 4, :], window, 16 * j)
                pacer.issued(sc, j, WA)
                if kt == qt:
                    sc = sc + bias[0]
                m8 = jnp.max(sc.reshape(-1, 8, T), axis=0)
                run_max[qt, j] = m8 if kt == 0 else jnp.maximum(run_max[qt, j], m8)
                if kt == qt:
                    extra = corner_max[qt, j // 2]
                    if j % 2 == 0:
                        extra = pltpu.roll(extra, T // 2, 1)
                    top = jnp.maximum(run_max[qt, j], jnp.where(left, NEG, extra))
                    col_max[qt, j] = jnp.broadcast_to(
                        jnp.max(top, axis=0, keepdims=True), (8, T))
                logits[t, j] = sc
            if kt == qt:
                for pr in range(2):
                    top = jnp.where(left, pltpu.roll(col_max[qt, 2 * pr], T // 2, 1),
                                    col_max[qt, 2 * pr + 1])
                    words = _as_words(jnp.exp2(
                        corner[qt, pr].reshape(8, 8, T) - top[None]).reshape(T // 2, T))
                    for j, shifted in enumerate((pltpu.roll(words, T // 2, 1), words)):
                        corner_p[qt, 2 * pr + j] = _as_bf16(jnp.where(
                            left[None], jnp.uint32(0), shifted.reshape(4, 8, T)).reshape(32, T))

        def values(t):
            qt, kt = tiles[t]
            tops = [pacer.hold(col_max[qt, j], lead - stagger * j) for j in range(4)]
            for j in range(4):
                p = jnp.exp2(logits[t, j].reshape(-1, 8, T) - tops[j][None])
                p = p.reshape(-1, T).astype(bf16)
                if kt == qt:
                    p = jnp.concatenate([p, corner_p[qt, j]], axis=0)
                first = (0, 16, 40, 56)[j]
                v = [vt[slot, kt, first + 8 * i:first + 8 * i + 8, :] for i in range(3)]
                if j % 2 == 0:
                    v[2] = jnp.where(low, v[2], 1.0)
                else:
                    v[0] = jnp.where(low, 1.0, v[0])
                part = _dot(jnp.concatenate(v, axis=0), p)
                pacer.issued(part, j)
                acc[qt, j] = part if kt == 0 else acc[qt, j] + part
            if kt == qt:
                done.append(qt)
                finish()

        def finish():
            while done and (not memory or done[0] in mem):
                qt = done.pop(0)
                w = [[acc[qt, j][8 * i:8 * i + 8] for i in range(3)] for j in range(4)]
                sums = jnp.where(
                    low_pair, jnp.where(low, w[1][0], w[0][2]),
                    pltpu.roll(jnp.where(low, w[3][0], w[2][2]), 2, 0))
                coef = rest_rows / sums
                c0, c1, c2, c3 = (
                    jnp.broadcast_to(coef[r:r + 1], (8, T)) for r in (4, 0, 6, 2))
                o = [w[0][0] * c0, w[0][1] * c0,
                     jnp.where(low, w[0][2] * c0, w[1][0] * c1), w[1][1] * c1, w[1][2] * c1,
                     w[2][0] * c2, w[2][1] * c2,
                     jnp.where(low, w[2][2] * c2, w[3][0] * c3), w[3][1] * c3, w[3][2] * c3]
                if memory:
                    o = [mem[qt][i] + o[i] for i in range(10)]
                ot[s % 2, qt, _ds(g * (GW // 2), GW // 2, 8), :] = _as_words(
                    jnp.concatenate(o, axis=0))

        return {"D": corners, "Q": scores, "V": values, "R": read}

    def wo_tile(c, m):
        return wraw[3, m, c * T:(c + 1) * T, :]

    def out_project(s, n, pacer):
        acc, done = [None] * 4, []

        def step(i):
            for lane in range(4):
                m, c = divmod(4 * i + lane, NC)
                part = _dot(_as_bf16(wot[c, 80 * m:80 * (m + 1), :]),
                            _as_bf16(ot[s % 2, n, c * 64:(c + 1) * 64, :]))
                pacer.issued(part, lane, WO)
                acc[m] = part if c == 0 else acc[m] + part
                if c == NC - 1:
                    acc[m] = acc[m].astype(bf16)
                    while T * (len(done) + 1) <= 160 * (m + 1):
                        i0 = T * len(done)
                        pieces = [acc[k][max(i0 - 160 * k, 0):min(i0 + T - 160 * k, 160)]
                                  for k in range(i0 // 160, (i0 + T - 1) // 160 + 1)]
                        tile = jnp.concatenate(pieces, axis=0).T
                        outb[s, _ds(n * T, T, T), i0:i0 + T] = tile
                        done.append(True)

        return step

    def outb_copy(s, n):
        return pltpu.make_async_copy(
            outb.at[s, _ds(n * T, T, T)],
            out_hbm.at[0, _ds(s * L + n * T, T, T), pl.ds(D, D)], sem_out.at[0])

    def conv_forward(c):
        cols = slice(c * T, (c + 1) * T)
        taps = shift_ref[:, cols].astype(f32)
        taps = [jnp.broadcast_to(taps[j:j + 1], (T, T)) for j in range(4)]
        skip = ssmd_ref[...].astype(f32)[c:c + 1]
        slices = pl.ds(c * NFV, NFV)

        def transform(even, odd):
            e, o = (_dot(_as_bf16(fwd[i]), x) for i, x in enumerate((even, odd)))
            return [x.reshape(NFV, 2, 8, T) for x in (e + o, e - o)]

        tail = jnp.zeros((8, T), u32)
        prev = None
        for b in range(NB):
            k0 = pltpu.bitcast(ka[2 * b * T:2 * (b + 1) * T, cols], u32)
            ext = jnp.concatenate([tail, k0], axis=0)
            tail = k0[T - 8:]
            k1, k2 = ext[7:7 + T], ext[6:6 + T]
            e0, o0, e1, o1, o2 = (
                _even_rows(k0), _odd_rows(k0), _even_rows(k1), _odd_rows(k1), _odd_rows(k2))
            v0 = pltpu.bitcast(va[2 * b * T:2 * (b + 1) * T, cols], u32)
            sig = transform(
                (e0 * taps[0] + o1 * taps[1] + e1 * taps[2] + o2 * taps[3]) * _even_rows(v0),
                (o0 * taps[0] + e0 * taps[1] + o1 * taps[2] + e1 * taps[3]) * _odd_rows(v0))
            taps_t = jnp.concatenate([
                pltpu.bitcast(ssk[cols, (2 * b + i) * T:(2 * b + i + 1) * T].T, u32)
                for i in range(2)], axis=0)
            filt = transform(_even_rows(taps_t), _odd_rows(taps_t))
            for sign in range(2):
                spec_buf[slices, 0, sign, b] = sig[sign].reshape(NFV, 16, T)
                re, im = filt[sign][:, 0], filt[sign][:, 1]
                if prev is None:
                    re = re + skip[None]
                else:
                    half = NFV // 2
                    pre, pim = prev[sign][:, 0], prev[sign][:, 1]
                    re = jnp.concatenate([re[:half] - pim[:half], re[half:] + pim[half:]], axis=0)
                    im = jnp.concatenate([im[:half] + pre[:half], im[half:] - pre[half:]], axis=0)
                spec_buf[slices, 1, sign, b, 0:8, :] = re
                spec_buf[slices, 1, sign, b, 8:16, :] = im
            prev = filt

    def conv_mix(first, count, never, blk=4):
        half = NFV // 2
        for item in range(count):
            idx = jnp.minimum(first + item, NC * half - 1)
            base = idx // half * NFV + idx % half

            def products(fv, sign, a0):
                def load(which, b):
                    return (spec_buf[fv, which, sign, b, 0:8, :],
                            spec_buf[fv, which, sign, b, 8:16, :])

                acc, kcache = [None] * blk, {}
                for b in range(a0 + blk):
                    token = yield
                    ur, ui = load(0, b)
                    ur = jnp.where(never, token, ur)
                    us = ur + ui
                    for a in range(max(a0, b), a0 + blk):
                        if a - b not in kcache:
                            kr, ki = load(1, a - b)
                            kcache[a - b] = (kr, ki - kr, kr + ki)
                        k1, k2, k3 = kcache[a - b]
                        terms = (us * k1, ur * k2, ui * k3)
                        old = acc[a - a0]
                        acc[a - a0] = terms if old is None else tuple(
                            o + t for o, t in zip(old, terms))
                return [(p1 - p3, p1 + p2) for p1, p2, p3 in acc]

            for a0 in range(0, NB, blk):
                parity = []
                for fv in (base, base + half):
                    plus = yield from products(fv, 0, a0)
                    minus = yield from products(fv, 1, a0)
                    parity.append((
                        [(pr + mr, pi + mi) for (pr, pi), (mr, mi) in zip(plus, minus)],
                        [(pr - mr, pi - mi) for (pr, pi), (mr, mi) in zip(plus, minus)]))
                for i in range(blk):
                    (ar, ai), (br, bi) = parity[0][0][i], parity[1][0][i]
                    (cr, ci), (dr, di) = parity[0][1][i], parity[1][1][i]
                    folded = ((ar + br, ai - bi), (cr - di, ci - dr),
                              (ar - br, ai + bi), (cr + di, ci + dr))
                    for r in range(4):
                        yf[idx, a0 + i, r] = _as_words(jnp.concatenate(folded[r], axis=0))

    def outa_copy(k):
        c, part = divmod(k, APARTS)
        rows = pl.ds(part * (S // APARTS), S // APARTS)
        return pltpu.make_async_copy(
            outa.at[c, rows], out_hbm.at[0, rows, pl.ds(c * T, T)], sem_out.at[0])

    def conv_inverse(pacer, zero):
        pending, pin, hold = [], [], []

        def send(c):
            outa_copy(c).start()
            pin.append(True)

        def flush(_):
            while pending:
                c, a, y = pending.pop(0)
                tile = c + zero if pin else c
                rows = slice(2 * a * T, 2 * (a + 1) * T)
                w01, w23 = _interleave(y[0], y[1]), _interleave(y[2], y[3])
                words = jnp.concatenate([
                    jnp.where(sub % 2 == 0, *(
                        jnp.take_along_axis(w[8 * v:8 * v + 8], sub // 2 + 4 * h, axis=0)
                        for w in (w01, w23)))
                    for v in range(8) for h in range(2)], axis=0)
                conv = _as_bf16(words).astype(f32)
                outa[tile, rows, :] = (qa[c, rows, :].astype(f32) * conv).astype(bf16)
                if pin:
                    hold.append(pltpu.bitcast(outa[tile, rows.start:rows.start + 16, :], u32))
                    pin.clear()

        def step(i):
            c, a = divmod(i, NB)
            res = []
            for r in range(4):
                words = yf[pl.ds(c * NFV // 2, NFV // 2), a, r].reshape(T // 2, T)
                if hold:
                    words = jnp.concatenate(
                        [jnp.where(pacer.never, hold.pop(), words[:8]), words[8:]], axis=0)
                res.append(_dot(
                    _as_bf16(inv[r]), _as_bf16(words)))
                pacer.issued(res[-1], r)
            flush(0)
            pending.append((c, a, res))

        return step, flush, send

    def out_project_last(pacer, zero):
        s = NSEG - 1
        o_rows, acc = {}, {}

        def transpose(n):
            for c in range(NC):
                o_rows[n, c] = _as_bf16(ot[s % 2, n, c * 64:(c + 1) * 64, :]).T

        def step(i):
            for lane in range(4):
                tile, c = divmod(4 * i + lane, NC)
                n, m = divmod(tile, NC)
                part = _dot(o_rows[n, c], wo_tile(c, m))
                pacer.issued(part, lane)
                acc[tile] = part if c == 0 else acc[tile] + part

        def store(part):
            n = min(part, NQ - 1)
            for m in range(NC) if part < NQ - 1 else ((0, 1, 2), (3, 4))[part - n]:
                seg = s + zero if m == 0 else s
                outb[seg, n * T:(n + 1) * T, m * T:(m + 1) * T] = acc[n * NC + m].astype(bf16)

        return transpose, step, store

    def new_pacer():
        return _Pacer(gate[0:8, :] > 2.0)

    def pair(s, p, plan, pacer, mix=None):
        memory = "Ra" in plan
        if mix is not None:
            first, count, cycles = mix
            pacer.attach(conv_mix(first, count, pacer.never), count * 96 / cycles)
        steps = {"a": attend(s, 2 * p, 0, pacer, memory),
                 "b": attend(s, 2 * p + 1, 1, pacer, memory)}
        steps["a"]["P"] = project(s, 2 * p + 1, 1, pacer)
        next_s, next_g = s + (p + 1) // 4, (2 * p + 2) % NG
        steps["b"]["P"] = project(next_s, next_g, 0, pacer)
        steps["a"]["U"] = lambda _: update(s, 2 * p + 1, pacer)
        steps["b"]["U"] = lambda _: update(next_s, next_g, pacer)
        steps["a"]["O"] = out_project(s - 1, p, pacer)
        steps["x"] = {
            "T": transpose_qkv,
            "K": repack_tables,
            "W": wait,
            "C": lambda _: outb_copy(s - 1, p).start(),
        }
        if "Jx" in plan:
            zero = pacer.never.astype(i32)[0, 0]
            steps["x"]["I"], steps["x"]["J"], steps["x"]["A"] = conv_inverse(pacer, zero)
            steps["x"]["L"], steps["x"]["E"], steps["x"]["G"] = out_project_last(pacer, zero)
        steps["x"]["F"] = lambda n: outb_copy(s, n).start()
        for item in plan:
            steps[item[1]][item[0]](int(item[2:] or 0))
        assert pacer.side is None

    def memory_pair(s, p):
        first = ((s - 1) * 4 + p) * MIX_PER_ITER
        pair(s, p, PLAN1, new_pacer(), (first, MIX_PER_ITER, MIX_CYCLES))

    wait(0)
    start(3, 4)
    for part in range(3):
        transpose_qkv(part)
    wait(1)
    start(4, len(loads))
    setup_gate()
    step = project(0, 0, 0, _Pacer(None))
    for i in range(NC):
        step(i)
    pacer = new_pacer()
    pair(0, 0, PLAN_FIRST, pacer)
    for p in range(1, 4):
        plan = ["Pa0"] + [item for item in PLAN0 if item != "Pa0"]
        if p == 1:
            plan.insert(plan.index("Qa5") + 1, "Wx4")
        pair(0, p, plan, pacer)

    wait(5)
    update(1, 0, _Pacer(None))
    for c in range(NC):
        conv_forward(c)
        transpose_wo(c)
    wait(6)

    @pl.loop(0, 11)
    def _(i):
        memory_pair(1 + i // 4, i % 4)

    wait(7)
    pair(NSEG - 1, 3, PLAN_LAST, new_pacer())

    outb_copy(NSEG - 1, NQ - 1).start()
    for k in range(NC * APARTS):
        outa_copy(k).wait()
    for s in range(NSEG):
        for n in range(NQ):
            outb_copy(s, n).wait()


@jax.jit
def pallas_concat_heads__ssm_conv_h3__memory_aug_infini_attn__prompt_kernel(
    A_q: jax.Array,
    A_k: jax.Array,
    A_v: jax.Array,
    A_shift_k: jax.Array,
    A_ssm_k: jax.Array,
    A_ssm_D: jax.Array,
    B_x: jax.Array,
    B_wq: jax.Array,
    B_wk: jax.Array,
    B_wv: jax.Array,
    B_wo: jax.Array,
    B_beta: jax.Array,
):
    hbm = pl.BlockSpec(memory_space=pl.ANY)
    scratch = [
        pltpu.VMEM((4, D), bf16),
        pltpu.VMEM((NC, T), bf16),
        pltpu.VMEM((H,), bf16),
        pltpu.VMEM((2, 2 * T, T), bf16),
        pltpu.VMEM((4, T // 2, T), bf16),
        pltpu.VMEM((NC, S, T), bf16),
        pltpu.VMEM((4, NC, D, T), bf16),
        pltpu.VMEM((3, NC, D // 2, T), u32),
        pltpu.VMEM((NC, D // 2, T), u32),
        pltpu.VMEM((NC, S, T), bf16),
        pltpu.VMEM((S, D), bf16),
        pltpu.VMEM((S, D), bf16),
        pltpu.VMEM((D, S), bf16),
        pltpu.VMEM((NC * NFV, 2, 2, NB, 16, T), f32),
        pltpu.VMEM((NC * NFV // 2, NB, 4, 8, T), u32),
        pltpu.VMEM((NC, S, T), bf16),
        pltpu.VMEM((NSEG, L, D), bf16),
        pltpu.VMEM((2, T, T), u32),
        pltpu.VMEM((4, T // 4, T), u32),
        pltpu.VMEM((H, T), f32),
        pltpu.VMEM((2, T // 2, T), f32),
        pltpu.VMEM((2, NQ, 64, T), u32),
        pltpu.VMEM((2, NQ, 48, T), u32),
        pltpu.VMEM((2, NQ, GW // 2, T), u32),
        pltpu.VMEM((2, NQ, T // 2, T), u32),
        pltpu.VMEM((2, NQ, GW, T), f32),
        pltpu.VMEM((2, NG, NQ, GW // 2, T), u32),
        pltpu.VMEM((2, NG, NQ, GW, T), f32),
        pltpu.VMEM((2, NQ, D // 2, T), u32),
        pltpu.VMEM((NG, GW + 8, T), f32),
        pltpu.SemaphoreType.DMA((8,)),
        pltpu.SemaphoreType.DMA((1,)),
    ]
    return pl.pallas_call(
        _kernel,
        out_shape=jax.ShapeDtypeStruct((1, S, 2 * D), bf16),
        in_specs=[hbm] * 14,
        out_specs=hbm,
        scratch_shapes=scratch,
        compiler_params=pltpu.CompilerParams(vmem_limit_bytes=100 * 2**20),
    )(
        A_shift_k.T, A_ssm_D.reshape(NC, T), B_beta, _FWD, _INV,
        A_q, A_k, A_v, A_ssm_k, B_x, B_wq, B_wk, B_wv, B_wo,
    )
```

```python
import jax
import jax.numpy as jnp
import numpy as np
from jax import lax
from jax.experimental import pallas as pl
from jax.experimental.pallas import tpu as pltpu

f32, bf16, u32, i32 = jnp.float32, jnp.bfloat16, jnp.uint32, jnp.int32

S, D, H, DH = 2048, 640, 32, 20
NSEG, L = 4, 512
T = 128
NC = D // T
NB = S // (2 * T)
NQ = L // T
NG = 8
GW = 4 * DH
APARTS = 2
NFV = 16
LOG2E = 1.4426950408889634
NEG = -1e30
MIX_PER_ITER = 4

PLAN_FIRST = (
    "Wx2 Qa0 Da0 Tx3 Tx4 Tx5 Qa1 Qa2 Qa3 Pa0 Qa4 Pa1 Va0 Pa2 Va1 Qa5 Pa3 Qa6 Pa4 Da1 Va2 Qa7 Va3 "
    "Qa8 Qa9 Va4 Qb0 Va5 Qb1 Va6 Db0 Va7 Qb2 Wx3 Tx6 Tx7 Tx8 Va8 Qb3 Vb0 Va9 Qb4 Pb0 Tx9 Tx10 "
    "Tx11 Qb5 Vb1 Qb6 Vb2 Db1 Vb3 Qb7 Tx12 Tx13 Tx14 Pb1 Kx Pb2 Vb4 Qb8 Vb5 Qb9 Pb3 Pb4 Vb6 Vb7 "
    "Vb8 Vb9"
).split()
PLAN0 = (
    "Qa0 Da0 Pa0 Qa1 Pa1 Qa2 Qa3 Pa2 Pa3 Qa4 Va0 Va1 Qa5 Qa6 Pa4 Da1 Va2 Qa7 Va3 Qa8 Qa9 Va4 Qb0 "
    "Va5 Qb1 Va6 Db0 Va7 Qb2 Va8 Qb3 Va9 Qb4 Pb0 Qb5 Vb0 Vb1 Qb6 Vb2 Db1 Vb3 Qb7 Pb1 Pb2 Vb4 Qb8 "
    "Vb5 Qb9 Pb3 Pb4 Vb6 Vb7 Vb8 Vb9"
).split()
PLAN1 = (
    "Qa0 Pa0 Da0 Pa1 Qa1 Qa2 Qa3 Pa2 Pa3 Pa4 Oa0 Qa4 Qa5 Qa6 Va0 Va1 Qa7 Va2 Oa1 Da1 Va3 Qa8 Qb0 "
    "Oa2 Ua Oa3 Oa4 Qa9 Va4 Ra Va5 Qb1 Va6 Va7 Db0 Qb2 Qb3 Va8 Qb4 Pb0 Qb5 Va9 Pb1 Qb6 Vb0 Vb1 "
    "Db1 Vb2 Qb7 Vb3 Pb2 Qb8 Vb4 Vb5 Qb9 Pb3 Vb6 Cx Pb4 Rb Vb7 Vb8 Vb9 Ub"
).split()
PLAN_LAST = (
    "Qa0 Da0 Pa0 Pa1 Qa1 Qa2 Qa3 Pa2 Pa3 Pa4 Qa4 Ix0 Qa5 Ix1 Va0 Ix2 Va1 Qa6 Ix3 Oa0 Va2 Qa7 Ix4 "
    "Ax0 Da1 Va3 Oa1 Ix5 Oa2 Qa8 Ix6 Va4 Oa3 Ix7 Oa4 Va5 Qa9 Ix8 Ax1 Ra Ua Va6 Ix9 Cx Qb0 Ix10 "
    "Va7 Qb1 Ix11 Db0 Ix12 Ax2 Qb2 Va8 Ix13 Qb3 Ix14 Vb0 Va9 Ix15 Qb4 Ix16 Ax3 Qb5 Ix17 Vb1 Qb6 "
    "Ix18 Db1 Ix19 Vb2 Qb7 Ix20 Ax4 Vb3 Ix21 Qb8 Ix22 Vb4 Ix23 Vb5 Qb9 Ix24 Ax5 Ix25 Ix26 Vb6 "
    "Ix27 Rb Ix28 Ax6 Vb7 Ix29 Ix30 Vb8 Ix31 Ix32 Ax7 Vb9 Ix33 Lx3 Ix34 Lx2 Ix35 Ix36 Ax8 Lx1 "
    "Ix37 Ix38 Lx0 Ix39 Ex0 Jx Ax9 Ex1 Ex2 Ex3 Ex4 Ex5 Ex6 Gx0 Fx0 Ex7 Ex8 Ex9 Ex10 Ex11 Ex12 Gx1 "
    "Fx1 Ex13 Ex14 Ex15 Ex16 Ex17 Ex18 Gx2 Fx2 Ex19 Ex20 Ex21 Ex22 Gx3 Ex23 Ex24 Gx4"
).split()
ORDER = (3, 2, 1, 0)
LEAD = {False: (400, 56), True: (380, 32)}
WA, WP, WO, WM = 1.2, 1.0, 1.2, 1.6
MIX_CYCLES = (2 * (1152 * WA + 1200 * WP + 176 * WM) + 800 * WO) * 0.965

NN = (((1,), (0,)), ((), ()))
NT = (((1,), (1,)), ((), ()))


def _dft_tables():
    freq = np.concatenate([np.arange(0, T, 2), T - 1 - np.arange(0, T, 2)])

    def table(freq, n):
        theta = 2.0 * np.pi * (freq[:, None] + 0.5) * n[None, :] / (4 * T)
        parts = [f(theta).reshape(-1, 8, len(n)) for f in (np.cos, lambda t: -np.sin(t))]
        return np.stack(parts, axis=1).reshape(-1, len(n))

    fwd = np.stack([table(freq, 2 * np.arange(T) + r) for r in range(2)])
    inv = np.stack([table(freq[:T // 2], 4 * np.arange(T // 2) + r).T / (2 * T) for r in range(4)])
    return fwd.astype(np.float32).astype(bf16), inv.astype(np.float32).astype(bf16)


_FWD, _INV = _dft_tables()


def _as_bf16(words):
    return pltpu.bitcast(words, bf16)


def _as_words(x):
    return pltpu.bitcast(x.astype(bf16), u32)


def _even_rows(words):
    return pltpu.bitcast(words << 16, f32)


def _odd_rows(words):
    return pltpu.bitcast(words & np.uint32(0xFFFF0000), f32)


def _interleave(even, odd):
    even, odd = (pltpu.bitcast(x.astype(bf16).astype(f32), u32) for x in (even, odd))
    return (even >> 16) | odd


def _dot(a, b):
    return lax.dot_general(a, b, NN, preferred_element_type=f32)


def _dot_nt(a, b):
    return lax.dot_general(a, b, NT, preferred_element_type=f32)


def _phi(t):
    return jnp.maximum(t, 0.0) + jnp.exp(jnp.minimum(t, 0.0))


def _ds(start, size, align):
    if isinstance(start, int):
        return pl.ds(start, size)
    return pl.ds(pl.multiple_of(start, align), size)


class _Pacer:
    def __init__(self, never):
        self.never, self.side, self.rate = never, None, 0.0
        self.credit, self.clock, self.history = 0.0, 0.0, []

    def attach(self, side, rate):
        self.side, self.rate, self.credit = side, rate, 0.0
        next(side)

    def issued(self, result, lane, weight=0.0):
        rows = result.shape[0]
        self.history.append((self.clock, result))
        if lane == 3:
            self.clock += rows
        self.credit += self.rate * rows / 4 * weight
        count = int(self.credit)
        self.credit -= count
        for i in range(count):
            if self.side is not None:
                v = min(rows // 8 - 1, int(rows // 8 * (lane + (i + 0.5) / count) / 4))
                try:
                    self.side.send(result[8 * v:8 * v + 8])
                except StopIteration:
                    self.side = None

    def hold(self, value, lead):
        target = self.clock - lead
        if target < 0 or self.never is None:
            return value
        for start, result in reversed(self.history):
            if start <= target:
                v = min(result.shape[0] // 8 - 1, int(target - start) // 8)
                return jnp.where(self.never, result[8 * v:8 * v + 8], value)
        return value


def _kernel(
    shift_hbm, ssmd_hbm, beta_hbm, fwd_hbm, inv_hbm,
    q_hbm, k_hbm, v_hbm, ssm_hbm, x_hbm, wq_hbm, wk_hbm, wv_hbm, wo_hbm, out_hbm,
    shift_ref, ssmd_ref, beta_ref, fwd_ref, inv_ref,
    xs, wraw, wrest, wo_raw, wt, wot, qa, ka, va, ssk, spec_buf, yf, outa, outb,
    fwd, inv, gate, bias, qm, qd, pq, kk, vt, pk_keep, vt_keep, ot, mz, sem_in, sem_out,
):
    def w_copies(n, sem):
        return [
            pltpu.make_async_copy(src.at[:, pl.ds(n * T, T)], wraw.at[i, n], sem)
            for i, src in enumerate((wq_hbm, wk_hbm, wv_hbm))
        ]

    def x_copies(lo, hi, sem):
        rows = pl.ds(lo * L, (hi - lo) * L)
        return [
            pltpu.make_async_copy(x_hbm.at[0, rows, pl.ds(c * T, T)], xs.at[c, rows], sem)
            for c in range(NC)
        ]

    def column_tiles(src, dst, sem):
        return [
            pltpu.make_async_copy(src.at[0, :, pl.ds(c * T, T)], dst.at[c], sem)
            for c in range(NC)
        ]

    loads = [
        w_copies(0, sem_in.at[0]),
        x_copies(0, 1, sem_in.at[1])
        + [pltpu.make_async_copy(beta_hbm, beta_ref, sem_in.at[1])],
        w_copies(1, sem_in.at[2]),
        [pltpu.make_async_copy(fwd_hbm, fwd_ref, sem_in.at[3]),
         pltpu.make_async_copy(inv_hbm, inv_ref, sem_in.at[3])]
        + [pltpu.make_async_copy(src.at[:, pl.ds(2 * T, 3 * T)], wrest.at[i], sem_in.at[3])
           for i, src in enumerate((wq_hbm, wk_hbm, wv_hbm))],
        x_copies(1, 2, sem_in.at[4]),
        [pltpu.make_async_copy(src, dst, sem_in.at[5]) for src, dst in (
            (shift_hbm, shift_ref), (ssmd_hbm, ssmd_ref),
            (ssm_hbm, ssk))]
        + [pltpu.make_async_copy(k_hbm.at[0], ka, sem_in.at[5]), pltpu.make_async_copy(v_hbm.at[0], va, sem_in.at[5])]
        + [pltpu.make_async_copy(wo_hbm, wo_raw, sem_in.at[5])],
        x_copies(2, NSEG, sem_in.at[6]),
        column_tiles(q_hbm, qa, sem_in.at[7]),
    ]

    def start(lo, hi):
        for copies in loads[lo:hi]:
            for cp in copies:
                cp.start()

    start(0, 3)

    def wait(i):
        for cp in loads[i]:
            cp.wait()

    mz[...] = jnp.zeros(mz.shape, f32)
    row = lax.broadcasted_iota(i32, (T // 2, T), 0)
    col = lax.broadcasted_iota(i32, (T // 2, T), 1)
    bias[0] = jnp.where(row <= col, 0.0, NEG)
    bias[1] = jnp.where(row <= col % (T // 2), 0.0, NEG)

    def setup_gate():
        beta = jnp.concatenate(
            [beta_ref[...].astype(f32)[None, :], jnp.zeros((1, T - H), f32)], axis=1)
        gate[...] = jax.nn.sigmoid(jnp.broadcast_to(beta, (T, T)).T[:H])

    def transpose_qkv(part):
        n, i = divmod(part, 3)
        for c in range(NC):
            tile = (wraw[i, n, c * T:(c + 1) * T, :] if n < 2
                    else wrest[i, c * T:(c + 1) * T, (n - 2) * T:(n - 1) * T])
            wt[i, c, n * T // 2:(n + 1) * T // 2, :] = pltpu.bitcast(tile.T, u32)

    def repack_tables(_):
        for i in range(2):
            fwd[i] = pltpu.bitcast(fwd_ref[i], u32)
        for i in range(4):
            inv[i] = pltpu.bitcast(inv_ref[i], u32)

    def transpose_wo(n):
        for c in range(NC):
            wot[c, n * T // 2:(n + 1) * T // 2, :] = pltpu.bitcast(wo_tile(c, n).T, u32)

    sub = lax.broadcasted_iota(i32, (8, T), 0)
    low = sub < 4
    left = lax.broadcasted_iota(i32, (8, T), 1) < T // 2

    def project(s, g, slot, pacer):
        rows = _ds(g * (GW // 2), GW // 2, 8)
        acc = [None] * NQ

        def store(n):
            q_t, k_t, v_t = acc[n][:GW], acc[n][GW:2 * GW], acc[n][2 * GW:]
            k_pad = jnp.concatenate([k_t.astype(bf16), jnp.zeros((T - GW, T), bf16)], axis=0)
            kk[slot, n] = pltpu.bitcast(k_pad.T, u32)
            qs = q_t * (DH ** -0.5 * LOG2E)
            r = [qs[8 * i:8 * i + 8] for i in range(10)]
            zero = jnp.zeros((8, T), f32)
            heads = [
                r[0], r[1], jnp.where(low, r[2], 0.0), zero,
                jnp.where(low, 0.0, r[2]), r[3], r[4], zero,
                zero, r[5], r[6], jnp.where(low, r[7], 0.0),
                zero, jnp.where(low, 0.0, r[7]), r[8], r[9],
            ]
            qm[slot, n] = _as_words(jnp.concatenate(heads, axis=0))
            e = {i: jnp.where(left, pltpu.roll(r[i], 64, 1), 0.0) for i in (0, 1, 2, 5, 6, 7)}
            o = {i: jnp.where(left, 0.0, r[i]) for i in (2, 3, 4, 7, 8, 9)}
            pairs = [
                e[0], e[1], jnp.where(low, e[2], o[2]), o[3], o[4], zero,
                zero, e[5], e[6], jnp.where(low, e[7], o[7]), o[8], o[9],
            ]
            qd[slot, n] = _as_words(jnp.concatenate(pairs, axis=0))
            pq[slot, n] = _as_words(_phi(q_t))
            pk_keep[s % 2, g, n] = _as_words(_phi(k_t))
            vt[slot, n] = v_t
            vt_keep[s % 2, g, n] = v_t

        def step(i):
            for lane in range(4):
                n, c = divmod(4 * i + lane, NC)
                w = _as_bf16(jnp.concatenate([wt[m, c, rows, :] for m in range(3)], axis=0))
                part = _dot_nt(w, xs[c, _ds(s * L + n * T, T, T), :])
                pacer.issued(part, lane, WP)
                acc[n] = part if c == 0 else acc[n] + part
                if c == NC - 1:
                    store(n)

        return step

    def masked_dot(key_words, window, first):
        end = first + window.shape[0]
        parts = [window, jnp.zeros((T - end, T), bf16)]
        if first:
            parts.insert(0, jnp.zeros((first, T), bf16))
        return _dot(_as_bf16(key_words), jnp.concatenate(parts, axis=0))

    def update(s, g, pacer):
        state = mz[g]
        for kt in range(NQ):
            v_one = jnp.concatenate(
                [vt_keep[(s + 1) % 2, g, kt], jnp.ones((8, T), f32)], axis=0)
            pk_t = jnp.concatenate(
                [_as_bf16(pk_keep[(s + 1) % 2, g, kt]), jnp.zeros((T - GW, T), bf16)], axis=0)
            part = _dot_nt(v_one, pk_t)
            pacer.issued(part, kt, WM)
            state = state + part
        mz[g] = state

    def attend(s, g, slot, pacer, memory):
        lead, stagger = LEAD[memory]
        tiles = [(qt, kt) for qt in ORDER for kt in range(qt + 1)]
        logits, run_max, col_max, acc, mem, done = {}, {}, {}, {}, {}, []
        corner, corner_max, corner_p = {}, {}, {}
        gates = [jnp.broadcast_to(gate[pl.ds(4 * g + j, 1), :], (8, T)) for j in range(4)]
        low_pair = sub % 4 < 2
        rest_rows = 1.0 - jnp.where(low, jnp.where(low_pair, gates[1], gates[3]),
                                    jnp.where(low_pair, gates[0], gates[2]))

        def read(_):
            def head_of(i):
                return (i >= DH).astype(i32) + (i >= 2 * DH).astype(i32) + (i >= 3 * DH).astype(i32)

            state = mz[g]
            row_m = lax.broadcasted_iota(i32, (GW, T), 0)
            col_m = lax.broadcasted_iota(i32, (GW, T), 1)
            weights = jnp.where(head_of(row_m) == head_of(col_m), state[:GW], 0.0)
            lane_head = head_of(lax.broadcasted_iota(i32, (8, T), 1))
            pair_of = sub // 2
            z_rows = jnp.where(lane_head == pair_of, state[GW:], 0.0)
            mem_w = jnp.concatenate([weights, z_rows], axis=0)
            g_rows = jnp.where(low, jnp.where(sub < 2, gates[0], gates[1]),
                               jnp.where(sub < 6, gates[2], gates[3]))
            for qt in range(NQ):
                res = _dot(mem_w, jnp.concatenate(
                    [_as_bf16(pq[slot, qt]), jnp.zeros((T - GW, T), bf16)], axis=0))
                pacer.issued(res, qt, WM)
                coef = g_rows / (res[GW:] + 1e-6)
                c0, c1, c2, c3 = (
                    jnp.broadcast_to(coef[2 * j:2 * j + 1], (8, T)) for j in range(4))
                cm = [c0, c0, jnp.where(low, c0, c1), c1, c1,
                      c2, c2, jnp.where(low, c2, c3), c3, c3]
                mem[qt] = [res[8 * i:8 * i + 8] * cm[i] for i in range(10)]
            finish()

        def corners(i):
            for lane in range(4):
                qt, pr = ORDER[2 * i + lane // 2], lane % 2
                window = _as_bf16(qd[slot, qt, 24 * pr:24 * pr + 24, :])
                sc = masked_dot(kk[slot, qt, T // 4:, :], window, 32 * pr)
                pacer.issued(sc, lane, WA)
                corner[qt, pr] = sc + bias[1]
                corner_max[qt, pr] = jnp.max(corner[qt, pr].reshape(8, 8, T), axis=0)

        def scores(t):
            qt, kt = tiles[t]
            for j in range(4):
                window = _as_bf16(qm[slot, qt, 16 * j:16 * j + 16, :])
                sc = masked_dot(
                    kk[slot, kt] if kt < qt else kk[slot, kt, :T // 4, :], window, 16 * j)
                pacer.issued(sc, j, WA)
                if kt == qt:
                    sc = sc + bias[0]
                m8 = jnp.max(sc.reshape(-1, 8, T), axis=0)
                run_max[qt, j] = m8 if kt == 0 else jnp.maximum(run_max[qt, j], m8)
                if kt == qt:
                    extra = corner_max[qt, j // 2]
                    if j % 2 == 0:
                        extra = pltpu.roll(extra, T // 2, 1)
                    top = jnp.maximum(run_max[qt, j], jnp.where(left, NEG, extra))
                    col_max[qt, j] = jnp.broadcast_to(
                        jnp.max(top, axis=0, keepdims=True), (8, T))
                logits[t, j] = sc
            if kt == qt:
                for pr in range(2):
                    top = jnp.where(left, pltpu.roll(col_max[qt, 2 * pr], T // 2, 1),
                                    col_max[qt, 2 * pr + 1])
                    words = _as_words(jnp.exp2(
                        corner[qt, pr].reshape(8, 8, T) - top[None]).reshape(T // 2, T))
                    for j, shifted in enumerate((pltpu.roll(words, T // 2, 1), words)):
                        corner_p[qt, 2 * pr + j] = _as_bf16(jnp.where(
                            left[None], jnp.uint32(0), shifted.reshape(4, 8, T)).reshape(32, T))

        def values(t):
            qt, kt = tiles[t]
            tops = [pacer.hold(col_max[qt, j], lead - stagger * j) for j in range(4)]
            for j in range(4):
                p = jnp.exp2(logits[t, j].reshape(-1, 8, T) - tops[j][None])
                p = p.reshape(-1, T).astype(bf16)
                if kt == qt:
                    p = jnp.concatenate([p, corner_p[qt, j]], axis=0)
                first = (0, 16, 40, 56)[j]
                v = [vt[slot, kt, first + 8 * i:first + 8 * i + 8, :] for i in range(3)]
                if j % 2 == 0:
                    v[2] = jnp.where(low, v[2], 1.0)
                else:
                    v[0] = jnp.where(low, 1.0, v[0])
                part = _dot(jnp.concatenate(v, axis=0), p)
                pacer.issued(part, j)
                acc[qt, j] = part if kt == 0 else acc[qt, j] + part
            if kt == qt:
                done.append(qt)
                finish()

        def finish():
            while done and (not memory or done[0] in mem):
                qt = done.pop(0)
                w = [[acc[qt, j][8 * i:8 * i + 8] for i in range(3)] for j in range(4)]
                sums = jnp.where(
                    low_pair, jnp.where(low, w[1][0], w[0][2]),
                    pltpu.roll(jnp.where(low, w[3][0], w[2][2]), 2, 0))
                coef = rest_rows / sums
                c0, c1, c2, c3 = (
                    jnp.broadcast_to(coef[r:r + 1], (8, T)) for r in (4, 0, 6, 2))
                o = [w[0][0] * c0, w[0][1] * c0,
                     jnp.where(low, w[0][2] * c0, w[1][0] * c1), w[1][1] * c1, w[1][2] * c1,
                     w[2][0] * c2, w[2][1] * c2,
                     jnp.where(low, w[2][2] * c2, w[3][0] * c3), w[3][1] * c3, w[3][2] * c3]
                if memory:
                    o = [mem[qt][i] + o[i] for i in range(10)]
                ot[s % 2, qt, _ds(g * (GW // 2), GW // 2, 8), :] = _as_words(
                    jnp.concatenate(o, axis=0))

        return {"D": corners, "Q": scores, "V": values, "R": read}

    def wo_tile(c, m):
        return wo_raw[c * T:(c + 1) * T, m * T:(m + 1) * T]

    def out_project(s, n, pacer):
        acc, done = [None] * 4, []

        def step(i):
            for lane in range(4):
                m, c = divmod(4 * i + lane, NC)
                part = _dot(_as_bf16(wot[c, 80 * m:80 * (m + 1), :]),
                            _as_bf16(ot[s % 2, n, c * 64:(c + 1) * 64, :]))
                pacer.issued(part, lane, WO)
                acc[m] = part if c == 0 else acc[m] + part
                if c == NC - 1:
                    acc[m] = acc[m].astype(bf16)
                    while T * (len(done) + 1) <= 160 * (m + 1):
                        i0 = T * len(done)
                        pieces = [acc[k][max(i0 - 160 * k, 0):min(i0 + T - 160 * k, 160)]
                                  for k in range(i0 // 160, (i0 + T - 1) // 160 + 1)]
                        tile = jnp.concatenate(pieces, axis=0).T
                        outb[s, _ds(n * T, T, T), i0:i0 + T] = tile
                        done.append(True)

        return step

    def outb_copy(s, n):
        return pltpu.make_async_copy(
            outb.at[s, _ds(n * T, T, T)],
            out_hbm.at[0, _ds(s * L + n * T, T, T), pl.ds(D, D)], sem_out.at[0])

    def conv_forward(c):
        cols = slice(c * T, (c + 1) * T)
        taps = shift_ref[:, cols].astype(f32)
        taps = [jnp.broadcast_to(taps[j:j + 1], (T, T)) for j in range(4)]
        skip = ssmd_ref[...].astype(f32)[c:c + 1]
        slices = pl.ds(c * NFV, NFV)

        def transform(even, odd):
            e, o = (_dot(_as_bf16(fwd[i]), x) for i, x in enumerate((even, odd)))
            return [x.reshape(NFV, 2, 8, T) for x in (e + o, e - o)]

        tail = jnp.zeros((8, T), u32)
        prev = None
        for b in range(NB):
            k0 = pltpu.bitcast(ka[2 * b * T:2 * (b + 1) * T, cols], u32)
            ext = jnp.concatenate([tail, k0], axis=0)
            tail = k0[T - 8:]
            k1, k2 = ext[7:7 + T], ext[6:6 + T]
            e0, o0, e1, o1, o2 = (
                _even_rows(k0), _odd_rows(k0), _even_rows(k1), _odd_rows(k1), _odd_rows(k2))
            v0 = pltpu.bitcast(va[2 * b * T:2 * (b + 1) * T, cols], u32)
            sig = transform(
                (e0 * taps[0] + o1 * taps[1] + e1 * taps[2] + o2 * taps[3]) * _even_rows(v0),
                (o0 * taps[0] + e0 * taps[1] + o1 * taps[2] + e1 * taps[3]) * _odd_rows(v0))
            taps_t = jnp.concatenate([
                pltpu.bitcast(ssk[cols, (2 * b + i) * T:(2 * b + i + 1) * T].T, u32)
                for i in range(2)], axis=0)
            filt = transform(_even_rows(taps_t), _odd_rows(taps_t))
            for sign in range(2):
                spec_buf[slices, 0, sign, b] = sig[sign].reshape(NFV, 16, T)
                re, im = filt[sign][:, 0], filt[sign][:, 1]
                if prev is None:
                    re = re + skip[None]
                else:
                    half = NFV // 2
                    pre, pim = prev[sign][:, 0], prev[sign][:, 1]
                    re = jnp.concatenate([re[:half] - pim[:half], re[half:] + pim[half:]], axis=0)
                    im = jnp.concatenate([im[:half] + pre[:half], im[half:] - pre[half:]], axis=0)
                spec_buf[slices, 1, sign, b, 0:8, :] = re
                spec_buf[slices, 1, sign, b, 8:16, :] = im
            prev = filt

    def conv_mix(first, count, never, blk=4):
        half = NFV // 2
        for item in range(count):
            idx = jnp.minimum(first + item, NC * half - 1)
            base = idx // half * NFV + idx % half

            def products(fv, sign, a0):
                def load(which, b):
                    return (spec_buf[fv, which, sign, b, 0:8, :],
                            spec_buf[fv, which, sign, b, 8:16, :])

                acc, kcache = [None] * blk, {}
                for b in range(a0 + blk):
                    token = yield
                    ur, ui = load(0, b)
                    ur = jnp.where(never, token, ur)
                    us = ur + ui
                    for a in range(max(a0, b), a0 + blk):
                        if a - b not in kcache:
                            kr, ki = load(1, a - b)
                            kcache[a - b] = (kr, ki - kr, kr + ki)
                        k1, k2, k3 = kcache[a - b]
                        terms = (us * k1, ur * k2, ui * k3)
                        old = acc[a - a0]
                        acc[a - a0] = terms if old is None else tuple(
                            o + t for o, t in zip(old, terms))
                return [(p1 - p3, p1 + p2) for p1, p2, p3 in acc]

            for a0 in range(0, NB, blk):
                parity = []
                for fv in (base, base + half):
                    plus = yield from products(fv, 0, a0)
                    minus = yield from products(fv, 1, a0)
                    parity.append((
                        [(pr + mr, pi + mi) for (pr, pi), (mr, mi) in zip(plus, minus)],
                        [(pr - mr, pi - mi) for (pr, pi), (mr, mi) in zip(plus, minus)]))
                for i in range(blk):
                    (ar, ai), (br, bi) = parity[0][0][i], parity[1][0][i]
                    (cr, ci), (dr, di) = parity[0][1][i], parity[1][1][i]
                    folded = ((ar + br, ai - bi), (cr - di, ci - dr),
                              (ar - br, ai + bi), (cr + di, ci + dr))
                    for r in range(4):
                        yf[idx, a0 + i, r] = _as_words(jnp.concatenate(folded[r], axis=0))

    def outa_copy(k):
        c, part = divmod(k, APARTS)
        rows = pl.ds(part * (S // APARTS), S // APARTS)
        return pltpu.make_async_copy(
            outa.at[c, rows], out_hbm.at[0, rows, pl.ds(c * T, T)], sem_out.at[0])

    def conv_inverse(pacer, zero):
        pending, pin, hold = [], [], []

        def send(c):
            outa_copy(c).start()
            pin.append(True)

        def flush(_):
            while pending:
                c, a, y = pending.pop(0)
                tile = c + zero if pin else c
                rows = slice(2 * a * T, 2 * (a + 1) * T)
                w01, w23 = _interleave(y[0], y[1]), _interleave(y[2], y[3])
                words = jnp.concatenate([
                    jnp.where(sub % 2 == 0, *(
                        jnp.take_along_axis(w[8 * v:8 * v + 8], sub // 2 + 4 * h, axis=0)
                        for w in (w01, w23)))
                    for v in range(8) for h in range(2)], axis=0)
                conv = _as_bf16(words).astype(f32)
                outa[tile, rows, :] = (qa[c, rows, :].astype(f32) * conv).astype(bf16)
                if pin:
                    hold.append(pltpu.bitcast(outa[tile, rows.start:rows.start + 16, :], u32))
                    pin.clear()

        def step(i):
            c, a = divmod(i, NB)
            res = []
            for r in range(4):
                words = yf[pl.ds(c * NFV // 2, NFV // 2), a, r].reshape(T // 2, T)
                if hold:
                    words = jnp.concatenate(
                        [jnp.where(pacer.never, hold.pop(), words[:8]), words[8:]], axis=0)
                res.append(_dot(
                    _as_bf16(inv[r]), _as_bf16(words)))
                pacer.issued(res[-1], r)
            flush(0)
            pending.append((c, a, res))

        return step, flush, send

    def out_project_last(pacer, zero):
        s = NSEG - 1
        o_rows, acc = {}, {}

        def transpose(n):
            for c in range(NC):
                o_rows[n, c] = _as_bf16(ot[s % 2, n, c * 64:(c + 1) * 64, :]).T

        def step(i):
            for lane in range(4):
                tile, c = divmod(4 * i + lane, NC)
                n, m = divmod(tile, NC)
                part = _dot(o_rows[n, c], wo_tile(c, m))
                pacer.issued(part, lane)
                acc[tile] = part if c == 0 else acc[tile] + part

        def store(part):
            n = min(part, NQ - 1)
            for m in range(NC) if part < NQ - 1 else ((0, 1, 2), (3, 4))[part - n]:
                seg = s + zero if m == 0 else s
                outb[seg, n * T:(n + 1) * T, m * T:(m + 1) * T] = acc[n * NC + m].astype(bf16)

        return transpose, step, store

    def new_pacer():
        return _Pacer(gate[0:8, :] > 2.0)

    def pair(s, p, plan, pacer, mix=None):
        memory = "Ra" in plan
        if mix is not None:
            first, count, cycles = mix
            pacer.attach(conv_mix(first, count, pacer.never), count * 96 / cycles)
        steps = {"a": attend(s, 2 * p, 0, pacer, memory),
                 "b": attend(s, 2 * p + 1, 1, pacer, memory)}
        steps["a"]["P"] = project(s, 2 * p + 1, 1, pacer)
        next_s, next_g = s + (p + 1) // 4, (2 * p + 2) % NG
        steps["b"]["P"] = project(next_s, next_g, 0, pacer)
        steps["a"]["U"] = lambda _: update(s, 2 * p + 1, pacer)
        steps["b"]["U"] = lambda _: update(next_s, next_g, pacer)
        steps["a"]["O"] = out_project(s - 1, p, pacer)
        steps["x"] = {
            "T": transpose_qkv,
            "K": repack_tables,
            "W": wait,
            "C": lambda _: outb_copy(s - 1, p).start(),
        }
        if "Jx" in plan:
            zero = pacer.never.astype(i32)[0, 0]
            steps["x"]["I"], steps["x"]["J"], steps["x"]["A"] = conv_inverse(pacer, zero)
            steps["x"]["L"], steps["x"]["E"], steps["x"]["G"] = out_project_last(pacer, zero)
        steps["x"]["F"] = lambda n: outb_copy(s, n).start()
        for item in plan:
            steps[item[1]][item[0]](int(item[2:] or 0))
        assert pacer.side is None

    def memory_pair(s, p):
        first = ((s - 1) * 4 + p) * MIX_PER_ITER
        pair(s, p, PLAN1, new_pacer(), (first, MIX_PER_ITER, MIX_CYCLES))

    wait(0)
    start(3, 4)
    for part in range(3):
        transpose_qkv(part)
    wait(1)
    start(4, len(loads))
    setup_gate()
    step = project(0, 0, 0, _Pacer(None))
    for i in range(NC):
        step(i)
    pacer = new_pacer()
    pair(0, 0, PLAN_FIRST, pacer)
    for p in range(1, 4):
        plan = ["Pa0"] + [item for item in PLAN0 if item != "Pa0"]
        if p == 1:
            plan.insert(plan.index("Qa5") + 1, "Wx4")
        pair(0, p, plan, pacer)

    wait(5)
    update(1, 0, _Pacer(None))
    for c in range(NC):
        conv_forward(c)
        transpose_wo(c)
    wait(6)

    @pl.loop(0, 11)
    def _(i):
        memory_pair(1 + i // 4, i % 4)

    wait(7)
    pair(NSEG - 1, 3, PLAN_LAST, new_pacer())

    outb_copy(NSEG - 1, NQ - 1).start()
    for k in range(NC * APARTS):
        outa_copy(k).wait()
    for s in range(NSEG):
        for n in range(NQ):
            outb_copy(s, n).wait()


@jax.jit
def pallas_concat_heads__ssm_conv_h3__memory_aug_infini_attn__prompt_kernel(
    A_q: jax.Array,
    A_k: jax.Array,
    A_v: jax.Array,
    A_shift_k: jax.Array,
    A_ssm_k: jax.Array,
    A_ssm_D: jax.Array,
    B_x: jax.Array,
    B_wq: jax.Array,
    B_wk: jax.Array,
    B_wv: jax.Array,
    B_wo: jax.Array,
    B_beta: jax.Array,
):
    hbm = pl.BlockSpec(memory_space=pl.ANY)
    scratch = [
        pltpu.VMEM((4, D), bf16),
        pltpu.VMEM((NC, T), bf16),
        pltpu.VMEM((H,), bf16),
        pltpu.VMEM((2, 2 * T, T), bf16),
        pltpu.VMEM((4, T // 2, T), bf16),
        pltpu.VMEM((NC, S, T), bf16),
        pltpu.VMEM((3, 2, D, T), bf16),
        pltpu.VMEM((3, D, 3 * T), bf16),
        pltpu.VMEM((D, D), bf16),
        pltpu.VMEM((3, NC, D // 2, T), u32),
        pltpu.VMEM((NC, D // 2, T), u32),
        pltpu.VMEM((NC, S, T), bf16),
        pltpu.VMEM((S, D), bf16),
        pltpu.VMEM((S, D), bf16),
        pltpu.VMEM((D, S), bf16),
        pltpu.VMEM((NC * NFV, 2, 2, NB, 16, T), f32),
        pltpu.VMEM((NC * NFV // 2, NB, 4, 8, T), u32),
        pltpu.VMEM((NC, S, T), bf16),
        pltpu.VMEM((NSEG, L, D), bf16),
        pltpu.VMEM((2, T, T), u32),
        pltpu.VMEM((4, T // 4, T), u32),
        pltpu.VMEM((H, T), f32),
        pltpu.VMEM((2, T // 2, T), f32),
        pltpu.VMEM((2, NQ, 64, T), u32),
        pltpu.VMEM((2, NQ, 48, T), u32),
        pltpu.VMEM((2, NQ, GW // 2, T), u32),
        pltpu.VMEM((2, NQ, T // 2, T), u32),
        pltpu.VMEM((2, NQ, GW, T), f32),
        pltpu.VMEM((2, NG, NQ, GW // 2, T), u32),
        pltpu.VMEM((2, NG, NQ, GW, T), f32),
        pltpu.VMEM((2, NQ, D // 2, T), u32),
        pltpu.VMEM((NG, GW + 8, T), f32),
        pltpu.SemaphoreType.DMA((8,)),
        pltpu.SemaphoreType.DMA((1,)),
    ]
    return pl.pallas_call(
        _kernel,
        out_shape=jax.ShapeDtypeStruct((1, S, 2 * D), bf16),
        in_specs=[hbm] * 14,
        out_specs=hbm,
        scratch_shapes=scratch,
        compiler_params=pltpu.CompilerParams(vmem_limit_bytes=100 * 2**20),
    )(
        A_shift_k.T, A_ssm_D.reshape(NC, T), B_beta, _FWD, _INV,
        A_q, A_k, A_v, A_ssm_k, B_x, B_wq, B_wk, B_wv, B_wo,
    )
```
